```python
import jax
import jax.numpy as jnp

def _softmax(x, axis=-1):
    return jax.nn.softmax(x, axis=axis)
def _gelu(x):
    return jax.nn.gelu(x, approximate=True)
def _silu(x):
    return jax.nn.silu(x)
def _sigmoid(x):
    return jax.nn.sigmoid(x)
def _layernorm(x, axis=-1, eps=1e-5):
    m = jnp.mean(x, axis=axis, keepdims=True)
    v = jnp.var(x, axis=axis, keepdims=True)
    return (x - m) / jnp.sqrt(v + eps)
def _scatter_add(tgt, idx, src, axis=0):
    return tgt.at[idx].add(src)
def _segment_sum(src, seg, n):
    return jax.ops.segment_sum(src, seg, n)
class _Rng:
    def __init__(self, key):
        self._k = key
    def _next(self):
        self._k, sub = jax.random.split(self._k)
        return sub
    def normal(self, shape):
        return jax.random.normal(self._next(), shape, dtype=jnp.bfloat16)
    def randint(self, lo, hi, shape):
        return jax.random.randint(self._next(), shape, lo, hi, dtype=jnp.int32)
    def uniform(self, shape, lo=0.0, hi=1.0):
        return jax.random.uniform(self._next(), shape, jnp.bfloat16, lo, hi)
    def permutation(self, n):
        return jax.random.permutation(self._next(), n)


kernel_name = 'gated_mix__compressed_kv_cla__ssm_conv_s5__prompt'

def setup_inputs():
    _rng = _Rng(jax.random.key(int.from_bytes(__import__("os").urandom(4), "little")))
    _w = (lambda a: (lambda t: t.astype(jnp.bfloat16) if jnp.issubdtype(t.dtype, jnp.floating) else t)(jnp.asarray(a)))
    def _A_setup():
        B, H, Sq, Sk, D, M = 1, 16, 2048, 2048, 256, 448
        Dc = 4 * D
        return {
            "x": _w((lambda *s: _rng.normal(s) * 0.05)(B, Sq, M)),
            "c_kv": _w((lambda *s: _rng.normal(s) * 0.05)(B, Sk, Dc)),
            "w_q": _w((lambda *s: _rng.normal(s) * 0.05)(M, H, D) * (M ** -0.5)),
            "w_uk": _w((lambda *s: _rng.normal(s) * 0.05)(Dc, H, D) * (Dc ** -0.5)),
            "w_uv": _w((lambda *s: _rng.normal(s) * 0.05)(Dc, H, D) * (Dc ** -0.5)),
            "w_o": _w((lambda *s: _rng.normal(s) * 0.05)(H, D, M) * ((H * D) ** -0.5)),
        }
    _A_in = _A_setup()

    def _B_setup():
        B, S, D = 1, 2048, 448
        P = D
        Lambda_re = -0.5 * jnp.exp((lambda *s: _rng.normal(s) * 0.05)(P))
        Lambda_im = (lambda *s: _rng.normal(s) * 0.05)(P) * 1.0
        B_re = (lambda *s: _rng.normal(s) * 0.05)(P, D) * (D ** -0.5)
        B_im = (lambda *s: _rng.normal(s) * 0.05)(P, D) * (D ** -0.5)
        C_re = (lambda *s: _rng.normal(s) * 0.05)(D, P) * (P ** -0.5)
        C_im = (lambda *s: _rng.normal(s) * 0.05)(D, P) * (P ** -0.5)
        log_dt = (lambda *s: _rng.normal(s) * 0.05)(P) * 0.3 - 2.0
        Dskip = (lambda *s: _rng.normal(s) * 0.05)(D)
        return {
            "x": _w((lambda *s: _rng.normal(s) * 0.05)(B, S, D)),
            "Lambda_re": _w(Lambda_re),
            "Lambda_im": _w(Lambda_im),
            "B_re": _w(B_re),
            "B_im": _w(B_im),
            "C_re": _w(C_re),
            "C_im": _w(C_im),
            "log_dt": _w(log_dt),
            "Dskip": _w(Dskip),
        }
    _B_in = _B_setup()

    return {
        "A_x": _A_in["x"],
        "A_c_kv": _A_in["c_kv"],
        "A_w_q": _A_in["w_q"],
        "A_w_uk": _A_in["w_uk"],
        "A_w_uv": _A_in["w_uv"],
        "A_w_o": _A_in["w_o"],
        "B_x": _B_in["x"],
        "B_Lambda_re": _B_in["Lambda_re"],
        "B_Lambda_im": _B_in["Lambda_im"],
        "B_B_re": _B_in["B_re"],
        "B_B_im": _B_in["B_im"],
        "B_C_re": _B_in["C_re"],
        "B_C_im": _B_in["C_im"],
        "B_log_dt": _B_in["log_dt"],
        "B_Dskip": _B_in["Dskip"],
        "gate_w": _w((lambda *s: _rng.normal(s) * 0.05)(448)),
    }

def reference(A_x, A_c_kv, A_w_q, A_w_uk, A_w_uv, A_w_o, B_x, B_Lambda_re, B_Lambda_im, B_B_re, B_B_im, B_C_re, B_C_im, B_log_dt, B_Dskip, gate_w):
    def _A_ref(x, c_kv, w_q, w_uk, w_uv, w_o):
        B, Sq, M = x.shape[0], x.shape[1], x.shape[2]
        Sk = c_kv.shape[1]
        H, D = w_q.shape[1], w_q.shape[2]
        q = jnp.einsum("bqm,mhd->bhqd", x, w_q)
        k = jnp.einsum("bkc,chd->bhkd", c_kv, w_uk)
        v = jnp.einsum("bkc,chd->bhkd", c_kv, w_uv)
        scores = jnp.einsum("bhqd,bhkd->bhqk", q, k) * (D ** -0.5)
        off = Sk - Sq
        qi = jnp.arange(Sq)[:, None]
        kj = jnp.arange(Sk)[None, :]
        cmask = kj <= (qi + off)
        scores = jnp.where(cmask[None, None], scores, -1e9)
        p = _softmax(scores, axis=-1)
        ctx = jnp.einsum("bhqk,bhkd->bhqd", p, v)
        return jnp.einsum("bhqd,hdm->bqm", ctx, w_o)

    def _B_ref(x, Lambda_re, Lambda_im, B_re, B_im, C_re, C_im, log_dt, Dskip):
        Bsz, L, H = x.shape
        Lam = Lambda_re + 1j * Lambda_im
        Bmat = B_re + 1j * B_im
        Cmat = C_re + 1j * C_im
        dt = jnp.exp(log_dt)
        Lam_bar = jnp.exp(dt * Lam)
        B_bar = ((Lam_bar - 1.0) / Lam)[:, None] * Bmat
        Bu = jnp.einsum("bld,pd->blp", x + 0j, B_bar)
        h = jnp.zeros_like(Bu[:, 0, :])
        hs = []
        for t in range(L):
            h = Lam_bar[None, :] * h + Bu[:, t, :]
            hs.append(h)
        hseq = jnp.stack(hs, 1)
        y = 2.0 * jnp.einsum("blp,dp->bld", hseq, Cmat).real + x * Dskip[None, None, :]
        return y

    x = A_x
    g = _sigmoid((x * gate_w).sum(-1, keepdims=True))
    a = _A_ref(x, A_c_kv, A_w_q, A_w_uk, A_w_uv, A_w_o)
    b = _B_ref(x, B_Lambda_re, B_Lambda_im, B_B_re, B_B_im, B_C_re, B_C_im, B_log_dt, B_Dskip)
    return g * a + (1 - g) * b
```

```python
import functools
import math

import jax
import jax.numpy as jnp
from jax import lax
import jax.experimental.pallas as pl
import jax.experimental.pallas.tpu as pltpu

F32 = jnp.float32
BF16 = jnp.bfloat16
U32 = jnp.uint32

S = 2048
M = 448
DC = 1024
H = 16
D = 256
TQ = 128
NSEG = 8
LSEG = S // NSEG
SEG_STRIDE = LSEG + 8
STEPS = 2 * LSEG // H
MA = 384
MR = M - MA
NT = (((1,), (1,)), ((), ()))
O_LAG = 2


def _unpack_head(even, odd, shift):
    lo = (even >> shift) & jnp.uint32(0xFFFF)
    hi = (odd >> shift) << jnp.uint32(16)
    return pltpu.bitcast(lo | hi, BF16)


def _cmul(pr, pi, hr, hi):
    return ([pr[t] * hr[t] - pi[t] * hi[t] for t in range(4)],
            [pr[t] * hi[t] + pi[t] * hr[t] for t in range(4)])


def _column(row):
    row = jnp.concatenate([row, jnp.zeros((1, 512 - M), F32)], axis=1)
    return jnp.broadcast_to(row, (128, 512)).T[:M]


def _kernel(xt_hbm, c_hbm, wq_hbm, wk_hbm, wv_hbm, wot_hbm,
            lre_hbm, lim_hbm, bre_hbm, bim_hbm, cre_hbm, cim_hbm, ldt_hbm,
            dsk_hbm, gw_hbm,
            out_hbm,
            xt_v, x_v, c_v, wot_v, wq_b, wk_b, wv_b, bcat_v, cre_v, cim_v, ccat_v,
            lre_v, lim_v, ldt_v, dsk_v, gw_v, col_v,
            u_v, h_v, a_v, st_v, acc_v, xsem, sem, wsem, osem):
    wq32 = wq_hbm.bitcast(U32)
    wk32 = wk_hbm.bitcast(U32)
    wv32 = wv_hbm.bitcast(U32)

    def w_copies(j, sl):
        cps = []
        for n, (src, dst) in enumerate(((wq32, wq_b), (wk32, wk_b), (wv32, wv_b))):
            for e in range(2):
                cps.append(pltpu.make_async_copy(
                    src.at[:, 8 * e + j, :], dst.at[sl, e],
                    wsem.at[sl * 6 + n * 2 + e]))
        return cps

    x_cps = [pltpu.make_async_copy(xt_hbm.at[:, s * LSEG:(s + 1) * LSEG],
                                   xt_v.at[:, s * LSEG:(s + 1) * LSEG], xsem.at[s])
             for s in range(NSEG)]
    b_cps = [
        pltpu.make_async_copy(bre_hbm.at[0:MA], bcat_v.at[0:MA], sem.at[0]),
        pltpu.make_async_copy(bim_hbm.at[0:MA], bcat_v.at[MA:2 * MA], sem.at[1]),
        pltpu.make_async_copy(bre_hbm.at[MA:M], bcat_v.at[2 * MA:2 * MA + MR], sem.at[2]),
        pltpu.make_async_copy(bim_hbm.at[MA:M], bcat_v.at[2 * MA + MR:2 * M], sem.at[3]),
    ]
    vec_cps = [pltpu.make_async_copy(src, dst, sem.at[4 + n]) for n, (src, dst) in enumerate(
        ((lre_hbm, lre_v), (lim_hbm, lim_v), (ldt_hbm, ldt_v), (dsk_hbm, dsk_v), (gw_hbm, gw_v)))]
    cc_cps = [pltpu.make_async_copy(cre_hbm, cre_v, sem.at[9]),
              pltpu.make_async_copy(cim_hbm, cim_v, sem.at[10])]
    c_cp = pltpu.make_async_copy(c_hbm, c_v, sem.at[11])
    wo_cp = pltpu.make_async_copy(wot_hbm, wot_v, sem.at[12])

    @jax.named_scope('prologue')
    def _prologue():
        x_cps[0].start()
        for cp in b_cps + vec_cps + x_cps[1:] + cc_cps + w_copies(0, 0) + [c_cp, wo_cp]:
            cp.start()
        acc_v[...] = jnp.zeros_like(acc_v)
        st_v[...] = jnp.zeros_like(st_v)

        for cp in b_cps:
            cp.wait()
        b_cat = bcat_v[...]
        for s in range(NSEG):
            x_cps[s].wait()
            xs = xt_v[:, s * LSEG:(s + 1) * LSEG].T
            x_v[s * LSEG:(s + 1) * LSEG, :] = xs
            u = lax.dot_general(xs, b_cat, NT, preferred_element_type=F32)
            rows = slice(s * SEG_STRIDE, s * SEG_STRIDE + LSEG)
            for t in range(7):
                u_v[t, rows, :] = u[:, t * 128:(t + 1) * 128]
            u_v[7, rows, :] = pltpu.roll(u[:, 2 * MA:], MR, 1)
            if s == NSEG - 3:
                for cp in vec_cps + cc_cps:
                    cp.wait()
                lre = lre_v[...].astype(F32).reshape(1, M)
                lim = lim_v[...].astype(F32).reshape(1, M)
                dt = jnp.exp(ldt_v[...].astype(F32)).astype(BF16).astype(F32).reshape(1, M)
                er = jnp.exp(dt * lre)
                ar = er * jnp.cos(dt * lim)
                ai = er * jnp.sin(dt * lim)
                den = lre * lre + lim * lim
                cr = ((ar - 1.0) * lre + ai * lim) / den
                ci = (ai * lre - (ar - 1.0) * lim) / den
                cre = cre_v[...].astype(F32)
                cim = cim_v[...].astype(F32)
                c_r = 2.0 * (cre * cr - cim * ci)
                c_i = -2.0 * (cre * ci + cim * cr)
                ccat_v[...] = jnp.concatenate(
                    [c_r[:, :MA], c_i[:, :MA], c_r[:, MA:], c_i[:, MA:]], axis=1).astype(BF16)

                def bc(v):
                    return jnp.broadcast_to(v, (NSEG, 128))

                for t in range(3):
                    a_v[t] = bc(ar[:, t * 128:(t + 1) * 128])
                    a_v[4 + t] = bc(ai[:, t * 128:(t + 1) * 128])
                a_v[3] = bc(jnp.concatenate([ar[:, MA:], ar[:, MA:]], axis=1))
                a_v[7] = bc(jnp.concatenate([ai[:, MA:], -ai[:, MA:]], axis=1))
                col_v[0] = _column(dsk_v[...].astype(F32).reshape(1, M))
                col_v[1] = _column(gw_v[...].astype(F32).reshape(1, M))
        c_cp.wait()
        wo_cp.wait()

    _prologue()

    def head(h, _):
        pair = lax.shift_right_logical(h, 1)
        slot = lax.bitwise_and(pair, 1)
        odd = lax.bitwise_and(h, 1)

        @pl.when(h == H // 2)
        def _segment_carry():
            pr = [a_v[t] for t in range(4)]
            pi = [a_v[4 + t] for t in range(4)]
            for _ in range(int(math.log2(LSEG))):
                pr, pi = ([pr[t] * pr[t] - pi[t] * pi[t] for t in range(4)],
                          [2.0 * pr[t] * pi[t] for t in range(4)])
            row = lax.broadcasted_iota(jnp.int32, (NSEG, 128), 0)
            e_r = [st_v[t] for t in range(4)]
            e_i = [st_v[4 + t] for t in range(4)]
            ir = [jnp.zeros((NSEG, 128), F32)] * 4
            ii = ir
            for s in range(1, NSEG):
                mr, mi = _cmul(pr, pi, ir, ii)
                fr = [pltpu.roll(mr[k] + e_r[k], 1, 0) for k in range(4)]
                fi = [pltpu.roll(mi[k] + e_i[k], 1, 0) for k in range(4)]
                ir = [jnp.where(row == s, fr[k], ir[k]) for k in range(4)]
                ii = [jnp.where(row == s, fi[k], ii[k]) for k in range(4)]
            for t in range(4):
                st_v[t] = ir[t]
                st_v[4 + t] = ii[t]

        @pl.when(odd == 0)
        def _weights():
            for cp in w_copies(pair, slot):
                cp.wait()

        @pl.when(jnp.logical_and(odd == 0, h + 2 < H))
        def _prefetch():
            for cp in w_copies(pair + 1, 1 - slot):
                cp.start()

        shift = (odd * 16).astype(U32)
        wq = _unpack_head(wq_b[slot, 0], wq_b[slot, 1], shift)
        wk = _unpack_head(wk_b[slot, 0], wk_b[slot, 1], shift)
        wv = _unpack_head(wv_b[slot, 0], wv_b[slot, 1], shift)
        qscale = (D ** -0.5) * math.log2(math.e)
        q = (jnp.dot(x_v[...], wq, preferred_element_type=F32) * qscale).astype(BF16)
        c = c_v[...]
        k = jnp.dot(c, wk, preferred_element_type=F32).astype(BF16)
        v = jnp.dot(c, wv, preferred_element_type=F32).astype(BF16)

        t0 = lax.bitwise_and(h, H // 2 - 1) * STEPS
        a_r = [a_v[t] for t in range(4)]
        a_i = [a_v[4 + t] for t in range(4)]
        hr = [st_v[t] for t in range(4)]
        hi = [st_v[4 + t] for t in range(4)]
        for j in range(STEPS):
            us = [u_v[kk, pl.ds(t0 + j, NSEG, stride=SEG_STRIDE), :] for kk in range(8)]
            mr, mi = _cmul(a_r, a_i, hr, hi)
            hr = [mr[0] + us[0], mr[1] + us[1], mr[2] + us[2], mr[3] + us[6]]
            hi = [mi[0] + us[3], mi[1] + us[4], mi[2] + us[5], mi[3] + us[7]]
            r0 = pl.multiple_of((t0 + j) * NSEG, NSEG)
            for kk, val in enumerate(hr[:3] + hi[:3] + [hr[3]]):
                h_v[kk, pl.ds(r0, NSEG), :] = val
        for t in range(4):
            st_v[t] = hr[t]
            st_v[4 + t] = hi[t]

        nb = S // TQ
        causal = (lax.broadcasted_iota(jnp.int32, (TQ, TQ), 1)
                  <= lax.broadcasted_iota(jnp.int32, (TQ, TQ), 0))
        wot = wot_v[h]

        def scores(i):
            return lax.dot_general(q[i * TQ:(i + 1) * TQ], k[:(i + 1) * TQ], NT,
                                   preferred_element_type=F32)

        def out_proj(i, ctx):
            cols = slice(i * TQ, (i + 1) * TQ)
            acc_v[:, cols] += lax.dot_general(wot, ctx, NT, preferred_element_type=F32)

        ctxs = {}
        s_next = scores(0)
        for i in range(nb):
            s = s_next
            if i + 1 < nb:
                s_next = scores(i + 1)
            diag = jnp.where(causal, s[:, i * TQ:], -1e9)
            if i > 0:
                s = jnp.concatenate([s[:, :i * TQ], diag], axis=1)
            else:
                s = diag
            m = jnp.max(s, axis=1, keepdims=True)
            p = jnp.exp2(s - m)
            l = jnp.sum(p, axis=1, keepdims=True)
            ctx = jnp.dot(p.astype(BF16), v[:(i + 1) * TQ], preferred_element_type=F32)
            ctxs[i] = (ctx * (1.0 / l)).astype(BF16)
            if i >= O_LAG:
                out_proj(i - O_LAG, ctxs.pop(i - O_LAG))
        for i in sorted(ctxs):
            out_proj(i, ctxs[i])
        return 0

    with jax.named_scope('heads'):
        lax.fori_loop(0, H, head, 0)

    @jax.named_scope('epilogue')
    def _epilogue():
        c_cat = ccat_v[...]
        o_cps = []
        for s in range(NSEG):
            cols = slice(s * LSEG, (s + 1) * LSEG)
            hs = jnp.concatenate(
                [h_v[kk, pl.ds(s, LSEG, stride=NSEG), :] for kk in range(7)], axis=1).astype(BF16)
            yt = lax.dot_general(c_cat, hs, NT, preferred_element_type=F32)
            xf = xt_v[:, cols].astype(F32)
            dsk = jnp.concatenate([col_v[0]] * (LSEG // 128), axis=1)
            gw = jnp.concatenate([col_v[1]] * (LSEG // 128), axis=1)
            g = jax.nn.sigmoid(jnp.sum(xf * gw, axis=0, keepdims=True))
            acc_v[:, cols] = g * acc_v[:, cols] + (1.0 - g) * (yt + xf * dsk)
            cp = pltpu.make_async_copy(acc_v.at[:, cols], out_hbm.at[:, cols], osem.at[s])
            cp.start()
            o_cps.append(cp)
        for cp in o_cps:
            cp.wait()

    _epilogue()


@jax.jit
def pallas_gated_mix__compressed_kv_cla__ssm_conv_s5__prompt_kernel(
    A_x: jax.Array,
    A_c_kv: jax.Array,
    A_w_q: jax.Array,
    A_w_uk: jax.Array,
    A_w_uv: jax.Array,
    A_w_o: jax.Array,
    B_x: jax.Array,
    B_Lambda_re: jax.Array,
    B_Lambda_im: jax.Array,
    B_B_re: jax.Array,
    B_B_im: jax.Array,
    B_C_re: jax.Array,
    B_C_im: jax.Array,
    B_log_dt: jax.Array,
    B_Dskip: jax.Array,
    gate_w: jax.Array,
):
    del B_x
    hbm_spec = pl.BlockSpec(memory_space=pltpu.HBM)
    out_t = pl.pallas_call(
        _kernel,
        in_specs=[hbm_spec] * 15,
        out_specs=hbm_spec,
        out_shape=jax.ShapeDtypeStruct((M, S), F32),
        scratch_shapes=[
            pltpu.VMEM((M, S), BF16),
            pltpu.VMEM((S, M), BF16),
            pltpu.VMEM((S, DC), BF16),
            pltpu.VMEM((H, M, D), BF16),
            pltpu.VMEM((2, 2, M // 2, D), U32),
            pltpu.VMEM((2, 2, DC // 2, D), U32),
            pltpu.VMEM((2, 2, DC // 2, D), U32),
            pltpu.VMEM((2 * M, M), BF16),
            pltpu.VMEM((M, M), BF16),
            pltpu.VMEM((M, M), BF16),
            pltpu.VMEM((M, 2 * M), BF16),
            pltpu.VMEM((M,), BF16), pltpu.VMEM((M,), BF16), pltpu.VMEM((M,), BF16),
            pltpu.VMEM((M,), BF16), pltpu.VMEM((M,), BF16),
            pltpu.VMEM((2, M, 128), F32),
            pltpu.VMEM((8, NSEG * SEG_STRIDE, 128), F32),
            pltpu.VMEM((7, S, 128), F32),
            pltpu.VMEM((8, NSEG, 128), F32),
            pltpu.VMEM((8, NSEG, 128), F32),
            pltpu.VMEM((M, S), F32),
            pltpu.SemaphoreType.DMA((NSEG,)),
            pltpu.SemaphoreType.DMA((13,)),
            pltpu.SemaphoreType.DMA((12,)),
            pltpu.SemaphoreType.DMA((NSEG,)),
        ],
        compiler_params=pltpu.CompilerParams(vmem_limit_bytes=110 * 1024 * 1024),
        name="gated_mix",
    )(
        A_x.reshape(S, M).T, A_c_kv.reshape(S, DC),
        A_w_q.reshape(M // 2, 2 * H, D), A_w_uk.reshape(DC // 2, 2 * H, D),
        A_w_uv.reshape(DC // 2, 2 * H, D), jnp.swapaxes(A_w_o, 1, 2),
        B_Lambda_re, B_Lambda_im, B_B_re, B_B_im, B_C_re, B_C_im, B_log_dt,
        B_Dskip, gate_w,
    )
    return out_t.T.reshape(1, S, M)
```

```python
import functools
import math
import os

import jax
import jax.numpy as jnp
from jax import lax
import jax.experimental.pallas as pl
import jax.experimental.pallas.tpu as pltpu

F32 = jnp.float32
BF16 = jnp.bfloat16
U32 = jnp.uint32

S = 2048
HS = S // 2
M = 448
DC = 1024
H = 16
D = 256
TQ = 128
NB = S // TQ
NSEG = 8
LSEG = S // NSEG
SEG_STRIDE = LSEG + 8
STEPS = 2 * LSEG // H
MA = 384
MR = M - MA
NT = (((1,), (1,)), ((), ()))
O_LAG = int(os.environ.get('O_LAG', 4))
NPRO = NSEG // 2
EC = 4
_om = os.environ.get('ORDER', 'desc')
if _om == 'asc':
    ORDER = list(range(NB))
elif _om == 'desc':
    ORDER = list(range(NB))[::-1]
else:
    ORDER = [int(t) for t in _om.split(',')]
LOOK = int(os.environ.get('LOOK', 2))
PRE_S = int(os.environ.get('PRE_S', 2))
KV_JOINT = int(os.environ.get('KV_JOINT', 0))
SEM_W = 3
SEM_X = 5
CROWS = 32


def _lhs_terms(a11, a12, a21, a22):
    return [t.astype(BF16) for t in
            (a11 + a22, a21 + a22, a11, a22, a11 + a12, a21 - a11, a12 - a22)]


def _rhs_terms(b11, b12, b21, b22):
    return [t.astype(BF16) for t in
            (b11 + b22, b11, b12 - b22, b21 - b11, b22, b11 + b12, b21 + b22)]


def _strassen(lhs, rhs):
    def mm(i):
        return jnp.dot(lhs(i), rhs[i], preferred_element_type=F32)
    m1 = mm(0)
    m4 = mm(3)
    c11 = m1 + m4
    m2 = mm(1)
    c21 = m2 + m4
    c22 = m1 - m2
    m5 = mm(4)
    c11 = c11 - m5
    m3 = mm(2)
    c12 = m3 + m5
    c22 = c22 + m3
    c11 = c11 + mm(6)
    c22 = c22 + mm(5)
    return c11, c12, c21, c22


def _cmul(pr, pi, hr, hi):
    return ([pr[t] * hr[t] - pi[t] * hi[t] for t in range(4)],
            [pr[t] * hi[t] + pi[t] * hr[t] for t in range(4)])


def _column(row):
    row = jnp.concatenate([row, jnp.zeros((1, 512 - M), F32)], axis=1)
    return jnp.broadcast_to(row, (128, 512)).T[:M]


def _kernel(xt_hbm, c_hbm, wq_hbm, wk_hbm, wv_hbm, wot_hbm,
            lre_hbm, lim_hbm, bre_hbm, bim_hbm, cre_hbm, cim_hbm, ldt_hbm,
            dsk_hbm, gw_hbm,
            out_hbm,
            xt_v, xs_v, c_v, cs_v, wot_v, wq_b, wk_b, wv_b, bcat_v, cre_v, cim_v, ccat_v,
            lre_v, lim_v, ldt_v, dsk_v, gw_v, col_v, coef_v,
            u_v, h_v, a_v, st_v, acc_v, ctxc_v, never_v, sem):
    wq32 = wq_hbm.bitcast(U32)
    wk32 = wk_hbm.bitcast(U32)
    wv32 = wv_hbm.bitcast(U32)

    def w_copies(h, h_dst, sl):
        j = lax.shift_right_logical(h, 1)
        cps = [pltpu.make_async_copy(src.at[:, j, :], dst.at[sl], sem.at[SEM_W + sl])
               for src, dst in ((wq32, wq_b), (wk32, wk_b), (wv32, wv_b))]
        return cps + [pltpu.make_async_copy(wot_hbm.at[h], wot_v.at[h_dst], sem.at[SEM_W + sl])]

    def x_copies(s):
        spans = [pl.ds(pl.multiple_of(s * LSEG + e * HS, LSEG), LSEG) for e in range(2)]
        return [pltpu.make_async_copy(xt_hbm.at[:, sp], xt_v.at[:, sp], sem.at[SEM_X + s])
                for sp in spans]

    def c_copies(s):
        spans = [pl.ds(pl.multiple_of(s * LSEG + e * HS, LSEG), LSEG) for e in range(2)]
        return [pltpu.make_async_copy(c_hbm.at[sp], c_v.at[sp], sem.at[SEM_X + 1 + s])
                for sp in spans]

    b_cps = [
        pltpu.make_async_copy(bre_hbm.at[0:MA], bcat_v.at[0:MA], sem.at[SEM_X]),
        pltpu.make_async_copy(bim_hbm.at[0:MA], bcat_v.at[MA:2 * MA], sem.at[SEM_X]),
        pltpu.make_async_copy(bre_hbm.at[MA:M], bcat_v.at[2 * MA:2 * MA + MR], sem.at[SEM_X]),
        pltpu.make_async_copy(bim_hbm.at[MA:M], bcat_v.at[2 * MA + MR:2 * M], sem.at[SEM_X]),
    ]
    vec_cps = [pltpu.make_async_copy(src, dst, sem.at[1]) for src, dst in
               ((lre_hbm, lre_v), (lim_hbm, lim_v), (ldt_hbm, ldt_v), (dsk_hbm, dsk_v),
                (gw_hbm, gw_v))]
    late_cps = [pltpu.make_async_copy(cre_hbm, cre_v, sem.at[2]),
                pltpu.make_async_copy(cim_hbm, cim_v, sem.at[2])]

    @jax.named_scope('prologue')
    def _prologue():
        zero = jnp.int32(0)
        first = vec_cps + x_copies(0) + b_cps
        for s in range(1, NPRO):
            first = first + x_copies(s) + c_copies(s - 1)
        for cp in first + c_copies(NPRO - 1) + w_copies(zero, 0, 0) + late_cps:
            cp.start()
        acc_v[...] = jnp.zeros_like(acc_v)
        st_v[...] = jnp.zeros_like(st_v)
        ctxc_v[...] = jnp.zeros_like(ctxc_v)
        never_v[...] = jnp.zeros_like(never_v)

        for cp in vec_cps:
            cp.wait()
        lre = lre_v[...].astype(F32).reshape(1, M)
        lim = lim_v[...].astype(F32).reshape(1, M)
        dt = jnp.exp(ldt_v[...].astype(F32)).astype(BF16).astype(F32).reshape(1, M)
        er = jnp.exp(dt * lre)
        ar = er * jnp.cos(dt * lim)
        ai = er * jnp.sin(dt * lim)
        den = lre * lre + lim * lim
        coef_v[0] = jnp.broadcast_to(2.0 * ((ar - 1.0) * lre + ai * lim) / den, (8, M))
        coef_v[1] = jnp.broadcast_to(2.0 * (ai * lre - (ar - 1.0) * lim) / den, (8, M))

        def bc(v):
            return jnp.broadcast_to(v, (NSEG, 128))

        for t in range(3):
            a_v[t] = bc(ar[:, t * 128:(t + 1) * 128])
            a_v[4 + t] = bc(ai[:, t * 128:(t + 1) * 128])
        a_v[3] = bc(jnp.concatenate([ar[:, MA:], ar[:, MA:]], axis=1))
        a_v[7] = bc(jnp.concatenate([ai[:, MA:], -ai[:, MA:]], axis=1))
        col_v[0] = _column(dsk_v[...].astype(F32).reshape(1, M))
        col_v[1] = _column(gw_v[...].astype(F32).reshape(1, M))

        never = never_v[...] != 0

        def bu(s):
            b_cat = bcat_v[...]
            r = pl.ds(pl.multiple_of(s * (LSEG // 2), LSEG // 2), LSEG // 2)
            xs = []
            us = []
            for e in range(2):
                c0 = pl.multiple_of(s * LSEG + e * HS, LSEG)
                xe = xt_v[:, pl.ds(c0, LSEG)].T
                u = lax.dot_general(xe, b_cat, NT, preferred_element_type=F32)
                us.append(u)
                rows = pl.ds(pl.multiple_of((s + e * NPRO) * SEG_STRIDE, 8), LSEG)
                u_v[7, rows, :] = pltpu.roll(u[:, 2 * MA:], MR, 1)
                for t in range(7):
                    u_v[t, rows, :] = u[:, t * 128:(t + 1) * 128]
                xe = xe.astype(F32)
                xs.append((xe[:, :D], jnp.concatenate(
                    [xe[:, D:], jnp.zeros((LSEG, 2 * D - M), F32)], axis=1)))
            for i, t in enumerate(_lhs_terms(xs[0][0], xs[0][1], xs[1][0], xs[1][1])):
                t = pltpu.bitcast(t, U32)
                for kt in range(2):
                    xs_v[i, kt, r, :] = t[:, kt * 128:(kt + 1) * 128]
            return us

        def c_terms(s, us):
            hc = DC // 2
            r = pl.ds(pl.multiple_of(s * (LSEG // 2), LSEG // 2), LSEG // 2)
            rt = pl.ds(pl.multiple_of(s * LSEG, LSEG), LSEG)
            rb = pl.ds(pl.multiple_of(s * LSEG + HS, LSEG), LSEG)
            a11, a12, a21, a22 = c_v[rt, :hc], c_v[rt, hc:], c_v[rb, :hc], c_v[rb, hc:]
            if us is not None:
                cols = []
                for kt in range(4):
                    vr = []
                    for g in range(16):
                        n = ((kt * 16 + g) * 13) // 2
                        e, t, rg = n // 224, (n % 224) // 32, n % 32
                        vr.append(us[e][8 * rg:8 * rg + 8, 128 * t:128 * t + 128])
                    cols.append(jnp.concatenate(vr, axis=0))
                dep = pltpu.bitcast(jnp.concatenate(cols, axis=1), U32)
                nv = jnp.concatenate([jnp.concatenate([never] * 16, axis=0)] * 4, axis=1)
                a11 = pltpu.bitcast(jnp.where(nv, dep, pltpu.bitcast(a11, U32)), BF16)
                a22 = pltpu.bitcast(jnp.where(nv, dep, pltpu.bitcast(a22, U32)), BF16)
            terms = _lhs_terms(*(a.astype(F32) for a in (a11, a12, a21, a22)))
            for i, t in enumerate(terms):
                t = pltpu.bitcast(t, U32)
                for kt in range(4):
                    cs_v[i, kt, r, :] = t[:, kt * 128:(kt + 1) * 128]

        for cp in x_copies(0) + b_cps:
            cp.wait()
        bu(0)

        def pro_step(s, _):
            for cp in x_copies(s) + c_copies(s - 1):
                cp.wait()
            c_terms(s - 1, bu(s))
            return 0

        lax.fori_loop(1, NPRO, pro_step, 0)
        for cp in c_copies(NPRO - 1):
            cp.wait()
        c_terms(NPRO - 1, None)
        for cp in late_cps:
            cp.wait()

    _prologue()

    def out_proj(wot, i, ctx):
        cols = slice(i * TQ, (i + 1) * TQ)
        acc_v[:, cols] += lax.dot_general(wot, ctx, NT, preferred_element_type=F32)

    def head(h, _):
        slot = lax.bitwise_and(h, 1)

        @pl.when(h == H // 2)
        def _segment_carry():
            pr = [a_v[t] for t in range(4)]
            pi = [a_v[4 + t] for t in range(4)]
            for _ in range(int(math.log2(LSEG))):
                pr, pi = ([pr[t] * pr[t] - pi[t] * pi[t] for t in range(4)],
                          [2.0 * pr[t] * pi[t] for t in range(4)])
            row = lax.broadcasted_iota(jnp.int32, (NSEG, 128), 0)
            e_r = [st_v[t] for t in range(4)]
            e_i = [st_v[4 + t] for t in range(4)]
            ir = [jnp.zeros((NSEG, 128), F32)] * 4
            ii = ir
            for s in range(1, NSEG):
                mr, mi = _cmul(pr, pi, ir, ii)
                fr = [pltpu.roll(mr[k] + e_r[k], 1, 0) for k in range(4)]
                fi = [pltpu.roll(mi[k] + e_i[k], 1, 0) for k in range(4)]
                ir = [jnp.where(row == s, fr[k], ir[k]) for k in range(4)]
                ii = [jnp.where(row == s, fi[k], ii[k]) for k in range(4)]
            for t in range(4):
                st_v[t] = ir[t]
                st_v[4 + t] = ii[t]

        for cp in w_copies(h, h, slot):
            cp.wait()

        wot_prev = wot_v[jnp.maximum(h - 1, 0)]
        o_prev = [lax.dot_general(wot_prev, ctxc_v[e], NT, preferred_element_type=F32)
                  for e in range(O_LAG)]
        for cp in w_copies(jnp.minimum(h + 1, H - 1), h + 1, 1 - slot):
            cp.start()
        for e in range(O_LAG):
            i = ORDER[NB - O_LAG + e]
            acc_v[:, i * TQ:(i + 1) * TQ] += o_prev[e]

        up = ((1 - slot) * 16).astype(U32)

        def weight(buf):
            return pltpu.bitcast((buf[slot] << up) & jnp.uint32(0xFFFF0000), F32)

        def quads(w, kh):
            return w[:kh, :128], w[:kh, 128:], w[kh:, :128], w[kh:, 128:]

        def assemble(c11, c12, c21, c22):
            return jnp.concatenate([jnp.concatenate([c11, c12], axis=1),
                                    jnp.concatenate([c21, c22], axis=1)], axis=0)

        def x_term(i):
            return pltpu.bitcast(jnp.concatenate([xs_v[i, kt] for kt in range(2)], axis=1), BF16)

        def c_term(i):
            return pltpu.bitcast(jnp.concatenate([cs_v[i, kt] for kt in range(4)], axis=1), BF16)

        wq = jnp.concatenate([weight(wq_b), jnp.zeros((2 * D - M, D), F32)], axis=0)
        qscale = (D ** -0.5) * math.log2(math.e)
        q = (assemble(*_strassen(x_term, _rhs_terms(*quads(wq, D)))) * qscale).astype(BF16)

        k = assemble(*_strassen(c_term, _rhs_terms(*quads(weight(wk_b), DC // 2)))).astype(BF16)

        def scores(i):
            return lax.dot_general(q[i * TQ:(i + 1) * TQ], k[:(i + 1) * TQ], NT,
                                   preferred_element_type=F32)

        pending = {}
        for n in range(PRE_S):
            pending[ORDER[n]] = scores(ORDER[n])
        v = assemble(*_strassen(c_term, _rhs_terms(*quads(weight(wv_b), DC // 2)))).astype(BF16)

        r0 = pl.multiple_of(jnp.minimum(h, M // CROWS - 1) * CROWS, CROWS)
        cre = cre_v[pl.ds(r0, CROWS), :].astype(F32)
        cim = cim_v[pl.ds(r0, CROWS), :].astype(F32)
        cr = coef_v[0, 0:1, :]
        ci = coef_v[1, 0:1, :]
        c_r = cre * cr - cim * ci
        c_i = -(cre * ci + cim * cr)
        ccat_v[pl.ds(r0, CROWS), :] = jnp.concatenate(
            [c_r[:, :MA], c_i[:, :MA], c_r[:, MA:], c_i[:, MA:]], axis=1).astype(BF16)

        t0 = lax.bitwise_and(h, H // 2 - 1) * STEPS
        never = never_v[...] != 0
        a_r = [a_v[t] for t in range(4)]
        a_i = [a_v[4 + t] for t in range(4)]
        hr = [st_v[t] for t in range(4)]
        hi = [st_v[4 + t] for t in range(4)]

        def scan_steps(j0, n, hr, hi):
            for j in range(j0, j0 + n):
                us = [u_v[kk, pl.ds(t0 + j, NSEG, stride=SEG_STRIDE), :] for kk in range(8)]
                mr, mi = _cmul(a_r, a_i, hr, hi)
                hr = [mr[0] + us[0], mr[1] + us[1], mr[2] + us[2], mr[3] + us[6]]
                hi = [mi[0] + us[3], mi[1] + us[4], mi[2] + us[5], mi[3] + us[7]]
                r0 = pl.multiple_of((t0 + j) * NSEG, NSEG)
                for kk, val in enumerate(hr[:3] + hi[:3] + [hr[3]]):
                    h_v[kk, pl.ds(r0, NSEG), :] = val
            return hr, hi

        causal = (lax.broadcasted_iota(jnp.int32, (TQ, TQ), 1)
                  <= lax.broadcasted_iota(jnp.int32, (TQ, TQ), 0))
        wot = wot_v[h]

        ctxs = []
        for n, i in enumerate(ORDER):
            for nn in range(n, min(n + LOOK + 1, NB)):
                if ORDER[nn] not in pending:
                    pending[ORDER[nn]] = scores(ORDER[nn])
            s = pending[i]
            hr = [jnp.where(never, s[8 * t:8 * t + 8, 0:128], hr[t]) for t in range(4)]
            hr, hi = scan_steps(n * (STEPS // NB), STEPS // NB, hr, hi)
            diag = jnp.where(causal, s[:, i * TQ:], -1e9)
            if i > 0:
                s = jnp.concatenate([s[:, :i * TQ], diag], axis=1)
            else:
                s = diag
            m = jnp.max(s, axis=1, keepdims=True)
            p = jnp.exp2(s - m)
            l = jnp.sum(p, axis=1, keepdims=True)
            ctx = jnp.dot(p.astype(BF16), v[:(i + 1) * TQ], preferred_element_type=F32)
            ctxs.append((ctx * (1.0 / l)).astype(BF16))
            if n >= O_LAG:
                out_proj(wot, ORDER[n - O_LAG], ctxs[n - O_LAG])
        for t in range(4):
            st_v[t] = hr[t]
            st_v[4 + t] = hi[t]
        for e in range(O_LAG):
            ctxc_v[e] = ctxs[NB - O_LAG + e]
        return 0

    with jax.named_scope('heads'):
        lax.fori_loop(0, H, head, 0)

    @jax.named_scope('epilogue')
    def _epilogue():
        for cp in w_copies(jnp.int32(H - 1), H, 0):
            cp.wait()
        wot = wot_v[H - 1]
        for e in range(O_LAG):
            out_proj(wot, ORDER[NB - O_LAG + e], ctxc_v[e])

        def o_copy(s):
            cols = pl.ds(pl.multiple_of(s * LSEG, LSEG), LSEG)
            return pltpu.make_async_copy(acc_v.at[:, cols], out_hbm.at[:, cols], sem.at[0])

        def out_step(it, _):
            c_cat = ccat_v[...]
            for e in range(EC):
                s = it * EC + e
                cols = pl.ds(pl.multiple_of(s * LSEG, LSEG), LSEG)
                hs = jnp.concatenate(
                    [h_v[kk, pl.ds(s, LSEG, stride=NSEG), :] for kk in range(7)],
                    axis=1).astype(BF16)
                yt = lax.dot_general(c_cat, hs, NT, preferred_element_type=F32)
                xf = xt_v[:, cols].astype(F32)
                dsk = jnp.concatenate([col_v[0]] * (LSEG // 128), axis=1)
                gw = jnp.concatenate([col_v[1]] * (LSEG // 128), axis=1)
                g = jax.nn.sigmoid(jnp.sum(xf * gw, axis=0, keepdims=True))
                acc_v[:, cols] = g * acc_v[:, cols] + (1.0 - g) * (yt + xf * dsk)
                o_copy(s).start()
            return 0

        lax.fori_loop(0, NSEG // EC, out_step, 0)
        for s in range(NSEG):
            o_copy(s).wait()

    _epilogue()


@jax.jit
def pallas_gated_mix__compressed_kv_cla__ssm_conv_s5__prompt_kernel(
    A_x: jax.Array,
    A_c_kv: jax.Array,
    A_w_q: jax.Array,
    A_w_uk: jax.Array,
    A_w_uv: jax.Array,
    A_w_o: jax.Array,
    B_x: jax.Array,
    B_Lambda_re: jax.Array,
    B_Lambda_im: jax.Array,
    B_B_re: jax.Array,
    B_B_im: jax.Array,
    B_C_re: jax.Array,
    B_C_im: jax.Array,
    B_log_dt: jax.Array,
    B_Dskip: jax.Array,
    gate_w: jax.Array,
):
    del B_x
    hbm_spec = pl.BlockSpec(memory_space=pltpu.HBM)
    out_t = pl.pallas_call(
        _kernel,
        in_specs=[hbm_spec] * 15,
        out_specs=hbm_spec,
        out_shape=jax.ShapeDtypeStruct((M, S), F32),
        scratch_shapes=[
            pltpu.VMEM((M, S), BF16),
            pltpu.VMEM((7, 2, HS // 2, 128), U32),
            pltpu.VMEM((S, DC), BF16),
            pltpu.VMEM((7, 4, HS // 2, 128), U32),
            pltpu.VMEM((H + 1, M, D), BF16),
            pltpu.VMEM((2, M, D), U32),
            pltpu.VMEM((2, DC, D), U32),
            pltpu.VMEM((2, DC, D), U32),
            pltpu.VMEM((2 * M, M), BF16),
            pltpu.VMEM((M, M), BF16),
            pltpu.VMEM((M, M), BF16),
            pltpu.VMEM((M, 2 * M), BF16),
            pltpu.VMEM((M,), BF16), pltpu.VMEM((M,), BF16), pltpu.VMEM((M,), BF16),
            pltpu.VMEM((M,), BF16), pltpu.VMEM((M,), BF16),
            pltpu.VMEM((2, M, 128), F32),
            pltpu.VMEM((2, 8, M), F32),
            pltpu.VMEM((8, NSEG * SEG_STRIDE, 128), F32),
            pltpu.VMEM((7, S, 128), F32),
            pltpu.VMEM((8, NSEG, 128), F32),
            pltpu.VMEM((8, NSEG, 128), F32),
            pltpu.VMEM((M, S), F32),
            pltpu.VMEM((O_LAG, TQ, D), BF16),
            pltpu.VMEM((8, 128), jnp.int32),
            pltpu.SemaphoreType.DMA((SEM_X + NPRO + 1,)),
        ],
        compiler_params=pltpu.CompilerParams(vmem_limit_bytes=110 * 1024 * 1024),
        name="gated_mix",
    )(
        A_x.reshape(S, M).T, A_c_kv.reshape(S, DC),
        A_w_q, A_w_uk, A_w_uv, jnp.swapaxes(A_w_o, 1, 2),
        B_Lambda_re, B_Lambda_im, B_B_re, B_B_im, B_C_re, B_C_im, B_log_dt,
        B_Dskip, gate_w,
    )
    return out_t.T.reshape(1, S, M)
```

```python
import functools
import math
import os

import jax
import jax.numpy as jnp
from jax import lax
import jax.experimental.pallas as pl
import jax.experimental.pallas.tpu as pltpu

F32 = jnp.float32
BF16 = jnp.bfloat16
U32 = jnp.uint32

S = 2048
HS = S // 2
M = 448
DC = 1024
H = 16
D = 256
TQ = 128
NB = S // TQ
NS = NB // 2
NSEG = 8
LSEG = S // NSEG
SEG_STRIDE = LSEG + 8
STEPS = 2 * LSEG // H
MA = 384
MR = M - MA
NT = (((1,), (1,)), ((), ()))
O_LAG = int(os.environ.get('O_LAG', 1))
NPRO = NSEG // 2
EC = 4
_om = os.environ.get('ORDER', 'desc')
if _om == 'asc':
    ORDER = list(range(NS))
elif _om == 'desc':
    ORDER = list(range(NS))[::-1]
else:
    ORDER = [int(t) for t in _om.split(',')]
LOOK = int(os.environ.get('LOOK', 1))
PRE_S = int(os.environ.get('PRE_S', 2))
KV_JOINT = int(os.environ.get('KV_JOINT', 0))
SEM_W = 3
SEM_X = 5
PV_K = int(os.environ.get('PV_K', 256))
O_SPLIT = int(os.environ.get('O_SPLIT', 0))
O_POS = int(os.environ.get('O_POS', 1))
S_AB = int(os.environ.get('S_AB', 1))
PV_SEQ = int(os.environ.get('PV_SEQ', 0))
S_AT = int(os.environ.get('S_AT', 6))
PINS = [int(t) for t in os.environ.get('PINS', '2222222')]
RCP_EUP = int(os.environ.get('RCP_EUP', 1))
MG = int(os.environ.get('MG', 1))
MLAG = int(os.environ.get('MLAG', 2))
SG = int(os.environ.get('SG', 0))
SLAG = int(os.environ.get('SLAG', 1))
D_FIRST = int(os.environ.get('D_FIRST', 0))
HEAD = int(os.environ.get('HEAD', 2))
BPIN = int(os.environ.get('BPIN', 0))
BLAG = int(os.environ.get('BLAG', 1))
BALT = int(os.environ.get('BALT', 1))
DSUM = int(os.environ.get('DSUM', 1))
DS0 = int(os.environ.get('DS0', 0))
DS1 = int(os.environ.get('DS1', 2))
O_TOP = int(os.environ.get('O_TOP', 1))
DMAX = int(os.environ.get('DMAX', 1))
DM0 = int(os.environ.get('DM0', 0))
DM1 = int(os.environ.get('DM1', 1))
CROWS = 32


def _lhs_terms(a11, a12, a21, a22):
    return [t.astype(BF16) for t in
            (a11 + a22, a21 + a22, a11, a22, a11 + a12, a21 - a11, a12 - a22)]


def _rhs_terms(b11, b12, b21, b22):
    return [t.astype(BF16) for t in
            (b11 + b22, b11, b12 - b22, b21 - b11, b22, b11 + b12, b21 + b22)]


def _strassen(lhs, rhs):
    def mm(i):
        return jnp.dot(lhs(i), rhs[i], preferred_element_type=F32)
    m1 = mm(0)
    m4 = mm(3)
    c11 = m1 + m4
    m2 = mm(1)
    c21 = m2 + m4
    c22 = m1 - m2
    m5 = mm(4)
    c11 = c11 - m5
    m3 = mm(2)
    c12 = m3 + m5
    c22 = c22 + m3
    c11 = c11 + mm(6)
    c22 = c22 + mm(5)
    return c11, c12, c21, c22


def _recip(l):
    if RCP_EUP:
        r = pl.reciprocal(l, approx=True)
        return r * (2.0 - l * r)
    r = pltpu.bitcast(jnp.int32(0x7EF311C3) - pltpu.bitcast(l, jnp.int32), F32)
    for _ in range(3):
        r = r * (2.0 - l * r)
    return r


def _cmul(pr, pi, hr, hi):
    return ([pr[t] * hr[t] - pi[t] * hi[t] for t in range(4)],
            [pr[t] * hi[t] + pi[t] * hr[t] for t in range(4)])


def _column(row):
    row = jnp.concatenate([row, jnp.zeros((1, 512 - M), F32)], axis=1)
    return jnp.broadcast_to(row, (128, 512)).T[:M]


def _kernel(xt_hbm, c_hbm, wq_hbm, wk_hbm, wv_hbm, wot_hbm,
            lre_hbm, lim_hbm, bre_hbm, bim_hbm, cre_hbm, cim_hbm, ldt_hbm,
            dsk_hbm, gw_hbm,
            out_hbm,
            xt_v, xs_v, c_v, cs_v, wot_v, wq_b, wk_b, wv_b, bcat_v, cre_v, cim_v, ccat_v,
            lre_v, lim_v, ldt_v, dsk_v, gw_v, col_v, coef_v,
            u_v, h_v, a_v, st_v, acc_v, ctxc_v, never_v, sem):
    wq32 = wq_hbm.bitcast(U32)
    wk32 = wk_hbm.bitcast(U32)
    wv32 = wv_hbm.bitcast(U32)

    def w_copies(h, h_dst, sl):
        j = lax.shift_right_logical(h, 1)
        cps = [pltpu.make_async_copy(src.at[:, j, :], dst.at[sl], sem.at[SEM_W + sl])
               for src, dst in ((wq32, wq_b), (wk32, wk_b), (wv32, wv_b))]
        return cps + [pltpu.make_async_copy(wot_hbm.at[h], wot_v.at[h_dst], sem.at[SEM_W + sl])]

    def x_copies(s):
        spans = [pl.ds(pl.multiple_of(s * LSEG + e * HS, LSEG), LSEG) for e in range(2)]
        return [pltpu.make_async_copy(xt_hbm.at[:, sp], xt_v.at[:, sp], sem.at[SEM_X + s])
                for sp in spans]

    def c_copies(s):
        spans = [pl.ds(pl.multiple_of(s * LSEG + e * HS, LSEG), LSEG) for e in range(2)]
        return [pltpu.make_async_copy(c_hbm.at[sp], c_v.at[sp], sem.at[SEM_X + 1 + s])
                for sp in spans]

    b_cps = [
        pltpu.make_async_copy(bre_hbm.at[0:MA], bcat_v.at[0:MA], sem.at[SEM_X]),
        pltpu.make_async_copy(bim_hbm.at[0:MA], bcat_v.at[MA:2 * MA], sem.at[SEM_X]),
        pltpu.make_async_copy(bre_hbm.at[MA:M], bcat_v.at[2 * MA:2 * MA + MR], sem.at[SEM_X]),
        pltpu.make_async_copy(bim_hbm.at[MA:M], bcat_v.at[2 * MA + MR:2 * M], sem.at[SEM_X]),
    ]
    vec_cps = [pltpu.make_async_copy(src, dst, sem.at[1]) for src, dst in
               ((lre_hbm, lre_v), (lim_hbm, lim_v), (ldt_hbm, ldt_v), (dsk_hbm, dsk_v),
                (gw_hbm, gw_v))]
    late_cps = [pltpu.make_async_copy(cre_hbm, cre_v, sem.at[2]),
                pltpu.make_async_copy(cim_hbm, cim_v, sem.at[2])]

    @jax.named_scope('prologue')
    def _prologue():
        zero = jnp.int32(0)
        first = vec_cps + x_copies(0) + b_cps
        for s in range(1, NPRO):
            first = first + x_copies(s) + c_copies(s - 1)
        for cp in first + c_copies(NPRO - 1) + w_copies(zero, 0, 0) + late_cps:
            cp.start()
        acc_v[...] = jnp.zeros_like(acc_v)
        st_v[...] = jnp.zeros_like(st_v)
        ctxc_v[...] = jnp.zeros_like(ctxc_v)
        never_v[...] = jnp.zeros_like(never_v)

        for cp in vec_cps:
            cp.wait()
        lre = lre_v[...].astype(F32).reshape(1, M)
        lim = lim_v[...].astype(F32).reshape(1, M)
        dt = jnp.exp(ldt_v[...].astype(F32)).astype(BF16).astype(F32).reshape(1, M)
        er = jnp.exp(dt * lre)
        ar = er * jnp.cos(dt * lim)
        ai = er * jnp.sin(dt * lim)
        den = lre * lre + lim * lim
        coef_v[0] = jnp.broadcast_to(2.0 * ((ar - 1.0) * lre + ai * lim) / den, (8, M))
        coef_v[1] = jnp.broadcast_to(2.0 * (ai * lre - (ar - 1.0) * lim) / den, (8, M))

        def bc(v):
            return jnp.broadcast_to(v, (NSEG, 128))

        for t in range(3):
            a_v[t] = bc(ar[:, t * 128:(t + 1) * 128])
            a_v[4 + t] = bc(ai[:, t * 128:(t + 1) * 128])
        a_v[3] = bc(jnp.concatenate([ar[:, MA:], ar[:, MA:]], axis=1))
        a_v[7] = bc(jnp.concatenate([ai[:, MA:], -ai[:, MA:]], axis=1))
        col_v[0] = _column(dsk_v[...].astype(F32).reshape(1, M))
        col_v[1] = _column(gw_v[...].astype(F32).reshape(1, M))

        never = never_v[...] != 0

        def bu(s):
            b_cat = bcat_v[...]
            r = pl.ds(pl.multiple_of(s * (LSEG // 2), LSEG // 2), LSEG // 2)
            xs = []
            us = []
            for e in range(2):
                c0 = pl.multiple_of(s * LSEG + e * HS, LSEG)
                xe = xt_v[:, pl.ds(c0, LSEG)].T
                u = lax.dot_general(xe, b_cat, NT, preferred_element_type=F32)
                us.append(u)
                rows = pl.ds(pl.multiple_of((s + e * NPRO) * SEG_STRIDE, 8), LSEG)
                u_v[7, rows, :] = pltpu.roll(u[:, 2 * MA:], MR, 1)
                for t in range(7):
                    u_v[t, rows, :] = u[:, t * 128:(t + 1) * 128]
                xe = xe.astype(F32)
                xs.append((xe[:, :D], jnp.concatenate(
                    [xe[:, D:], jnp.zeros((LSEG, 2 * D - M), F32)], axis=1)))
            for i, t in enumerate(_lhs_terms(xs[0][0], xs[0][1], xs[1][0], xs[1][1])):
                t = pltpu.bitcast(t, U32)
                for kt in range(2):
                    xs_v[i, kt, r, :] = t[:, kt * 128:(kt + 1) * 128]
            return us

        def c_terms(s, us):
            hc = DC // 2
            r = pl.ds(pl.multiple_of(s * (LSEG // 2), LSEG // 2), LSEG // 2)
            rt = pl.ds(pl.multiple_of(s * LSEG, LSEG), LSEG)
            rb = pl.ds(pl.multiple_of(s * LSEG + HS, LSEG), LSEG)
            a11, a12, a21, a22 = c_v[rt, :hc], c_v[rt, hc:], c_v[rb, :hc], c_v[rb, hc:]
            if us is not None:
                cols = []
                for kt in range(4):
                    vr = []
                    for g in range(16):
                        n = ((kt * 16 + g) * 13) // 2
                        e, t, rg = n // 224, (n % 224) // 32, n % 32
                        vr.append(us[e][8 * rg:8 * rg + 8, 128 * t:128 * t + 128])
                    cols.append(jnp.concatenate(vr, axis=0))
                dep = pltpu.bitcast(jnp.concatenate(cols, axis=1), U32)
                nv = jnp.concatenate([jnp.concatenate([never] * 16, axis=0)] * 4, axis=1)
                a11 = pltpu.bitcast(jnp.where(nv, dep, pltpu.bitcast(a11, U32)), BF16)
                a22 = pltpu.bitcast(jnp.where(nv, dep, pltpu.bitcast(a22, U32)), BF16)
            terms = _lhs_terms(*(a.astype(F32) for a in (a11, a12, a21, a22)))
            for i, t in enumerate(terms):
                t = pltpu.bitcast(t, U32)
                for kt in range(4):
                    cs_v[i, kt, r, :] = t[:, kt * 128:(kt + 1) * 128]

        for cp in x_copies(0) + b_cps:
            cp.wait()
        bu(0)

        def pro_step(s, _):
            for cp in x_copies(s) + c_copies(s - 1):
                cp.wait()
            c_terms(s - 1, bu(s))
            return 0

        lax.fori_loop(1, NPRO, pro_step, 0)
        for cp in c_copies(NPRO - 1):
            cp.wait()
        c_terms(NPRO - 1, None)
        for cp in late_cps:
            cp.wait()

    _prologue()

    def out_proj(wot, i, ctx):
        cols = slice(2 * i * TQ, (2 * i + 2) * TQ)
        o = lax.dot_general(wot, ctx, NT, preferred_element_type=F32)
        acc_v[:, cols] += o
        return o

    def head(h, _):
        slot = lax.bitwise_and(h, 1)

        @pl.when(h == H // 2)
        def _segment_carry():
            pr = [a_v[t] for t in range(4)]
            pi = [a_v[4 + t] for t in range(4)]
            for _ in range(int(math.log2(LSEG))):
                pr, pi = ([pr[t] * pr[t] - pi[t] * pi[t] for t in range(4)],
                          [2.0 * pr[t] * pi[t] for t in range(4)])
            row = lax.broadcasted_iota(jnp.int32, (NSEG, 128), 0)
            e_r = [st_v[t] for t in range(4)]
            e_i = [st_v[4 + t] for t in range(4)]
            ir = [jnp.zeros((NSEG, 128), F32)] * 4
            ii = ir
            for s in range(1, NSEG):
                mr, mi = _cmul(pr, pi, ir, ii)
                fr = [pltpu.roll(mr[k] + e_r[k], 1, 0) for k in range(4)]
                fi = [pltpu.roll(mi[k] + e_i[k], 1, 0) for k in range(4)]
                ir = [jnp.where(row == s, fr[k], ir[k]) for k in range(4)]
                ii = [jnp.where(row == s, fi[k], ii[k]) for k in range(4)]
            for t in range(4):
                st_v[t] = ir[t]
                st_v[4 + t] = ii[t]

        for cp in w_copies(h, h, slot):
            cp.wait()

        if O_TOP:
            wot_prev = wot_v[jnp.maximum(h - 1, 0)]
            o_prev = [lax.dot_general(wot_prev, ctxc_v[e], NT, preferred_element_type=F32)
                      for e in range(O_LAG)]
        for cp in w_copies(jnp.minimum(h + 1, H - 1), h + 1, 1 - slot):
            cp.start()
        for e in range(O_LAG if O_TOP else 0):
            i = ORDER[NS - O_LAG + e]
            acc_v[:, 2 * i * TQ:(2 * i + 2) * TQ] += o_prev[e]

        up = ((1 - slot) * 16).astype(U32)

        def weight(buf):
            return pltpu.bitcast((buf[slot] << up) & jnp.uint32(0xFFFF0000), F32)

        def quads(w, kh):
            return w[:kh, :128], w[:kh, 128:], w[kh:, :128], w[kh:, 128:]

        def assemble(c11, c12, c21, c22):
            return jnp.concatenate([jnp.concatenate([c11, c12], axis=1),
                                    jnp.concatenate([c21, c22], axis=1)], axis=0)

        def x_term(i):
            return pltpu.bitcast(jnp.concatenate([xs_v[i, kt] for kt in range(2)], axis=1), BF16)

        def c_term(i):
            return pltpu.bitcast(jnp.concatenate([cs_v[i, kt] for kt in range(4)], axis=1), BF16)

        wq = jnp.concatenate([weight(wq_b), jnp.zeros((2 * D - M, D), F32)], axis=0)
        qscale = (D ** -0.5) * math.log2(math.e)
        kf = assemble(*_strassen(c_term, _rhs_terms(*quads(weight(wk_b), DC // 2))))
        qf = assemble(*_strassen(x_term, _rhs_terms(*quads(wq, D)))) * qscale
        never = never_v[...] != 0

        def sup(a, j):
            return quads(a[2 * j * TQ:(2 * j + 2) * TQ], TQ)

        q = qf.astype(BF16)
        k = kf.astype(BF16)
        qt = [None] + [_lhs_terms(*sup(qf, j)) for j in range(1, NS)]
        kt = []
        for j in range(NS - 1):
            k11, k12, k21, k22 = sup(kf, j)
            kt.append(_rhs_terms(k11, k21, k12, k22))

        causal = (lax.broadcasted_iota(jnp.int32, (TQ, TQ), 1)
                  <= lax.broadcasted_iota(jnp.int32, (TQ, TQ), 0))

        def nt(a, b):
            return lax.dot_general(a, b, NT, preferred_element_type=F32)

        never64 = jnp.concatenate([never] * 8, axis=0)
        never128 = jnp.concatenate([never] * 16, axis=0)

        lpins = []

        def tmax(x):
            return jnp.maximum(x[:, :TQ], x[:, TQ:]) if x.shape[1] > TQ else x

        def score_jobs(i):
            top, bot = [None] * (i + 1), [None] * (i + 1)
            mx = [None, None]
            tmp = {}
            hist = []

            def note(half, x):
                mx[half] = tmax(x) if mx[half] is None else jnp.maximum(mx[half], tmax(x))

            def job_a(j):
                lhs = [qt[i][t] for t in (1, 2, 3, 4)]
                jj = j - MLAG
                if MG and jj >= 0 and jj % MG == MG - 1:
                    pins = [pltpu.bitcast(x, U32) for x in hist[jj]]
                    pins = [pins[0][:64], pins[0][64:], pins[1][:64], pins[1][64:]]
                    lhs = [pltpu.bitcast(jnp.where(never64, pn, pltpu.bitcast(x, U32)), BF16)
                           for pn, x in zip(pins, lhs)]
                m2, m3, m4, m5 = (nt(x, kt[j][t]) for x, t in zip(lhs, (1, 2, 3, 4)))
                tmp[j] = (m4 - m5, m3 + m5, m2 + m4, m3 - m2)

            def job_b(j):
                t11, c12, c21, t22 = tmp.pop(j)
                lhs = [qt[i][t] for t in (0, 5, 6)]
                if BPIN and len(lpins) > BLAG + 1:
                    pn = pltpu.bitcast(lpins[-1 - BLAG - (j % 2 if BALT else 0)], U32)
                    lhs[1:] = [pltpu.bitcast(jnp.where(never64, x, pltpu.bitcast(y, U32)), BF16)
                               for x, y in zip((pn[:64], pn[64:]), lhs[1:])]
                m1, m6, m7 = (nt(x, kt[j][t]) for x, t in zip(lhs, (0, 5, 6)))
                top[j] = jnp.concatenate([t11 + (m1 + m7), c12], axis=1)
                bot[j] = jnp.concatenate([c21, t22 + (m1 + m6)], axis=1)
                note(0, top[j])
                note(1, bot[j])
                hist.append(tuple(mx))

            def diag_b():
                r0 = 2 * i * TQ
                sb = nt(q[r0 + TQ:r0 + 2 * TQ], k[r0:r0 + 2 * TQ])
                bot[i] = jnp.concatenate(
                    [sb[:, :TQ], jnp.where(causal, sb[:, TQ:], -1e9)], axis=1)
                note(1, bot[i])

            def diag_t():
                r0 = 2 * i * TQ
                top[i] = jnp.where(causal, nt(q[r0:r0 + TQ], k[r0:r0 + TQ]), -1e9)
                note(0, top[i])

            jobs = []
            for j in range(i):
                jobs += [functools.partial(job_a, j), functools.partial(job_b, j)]
            if D_FIRST:
                return (top, bot, mx, hist), [diag_b, diag_t] + jobs
            return (top, bot, mx, hist), jobs + [diag_b, diag_t]

        pending = {}
        calls = [0]
        never_col = jnp.concatenate([never] * 56, axis=0)
        pin_list = [kt[j] for j in range(NS - 1)] + [qt[j] for j in range(NS - 1, 0, -1)]

        def v_lhs(i):
            n = calls[0]
            calls[0] += 1
            if n == S_AT:
                for nn in range(LOOK):
                    pending[ORDER[nn]], jobs = score_jobs(ORDER[nn])
                    for job in jobs:
                        job()
            cols = [cs_v[i, kt_] for kt_ in range(4)]
            for c in range(PINS[n]):
                pin = jnp.concatenate([pltpu.bitcast(t, U32) for t in pin_list.pop(0)], axis=0)
                cols[c] = jnp.concatenate(
                    [cols[c][:64], jnp.where(never_col, pin, cols[c][64:])], axis=0)
            return pltpu.bitcast(jnp.concatenate(cols, axis=1), BF16)

        v = assemble(*_strassen(v_lhs, _rhs_terms(*quads(weight(wv_b), DC // 2)))).astype(BF16)

        r0 = pl.multiple_of(jnp.minimum(h, M // CROWS - 1) * CROWS, CROWS)
        cre = cre_v[pl.ds(r0, CROWS), :].astype(F32)
        cim = cim_v[pl.ds(r0, CROWS), :].astype(F32)
        cr = coef_v[0, 0:1, :]
        ci = coef_v[1, 0:1, :]
        c_r = cre * cr - cim * ci
        c_i = -(cre * ci + cim * cr)
        ccat_v[pl.ds(r0, CROWS), :] = jnp.concatenate(
            [c_r[:, :MA], c_i[:, :MA], c_r[:, MA:], c_i[:, MA:]], axis=1).astype(BF16)

        t0 = lax.bitwise_and(h, H // 2 - 1) * STEPS
        a_r = [a_v[t] for t in range(4)]
        a_i = [a_v[4 + t] for t in range(4)]
        hr = [st_v[t] for t in range(4)]
        hi = [st_v[4 + t] for t in range(4)]

        def scan_steps(j0, n, hr, hi):
            for j in range(j0, j0 + n):
                us = [u_v[kk, pl.ds(t0 + j, NSEG, stride=SEG_STRIDE), :] for kk in range(8)]
                mr, mi = _cmul(a_r, a_i, hr, hi)
                hr = [mr[0] + us[0], mr[1] + us[1], mr[2] + us[2], mr[3] + us[6]]
                hi = [mi[0] + us[3], mi[1] + us[4], mi[2] + us[5], mi[3] + us[7]]
                r0 = pl.multiple_of((t0 + j) * NSEG, NSEG)
                for kk, val in enumerate(hr[:3] + hi[:3] + [hr[3]]):
                    h_v[kk, pl.ds(r0, NSEG), :] = val
            return hr, hi

        wot = wot_v[h]

        def normalise(ls, ctx, tiles, o):
            if DSUM and o is not None:
                ls = []
                for half, tl in enumerate(tiles):
                    dep = jnp.concatenate(
                        [o[8 * (DS0 + g * DS1):8 * (DS0 + g * DS1) + 8, half * TQ:(half + 1) * TQ]
                         for g in range(16)], axis=0)
                    l = jnp.where(never128, dep, tl[0])
                    for t in tl[1:]:
                        l = l + t
                    ls.append(l)
            out = [c * _recip(jnp.sum(l, axis=1, keepdims=True)) for l, c in zip(ls, ctx)]
            return jnp.concatenate(out, axis=0).astype(BF16)

        ctxs = []
        o = None
        for n, i in enumerate(ORDER):
            ms = []
            cur = pending.pop(i)
            for half in range(2):
                s = cur[half][0]
                hr = [jnp.where(never, s[8 * t:8 * t + 8, 0:128], hr[t]) for t in range(4)]
                hr, hi = scan_steps((2 * n + half) * (STEPS // NB), STEPS // NB, hr, hi)
                mx = cur[2][half]
                if DMAX and o is not None and i > 0:
                    done = max(i - MLAG, 0)
                    dep = jnp.concatenate(
                        [o[8 * (DM0 + g * DM1):8 * (DM0 + g * DM1) + 8, half * TQ:(half + 1) * TQ]
                         for g in range(16)], axis=0)
                    rest = [x[:, c * TQ:(c + 1) * TQ] for x in cur[half][done:]
                            for c in range(x.shape[1] // TQ)]
                    if done:
                        rest = [cur[3][done - 1][half]] + rest
                    mx = jnp.where(never128, dep, rest[0])
                    for t in rest[1:]:
                        mx = jnp.maximum(mx, t)
                ms.append(jnp.max(mx, axis=1, keepdims=True))
            if n >= 1:
                ctxs[n - 1] = normalise(*ctxs[n - 1])
            todo = []
            if n + LOOK < NS:
                pending[ORDER[n + LOOK]], todo = score_jobs(ORDER[n + LOOK])
            for _ in range(HEAD):
                if todo:
                    todo.pop(0)()
            ctx = [None, None]
            ls = [None, None]
            lhist = []
            tiles = [[], []]
            o = None
            if PV_SEQ:
                seq = [(half, j) for half in range(2) for j in range(i + 1)]
            else:
                seq = [(half, j) for j in range(i + 1) for half in range(2)]
            for cn, (half, j) in enumerate(seq):
                if todo:
                    todo.pop(0)()
                p = jnp.exp2(cur[half][j] - ms[half])
                psum = p[:, :TQ] + p[:, TQ:] if p.shape[1] > TQ else p
                ls[half] = psum if ls[half] is None else ls[half] + psum
                lhist.append((ls[half], j))
                tiles[half] += [p[:, c * TQ:(c + 1) * TQ] for c in range(p.shape[1] // TQ)]
                lpins.append(ls[half])
                cc = cn - SLAG
                if SG and cc >= 0 and lhist[cc][1] % SG == SG - 1:
                    last = jnp.where(never128, lhist[cc][0], p[:, -TQ:])
                    p = jnp.concatenate([p[:, :TQ], last], axis=1) if p.shape[1] > TQ else last
                j0 = j * 2 * TQ
                part = jnp.dot(p.astype(BF16), v[j0:j0 + p.shape[1]], preferred_element_type=F32)
                ctx[half] = part if ctx[half] is None else ctx[half] + part
                if n >= O_LAG and cn == (len(seq) - 1 if O_POS else 0):
                    o = out_proj(wot, ORDER[n - O_LAG], ctxs[n - O_LAG])
                if n < O_LAG and not O_TOP and cn == len(seq) - 1:
                    o = out_proj(wot_v[jnp.maximum(h - 1, 0)], ORDER[NS - O_LAG + n], ctxc_v[n])
            for job in todo:
                job()
            ctxs.append((ls, ctx, tiles, o if n < NS - 1 else None))
        ctxs[NS - 1] = normalise(*ctxs[NS - 1])
        for t in range(4):
            st_v[t] = hr[t]
            st_v[4 + t] = hi[t]
        for e in range(O_LAG):
            ctxc_v[e] = ctxs[NS - O_LAG + e]
        return 0

    with jax.named_scope('heads'):
        lax.fori_loop(0, H, head, 0)

    @jax.named_scope('epilogue')
    def _epilogue():
        for cp in w_copies(jnp.int32(H - 1), H, 0):
            cp.wait()
        wot = wot_v[H - 1]
        for e in range(O_LAG):
            out_proj(wot, ORDER[NS - O_LAG + e], ctxc_v[e])

        def o_copy(s):
            cols = pl.ds(pl.multiple_of(s * LSEG, LSEG), LSEG)
            return pltpu.make_async_copy(acc_v.at[:, cols], out_hbm.at[:, cols], sem.at[0])

        def out_step(it, _):
            c_cat = ccat_v[...]
            for e in range(EC):
                s = it * EC + e
                cols = pl.ds(pl.multiple_of(s * LSEG, LSEG), LSEG)
                hs = jnp.concatenate(
                    [h_v[kk, pl.ds(s, LSEG, stride=NSEG), :] for kk in range(7)],
                    axis=1).astype(BF16)
                yt = lax.dot_general(c_cat, hs, NT, preferred_element_type=F32)
                xf = xt_v[:, cols].astype(F32)
                dsk = jnp.concatenate([col_v[0]] * (LSEG // 128), axis=1)
                gw = jnp.concatenate([col_v[1]] * (LSEG // 128), axis=1)
                g = jax.nn.sigmoid(jnp.sum(xf * gw, axis=0, keepdims=True))
                acc_v[:, cols] = g * acc_v[:, cols] + (1.0 - g) * (yt + xf * dsk)
                o_copy(s).start()
            return 0

        lax.fori_loop(0, NSEG // EC, out_step, 0)
        for s in range(NSEG):
            o_copy(s).wait()

    _epilogue()


@jax.jit
def pallas_gated_mix__compressed_kv_cla__ssm_conv_s5__prompt_kernel(
    A_x: jax.Array,
    A_c_kv: jax.Array,
    A_w_q: jax.Array,
    A_w_uk: jax.Array,
    A_w_uv: jax.Array,
    A_w_o: jax.Array,
    B_x: jax.Array,
    B_Lambda_re: jax.Array,
    B_Lambda_im: jax.Array,
    B_B_re: jax.Array,
    B_B_im: jax.Array,
    B_C_re: jax.Array,
    B_C_im: jax.Array,
    B_log_dt: jax.Array,
    B_Dskip: jax.Array,
    gate_w: jax.Array,
):
    del B_x
    hbm_spec = pl.BlockSpec(memory_space=pltpu.HBM)
    out_t = pl.pallas_call(
        _kernel,
        in_specs=[hbm_spec] * 15,
        out_specs=hbm_spec,
        out_shape=jax.ShapeDtypeStruct((M, S), F32),
        scratch_shapes=[
            pltpu.VMEM((M, S), BF16),
            pltpu.VMEM((7, 2, HS // 2, 128), U32),
            pltpu.VMEM((S, DC), BF16),
            pltpu.VMEM((7, 4, HS // 2, 128), U32),
            pltpu.VMEM((H + 1, M, D), BF16),
            pltpu.VMEM((2, M, D), U32),
            pltpu.VMEM((2, DC, D), U32),
            pltpu.VMEM((2, DC, D), U32),
            pltpu.VMEM((2 * M, M), BF16),
            pltpu.VMEM((M, M), BF16),
            pltpu.VMEM((M, M), BF16),
            pltpu.VMEM((M, 2 * M), BF16),
            pltpu.VMEM((M,), BF16), pltpu.VMEM((M,), BF16), pltpu.VMEM((M,), BF16),
            pltpu.VMEM((M,), BF16), pltpu.VMEM((M,), BF16),
            pltpu.VMEM((2, M, 128), F32),
            pltpu.VMEM((2, 8, M), F32),
            pltpu.VMEM((8, NSEG * SEG_STRIDE, 128), F32),
            pltpu.VMEM((7, S, 128), F32),
            pltpu.VMEM((8, NSEG, 128), F32),
            pltpu.VMEM((8, NSEG, 128), F32),
            pltpu.VMEM((M, S), F32),
            pltpu.VMEM((O_LAG, 2 * TQ, D), BF16),
            pltpu.VMEM((8, 128), jnp.int32),
            pltpu.SemaphoreType.DMA((SEM_X + NPRO + 1,)),
        ],
        compiler_params=pltpu.CompilerParams(vmem_limit_bytes=110 * 1024 * 1024),
        name="gated_mix",
    )(
        A_x.reshape(S, M).T, A_c_kv.reshape(S, DC),
        A_w_q, A_w_uk, A_w_uv, jnp.swapaxes(A_w_o, 1, 2),
        B_Lambda_re, B_Lambda_im, B_B_re, B_B_im, B_C_re, B_C_im, B_log_dt,
        B_Dskip, gate_w,
    )
    return out_t.T.reshape(1, S, M)
```

```python
import functools
import math
import os

import jax
import jax.numpy as jnp
from jax import lax
import jax.experimental.pallas as pl
import jax.experimental.pallas.tpu as pltpu

F32 = jnp.float32
BF16 = jnp.bfloat16
U32 = jnp.uint32

S = 2048
HS = S // 2
M = 448
DC = 1024
H = 16
D = 256
TQ = 128
NB = S // TQ
NS = NB // 2
NSEG = 8
LSEG = S // NSEG
SEG_STRIDE = LSEG + 8
STEPS = 2 * LSEG // H
MA = 384
MR = M - MA
NT = (((1,), (1,)), ((), ()))
O_LAG = int(os.environ.get('O_LAG', 1))
NPRO = NSEG // 2
EC = int(os.environ.get('EC', 8))
_om = os.environ.get('ORDER', 'desc')
if _om == 'asc':
    ORDER = list(range(NS))
elif _om == 'desc':
    ORDER = list(range(NS))[::-1]
else:
    ORDER = [int(t) for t in _om.split(',')]
LOOK = int(os.environ.get('LOOK', 1))
PRE_S = int(os.environ.get('PRE_S', 2))
KV_JOINT = int(os.environ.get('KV_JOINT', 0))
SEM_W = 3
SEM_X = 5
PV_K = int(os.environ.get('PV_K', 256))
O_SPLIT = int(os.environ.get('O_SPLIT', 0))
O_POS = int(os.environ.get('O_POS', 1))
S_AB = int(os.environ.get('S_AB', 1))
PV_SEQ = int(os.environ.get('PV_SEQ', 0))
S_AT = int(os.environ.get('S_AT', 6))
PINS = [int(t) for t in os.environ.get('PINS', '2222222')]
RCP_EUP = int(os.environ.get('RCP_EUP', 1))
MG = int(os.environ.get('MG', 1))
MLAG = int(os.environ.get('MLAG', 2))
SG = int(os.environ.get('SG', 0))
SLAG = int(os.environ.get('SLAG', 1))
D_FIRST = int(os.environ.get('D_FIRST', 0))
HEAD = int(os.environ.get('HEAD', 1))
BPIN = int(os.environ.get('BPIN', 0))
BLAG = int(os.environ.get('BLAG', 1))
BALT = int(os.environ.get('BALT', 1))
DSUM = int(os.environ.get('DSUM', 1))
DS0 = int(os.environ.get('DS0', 0))
DS1 = int(os.environ.get('DS1', 2))
O_TOP = int(os.environ.get('O_TOP', 160))
DMAX = int(os.environ.get('DMAX', 1))
DM0 = int(os.environ.get('DM0', 0))
DM1 = int(os.environ.get('DM1', 1))
CW = 352
CSTEP = 336
XLO = int(os.environ.get('XLO', 40))
XHI = int(os.environ.get('XHI', 420))
CLO = int(os.environ.get('CLO', 0))
CHI = int(os.environ.get('CHI', 420))
DPIN = int(os.environ.get('DPIN', 1))
CROWS = 32


def _lhs_terms(a11, a12, a21, a22):
    return [t.astype(BF16) for t in
            (a11 + a22, a21 + a22, a11, a22, a11 + a12, a21 - a11, a12 - a22)]


def _rhs_terms(b11, b12, b21, b22):
    return [t.astype(BF16) for t in
            (b11 + b22, b11, b12 - b22, b21 - b11, b22, b11 + b12, b21 + b22)]


def _strassen(lhs, rhs):
    def mm(i):
        return jnp.dot(lhs(i), rhs[i], preferred_element_type=F32)
    m1 = mm(0)
    m4 = mm(3)
    c11 = m1 + m4
    m2 = mm(1)
    c21 = m2 + m4
    c22 = m1 - m2
    m5 = mm(4)
    c11 = c11 - m5
    m3 = mm(2)
    c12 = m3 + m5
    c22 = c22 + m3
    c11 = c11 + mm(6)
    c22 = c22 + mm(5)
    return c11, c12, c21, c22


def _recip(l):
    if RCP_EUP:
        r = pl.reciprocal(l, approx=True)
        return r * (2.0 - l * r)
    r = pltpu.bitcast(jnp.int32(0x7EF311C3) - pltpu.bitcast(l, jnp.int32), F32)
    for _ in range(3):
        r = r * (2.0 - l * r)
    return r


def _cmul(pr, pi, hr, hi):
    return ([pr[t] * hr[t] - pi[t] * hi[t] for t in range(4)],
            [pr[t] * hi[t] + pi[t] * hr[t] for t in range(4)])


def _column(row):
    row = jnp.concatenate([row, jnp.zeros((1, 512 - M), F32)], axis=1)
    return jnp.broadcast_to(row, (128, 512)).T[:M]


def _kernel(xt_hbm, c_hbm, wq_hbm, wk_hbm, wv_hbm, wot_hbm,
            lre_hbm, lim_hbm, bre_hbm, bim_hbm, cre_hbm, cim_hbm, ldt_hbm,
            dsk_hbm, gw_hbm,
            out_hbm,
            xt_v, xs_v, c_v, cs_v, wot_v, wq_b, wk_b, wv_b, bc_v, ccat_v,
            lre_v, lim_v, ldt_v, dsk_v, gw_v, col_v, coef_v,
            u_v, h_v, a_v, st_v, acc_v, ctxc_v, never_v, sem):
    wq32 = wq_hbm.bitcast(U32)
    wk32 = wk_hbm.bitcast(U32)
    wv32 = wv_hbm.bitcast(U32)
    wot32 = wot_hbm.bitcast(U32)

    def w_copies(h, h_dst, sl):
        j = lax.shift_right_logical(h, 1)
        cps = [pltpu.make_async_copy(src.at[:, j, :], dst.at[sl], sem.at[SEM_W + sl])
               for src, dst in ((wq32, wq_b), (wk32, wk_b), (wv32, wv_b))]
        return cps + [pltpu.make_async_copy(wot32.at[h], wot_v.at[h_dst], sem.at[SEM_W + sl])]

    def x_copies(s):
        spans = [pl.ds(pl.multiple_of(s * LSEG + e * HS, LSEG), LSEG) for e in range(2)]
        return [pltpu.make_async_copy(xt_hbm.at[:, sp], xt_v.at[:, sp], sem.at[SEM_X + s])
                for sp in spans]

    def c_copies(start, rows, s):
        spans = [pl.ds(pl.multiple_of(start + e * HS, 16), rows) for e in range(2)]
        return [pltpu.make_async_copy(c_hbm.at[sp], c_v.at[sp], sem.at[SEM_X + s])
                for sp in spans]

    def stage_copies(s):
        return x_copies(s) + c_copies(CW - CSTEP + (s - 1) * CSTEP, CSTEP, s)

    first_cps = x_copies(0) + [
        pltpu.make_async_copy(bre_hbm.at[MA:M], bc_v.at[0:MR], sem.at[SEM_X]),
        pltpu.make_async_copy(bim_hbm.at[MA:M], bc_v.at[MR:2 * MR], sem.at[SEM_X]),
        pltpu.make_async_copy(bre_hbm.at[0:MA], bc_v.at[2 * MR:2 * MR + MA], sem.at[SEM_X]),
        pltpu.make_async_copy(bim_hbm.at[0:MA], bc_v.at[2 * MR + MA:2 * M], sem.at[SEM_X]),
    ] + c_copies(0, CW - CSTEP, 0)
    vec_cps = [pltpu.make_async_copy(src, dst, sem.at[1]) for src, dst in
               ((lre_hbm, lre_v), (lim_hbm, lim_v), (ldt_hbm, ldt_v), (dsk_hbm, dsk_v),
                (gw_hbm, gw_v))]
    late_cps = [pltpu.make_async_copy(cre_hbm, bc_v.at[2 * M:3 * M], sem.at[2]),
                pltpu.make_async_copy(cim_hbm, bc_v.at[3 * M:4 * M], sem.at[2])]

    @jax.named_scope('prologue')
    def _prologue():
        zero = jnp.int32(0)
        first = vec_cps + first_cps
        for s in range(1, NPRO):
            first = first + stage_copies(s)
        for cp in first + w_copies(zero, 0, 0) + late_cps:
            cp.start()
        acc_v[...] = jnp.zeros_like(acc_v)
        st_v[...] = jnp.zeros_like(st_v)
        ctxc_v[...] = jnp.zeros_like(ctxc_v)
        never_v[...] = jnp.zeros_like(never_v)

        for cp in vec_cps:
            cp.wait()
        lre = lre_v[...].astype(F32).reshape(1, M)
        lim = lim_v[...].astype(F32).reshape(1, M)
        dt = jnp.exp(ldt_v[...].astype(F32)).astype(BF16).astype(F32).reshape(1, M)
        er = jnp.exp(dt * lre)
        ar = er * jnp.cos(dt * lim)
        ai = er * jnp.sin(dt * lim)
        den = lre * lre + lim * lim
        coef_v[0] = jnp.broadcast_to(2.0 * ((ar - 1.0) * lre + ai * lim) / den, (8, M))
        coef_v[1] = jnp.broadcast_to(2.0 * (ai * lre - (ar - 1.0) * lim) / den, (8, M))

        def bc(v):
            return jnp.broadcast_to(v, (NSEG, 128))

        for t in range(3):
            a_v[t] = bc(ar[:, t * 128:(t + 1) * 128])
            a_v[4 + t] = bc(ai[:, t * 128:(t + 1) * 128])
        a_v[3] = bc(jnp.concatenate([ar[:, MA:], ar[:, MA:]], axis=1))
        a_v[7] = bc(jnp.concatenate([ai[:, MA:], -ai[:, MA:]], axis=1))
        col_v[0] = _column(dsk_v[...].astype(F32).reshape(1, M))
        col_v[1] = _column(gw_v[...].astype(F32).reshape(1, M))

        never = never_v[...] != 0

        def spread(us, rows, cols, lo, hi):
            out = []
            for c in range(cols):
                vr = []
                for g in range(rows):
                    n = lo + ((c * rows + g) * (hi - lo)) // (rows * cols)
                    e, t, rg = n // 224, (n % 224) // 32, n % 32
                    vr.append(us[e][8 * rg:8 * rg + 8, 128 * t:128 * t + 128])
                out.append(jnp.concatenate(vr, axis=0))
            mask = jnp.concatenate([jnp.concatenate([never] * rows, axis=0)] * cols, axis=1)
            return mask, jnp.concatenate(out, axis=1)

        def bu(s):
            b_cat = bc_v[0:2 * M, :]
            r = pl.ds(pl.multiple_of(s * (LSEG // 2), LSEG // 2), LSEG // 2)
            xs = []
            us = []
            for e in range(2):
                c0 = pl.multiple_of(s * LSEG + e * HS, LSEG)
                xe = xt_v[:, pl.ds(c0, LSEG)].T
                u = lax.dot_general(xe, b_cat, NT, preferred_element_type=F32)
                us.append(u)
                rows = pl.ds(pl.multiple_of((s + e * NPRO) * SEG_STRIDE, 8), LSEG)
                u_v[6, rows, :] = u[:, :128]
                u_v[7, rows, :] = pltpu.roll(u[:, :128], MR, 1)
                for t in range(6):
                    u_v[t, rows, :] = u[:, (t + 1) * 128:(t + 2) * 128]
                xe = xe.astype(F32)
                xs.append((xe[:, :D], jnp.concatenate(
                    [xe[:, D:], jnp.zeros((LSEG, 2 * D - M), F32)], axis=1)))
            mask, dep = spread(us, 32, 2, XLO, XHI)
            a11 = jnp.where(mask, dep, xs[0][0])
            a22 = jnp.where(mask, dep, xs[1][1])
            for i, t in enumerate(_lhs_terms(a11, xs[0][1], xs[1][0], a22)):
                t = pltpu.bitcast(t, U32)
                for kt in range(2):
                    xs_v[i, kt, r, :] = t[:, kt * 128:(kt + 1) * 128]
            return us

        def c_terms(s, us):
            hc = DC // 2
            r = pl.ds(pl.multiple_of(s * (CSTEP // 2), 8), CW // 2)
            rt = pl.ds(pl.multiple_of(s * CSTEP, 16), CW)
            rb = pl.ds(pl.multiple_of(s * CSTEP + HS, 16), CW)
            a11, a12, a21, a22 = c_v[rt, :hc], c_v[rt, hc:], c_v[rb, :hc], c_v[rb, hc:]
            mask, dep = spread(us, CW // 16, 4, CLO, CHI)
            dep = pltpu.bitcast(dep, U32)
            a11 = pltpu.bitcast(jnp.where(mask, dep, pltpu.bitcast(a11, U32)), BF16)
            a22 = pltpu.bitcast(jnp.where(mask, dep, pltpu.bitcast(a22, U32)), BF16)
            terms = _lhs_terms(*(a.astype(F32) for a in (a11, a12, a21, a22)))
            for i, t in enumerate(terms):
                t = pltpu.bitcast(t, U32)
                for kt in range(4):
                    cs_v[i, kt, r, :] = t[:, kt * 128:(kt + 1) * 128]

        for cp in first_cps:
            cp.wait()
        bu(0)

        def pro_step(s, _):
            for cp in stage_copies(s):
                cp.wait()
            c_terms(s - 1, bu(s))
            return 0

        lax.fori_loop(1, NPRO, pro_step, 0)

    _prologue()

    def out_mm(h, ctx, r0=0, r1=M):
        wot = pltpu.bitcast(wot_v[h, r0 // 2:r1 // 2, :], BF16)
        return lax.dot_general(wot, ctx, NT, preferred_element_type=F32)

    def out_proj(h, i, ctx, r0=0, r1=M):
        o = out_mm(h, ctx, r0, r1)
        acc_v[r0:r1, 2 * i * TQ:(2 * i + 2) * TQ] += o
        return o

    def carried(e):
        return pltpu.bitcast(ctxc_v[e], BF16)

    def head(h, _):
        slot = lax.bitwise_and(h, 1)

        @pl.when(h == H // 2)
        def _segment_carry():
            pr = [a_v[t] for t in range(4)]
            pi = [a_v[4 + t] for t in range(4)]
            for _ in range(int(math.log2(LSEG))):
                pr, pi = ([pr[t] * pr[t] - pi[t] * pi[t] for t in range(4)],
                          [2.0 * pr[t] * pi[t] for t in range(4)])
            row = lax.broadcasted_iota(jnp.int32, (NSEG, 128), 0)
            e_r = [st_v[t] for t in range(4)]
            e_i = [st_v[4 + t] for t in range(4)]
            ir = [jnp.zeros((NSEG, 128), F32)] * 4
            ii = ir
            for s in range(1, NSEG):
                mr, mi = _cmul(pr, pi, ir, ii)
                fr = [pltpu.roll(mr[k] + e_r[k], 1, 0) for k in range(4)]
                fi = [pltpu.roll(mi[k] + e_i[k], 1, 0) for k in range(4)]
                ir = [jnp.where(row == s, fr[k], ir[k]) for k in range(4)]
                ii = [jnp.where(row == s, fi[k], ii[k]) for k in range(4)]
            for t in range(4):
                st_v[t] = ir[t]
                st_v[4 + t] = ii[t]

        @pl.when(h == 1)
        def _():
            for cp in late_cps:
                cp.wait()

        for cp in w_copies(h, h, slot):
            cp.wait()

        hprev = jnp.maximum(h - 1, 0)
        o_prev = out_mm(hprev, carried(0), 0, O_TOP) if O_TOP else None
        for cp in w_copies(jnp.minimum(h + 1, H - 1), h + 1, 1 - slot):
            cp.start()
        if O_TOP:
            acc_v[0:O_TOP, 2 * ORDER[-1] * TQ:(2 * ORDER[-1] + 2) * TQ] += o_prev

        up = ((1 - slot) * 16).astype(U32)

        def weight(buf):
            return pltpu.bitcast((buf[slot] << up) & jnp.uint32(0xFFFF0000), F32)

        def quads(w, kh):
            return w[:kh, :128], w[:kh, 128:], w[kh:, :128], w[kh:, 128:]

        def assemble(c11, c12, c21, c22):
            return jnp.concatenate([jnp.concatenate([c11, c12], axis=1),
                                    jnp.concatenate([c21, c22], axis=1)], axis=0)

        def x_term(i):
            return pltpu.bitcast(jnp.concatenate([xs_v[i, kt] for kt in range(2)], axis=1), BF16)

        def c_term(i):
            return pltpu.bitcast(jnp.concatenate([cs_v[i, kt] for kt in range(4)], axis=1), BF16)

        wq = jnp.concatenate([weight(wq_b), jnp.zeros((2 * D - M, D), F32)], axis=0)
        qscale = (D ** -0.5) * math.log2(math.e)
        kf = assemble(*_strassen(c_term, _rhs_terms(*quads(weight(wk_b), DC // 2))))
        qf = assemble(*_strassen(x_term, _rhs_terms(*quads(wq, D)))) * qscale
        never = never_v[...] != 0

        def sup(a, j):
            return quads(a[2 * j * TQ:(2 * j + 2) * TQ], TQ)

        q = qf.astype(BF16)
        k = kf.astype(BF16)
        qt = [None] + [_lhs_terms(*sup(qf, j)) for j in range(1, NS)]
        kt = []
        for j in range(NS - 1):
            k11, k12, k21, k22 = sup(kf, j)
            kt.append(_rhs_terms(k11, k21, k12, k22))

        causal = (lax.broadcasted_iota(jnp.int32, (TQ, TQ), 1)
                  <= lax.broadcasted_iota(jnp.int32, (TQ, TQ), 0))

        def nt(a, b):
            return lax.dot_general(a, b, NT, preferred_element_type=F32)

        never64 = jnp.concatenate([never] * 8, axis=0)
        never128 = jnp.concatenate([never] * 16, axis=0)

        lpins = []

        def tmax(x):
            return jnp.maximum(x[:, :TQ], x[:, TQ:]) if x.shape[1] > TQ else x

        def score_jobs(i):
            top, bot = [None] * (i + 1), [None] * (i + 1)
            mx = [None, None]
            tmp = {}
            hist = []

            def note(half, x):
                mx[half] = tmax(x) if mx[half] is None else jnp.maximum(mx[half], tmax(x))

            def job_a(j):
                lhs = [qt[i][t] for t in (1, 2, 3, 4)]
                jj = j - MLAG
                if MG and jj >= 0 and jj % MG == MG - 1:
                    pins = [pltpu.bitcast(x, U32) for x in hist[jj]]
                    pins = [pins[0][:64], pins[0][64:], pins[1][:64], pins[1][64:]]
                    lhs = [pltpu.bitcast(jnp.where(never64, pn, pltpu.bitcast(x, U32)), BF16)
                           for pn, x in zip(pins, lhs)]
                m2, m3, m4, m5 = (nt(x, kt[j][t]) for x, t in zip(lhs, (1, 2, 3, 4)))
                tmp[j] = (m4 - m5, m3 + m5, m2 + m4, m3 - m2)

            def job_b(j):
                t11, c12, c21, t22 = tmp.pop(j)
                lhs = [qt[i][t] for t in (0, 5, 6)]
                if BPIN and len(lpins) > BLAG + 1:
                    pn = pltpu.bitcast(lpins[-1 - BLAG - (j % 2 if BALT else 0)], U32)
                    lhs[1:] = [pltpu.bitcast(jnp.where(never64, x, pltpu.bitcast(y, U32)), BF16)
                               for x, y in zip((pn[:64], pn[64:]), lhs[1:])]
                m1, m6, m7 = (nt(x, kt[j][t]) for x, t in zip(lhs, (0, 5, 6)))
                top[j] = jnp.concatenate([t11 + (m1 + m7), c12], axis=1)
                bot[j] = jnp.concatenate([c21, t22 + (m1 + m6)], axis=1)
                note(0, top[j])
                note(1, bot[j])
                hist.append(tuple(mx))

            def dpin(x, half):
                if not DPIN or i < MLAG:
                    return x
                pn = pltpu.bitcast(hist[i - MLAG][half], U32)
                pn = jnp.concatenate([pn[:64], pn[64:]], axis=1)
                nv = jnp.concatenate([never64, never64], axis=1)
                return pltpu.bitcast(jnp.where(nv, pn, pltpu.bitcast(x, U32)), BF16)

            def diag_b():
                r0 = 2 * i * TQ
                sb = nt(dpin(q[r0 + TQ:r0 + 2 * TQ], 1), k[r0:r0 + 2 * TQ])
                bot[i] = jnp.concatenate(
                    [sb[:, :TQ], jnp.where(causal, sb[:, TQ:], -1e9)], axis=1)
                note(1, bot[i])

            def diag_t():
                r0 = 2 * i * TQ
                top[i] = jnp.where(causal, nt(dpin(q[r0:r0 + TQ], 0), k[r0:r0 + TQ]), -1e9)
                note(0, top[i])

            jobs = []
            for j in range(i):
                jobs += [functools.partial(job_a, j), functools.partial(job_b, j)]
            if D_FIRST:
                return (top, bot, mx, hist), [diag_b, diag_t] + jobs
            return (top, bot, mx, hist), jobs + [diag_b, diag_t]

        pending = {}
        calls = [0]
        never_col = jnp.concatenate([never] * 56, axis=0)
        pin_list = [kt[j] for j in range(NS - 1)] + [qt[j] for j in range(NS - 1, 0, -1)]

        def v_lhs(i):
            n = calls[0]
            calls[0] += 1
            if n == S_AT:
                for nn in range(LOOK):
                    pending[ORDER[nn]], jobs = score_jobs(ORDER[nn])
                    for job in jobs:
                        job()
            cols = [cs_v[i, kt_] for kt_ in range(4)]
            for c in range(PINS[n]):
                pin = jnp.concatenate([pltpu.bitcast(t, U32) for t in pin_list.pop(0)], axis=0)
                cols[c] = jnp.concatenate(
                    [cols[c][:64], jnp.where(never_col, pin, cols[c][64:])], axis=0)
            return pltpu.bitcast(jnp.concatenate(cols, axis=1), BF16)

        v = assemble(*_strassen(v_lhs, _rhs_terms(*quads(weight(wv_b), DC // 2)))).astype(BF16)

        r0 = pl.multiple_of(jnp.clip(h - 1, 0, M // CROWS - 1) * CROWS, CROWS)
        src = jnp.where(h == 0, 0, 2 * M) + r0
        cre = bc_v[pl.ds(pl.multiple_of(src, CROWS), CROWS), :].astype(F32)
        cim = bc_v[pl.ds(pl.multiple_of(src + M, CROWS), CROWS), :].astype(F32)
        cr = coef_v[0, 0:1, :]
        ci = coef_v[1, 0:1, :]
        c_r = cre * cr - cim * ci
        c_i = -(cre * ci + cim * cr)
        ccat_v[pl.ds(r0, CROWS), :] = jnp.concatenate(
            [c_r[:, :MA], c_i[:, :MA], c_r[:, MA:], c_i[:, MA:]], axis=1).astype(BF16)

        t0 = lax.bitwise_and(h, H // 2 - 1) * STEPS
        a_r = [a_v[t] for t in range(4)]
        a_i = [a_v[4 + t] for t in range(4)]
        hr = [st_v[t] for t in range(4)]
        hi = [st_v[4 + t] for t in range(4)]

        def scan_steps(j0, n, hr, hi):
            for j in range(j0, j0 + n):
                us = [u_v[kk, pl.ds(t0 + j, NSEG, stride=SEG_STRIDE), :] for kk in range(8)]
                mr, mi = _cmul(a_r, a_i, hr, hi)
                hr = [mr[0] + us[0], mr[1] + us[1], mr[2] + us[2], mr[3] + us[6]]
                hi = [mi[0] + us[3], mi[1] + us[4], mi[2] + us[5], mi[3] + us[7]]
                r0 = pl.multiple_of((t0 + j) * NSEG, NSEG)
                for kk, val in enumerate(hr[:3] + hi[:3] + [hr[3]]):
                    h_v[kk, pl.ds(r0, NSEG), :] = val
            return hr, hi

        def orow(o, g, half):
            g = min(g, o.shape[0] // 8 - 1)
            return o[8 * g:8 * g + 8, half * TQ:(half + 1) * TQ]

        def normalise(ls, ctx, tiles, o):
            if DSUM and o is not None:
                ls = []
                for half, tl in enumerate(tiles):
                    dep = jnp.concatenate(
                        [orow(o, DS0 + g * DS1, half)
                         for g in range(16)], axis=0)
                    l = jnp.where(never128, dep, tl[0])
                    for t in tl[1:]:
                        l = l + t
                    ls.append(l)
            out = [c * _recip(jnp.sum(l, axis=1, keepdims=True)) for l, c in zip(ls, ctx)]
            return jnp.concatenate(out, axis=0).astype(BF16)

        ctxs = []
        o = None
        for n, i in enumerate(ORDER):
            ms = []
            cur = pending.pop(i)
            for half in range(2):
                s = cur[half][0]
                hr = [jnp.where(never, s[8 * t:8 * t + 8, 0:128], hr[t]) for t in range(4)]
                hr, hi = scan_steps((2 * n + half) * (STEPS // NB), STEPS // NB, hr, hi)
                mx = cur[2][half]
                if DMAX and o is not None and i > 0:
                    done = max(i - MLAG + DPIN, 0)
                    dep = jnp.concatenate(
                        [orow(o, DM0 + g * DM1, half)
                         for g in range(16)], axis=0)
                    rest = [x[:, c * TQ:(c + 1) * TQ] for x in cur[half][done:]
                            for c in range(x.shape[1] // TQ)]
                    if done:
                        rest = [cur[3][done - 1][half]] + rest
                    mx = jnp.where(never128, dep, rest[0])
                    for t in rest[1:]:
                        mx = jnp.maximum(mx, t)
                ms.append(jnp.max(mx, axis=1, keepdims=True))
            if n >= 1:
                ctxs[n - 1] = normalise(*ctxs[n - 1])
            todo = []
            if n + LOOK < NS:
                pending[ORDER[n + LOOK]], todo = score_jobs(ORDER[n + LOOK])
            for _ in range(HEAD):
                if todo:
                    todo.pop(0)()
            ctx = [None, None]
            ls = [None, None]
            lhist = []
            tiles = [[], []]
            o = None
            if PV_SEQ:
                seq = [(half, j) for half in range(2) for j in range(i + 1)]
            else:
                seq = [(half, j) for j in range(i + 1) for half in range(2)]
            for cn, (half, j) in enumerate(seq):
                if todo:
                    todo.pop(0)()
                p = jnp.exp2(cur[half][j] - ms[half])
                psum = p[:, :TQ] + p[:, TQ:] if p.shape[1] > TQ else p
                ls[half] = psum if ls[half] is None else ls[half] + psum
                lhist.append((ls[half], j))
                tiles[half] += [p[:, c * TQ:(c + 1) * TQ] for c in range(p.shape[1] // TQ)]
                lpins.append(ls[half])
                cc = cn - SLAG
                if SG and cc >= 0 and lhist[cc][1] % SG == SG - 1:
                    last = jnp.where(never128, lhist[cc][0], p[:, -TQ:])
                    p = jnp.concatenate([p[:, :TQ], last], axis=1) if p.shape[1] > TQ else last
                j0 = j * 2 * TQ
                part = jnp.dot(p.astype(BF16), v[j0:j0 + p.shape[1]], preferred_element_type=F32)
                ctx[half] = part if ctx[half] is None else ctx[half] + part
                if n >= O_LAG and cn == (len(seq) - 1 if O_POS else 0):
                    o = out_proj(h, ORDER[n - O_LAG], ctxs[n - O_LAG])
                if n == 0 and O_TOP < M and cn == len(seq) - 1:
                    o = out_proj(hprev, ORDER[-1], carried(0), O_TOP, M)
            for job in todo:
                job()
            ctxs.append((ls, ctx, tiles, o if n < NS - 1 else None))
        ctxs[NS - 1] = normalise(*ctxs[NS - 1])
        for t in range(4):
            st_v[t] = hr[t]
            st_v[4 + t] = hi[t]
        for e in range(O_LAG):
            ctxc_v[e] = pltpu.bitcast(ctxs[NS - O_LAG + e], U32)
        return 0

    with jax.named_scope('heads'):
        lax.fori_loop(0, H, head, 0)

    @jax.named_scope('epilogue')
    def _epilogue():
        for cp in w_copies(jnp.int32(H - 1), H, 0):
            cp.wait()
        out_proj(H - 1, ORDER[-1], carried(0))

        def o_copy(c0, width):
            cols = pl.ds(c0, width)
            return pltpu.make_async_copy(acc_v.at[:, cols], out_hbm.at[:, cols], sem.at[0])

        def segment(s, c_cat, pieces):
            c0 = s * LSEG if isinstance(s, int) else pl.multiple_of(s * LSEG, LSEG)
            hs = jnp.concatenate(
                [h_v[kk, pl.ds(s, LSEG, stride=NSEG), :] for kk in range(7)],
                axis=1).astype(BF16)
            yt = lax.dot_general(c_cat, hs, NT, preferred_element_type=F32)
            w = LSEG // pieces
            for e in range(pieces):
                ce = c0 + e * w
                cols = pl.ds(ce, w)
                xf = xt_v[:, cols].astype(F32)
                dsk = jnp.concatenate([col_v[0]] * (w // 128), axis=1)
                gw = jnp.concatenate([col_v[1]] * (w // 128), axis=1)
                g = jax.nn.sigmoid(jnp.sum(xf * gw, axis=0, keepdims=True))
                y = yt[:, e * w:(e + 1) * w] + xf * dsk
                acc_v[:, cols] = g * acc_v[:, cols] + (1.0 - g) * y
                o_copy(ce, w).start()

        if EC == NSEG:
            c_cat = ccat_v[...]
            for s in range(NSEG - 1, -1, -1):
                segment(s, c_cat, 2 if s == 0 else 1)
        else:
            def out_step(it, _):
                c_cat = ccat_v[...]
                for e in range(EC):
                    segment(it * EC + e, c_cat, 1)
                return 0

            lax.fori_loop(0, NSEG // EC, out_step, 0)
        o_copy(0, S).wait()

    _epilogue()


@jax.jit
def pallas_gated_mix__compressed_kv_cla__ssm_conv_s5__prompt_kernel(
    A_x: jax.Array,
    A_c_kv: jax.Array,
    A_w_q: jax.Array,
    A_w_uk: jax.Array,
    A_w_uv: jax.Array,
    A_w_o: jax.Array,
    B_x: jax.Array,
    B_Lambda_re: jax.Array,
    B_Lambda_im: jax.Array,
    B_B_re: jax.Array,
    B_B_im: jax.Array,
    B_C_re: jax.Array,
    B_C_im: jax.Array,
    B_log_dt: jax.Array,
    B_Dskip: jax.Array,
    gate_w: jax.Array,
):
    del B_x
    hbm_spec = pl.BlockSpec(memory_space=pltpu.HBM)
    out_t = pl.pallas_call(
        _kernel,
        in_specs=[hbm_spec] * 15,
        out_specs=hbm_spec,
        out_shape=jax.ShapeDtypeStruct((M, S), F32),
        scratch_shapes=[
            pltpu.VMEM((M, S), BF16),
            pltpu.VMEM((7, 2, HS // 2, 128), U32),
            pltpu.VMEM((S, DC), BF16),
            pltpu.VMEM((7, 4, HS // 2, 128), U32),
            pltpu.VMEM((H + 1, M // 2, D), U32),
            pltpu.VMEM((2, M, D), U32),
            pltpu.VMEM((2, DC, D), U32),
            pltpu.VMEM((2, DC, D), U32),
            pltpu.VMEM((4 * M, M), BF16),
            pltpu.VMEM((M, 2 * M), BF16),
            pltpu.VMEM((M,), BF16), pltpu.VMEM((M,), BF16), pltpu.VMEM((M,), BF16),
            pltpu.VMEM((M,), BF16), pltpu.VMEM((M,), BF16),
            pltpu.VMEM((2, M, 128), F32),
            pltpu.VMEM((2, 8, M), F32),
            pltpu.VMEM((8, NSEG * SEG_STRIDE, 128), F32),
            pltpu.VMEM((7, S, 128), F32),
            pltpu.VMEM((8, NSEG, 128), F32),
            pltpu.VMEM((8, NSEG, 128), F32),
            pltpu.VMEM((M, S), F32),
            pltpu.VMEM((O_LAG, TQ, D), U32),
            pltpu.VMEM((8, 128), jnp.int32),
            pltpu.SemaphoreType.DMA((SEM_X + NPRO,)),
        ],
        compiler_params=pltpu.CompilerParams(vmem_limit_bytes=110 * 1024 * 1024),
        name="gated_mix",
    )(
        A_x.reshape(S, M).T, A_c_kv.reshape(S, DC),
        A_w_q, A_w_uk, A_w_uv, jnp.swapaxes(A_w_o, 1, 2),
        B_Lambda_re, B_Lambda_im, B_B_re, B_B_im, B_C_re, B_C_im, B_log_dt,
        B_Dskip, gate_w,
    )
    return out_t.T.reshape(1, S, M)
```

```python
import functools
import math
import os

import jax
import jax.numpy as jnp
from jax import lax
import jax.experimental.pallas as pl
import jax.experimental.pallas.tpu as pltpu

F32 = jnp.float32
BF16 = jnp.bfloat16
U32 = jnp.uint32

S = 2048
HS = S // 2
M = 448
DC = 1024
H = 16
D = 256
TQ = 128
NB = S // TQ
NS = NB // 2
NSEG = 8
LSEG = S // NSEG
SEG_STRIDE = LSEG + 8
STEPS = 2 * LSEG // H
MA = 384
MR = M - MA
NT = (((1,), (1,)), ((), ()))
O_LAG = int(os.environ.get('O_LAG', 1))
NPRO = NSEG // 2
EC = int(os.environ.get('EC', 8))
_om = os.environ.get('ORDER', 'desc')
if _om == 'asc':
    ORDER = list(range(NS))
elif _om == 'desc':
    ORDER = list(range(NS))[::-1]
else:
    ORDER = [int(t) for t in _om.split(',')]
LOOK = int(os.environ.get('LOOK', 1))
PRE_S = int(os.environ.get('PRE_S', 2))
KV_JOINT = int(os.environ.get('KV_JOINT', 0))
SEM_W = 3
SEM_X = 5
PV_K = int(os.environ.get('PV_K', 256))
O_SPLIT = int(os.environ.get('O_SPLIT', 0))
O_POS = int(os.environ.get('O_POS', 1))
S_AB = int(os.environ.get('S_AB', 1))
PV_SEQ = int(os.environ.get('PV_SEQ', 0))
S_AT = int(os.environ.get('S_AT', 6))
PINS = [int(t) for t in os.environ.get('PINS', '2222222')]
RCP_EUP = int(os.environ.get('RCP_EUP', 1))
MG = int(os.environ.get('MG', 1))
MLAG = int(os.environ.get('MLAG', 2))
SG = int(os.environ.get('SG', 0))
SLAG = int(os.environ.get('SLAG', 1))
D_FIRST = int(os.environ.get('D_FIRST', 0))
HEAD = int(os.environ.get('HEAD', 4))
BPIN = int(os.environ.get('BPIN', 0))
BLAG = int(os.environ.get('BLAG', 1))
BALT = int(os.environ.get('BALT', 1))
DSUM = int(os.environ.get('DSUM', 1))
DS0 = int(os.environ.get('DS0', 0))
DS1 = int(os.environ.get('DS1', 2))
O_TOP = int(os.environ.get('O_TOP', 160))
DMAX = int(os.environ.get('DMAX', 1))
DM0 = int(os.environ.get('DM0', 0))
DM1 = int(os.environ.get('DM1', 1))
CW = 352
CSTEP = 336
XLO = int(os.environ.get('XLO', 40))
XHI = int(os.environ.get('XHI', 420))
CLO = int(os.environ.get('CLO', 0))
CHI = int(os.environ.get('CHI', 420))
DPIN = int(os.environ.get('DPIN', 1))
PS = int(os.environ.get('PS', 1))
VPIN = int(os.environ.get('VPIN', 12))
QPIN = int(os.environ.get('QPIN', 10))
SCAN_SPAN = int(os.environ.get('SCAN_SPAN', 5))
LREUSE = int(os.environ.get('LREUSE', 0))
PD_FIRST = int(os.environ.get('PD_FIRST', 0))
PORDER = [int(t) for t in os.environ.get('PORDER', '2301546')]
PG = int(os.environ.get('PG', 4))
PGROUPS = [[(j, min(j + PG, i)) for j in range(0, i, PG)] for i in range(8)]
if PG == 4:
    PGROUPS[7] = [(0, 4), (4, 6), (6, 7)]
    PGROUPS[3] = [(0, 2), (2, 3)]
LEAD0 = int(os.environ.get('LEAD0', 3))
LEAD = int(os.environ.get('LEAD', 5))
BAL = int(os.environ.get('BAL', 16))
FILL0 = int(os.environ.get('FILL0', 3))
CAP = int(os.environ.get('CAP', 96))
MCOST = int(os.environ.get('MCOST', 32))
PHOST = int(os.environ.get('PHOST', 1))
EARLY = int(os.environ.get('EARLY', 0))
VPIN2 = int(os.environ.get('VPIN2', 24))
RHOST = int(os.environ.get('RHOST', 0))
AGE = int(os.environ.get('AGE', 3))
ODELAY = int(os.environ.get('ODELAY', 0))
SUMPIN = int(os.environ.get('SUMPIN', 1))
OS0 = int(os.environ.get('OS0', 2))
XDEL = int(os.environ.get('XDEL', 1))
XD0 = int(os.environ.get('XD0', 0))
INDEL = int(os.environ.get('INDEL', 1))
INSTAG = int(os.environ.get('INSTAG', 1))
OPIN = int(os.environ.get('OPIN', 1))
CROWS = 32


_DIAG = {8: (1, 0), 5: (1, 1), 6: (0, 0), 7: (0, 1)}


def _plan():
    i = NS - 1
    sq = [(4, 'a', i, 0), (4, 'a', i, 1), (3, 'b', i, 0), (1, 's', i, (1, 5)),
          (4, 'a', i, 2), (3, 'b', i, 2), (1, 's', i, (1, 6)),
          (4, 'a', i, 3), (3, 'b', i, 3), (1, 's', i, (1, 0)),
          (4, 'a', i, 4), (4, 'a', i, 5), (3, 'b', i, 4), (1, 's', i, (5, 5)),
          (4, 'a', i, 6), (3, 'b', i, 6), (1, 's', i, (5, 6)),
          (2, 'd', i, (1, 0)), (2, 'd', i, (0, 0)),
          (4, 'a', i - 1, 0), (4, 'a', i - 1, 1),
          (1, 's', i, (5, 0)), (1, 's', i - 1, (1, 5)), (2, 'd', i, (1, 1)),
          (3, 'b', i - 1, 0), (1, 's', i - 1, (1, 6)),
          (4, 'a', i - 1, 2), (3, 'b', i - 1, 2), (1, 's', i - 1, (1, 0))]
    for i in range(NS - 2, -1, -1):
        for j in range(3 if i == NS - 2 else 0, i):
            sq += [(4, 'a', i, j), (3, 'b', i, j)]
        sq += [(2, 'd', i, hk) for hk in ((1, 0), (0, 0), (1, 1))]
    pq = {}
    for i in range(NS):
        pq[i] = [[j1 - j0, t, list(range(j0, j1))] for j0, j1 in PGROUPS[i] for t in PORDER]
        pq[i] += [[2, 8, [i, i + 1]], [2, 5, [i, i + 1]], [1, 6, [i]], [1, 7, [i]]]
    ready, rounds, events = {}, [], {}
    pi, fill = NS - 1, 0
    while sq or pi >= 0:
        free, fill, cur = 4 - fill, 0, []
        while free:
            p_ok = pi >= 0 and ready.get(pi, 1 << 30) <= len(rounds)
            s_fit = bool(sq) and sq[0][0] <= free
            s_left = sum(u[0] for u in sq if u[2] >= pi - 1)
            p_left = sum(u[0] for u in pq[pi]) if pi >= 0 else 0
            want_s = s_left + BAL >= p_left if s_left else (
                not rounds or all(u[0] == 'p' for u in rounds[-1]))
            if (s_fit and (not p_ok or (want_s and (free == 4 or sq[0][0] == free))
                           or sq[0][1] == 's')) or (sq and not p_ok):
                u = sq.pop(0)
                cur.append(u[1:])
                fill = max(u[0] - free, 0)
                free = max(free - u[0], 0)
                if all(v[2] != u[2] for v in sq):
                    events.setdefault(len(rounds) + 1, []).append(('m', u[2]))
                    ready[u[2]] = len(rounds) + 1 + (LEAD0 if u[2] == NS - 1 else LEAD)
            elif p_ok:
                us = pq[pi]
                size = us[0][0]
                if size > free or free < 4:
                    size = min(free, max(u[0] for u in us))
                same = [u for u in us if u[0] == size]
                if same:
                    us.remove(same[0])
                    cur.append(('p', pi, same[0][1], same[0][2]))
                else:
                    u = min((u for u in us if u[0] > size), key=lambda u: u[0])
                    cur.append(('p', pi, u[1], u[2][-size:]))
                    u[2], u[0] = u[2][:-size], u[0] - size
                free -= size
                if not us:
                    events.setdefault(len(rounds) + 1 + (ODELAY if pi else 0), []).append(('o', pi))
                    pi -= 1
            else:
                free = 0
        rounds.append(cur)
    return rounds, events


def _lhs_terms(a11, a12, a21, a22):
    return [t.astype(BF16) for t in
            (a11 + a22, a21 + a22, a11, a22, a11 + a12, a21 - a11, a12 - a22)]


def _rhs_terms(b11, b12, b21, b22):
    return [t.astype(BF16) for t in
            (b11 + b22, b11, b12 - b22, b21 - b11, b22, b11 + b12, b21 + b22)]


def _strassen(lhs, rhs, log):
    def mm(i):
        log.append(jnp.dot(lhs(i), rhs[i], preferred_element_type=F32))
        return log[-1]
    m1 = mm(0)
    m4 = mm(3)
    c11 = m1 + m4
    m2 = mm(1)
    c21 = m2 + m4
    c22 = m1 - m2
    m5 = mm(4)
    c11 = c11 - m5
    m3 = mm(2)
    c12 = m3 + m5
    c22 = c22 + m3
    c11 = c11 + mm(6)
    c22 = c22 + mm(5)
    return c11, c12, c21, c22


def _recip(l):
    if RCP_EUP:
        r = pl.reciprocal(l, approx=True)
        return r * (2.0 - l * r)
    r = pltpu.bitcast(jnp.int32(0x7EF311C3) - pltpu.bitcast(l, jnp.int32), F32)
    for _ in range(3):
        r = r * (2.0 - l * r)
    return r


def _cmul(pr, pi, hr, hi):
    return ([pr[t] * hr[t] - pi[t] * hi[t] for t in range(4)],
            [pr[t] * hi[t] + pi[t] * hr[t] for t in range(4)])


def _column(row):
    row = jnp.concatenate([row, jnp.zeros((1, 512 - M), F32)], axis=1)
    return jnp.broadcast_to(row, (128, 512)).T[:M]


def _kernel(xt_hbm, c_hbm, wq_hbm, wk_hbm, wv_hbm, wot_hbm,
            lre_hbm, lim_hbm, bre_hbm, bim_hbm, cre_hbm, cim_hbm, ldt_hbm,
            dsk_hbm, gw_hbm,
            out_hbm,
            xt_v, xs_v, c_v, cs_v, wot_v, wq_b, wk_b, wv_b, bc_v, ccat_v,
            lre_v, lim_v, ldt_v, dsk_v, gw_v, col_v, coef_v,
            u_v, h_v, a_v, st_v, acc_v, ctxc_v, never_v, sem):
    wq32 = wq_hbm.bitcast(U32)
    wk32 = wk_hbm.bitcast(U32)
    wv32 = wv_hbm.bitcast(U32)
    wot32 = wot_hbm.bitcast(U32)

    def w_copies(h, h_dst, sl):
        j = lax.shift_right_logical(h, 1)
        cps = [pltpu.make_async_copy(src.at[:, j, :], dst.at[sl], sem.at[SEM_W + sl])
               for src, dst in ((wq32, wq_b), (wk32, wk_b), (wv32, wv_b))]
        return cps + [pltpu.make_async_copy(wot32.at[h], wot_v.at[h_dst], sem.at[SEM_W + sl])]

    def x_copies(s):
        spans = [pl.ds(pl.multiple_of(s * LSEG + e * HS, LSEG), LSEG) for e in range(2)]
        return [pltpu.make_async_copy(xt_hbm.at[:, sp], xt_v.at[:, sp], sem.at[SEM_X + s])
                for sp in spans]

    def c_copies(start, rows, s):
        spans = [pl.ds(pl.multiple_of(start + e * HS, 16), rows) for e in range(2)]
        return [pltpu.make_async_copy(c_hbm.at[sp], c_v.at[sp], sem.at[SEM_X + s])
                for sp in spans]

    def stage_copies(s):
        return x_copies(s) + c_copies(CW - CSTEP + (s - 1) * CSTEP, CSTEP, s)

    first_cps = x_copies(0) + [
        pltpu.make_async_copy(bre_hbm.at[MA:M], bc_v.at[0:MR], sem.at[SEM_X]),
        pltpu.make_async_copy(bim_hbm.at[MA:M], bc_v.at[MR:2 * MR], sem.at[SEM_X]),
        pltpu.make_async_copy(bre_hbm.at[0:MA], bc_v.at[2 * MR:2 * MR + MA], sem.at[SEM_X]),
        pltpu.make_async_copy(bim_hbm.at[0:MA], bc_v.at[2 * MR + MA:2 * M], sem.at[SEM_X]),
    ] + c_copies(0, CW - CSTEP, 0)
    vec_cps = [pltpu.make_async_copy(src, dst, sem.at[1]) for src, dst in
               ((lre_hbm, lre_v), (lim_hbm, lim_v), (ldt_hbm, ldt_v), (dsk_hbm, dsk_v),
                (gw_hbm, gw_v))]
    late_cps = [pltpu.make_async_copy(cre_hbm, bc_v.at[2 * M:3 * M], sem.at[2]),
                pltpu.make_async_copy(cim_hbm, bc_v.at[3 * M:4 * M], sem.at[2])]

    @jax.named_scope('prologue')
    def _prologue():
        zero = jnp.int32(0)
        first = vec_cps + first_cps
        for s in range(1, NPRO):
            first = first + stage_copies(s)
        for cp in first + w_copies(zero, 0, 0) + late_cps:
            cp.start()
        acc_v[...] = jnp.zeros_like(acc_v)
        st_v[...] = jnp.zeros_like(st_v)
        ctxc_v[...] = jnp.zeros_like(ctxc_v)
        never_v[...] = jnp.zeros_like(never_v)

        for cp in vec_cps:
            cp.wait()
        lre = lre_v[...].astype(F32).reshape(1, M)
        lim = lim_v[...].astype(F32).reshape(1, M)
        dt = jnp.exp(ldt_v[...].astype(F32)).astype(BF16).astype(F32).reshape(1, M)
        er = jnp.exp(dt * lre)
        ar = er * jnp.cos(dt * lim)
        ai = er * jnp.sin(dt * lim)
        den = lre * lre + lim * lim
        coef_v[0] = jnp.broadcast_to(2.0 * ((ar - 1.0) * lre + ai * lim) / den, (8, M))
        coef_v[1] = jnp.broadcast_to(2.0 * (ai * lre - (ar - 1.0) * lim) / den, (8, M))

        def bc(v):
            return jnp.broadcast_to(v, (NSEG, 128))

        for t in range(3):
            a_v[t] = bc(ar[:, t * 128:(t + 1) * 128])
            a_v[4 + t] = bc(ai[:, t * 128:(t + 1) * 128])
        a_v[3] = bc(jnp.concatenate([ar[:, MA:], ar[:, MA:]], axis=1))
        a_v[7] = bc(jnp.concatenate([ai[:, MA:], -ai[:, MA:]], axis=1))
        col_v[0] = _column(dsk_v[...].astype(F32).reshape(1, M))
        col_v[1] = _column(gw_v[...].astype(F32).reshape(1, M))

        never = never_v[...] != 0

        def spread(us, rows, cols, lo, hi):
            out = []
            for c in range(cols):
                vr = []
                for g in range(rows):
                    n = lo + ((c * rows + g) * (hi - lo)) // (rows * cols)
                    e, t, rg = n // 224, (n % 224) // 32, n % 32
                    vr.append(us[e][8 * rg:8 * rg + 8, 128 * t:128 * t + 128])
                out.append(jnp.concatenate(vr, axis=0))
            mask = jnp.concatenate([jnp.concatenate([never] * rows, axis=0)] * cols, axis=1)
            return mask, jnp.concatenate(out, axis=1)

        def bu(s):
            b_cat = bc_v[0:2 * M, :]
            r = pl.ds(pl.multiple_of(s * (LSEG // 2), LSEG // 2), LSEG // 2)
            xs = []
            us = []
            for e in range(2):
                c0 = pl.multiple_of(s * LSEG + e * HS, LSEG)
                xe = xt_v[:, pl.ds(c0, LSEG)].T
                u = lax.dot_general(xe, b_cat, NT, preferred_element_type=F32)
                us.append(u)
                rows = pl.ds(pl.multiple_of((s + e * NPRO) * SEG_STRIDE, 8), LSEG)
                u_v[6, rows, :] = u[:, :128]
                u_v[7, rows, :] = pltpu.roll(u[:, :128], MR, 1)
                for t in range(6):
                    u_v[t, rows, :] = u[:, (t + 1) * 128:(t + 2) * 128]
                xe = xe.astype(F32)
                xs.append((xe[:, :D], jnp.concatenate(
                    [xe[:, D:], jnp.zeros((LSEG, 2 * D - M), F32)], axis=1)))
            mask, dep = spread(us, 32, 2, XLO, XHI)
            a11 = jnp.where(mask, dep, xs[0][0])
            a22 = jnp.where(mask, dep, xs[1][1])
            for i, t in enumerate(_lhs_terms(a11, xs[0][1], xs[1][0], a22)):
                t = pltpu.bitcast(t, U32)
                for kt in range(2):
                    xs_v[i, kt, r, :] = t[:, kt * 128:(kt + 1) * 128]
            return us

        def c_terms(s, us):
            hc = DC // 2
            r = pl.ds(pl.multiple_of(s * (CSTEP // 2), 8), CW // 2)
            rt = pl.ds(pl.multiple_of(s * CSTEP, 16), CW)
            rb = pl.ds(pl.multiple_of(s * CSTEP + HS, 16), CW)
            a11, a12, a21, a22 = c_v[rt, :hc], c_v[rt, hc:], c_v[rb, :hc], c_v[rb, hc:]
            mask, dep = spread(us, CW // 16, 4, CLO, CHI)
            dep = pltpu.bitcast(dep, U32)
            a11 = pltpu.bitcast(jnp.where(mask, dep, pltpu.bitcast(a11, U32)), BF16)
            a22 = pltpu.bitcast(jnp.where(mask, dep, pltpu.bitcast(a22, U32)), BF16)
            terms = _lhs_terms(*(a.astype(F32) for a in (a11, a12, a21, a22)))
            for i, t in enumerate(terms):
                t = pltpu.bitcast(t, U32)
                for kt in range(4):
                    cs_v[i, kt, r, :] = t[:, kt * 128:(kt + 1) * 128]

        for cp in first_cps:
            cp.wait()
        bu(0)

        def pro_step(s, _):
            for cp in stage_copies(s):
                cp.wait()
            c_terms(s - 1, bu(s))
            return 0

        lax.fori_loop(1, NPRO, pro_step, 0)

    _prologue()

    def out_mm(h, ctx, r0=0, r1=M):
        wot = pltpu.bitcast(wot_v[h, r0 // 2:r1 // 2, :], BF16)
        return lax.dot_general(wot, ctx, NT, preferred_element_type=F32)

    def out_proj(h, i, ctx, r0=0, r1=M):
        o = out_mm(h, ctx, r0, r1)
        acc_v[r0:r1, 2 * i * TQ:(2 * i + 2) * TQ] += o
        return o

    def carried(e):
        return pltpu.bitcast(ctxc_v[e], BF16)

    def head(h, _):
        slot = lax.bitwise_and(h, 1)

        @pl.when(h == H // 2)
        def _segment_carry():
            pr = [a_v[t] for t in range(4)]
            pi = [a_v[4 + t] for t in range(4)]
            for _ in range(int(math.log2(LSEG))):
                pr, pi = ([pr[t] * pr[t] - pi[t] * pi[t] for t in range(4)],
                          [2.0 * pr[t] * pi[t] for t in range(4)])
            row = lax.broadcasted_iota(jnp.int32, (NSEG, 128), 0)
            e_r = [st_v[t] for t in range(4)]
            e_i = [st_v[4 + t] for t in range(4)]
            ir = [jnp.zeros((NSEG, 128), F32)] * 4
            ii = ir
            for s in range(1, NSEG):
                mr, mi = _cmul(pr, pi, ir, ii)
                fr = [pltpu.roll(mr[k] + e_r[k], 1, 0) for k in range(4)]
                fi = [pltpu.roll(mi[k] + e_i[k], 1, 0) for k in range(4)]
                ir = [jnp.where(row == s, fr[k], ir[k]) for k in range(4)]
                ii = [jnp.where(row == s, fi[k], ii[k]) for k in range(4)]
            for t in range(4):
                st_v[t] = ir[t]
                st_v[4 + t] = ii[t]

        @pl.when(h == 1)
        def _():
            for cp in late_cps:
                cp.wait()

        for cp in w_copies(h, h, slot):
            cp.wait()

        hprev = jnp.maximum(h - 1, 0)
        o_prev = out_mm(hprev, carried(0), 0, O_TOP) if O_TOP else None
        for cp in w_copies(jnp.minimum(h + 1, H - 1), h + 1, 1 - slot):
            cp.start()
        if O_TOP:
            acc_v[0:O_TOP, 2 * ORDER[-1] * TQ:(2 * ORDER[-1] + 2) * TQ] += o_prev

        up = ((1 - slot) * 16).astype(U32)
        never = never_v[...] != 0
        never64 = jnp.concatenate([never] * 8, axis=0)
        never128 = jnp.concatenate([never] * 16, axis=0)

        def weight(buf):
            return pltpu.bitcast((buf[slot] << up) & jnp.uint32(0xFFFF0000), F32)

        def quads(w, kh):
            return w[:kh, :128], w[:kh, 128:], w[kh:, :128], w[kh:, 128:]

        def bf(rows):
            return pltpu.bitcast(jnp.concatenate(
                [jnp.concatenate(r, axis=1) for r in rows], axis=0), BF16)

        def pk(x):
            return pltpu.bitcast(x.astype(BF16), U32)

        def nt(a, b):
            return lax.dot_general(a, b, NT, preferred_element_type=F32)

        def nn(a, b):
            return jnp.dot(a, b, preferred_element_type=F32)

        pin_list = []

        def lhs_term(ref, i, npin, order=range(8)):
            ncol = ref.shape[1]
            rows = [[ref[i, c, g * 64:(g + 1) * 64, :] for c in range(ncol)] for g in order]
            nr = len(rows) - 1
            npin = min(npin, len(pin_list), nr * ncol)
            for n in range(npin):
                g, c = 1 + (n * nr) // npin, n % ncol
                rows[g][c] = jnp.where(never64, pin_list.pop(0), rows[g][c])
            return bf(rows)

        def sup(cq, j):
            l, r = (cq[0], cq[1]) if j < NS // 2 else (cq[2], cq[3])
            r0 = (j % (NS // 2)) * 2 * TQ
            return l[r0:r0 + TQ], r[r0:r0 + TQ], l[r0 + TQ:r0 + 2 * TQ], r[r0 + TQ:r0 + 2 * TQ]

        def rhs_tiles(b11, b12, b21, b22, with_terms):
            plain = [pk(b11), pk(b12), pk(b21), pk(b22)]
            if not with_terms:
                return None, plain, plain
            extra = [pk(b11 + b22), pk(b12 - b22), pk(b21 - b11), pk(b11 + b12), pk(b21 + b22)]
            terms = [extra[0], plain[0], extra[1], extra[2], plain[3], extra[3], extra[4]]
            return terms, plain, plain + extra

        def lhs_tiles(a11, a12, a21, a22, with_terms):
            plain = [pk(a11), pk(a12), pk(a21), pk(a22)]
            if not with_terms:
                return None, plain, plain
            extra = [pk(a11 + a22), pk(a21 + a22), pk(a11 + a12), pk(a21 - a11), pk(a12 - a22)]
            terms = [extra[0], extra[1], plain[0], plain[3], extra[2], extra[3], extra[4]]
            return terms, plain, plain + extra

        klog = []
        kq = _strassen(lambda i: lhs_term(cs_v, i, 0),
                       _rhs_terms(*quads(weight(wk_b), DC // 2)), klog)
        kt, kp = [], []
        for j in range(NS):
            k11, k12, k21, k22 = sup(kq, j)
            t, p_, allt = rhs_tiles(k11, k21, k12, k22, j < NS - 1)
            kt.append(t)
            kp.append(p_)
            pin_list += allt

        r0 = pl.multiple_of(jnp.clip(h - 1, 0, M // CROWS - 1) * CROWS, CROWS)
        src = jnp.where(h == 0, 0, 2 * M) + r0
        cre = bc_v[pl.ds(pl.multiple_of(src, CROWS), CROWS), :].astype(F32)
        cim = bc_v[pl.ds(pl.multiple_of(src + M, CROWS), CROWS), :].astype(F32)
        cr = coef_v[0, 0:1, :]
        ci = coef_v[1, 0:1, :]
        c_r = cre * cr - cim * ci
        c_i = -(cre * ci + cim * cr)
        ccat_v[pl.ds(r0, CROWS), :] = jnp.concatenate(
            [c_r[:, :MA], c_i[:, :MA], c_r[:, MA:], c_i[:, MA:]], axis=1).astype(BF16)

        t0 = lax.bitwise_and(h, H // 2 - 1) * STEPS
        a_r = [a_v[t] for t in range(4)]
        a_i = [a_v[4 + t] for t in range(4)]
        hr = [st_v[t] for t in range(4)]
        hi = [st_v[4 + t] for t in range(4)]
        for j in range(STEPS):
            pos = (j * SCAN_SPAN * 128) // STEPS
            dep = klog[pos // 128][8 * (pos % 128):8 * (pos % 128) + 8]
            hr = [jnp.where(never, dep, x) for x in hr]
            us = [u_v[kk, pl.ds(t0 + j, NSEG, stride=SEG_STRIDE), :] for kk in range(8)]
            mr, mi = _cmul(a_r, a_i, hr, hi)
            hr = [mr[0] + us[0], mr[1] + us[1], mr[2] + us[2], mr[3] + us[6]]
            hi = [mi[0] + us[3], mi[1] + us[4], mi[2] + us[5], mi[3] + us[7]]
            r0 = pl.multiple_of((t0 + j) * NSEG, NSEG)
            for kk, val in enumerate(hr[:3] + hi[:3] + [hr[3]]):
                h_v[kk, pl.ds(r0, NSEG), :] = val
        for t in range(4):
            st_v[t] = hr[t]
            st_v[4 + t] = hi[t]

        qscale = (D ** -0.5) * math.log2(math.e)
        wq = jnp.concatenate([weight(wq_b), jnp.zeros((2 * D - M, D), F32)], axis=0)
        wqt = _rhs_terms(*quads(wq, D))
        m4, m1, m2, m3, m6, m5 = (nn(lhs_term(xs_v, i, QPIN), wqt[i]) for i in (3, 0, 1, 2, 5, 4))
        m7 = jnp.concatenate([nn(lhs_term(xs_v, 6, QPIN // 2, range(4)), wqt[6]),
                              nn(lhs_term(xs_v, 6, QPIN // 2, range(4, 8)), wqt[6])], axis=0)
        qq = [x * qscale for x in ((m1 + m4) + (m7 - m5), m3 + m5, m2 + m4, (m1 - m2) + (m3 + m6))]
        qt, qp = [None] * NS, [None] * NS
        for j in range(NS - 1, -1, -1):
            qt[j], qp[j], allt = lhs_tiles(*sup(qq, j), j > 0)
            pin_list += allt

        wvt = _rhs_terms(*quads(weight(wv_b), DC // 2))
        m1, m4, m2, m5, m3, m7 = (nn(lhs_term(cs_v, i, VPIN), wvt[i]) for i in (0, 3, 1, 4, 2, 6))
        vq = [(m1 + m4) + (m7 - m5), m3 + m5, m2 + m4, None]
        del pin_list[:]
        vt, vp = [None] * NS, [None] * NS
        for j in range(NS // 2):
            vt[j], vp[j], allt = rhs_tiles(*sup(vq, j), True)
            pin_list += allt
        vq[3] = ((m1 - m2) + m3) + nn(lhs_term(cs_v, 5, VPIN2), wvt[5])
        for j in range(NS // 2, NS):
            vt[j], vp[j], allt = rhs_tiles(*sup(vq, j), j < NS - 1)
            pin_list += allt

        causal = (lax.broadcasted_iota(jnp.int32, (TQ, TQ), 1)
                  <= lax.broadcasted_iota(jnp.int32, (TQ, TQ), 0))

        class Block:
            def __init__(self):
                self.tiles = [{}, {}]
                self.mx = [None, None]
                self.tmp, self.acc, self.p = {}, {}, {}

            def note(self, half, n, x):
                self.tiles[half][n] = x
                self.mx[half] = x if self.mx[half] is None else jnp.maximum(self.mx[half], x)

        blks = [Block() for _ in range(NS)]
        rlog = []
        snaps = []

        def host_tile(x):
            return jnp.where(never64, pin_list.pop(0), x) if pin_list else x

        def smm(i, j, t, lhs=None):
            lhs = host_tile(qt[i][t]) if lhs is None else lhs
            rlog[-1] = nt(bf([[lhs]]), bf([[host_tile(kt[j][t]) if RHOST else kt[j][t]]]))
            return rlog[-1]

        def host_max(r, lhs):
            old = [sn for sn in snaps if sn[0] <= r - AGE]
            if not old:
                return lhs
            pick = [sn for sn in old if sn[1] == old[0][1]][-1]
            snaps[:] = [sn for sn in snaps if sn[1] != pick[1] or sn[0] > pick[0]]
            t_, b_ = (pltpu.bitcast(x, U32) for x in pick[2])
            return [jnp.where(never64, x, y)
                    for x, y in zip((t_[:64], t_[64:], b_[:64], b_[64:]), lhs)]

        def s_run(r, kind, i, arg):
            blk = blks[i]
            if kind == 'a':
                lhs = host_max(r, [qt[i][t] for t in (1, 2, 3, 4)])
                m2, m3, m4, m5 = (smm(i, arg, t, x) for x, t in zip(lhs, (1, 2, 3, 4)))
                blk.tmp[arg] = [m4 - m5, m3 - m2, m3 + m5, m2 + m4]
                return
            if kind == 'd':
                half, kr = arg
                x = nt(bf([qp[i][2 * half:2 * half + 2]]), bf([[kp[i][kr], kp[i][2 + kr]]]))
                rlog[-1] = x
                blk.note(half, 2 * i + kr, jnp.where(causal, x, -1e9) if half == kr else x)
                if kr == 0:
                    return
            else:
                j = arg if kind == 'b' else arg[0]
                tmp = blk.tmp[j]
                if kind == 'b':
                    m1, m6, m7 = (smm(i, j, t) for t in (0, 5, 6))
                    c11, c22 = tmp[0] + (m1 + m7), tmp[1] + (m1 + m6)
                elif arg[1] == 0:
                    m1 = smm(i, j, 0)
                    c11, c22 = tmp[0] + m1, tmp[1] + m1
                else:
                    tmp[6 - arg[1]] = tmp[6 - arg[1]] + smm(i, j, arg[1])
                    return
                blk.note(0, 2 * j + 1, tmp[2])
                blk.note(1, 2 * j, tmp[3])
                blk.note(0, 2 * j, c11)
                blk.note(1, 2 * j + 1, c22)
            snaps.append((r, i, tuple(blk.mx)))

        def row_shift(i):
            blk = blks[i]
            blk.m = []
            for lane in blk.mx:
                m = jnp.max(lane, axis=1, keepdims=True)
                if i > 0:
                    m = m + jnp.log2(jnp.sum(jnp.exp2(lane - m), axis=1, keepdims=True))
                blk.m.append(m)

        def prob(blk, half, n):
            if (half, n) not in blk.p:
                blk.p[half, n] = jnp.exp2(blk.tiles[half][n] - blk.m[half])
            return blk.p[half, n]

        def pv_run(i, t, js):
            blk = blks[i]
            lhs, rhs = [], []
            for j in js:
                if j >= i:
                    half, col = _DIAG[t]
                    lhs.append(prob(blk, half, 2 * i + j - i))
                    rhs.append(vp[i][2 * (j - i) + col])
                    continue
                a11, a12 = (lambda: prob(blk, 0, 2 * j)), (lambda: prob(blk, 0, 2 * j + 1))
                a21, a22 = (lambda: prob(blk, 1, 2 * j)), (lambda: prob(blk, 1, 2 * j + 1))
                lhs.append((
                    lambda: a11() + a22(), lambda: a21() + a22(), a11, a22,
                    lambda: a11() + a12(), lambda: a21() - a11(), lambda: a12() - a22())[t]())
                rhs.append(vt[j][t])
            x = nn(jnp.concatenate(lhs, axis=1).astype(BF16), bf([[r] for r in rhs]))
            blk.acc[t] = x if t not in blk.acc else blk.acc[t] + x
            rlog[-1] = x

        def lane_sums(i):
            out = []
            for half in range(2):
                tl = [p for (hf, _), p in blks[i].p.items() if hf == half]
                if i >= SUMPIN and INDEL:
                    tl[0] = jnp.where(never128, rlog[-INDEL - (INSTAG if half == 0 else 0)], tl[0])
                out.append(functools.reduce(jnp.add, tl))
            return out

        def normalise(i, lanes):
            m = blks[i].acc
            if i > 0:
                ctx = [[(m[0] + m[3]) + (m[6] - m[4]), (m[2] + m[4]) + m[7]],
                       [(m[1] + m[3]) + m[8], (m[0] - m[1]) + (m[2] + m[5])]]
            else:
                ctx = [[m[6], m[7]], [m[8], m[5]]]
            out = [jnp.concatenate(c, axis=1) * _recip(jnp.sum(l, axis=1, keepdims=True))
                   for c, l in zip(ctx, lanes)]
            return jnp.concatenate(out, axis=0).astype(BF16)

        def o_run(hh, i, ctx, r0, lanes):
            n = (M - r0) // 16
            rows = [[wot_v[hh, r0 // 2 + 8 * g:r0 // 2 + 8 * g + 8, c * 128:(c + 1) * 128]
                     for c in range(2)] for g in range(n)]
            if lanes is not None:
                for g in range(32 if OPIN else 0):
                    k = 2 * n - 1 - ((31 - g) * max(2 * (n - OS0), 32)) // 32
                    l = lanes[g // 16][8 * (g % 16):8 * (g % 16) + 8]
                    rows[k // 2][k % 2] = jnp.where(never, pltpu.bitcast(l, U32), rows[k // 2][k % 2])
            o = nt(bf(rows), ctx)
            acc_v[r0:M, 2 * i * TQ:(2 * i + 2) * TQ] += o
            return o

        rounds, events = _plan()
        ctx = None
        for r in range(max(events)):
            rlog.append(None)
            for u in (rounds[r] if r < len(rounds) else []):
                if u[0] == 'p':
                    pv_run(*u[1:])
                else:
                    s_run(r, *u)
            for kind, i in events.get(r + 1, []):
                if kind == 'm':
                    row_shift(i)
                    continue
                lanes = lane_sums(i)
                pins = lanes if i >= SUMPIN else None
                if ctx is None:
                    o = o_run(hprev, 0, carried(0), O_TOP, pins)
                else:
                    o = o_run(h, i + 1, ctx, 0, pins)
                if pins is not None and XDEL:
                    x0 = 8 * min(XD0, o.shape[0] // 8 - 16)
                    lanes = [jnp.where(never128, o[x0:x0 + TQ, c * TQ:(c + 1) * TQ], l)
                             for c, l in enumerate(lanes)]
                ctx = normalise(i, lanes)
        ctxc_v[0] = pltpu.bitcast(ctx, U32)
        return 0

    with jax.named_scope('heads'):
        lax.fori_loop(0, H, head, 0)

    @jax.named_scope('epilogue')
    def _epilogue():
        for cp in w_copies(jnp.int32(H - 1), H, 0):
            cp.wait()
        for e in range(O_LAG):
            out_proj(H - 1, e, carried(e))

        def o_copy(c0, width):
            cols = pl.ds(c0, width)
            return pltpu.make_async_copy(acc_v.at[:, cols], out_hbm.at[:, cols], sem.at[0])

        def segment(s, c_cat, pieces):
            c0 = s * LSEG if isinstance(s, int) else pl.multiple_of(s * LSEG, LSEG)
            hs = jnp.concatenate(
                [h_v[kk, pl.ds(s, LSEG, stride=NSEG), :] for kk in range(7)],
                axis=1).astype(BF16)
            yt = lax.dot_general(c_cat, hs, NT, preferred_element_type=F32)
            w = LSEG // pieces
            for e in range(pieces):
                ce = c0 + e * w
                cols = pl.ds(ce, w)
                xf = xt_v[:, cols].astype(F32)
                dsk = jnp.concatenate([col_v[0]] * (w // 128), axis=1)
                gw = jnp.concatenate([col_v[1]] * (w // 128), axis=1)
                g = jax.nn.sigmoid(jnp.sum(xf * gw, axis=0, keepdims=True))
                y = yt[:, e * w:(e + 1) * w] + xf * dsk
                acc_v[:, cols] = g * acc_v[:, cols] + (1.0 - g) * y
                o_copy(ce, w).start()

        if EC == NSEG:
            c_cat = ccat_v[...]
            for s in range(NSEG - 1, -1, -1):
                segment(s, c_cat, 2 if s == 0 else 1)
        else:
            def out_step(it, _):
                c_cat = ccat_v[...]
                for e in range(EC):
                    segment(it * EC + e, c_cat, 1)
                return 0

            lax.fori_loop(0, NSEG // EC, out_step, 0)
        o_copy(0, S).wait()

    _epilogue()


@jax.jit
def pallas_gated_mix__compressed_kv_cla__ssm_conv_s5__prompt_kernel(
    A_x: jax.Array,
    A_c_kv: jax.Array,
    A_w_q: jax.Array,
    A_w_uk: jax.Array,
    A_w_uv: jax.Array,
    A_w_o: jax.Array,
    B_x: jax.Array,
    B_Lambda_re: jax.Array,
    B_Lambda_im: jax.Array,
    B_B_re: jax.Array,
    B_B_im: jax.Array,
    B_C_re: jax.Array,
    B_C_im: jax.Array,
    B_log_dt: jax.Array,
    B_Dskip: jax.Array,
    gate_w: jax.Array,
):
    del B_x
    hbm_spec = pl.BlockSpec(memory_space=pltpu.HBM)
    out_t = pl.pallas_call(
        _kernel,
        in_specs=[hbm_spec] * 15,
        out_specs=hbm_spec,
        out_shape=jax.ShapeDtypeStruct((M, S), F32),
        scratch_shapes=[
            pltpu.VMEM((M, S), BF16),
            pltpu.VMEM((7, 2, HS // 2, 128), U32),
            pltpu.VMEM((S, DC), BF16),
            pltpu.VMEM((7, 4, HS // 2, 128), U32),
            pltpu.VMEM((H + 1, M // 2, D), U32),
            pltpu.VMEM((2, M, D), U32),
            pltpu.VMEM((2, DC, D), U32),
            pltpu.VMEM((2, DC, D), U32),
            pltpu.VMEM((4 * M, M), BF16),
            pltpu.VMEM((M, 2 * M), BF16),
            pltpu.VMEM((M,), BF16), pltpu.VMEM((M,), BF16), pltpu.VMEM((M,), BF16),
            pltpu.VMEM((M,), BF16), pltpu.VMEM((M,), BF16),
            pltpu.VMEM((2, M, 128), F32),
            pltpu.VMEM((2, 8, M), F32),
            pltpu.VMEM((8, NSEG * SEG_STRIDE, 128), F32),
            pltpu.VMEM((7, S, 128), F32),
            pltpu.VMEM((8, NSEG, 128), F32),
            pltpu.VMEM((8, NSEG, 128), F32),
            pltpu.VMEM((M, S), F32),
            pltpu.VMEM((O_LAG, TQ, D), U32),
            pltpu.VMEM((8, 128), jnp.int32),
            pltpu.SemaphoreType.DMA((SEM_X + NPRO,)),
        ],
        compiler_params=pltpu.CompilerParams(vmem_limit_bytes=110 * 1024 * 1024),
        name="gated_mix",
    )(
        A_x.reshape(S, M).T, A_c_kv.reshape(S, DC),
        A_w_q, A_w_uk, A_w_uv, jnp.swapaxes(A_w_o, 1, 2),
        B_Lambda_re, B_Lambda_im, B_B_re, B_B_im, B_C_re, B_C_im, B_log_dt,
        B_Dskip, gate_w,
    )
    return out_t.T.reshape(1, S, M)
```

```python
import functools
import math
import os

import jax
import jax.numpy as jnp
from jax import lax
import jax.experimental.pallas as pl
import jax.experimental.pallas.tpu as pltpu

F32 = jnp.float32
BF16 = jnp.bfloat16
U32 = jnp.uint32

S = 2048
HS = S // 2
M = 448
DC = 1024
H = 16
D = 256
TQ = 128
NB = S // TQ
NS = NB // 2
NSEG = 8
LSEG = S // NSEG
SEG_STRIDE = LSEG + 8
STEPS = 2 * LSEG // H
MA = 384
MR = M - MA
NT = (((1,), (1,)), ((), ()))
O_LAG = int(os.environ.get('O_LAG', 1))
NPRO = NSEG // 2
EC = int(os.environ.get('EC', 8))
_om = os.environ.get('ORDER', 'desc')
if _om == 'asc':
    ORDER = list(range(NS))
elif _om == 'desc':
    ORDER = list(range(NS))[::-1]
else:
    ORDER = [int(t) for t in _om.split(',')]
LOOK = int(os.environ.get('LOOK', 1))
PRE_S = int(os.environ.get('PRE_S', 2))
KV_JOINT = int(os.environ.get('KV_JOINT', 0))
SEM_W = 3
SEM_X = 5
PV_K = int(os.environ.get('PV_K', 256))
O_SPLIT = int(os.environ.get('O_SPLIT', 0))
O_POS = int(os.environ.get('O_POS', 1))
S_AB = int(os.environ.get('S_AB', 1))
PV_SEQ = int(os.environ.get('PV_SEQ', 0))
S_AT = int(os.environ.get('S_AT', 6))
PINS = [int(t) for t in os.environ.get('PINS', '2222222')]
RCP_EUP = int(os.environ.get('RCP_EUP', 1))
MG = int(os.environ.get('MG', 1))
MLAG = int(os.environ.get('MLAG', 2))
SG = int(os.environ.get('SG', 0))
SLAG = int(os.environ.get('SLAG', 1))
D_FIRST = int(os.environ.get('D_FIRST', 0))
HEAD = int(os.environ.get('HEAD', 4))
BPIN = int(os.environ.get('BPIN', 0))
BLAG = int(os.environ.get('BLAG', 1))
BALT = int(os.environ.get('BALT', 1))
DSUM = int(os.environ.get('DSUM', 1))
DS0 = int(os.environ.get('DS0', 0))
DS1 = int(os.environ.get('DS1', 2))
O_TOP = int(os.environ.get('O_TOP', 160))
DMAX = int(os.environ.get('DMAX', 1))
DM0 = int(os.environ.get('DM0', 0))
DM1 = int(os.environ.get('DM1', 1))
CW = 352
CSTEP = 336
XLO = int(os.environ.get('XLO', 40))
XHI = int(os.environ.get('XHI', 420))
CLO = int(os.environ.get('CLO', 0))
CHI = int(os.environ.get('CHI', 420))
DPIN = int(os.environ.get('DPIN', 1))
PS = int(os.environ.get('PS', 1))
VPIN = int(os.environ.get('VPIN', 12))
QPIN = int(os.environ.get('QPIN', 10))
SCAN_SPAN = int(os.environ.get('SCAN_SPAN', 5))
LREUSE = int(os.environ.get('LREUSE', 0))
PD_FIRST = int(os.environ.get('PD_FIRST', 0))
PORDER = [int(t) for t in os.environ.get('PORDER', '2301546')]
PG = int(os.environ.get('PG', 4))
PGROUPS = [[(j, min(j + PG, i)) for j in range(0, i, PG)] for i in range(8)]
if PG == 4:
    PGROUPS[7] = [(0, 4), (4, 6), (6, 7)]
    PGROUPS[3] = [(0, 2), (2, 3)]
LEAD0 = int(os.environ.get('LEAD0', 4))
LEAD = int(os.environ.get('LEAD', 5))
BAL = int(os.environ.get('BAL', 10))
FILL0 = int(os.environ.get('FILL0', 3))
CAP = int(os.environ.get('CAP', 112))
MCOST = int(os.environ.get('MCOST', 32))
PHOST = int(os.environ.get('PHOST', 1))
EARLY = int(os.environ.get('EARLY', 0))
VPIN2 = int(os.environ.get('VPIN2', 28))
RHOST = int(os.environ.get('RHOST', 0))
AGE = int(os.environ.get('AGE', 3))
ODELAY = int(os.environ.get('ODELAY', 0))
SUMPIN = int(os.environ.get('SUMPIN', 1))
OS0 = int(os.environ.get('OS0', 2))
XDEL = int(os.environ.get('XDEL', 0))
XD0 = int(os.environ.get('XD0', 0))
INDEL = int(os.environ.get('INDEL', 1))
INSTAG = int(os.environ.get('INSTAG', 1))
OPIN = int(os.environ.get('OPIN', 1))
SPLIT = [int(t) for t in os.environ.get('SPLIT', '73')]
CARRY = [(min(SPLIT), t) for t in (5, 6, 0)][min(SPLIT) - 1:]
W_LOAD = float(os.environ.get('W_LOAD', 1))
W_LATE = float(os.environ.get('W_LATE', 2))
W_NEW = float(os.environ.get('W_NEW', 1))
W_UNIT = float(os.environ.get('W_UNIT', 1))
RATIO = float(os.environ.get('RATIO', 0.85))
PTAIL = int(os.environ.get('PTAIL', 50))
OCOST = int(os.environ.get('OCOST', 48))
CROWS = 32


_NEEDS = {0: ((0, 0), (1, 1)), 1: ((1, 0), (1, 1)), 2: ((0, 0),), 3: ((1, 1),),
          4: ((0, 0), (0, 1)), 5: ((1, 0), (0, 0)), 6: ((0, 1), (1, 1))}
_DIAG = {8: (1, 0), 5: (1, 1), 6: (0, 0), 7: (0, 1)}


def _plan():
    i = NS - 1
    sq = [(4, 'a', i, 0), (4, 'a', i, 1), (3, 'b', i, 0), (1, 's', i, (1, 5)),
          (4, 'a', i, 2), (3, 'b', i, 2), (1, 's', i, (1, 6)),
          (4, 'a', i, 3), (3, 'b', i, 3), (1, 's', i, (1, 0)),
          (4, 'a', i, 4), (4, 'a', i, 5), (3, 'b', i, 4), (1, 's', i, (5, 5)),
          (4, 'a', i, 6), (3, 'b', i, 6), (1, 's', i, (5, 6)),
          (2, 'd', i, (1, 0)), (2, 'd', i, (0, 0)),
          (4, 'a', i - 1, 0), (4, 'a', i - 1, 1),
          (1, 's', i, (5, 0)), (1, 's', i - 1, (1, 5)), (2, 'd', i, (1, 1)),
          (3, 'b', i - 1, 0), (1, 's', i - 1, (1, 6)),
          (4, 'a', i - 1, 2), (3, 'b', i - 1, 2), (1, 's', i - 1, (1, 0))]
    for i in range(NS - 2, -1, -1):
        for j in range(3 if i == NS - 2 else 0, i):
            sq += [(4, 'a', i, j), (3, 'b', i, j)]
        sq += [(2, 'd', i, hk) for hk in ((1, 0), (0, 0), (1, 1))]
    pq = {}
    for i in range(NS):
        pq[i] = [[j1 - j0, t, list(range(j0, j1))] for j0, j1 in PGROUPS[i] for t in PORDER]
        pq[i] += [[2, 8, [i, i + 1]], [2, 5, [i, i + 1]], [1, 6, [i]], [1, 7, [i]]]
    ready, rounds, events, seen = {}, [], {}, set()

    def needs(i, t, js):
        out = set()
        for j in js:
            out |= ({(i, _DIAG[t][0], i + j)} if j >= i else
                    {(i, hf, 2 * j + c) for hf, c in _NEEDS[t]})
        return out

    def p_fill(free, pi, first):
        left = {i: [list(u) for u in pq[i]] for i in (pi, pi - 1) if i >= 0}
        got, new = [], set()
        while free and pi in left and ready.get(pi, 1 << 30) <= len(rounds):
            us = left[pi]
            if first is not None:
                u, first = us[first], None
            else:
                size = min(free, max(v[0] for v in us))
                fit = [v for v in us if v[0] == size] or [
                    v for v in us if v[0] == min(w[0] for w in us if w[0] > size)]
                u = min(fit, key=lambda v: len(needs(pi, v[1], v[2][-size:]) - seen - new))
            size = min(free, u[0])
            got.append(('p', pi, u[1], u[2][-size:]))
            new |= needs(pi, u[1], u[2][-size:]) - seen
            u[2], u[0] = u[2][:len(u[2]) - size], u[0] - size
            if not u[0]:
                us.remove(u)
            free -= size
            if not us:
                pi -= 1
        return got, new, free, left, pi

    pi, prev = NS - 1, 0
    while sq or pi >= 0:
        cands = []
        if sq:
            n, free = 0, 4
            while n < len(sq) and sq[n][0] <= free and (n == 0 or sq[n][1] == 's' or sq[n - 1][1] == 's'):
                free -= sq[n][0]
                n += 1
            cands.append((n,) + p_fill(free, pi, None))
            if free == 2 and n < len(sq) and sq[n][0] == 2:
                cands.append((n + 1,) + p_fill(0, pi, None))
        if pi >= 0:
            big = max(u[0] for u in pq[pi])
            grp = next(u[2] for u in pq[pi] if u[0] == big)
            cands += [(0,) + p_fill(4, pi, k) for k, u in enumerate(pq[pi]) if u[2] == grp]
        best = None
        for n, got, new, free, left, p2 in cands:
            s_left = sum(u[0] for u in sq[n:] if u[2] >= pi - 1)
            p_left = sum(u[0] for u in left.get(pi, []))
            s_all = sum(u[0] for u in sq[n:])
            p_all = sum(u[0] for i in range(pi + 1) for u in left.get(i, pq[i]))
            load = prev + 16 * len(new) + (MCOST if n and sq[0][1] == 'a' else 0)
            late = max(s_left + BAL - p_left, 0) if s_left else 0
            drift = abs(s_all - RATIO * max(p_all - PTAIL, 0))
            cost = (1000 * free + W_LOAD * max(load - CAP, 0) + W_LATE * late + drift
                    - W_NEW * len(new) + W_UNIT * len(got))
            if best is None or cost < best[0]:
                best = (cost, n, got, new, left, p2)
        _, n, got, new, left, p2 = best
        cur = [u[1:] for u in sq[:n]] + got
        done = {u[2] for u in sq[:n]}
        del sq[:n]
        seen |= new
        pq.update(left)
        rounds.append(cur)
        for i in done:
            if all(v[2] != i for v in sq):
                events.setdefault(len(rounds), []).append(('m', i))
                ready[i] = len(rounds) + (LEAD0 if i == NS - 1 else LEAD)
        prev = sum({'a': 64, 'b': 32, 'd': 16, 's': 24, 'p': 16}[u[0]] for u in cur)
        for i in range(pi, p2, -1):
            events.setdefault(len(rounds), []).append(('o', i))
            prev = OCOST
        pi = p2
    return rounds, events


def _lhs_terms(a11, a12, a21, a22):
    return [t.astype(BF16) for t in
            (a11 + a22, a21 + a22, a11, a22, a11 + a12, a21 - a11, a12 - a22)]


def _rhs_terms(b11, b12, b21, b22):
    return [t.astype(BF16) for t in
            (b11 + b22, b11, b12 - b22, b21 - b11, b22, b11 + b12, b21 + b22)]


def _strassen(lhs, rhs, log):
    def mm(i):
        log.append(jnp.dot(lhs(i), rhs[i], preferred_element_type=F32))
        return log[-1]
    m1 = mm(0)
    m4 = mm(3)
    c11 = m1 + m4
    m2 = mm(1)
    c21 = m2 + m4
    c22 = m1 - m2
    m5 = mm(4)
    c11 = c11 - m5
    m3 = mm(2)
    c12 = m3 + m5
    c22 = c22 + m3
    c11 = c11 + mm(6)
    c22 = c22 + mm(5)
    return c11, c12, c21, c22


def _recip(l):
    if RCP_EUP:
        r = pl.reciprocal(l, approx=True)
        return r * (2.0 - l * r)
    r = pltpu.bitcast(jnp.int32(0x7EF311C3) - pltpu.bitcast(l, jnp.int32), F32)
    for _ in range(3):
        r = r * (2.0 - l * r)
    return r


def _cmul(pr, pi, hr, hi):
    return ([pr[t] * hr[t] - pi[t] * hi[t] for t in range(4)],
            [pr[t] * hi[t] + pi[t] * hr[t] for t in range(4)])


def _column(row):
    row = jnp.concatenate([row, jnp.zeros((1, 512 - M), F32)], axis=1)
    return jnp.broadcast_to(row, (128, 512)).T[:M]


def _kernel(xt_hbm, c_hbm, wq_hbm, wk_hbm, wv_hbm, wot_hbm,
            lre_hbm, lim_hbm, bre_hbm, bim_hbm, cre_hbm, cim_hbm, ldt_hbm,
            dsk_hbm, gw_hbm,
            out_hbm,
            xt_v, xs_v, c_v, cs_v, wot_v, wt_v, wq_b, wk_b, wv_b, bc_v, ccat_v,
            lre_v, lim_v, ldt_v, dsk_v, gw_v, col_v, coef_v,
            u_v, h_v, a_v, st_v, acc_v, ctxc_v, never_v, sem):
    wq32 = wq_hbm.bitcast(U32)
    wk32 = wk_hbm.bitcast(U32)
    wv32 = wv_hbm.bitcast(U32)
    wot32 = wot_hbm.bitcast(U32)

    def w_copies(h, sl):
        j = lax.shift_right_logical(h, 1)
        cps = [pltpu.make_async_copy(src.at[:, j, :], dst.at[sl], sem.at[SEM_W + sl])
               for src, dst in ((wq32, wq_b), (wk32, wk_b), (wv32, wv_b))]
        return cps + [pltpu.make_async_copy(wot32.at[h], wot_v.at[sl], sem.at[SEM_W + sl])]

    def x_copies(s):
        spans = [pl.ds(pl.multiple_of(s * LSEG + e * HS, LSEG), LSEG) for e in range(2)]
        return [pltpu.make_async_copy(xt_hbm.at[:, sp], xt_v.at[:, sp], sem.at[SEM_X + s])
                for sp in spans]

    def c_copies(start, rows, s):
        spans = [pl.ds(pl.multiple_of(start + e * HS, 16), rows) for e in range(2)]
        return [pltpu.make_async_copy(c_hbm.at[sp], c_v.at[sp], sem.at[SEM_X + s])
                for sp in spans]

    def stage_copies(s):
        return x_copies(s) + c_copies(CW - CSTEP + (s - 1) * CSTEP, CSTEP, s)

    first_cps = x_copies(0) + [
        pltpu.make_async_copy(bre_hbm.at[MA:M], bc_v.at[0:MR], sem.at[SEM_X]),
        pltpu.make_async_copy(bim_hbm.at[MA:M], bc_v.at[MR:2 * MR], sem.at[SEM_X]),
        pltpu.make_async_copy(bre_hbm.at[0:MA], bc_v.at[2 * MR:2 * MR + MA], sem.at[SEM_X]),
        pltpu.make_async_copy(bim_hbm.at[0:MA], bc_v.at[2 * MR + MA:2 * M], sem.at[SEM_X]),
    ] + c_copies(0, CW - CSTEP, 0)
    vec_cps = [pltpu.make_async_copy(src, dst, sem.at[1]) for src, dst in
               ((lre_hbm, lre_v), (lim_hbm, lim_v), (ldt_hbm, ldt_v), (dsk_hbm, dsk_v),
                (gw_hbm, gw_v))]
    late_cps = [pltpu.make_async_copy(cre_hbm, bc_v.at[2 * M:3 * M], sem.at[2]),
                pltpu.make_async_copy(cim_hbm, bc_v.at[3 * M:4 * M], sem.at[2])]

    @jax.named_scope('prologue')
    def _prologue():
        zero = jnp.int32(0)
        first = vec_cps + first_cps
        for s in range(1, NPRO):
            first = first + stage_copies(s)
        for cp in first + w_copies(zero, 0) + late_cps:
            cp.start()
        acc_v[...] = jnp.zeros_like(acc_v)
        st_v[...] = jnp.zeros_like(st_v)
        ctxc_v[...] = jnp.zeros_like(ctxc_v)
        wt_v[1] = jnp.zeros(wt_v.shape[1:], U32)
        never_v[...] = jnp.zeros_like(never_v)

        for cp in vec_cps:
            cp.wait()
        lre = lre_v[...].astype(F32).reshape(1, M)
        lim = lim_v[...].astype(F32).reshape(1, M)
        dt = jnp.exp(ldt_v[...].astype(F32)).astype(BF16).astype(F32).reshape(1, M)
        er = jnp.exp(dt * lre)
        ar = er * jnp.cos(dt * lim)
        ai = er * jnp.sin(dt * lim)
        den = lre * lre + lim * lim
        coef_v[0] = jnp.broadcast_to(2.0 * ((ar - 1.0) * lre + ai * lim) / den, (8, M))
        coef_v[1] = jnp.broadcast_to(2.0 * (ai * lre - (ar - 1.0) * lim) / den, (8, M))

        def bc(v):
            return jnp.broadcast_to(v, (NSEG, 128))

        for t in range(3):
            a_v[t] = bc(ar[:, t * 128:(t + 1) * 128])
            a_v[4 + t] = bc(ai[:, t * 128:(t + 1) * 128])
        a_v[3] = bc(jnp.concatenate([ar[:, MA:], ar[:, MA:]], axis=1))
        a_v[7] = bc(jnp.concatenate([ai[:, MA:], -ai[:, MA:]], axis=1))
        col_v[0] = _column(dsk_v[...].astype(F32).reshape(1, M))
        col_v[1] = _column(gw_v[...].astype(F32).reshape(1, M))

        never = never_v[...] != 0

        def spread(us, rows, cols, lo, hi):
            out = []
            for c in range(cols):
                vr = []
                for g in range(rows):
                    n = lo + ((c * rows + g) * (hi - lo)) // (rows * cols)
                    e, t, rg = n // 224, (n % 224) // 32, n % 32
                    vr.append(us[e][8 * rg:8 * rg + 8, 128 * t:128 * t + 128])
                out.append(jnp.concatenate(vr, axis=0))
            mask = jnp.concatenate([jnp.concatenate([never] * rows, axis=0)] * cols, axis=1)
            return mask, jnp.concatenate(out, axis=1)

        def bu(s):
            b_cat = bc_v[0:2 * M, :]
            r = pl.ds(pl.multiple_of(s * (LSEG // 2), LSEG // 2), LSEG // 2)
            xs = []
            us = []
            for e in range(2):
                c0 = pl.multiple_of(s * LSEG + e * HS, LSEG)
                xe = xt_v[:, pl.ds(c0, LSEG)].T
                u = lax.dot_general(xe, b_cat, NT, preferred_element_type=F32)
                us.append(u)
                rows = pl.ds(pl.multiple_of((s + e * NPRO) * SEG_STRIDE, 8), LSEG)
                u_v[6, rows, :] = u[:, :128]
                u_v[7, rows, :] = pltpu.roll(u[:, :128], MR, 1)
                for t in range(6):
                    u_v[t, rows, :] = u[:, (t + 1) * 128:(t + 2) * 128]
                xe = xe.astype(F32)
                xs.append((xe[:, :D], jnp.concatenate(
                    [xe[:, D:], jnp.zeros((LSEG, 2 * D - M), F32)], axis=1)))
            mask, dep = spread(us, 32, 2, XLO, XHI)
            a11 = jnp.where(mask, dep, xs[0][0])
            a22 = jnp.where(mask, dep, xs[1][1])
            for i, t in enumerate(_lhs_terms(a11, xs[0][1], xs[1][0], a22)):
                t = pltpu.bitcast(t, U32)
                for kt in range(2):
                    xs_v[i, kt, r, :] = t[:, kt * 128:(kt + 1) * 128]
            return us

        def c_terms(s, us):
            hc = DC // 2
            r = pl.ds(pl.multiple_of(s * (CSTEP // 2), 8), CW // 2)
            rt = pl.ds(pl.multiple_of(s * CSTEP, 16), CW)
            rb = pl.ds(pl.multiple_of(s * CSTEP + HS, 16), CW)
            a11, a12, a21, a22 = c_v[rt, :hc], c_v[rt, hc:], c_v[rb, :hc], c_v[rb, hc:]
            mask, dep = spread(us, CW // 16, 4, CLO, CHI)
            dep = pltpu.bitcast(dep, U32)
            a11 = pltpu.bitcast(jnp.where(mask, dep, pltpu.bitcast(a11, U32)), BF16)
            a22 = pltpu.bitcast(jnp.where(mask, dep, pltpu.bitcast(a22, U32)), BF16)
            terms = _lhs_terms(*(a.astype(F32) for a in (a11, a12, a21, a22)))
            for i, t in enumerate(terms):
                t = pltpu.bitcast(t, U32)
                for kt in range(4):
                    cs_v[i, kt, r, :] = t[:, kt * 128:(kt + 1) * 128]

        for cp in first_cps:
            cp.wait()
        bu(0)

        def pro_step(s, _):
            for cp in stage_copies(s):
                cp.wait()
            c_terms(s - 1, bu(s))
            return 0

        lax.fori_loop(1, NPRO, pro_step, 0)

    _prologue()

    HM = M // 2

    def o_tiles(jobs, host=None):
        lhs = [[wt_v[sl, t, 8 * g:8 * g + 8, :] for g in range(HM // 16)] for sl, t, _ in jobs]
        if host is not None:
            host(lhs)
        return [lax.dot_general(pltpu.bitcast(jnp.concatenate(l, axis=0), BF16),
                                c, NT, preferred_element_type=F32)
                for l, (_, _, c) in zip(lhs, jobs)]

    def o_add(i, quad, x):
        r0, c0 = (quad // 2) * HM, (2 * i + quad % 2) * TQ
        acc_v[r0:r0 + HM, c0:c0 + TQ] += x

    def o_finish_a(i, m2, m3, m4, m5):
        o_add(i, 0, m4 - m5)
        o_add(i, 1, m3 + m5)
        o_add(i, 2, m2 + m4)
        o_add(i, 3, m3 - m2)

    def o_round_a(sl, i, ct, host=None):
        ms = o_tiles([(sl, t, ct[t]) for t in (1, 2, 3, 4)], host)
        o_finish_a(i, *ms)
        return ms

    def o_single(i, t, m):
        if t != 5:
            o_add(i, 0, m)
        if t != 6:
            o_add(i, 3, m)

    def o_round_b(sl, i, ct, extra, host=None):
        ms = o_tiles([(sl, t, ct[t]) for t in (0, 5, 6)] + [(e[0], e[2], e[3]) for e in extra], host)
        o_add(i, 0, ms[0] + ms[2])
        o_add(i, 3, ms[0] + ms[1])
        for e, m in zip(extra, ms[3:]):
            o_single(e[1], e[2], m)
        return ms

    def carried(sl):
        ct = [ctxc_v[t] for t in range(7)]
        return ct, [(sl, i, t, ctxc_v[7 + n]) for n, (i, t) in enumerate(CARRY)]

    def head(h, _):
        slot = lax.bitwise_and(h, 1)

        @pl.when(h == H // 2)
        def _segment_carry():
            pr = [a_v[t] for t in range(4)]
            pi = [a_v[4 + t] for t in range(4)]
            for _ in range(int(math.log2(LSEG))):
                pr, pi = ([pr[t] * pr[t] - pi[t] * pi[t] for t in range(4)],
                          [2.0 * pr[t] * pi[t] for t in range(4)])
            row = lax.broadcasted_iota(jnp.int32, (NSEG, 128), 0)
            e_r = [st_v[t] for t in range(4)]
            e_i = [st_v[4 + t] for t in range(4)]
            ir = [jnp.zeros((NSEG, 128), F32)] * 4
            ii = ir
            for s in range(1, NSEG):
                mr, mi = _cmul(pr, pi, ir, ii)
                fr = [pltpu.roll(mr[k] + e_r[k], 1, 0) for k in range(4)]
                fi = [pltpu.roll(mi[k] + e_i[k], 1, 0) for k in range(4)]
                ir = [jnp.where(row == s, fr[k], ir[k]) for k in range(4)]
                ii = [jnp.where(row == s, fi[k], ii[k]) for k in range(4)]
            for t in range(4):
                st_v[t] = ir[t]
                st_v[4 + t] = ii[t]

        @pl.when(h == 1)
        def _():
            for cp in late_cps:
                cp.wait()

        for cp in w_copies(h, slot):
            cp.wait()

        o_prev = o_tiles([(1 - slot, t, ctxc_v[t]) for t in (1, 2, 3, 4)])
        for cp in w_copies(jnp.minimum(h + 1, H - 1), 1 - slot):
            cp.start()
        o_finish_a(0, *o_prev)
        ct0, singles = carried(1 - slot)

        up = ((1 - slot) * 16).astype(U32)
        never = never_v[...] != 0
        never64 = jnp.concatenate([never] * 8, axis=0)
        never128 = jnp.concatenate([never] * 16, axis=0)

        def weight(buf):
            return pltpu.bitcast((buf[slot] << up) & jnp.uint32(0xFFFF0000), F32)

        def quads(w, kh):
            return w[:kh, :128], w[:kh, 128:], w[kh:, :128], w[kh:, 128:]

        def bf(rows):
            return pltpu.bitcast(jnp.concatenate(
                [jnp.concatenate(r, axis=1) for r in rows], axis=0), BF16)

        def pk(x):
            return pltpu.bitcast(x.astype(BF16), U32)

        def nt(a, b):
            return lax.dot_general(a, b, NT, preferred_element_type=F32)

        def nn(a, b):
            return jnp.dot(a, b, preferred_element_type=F32)

        pin_list = []

        def lhs_term(ref, i, npin, order=range(8)):
            ncol = ref.shape[1]
            rows = [[ref[i, c, g * 64:(g + 1) * 64, :] for c in range(ncol)] for g in order]
            nr = len(rows) - 1
            npin = min(npin, len(pin_list), nr * ncol)
            for n in range(npin):
                g, c = 1 + (n * nr) // npin, n % ncol
                rows[g][c] = jnp.where(never64, pin_list.pop(0), rows[g][c])
            return bf(rows)

        def sup(cq, j):
            l, r = (cq[0], cq[1]) if j < NS // 2 else (cq[2], cq[3])
            r0 = (j % (NS // 2)) * 2 * TQ
            return l[r0:r0 + TQ], r[r0:r0 + TQ], l[r0 + TQ:r0 + 2 * TQ], r[r0 + TQ:r0 + 2 * TQ]

        def rhs_tiles(b11, b12, b21, b22, with_terms):
            plain = [pk(b11), pk(b12), pk(b21), pk(b22)]
            if not with_terms:
                return None, plain, plain
            extra = [pk(b11 + b22), pk(b12 - b22), pk(b21 - b11), pk(b11 + b12), pk(b21 + b22)]
            terms = [extra[0], plain[0], extra[1], extra[2], plain[3], extra[3], extra[4]]
            return terms, plain, plain + extra

        def lhs_tiles(a11, a12, a21, a22, with_terms):
            plain = [pk(a11), pk(a12), pk(a21), pk(a22)]
            if not with_terms:
                return None, plain, plain
            extra = [pk(a11 + a22), pk(a21 + a22), pk(a11 + a12), pk(a21 - a11), pk(a12 - a22)]
            terms = [extra[0], extra[1], plain[0], plain[3], extra[2], extra[3], extra[4]]
            return terms, plain, plain + extra

        klog = []
        kq = _strassen(lambda i: lhs_term(cs_v, i, 0),
                       _rhs_terms(*quads(weight(wk_b), DC // 2)), klog)
        kt, kp = [], []
        for j in range(NS):
            k11, k12, k21, k22 = sup(kq, j)
            t, p_, allt = rhs_tiles(k11, k21, k12, k22, j < NS - 1)
            kt.append(t)
            kp.append(p_)
            pin_list += allt

        r0 = pl.multiple_of(jnp.clip(h - 1, 0, M // CROWS - 1) * CROWS, CROWS)
        src = jnp.where(h == 0, 0, 2 * M) + r0
        cre = bc_v[pl.ds(pl.multiple_of(src, CROWS), CROWS), :].astype(F32)
        cim = bc_v[pl.ds(pl.multiple_of(src + M, CROWS), CROWS), :].astype(F32)
        cr = coef_v[0, 0:1, :]
        ci = coef_v[1, 0:1, :]
        c_r = cre * cr - cim * ci
        c_i = -(cre * ci + cim * cr)
        ccat_v[pl.ds(r0, CROWS), :] = jnp.concatenate(
            [c_r[:, :MA], c_i[:, :MA], c_r[:, MA:], c_i[:, MA:]], axis=1).astype(BF16)

        t0 = lax.bitwise_and(h, H // 2 - 1) * STEPS
        a_r = [a_v[t] for t in range(4)]
        a_i = [a_v[4 + t] for t in range(4)]
        hr = [st_v[t] for t in range(4)]
        hi = [st_v[4 + t] for t in range(4)]
        for j in range(STEPS):
            pos = (j * SCAN_SPAN * 128) // STEPS
            dep = klog[pos // 128][8 * (pos % 128):8 * (pos % 128) + 8]
            hr = [jnp.where(never, dep, x) for x in hr]
            us = [u_v[kk, pl.ds(t0 + j, NSEG, stride=SEG_STRIDE), :] for kk in range(8)]
            mr, mi = _cmul(a_r, a_i, hr, hi)
            hr = [mr[0] + us[0], mr[1] + us[1], mr[2] + us[2], mr[3] + us[6]]
            hi = [mi[0] + us[3], mi[1] + us[4], mi[2] + us[5], mi[3] + us[7]]
            r0 = pl.multiple_of((t0 + j) * NSEG, NSEG)
            for kk, val in enumerate(hr[:3] + hi[:3] + [hr[3]]):
                h_v[kk, pl.ds(r0, NSEG), :] = val
        for t in range(4):
            st_v[t] = hr[t]
            st_v[4 + t] = hi[t]

        wo = pltpu.bitcast(wot_v[slot], BF16).astype(F32)
        w11, w12, w21, w22 = quads(wo, HM)
        dep = jnp.concatenate([klog[5][32 * g:32 * g + 8] for g in range(HM // 8)], axis=0)
        nv = jnp.concatenate([never] * (HM // 8), axis=0)
        for t, val in enumerate(_lhs_terms(jnp.where(nv, dep, w11), w12, w21,
                                           jnp.where(nv, dep, w22))):
            wt_v[slot, t] = pltpu.bitcast(val, U32)

        qscale = (D ** -0.5) * math.log2(math.e)
        wq = jnp.concatenate([weight(wq_b), jnp.zeros((2 * D - M, D), F32)], axis=0)
        wqt = _rhs_terms(*quads(wq, D))
        m4, m1, m2, m3, m6, m5 = (nn(lhs_term(xs_v, i, QPIN), wqt[i]) for i in (3, 0, 1, 2, 5, 4))
        m7 = jnp.concatenate([nn(lhs_term(xs_v, 6, QPIN // 2, range(4)), wqt[6]),
                              nn(lhs_term(xs_v, 6, QPIN // 2, range(4, 8)), wqt[6])], axis=0)
        qq = [x * qscale for x in ((m1 + m4) + (m7 - m5), m3 + m5, m2 + m4, (m1 - m2) + (m3 + m6))]
        qt, qp = [None] * NS, [None] * NS
        for j in range(NS - 1, -1, -1):
            qt[j], qp[j], allt = lhs_tiles(*sup(qq, j), j > 0)
            pin_list += allt

        wvt = _rhs_terms(*quads(weight(wv_b), DC // 2))
        m1, m4, m2, m5, m3, m7 = (nn(lhs_term(cs_v, i, VPIN), wvt[i]) for i in (0, 3, 1, 4, 2, 6))
        vq = [(m1 + m4) + (m7 - m5), m3 + m5, m2 + m4, None]
        del pin_list[:]
        vt, vp = [None] * NS, [None] * NS
        for j in range(NS // 2):
            vt[j], vp[j], allt = rhs_tiles(*sup(vq, j), True)
            pin_list += allt
        vq[3] = ((m1 - m2) + m3) + nn(lhs_term(cs_v, 5, VPIN2), wvt[5])
        for j in range(NS // 2, NS):
            vt[j], vp[j], allt = rhs_tiles(*sup(vq, j), j < NS - 1)
            pin_list += allt

        vn = [[x ^ jnp.uint32(0x80008000) for x in t] for t in vp]
        causal = (lax.broadcasted_iota(jnp.int32, (TQ, TQ), 1)
                  <= lax.broadcasted_iota(jnp.int32, (TQ, TQ), 0))

        class Block:
            def __init__(self):
                self.tiles = [{}, {}]
                self.mx = [None, None]
                self.tmp, self.acc, self.p = {}, {}, {}

            def note(self, half, n, x):
                self.tiles[half][n] = x
                self.mx[half] = x if self.mx[half] is None else jnp.maximum(self.mx[half], x)

        blks = [Block() for _ in range(NS)]
        rlog = []
        snaps = []

        def host_tile(x):
            return jnp.where(never64, pin_list.pop(0), x) if pin_list else x

        def smm(i, j, t, lhs=None):
            lhs = host_tile(qt[i][t]) if lhs is None else lhs
            rlog[-1] = nt(bf([[lhs]]), bf([[host_tile(kt[j][t]) if RHOST else kt[j][t]]]))
            return rlog[-1]

        def host_max(r, lhs):
            old = [sn for sn in snaps if sn[0] <= r - AGE]
            if not old:
                return lhs
            pick = [sn for sn in old if sn[1] == old[0][1]][-1]
            snaps[:] = [sn for sn in snaps if sn[1] != pick[1] or sn[0] > pick[0]]
            t_, b_ = (pltpu.bitcast(x, U32) for x in pick[2])
            return [jnp.where(never64, x, y)
                    for x, y in zip((t_[:64], t_[64:], b_[:64], b_[64:]), lhs)]

        def s_run(r, kind, i, arg):
            blk = blks[i]
            if kind == 'a':
                lhs = host_max(r, [qt[i][t] for t in (1, 2, 3, 4)])
                m2, m3, m4, m5 = (smm(i, arg, t, x) for x, t in zip(lhs, (1, 2, 3, 4)))
                blk.tmp[arg] = [m4 - m5, m3 - m2, m3 + m5, m2 + m4]
                return
            if kind == 'd':
                half, kr = arg
                x = nt(bf([qp[i][2 * half:2 * half + 2]]), bf([[kp[i][kr], kp[i][2 + kr]]]))
                rlog[-1] = x
                blk.note(half, 2 * i + kr, jnp.where(causal, x, -1e9) if half == kr else x)
                if kr == 0:
                    return
            else:
                j = arg if kind == 'b' else arg[0]
                tmp = blk.tmp[j]
                if kind == 'b':
                    m1, m6, m7 = (smm(i, j, t) for t in (0, 5, 6))
                    c11, c22 = tmp[0] + (m1 + m7), tmp[1] + (m1 + m6)
                elif arg[1] == 0:
                    m1 = smm(i, j, 0)
                    c11, c22 = tmp[0] + m1, tmp[1] + m1
                else:
                    tmp[6 - arg[1]] = tmp[6 - arg[1]] + smm(i, j, arg[1])
                    return
                blk.note(0, 2 * j + 1, tmp[2])
                blk.note(1, 2 * j, tmp[3])
                blk.note(0, 2 * j, c11)
                blk.note(1, 2 * j + 1, c22)
            snaps.append((r, i, tuple(blk.mx)))

        def row_shift(i):
            blk = blks[i]
            blk.m = []
            for lane in blk.mx:
                m = jnp.max(lane, axis=1, keepdims=True)
                if i > 0:
                    m = m + jnp.log2(jnp.sum(jnp.exp2(lane - m), axis=1, keepdims=True))
                blk.m.append(m)

        def prob(blk, half, n):
            if (half, n) not in blk.p:
                blk.p[half, n] = jnp.exp2(blk.tiles[half][n] - blk.m[half])
            return blk.p[half, n]

        def pv_run(i, t, js):
            blk = blks[i]
            lhs, rhs = [], []
            for j in js:
                if j >= i:
                    half, col = _DIAG[t]
                    lhs.append(prob(blk, half, 2 * i + j - i))
                    rhs.append((vn if t > 6 and i > 0 else vp)[i][2 * (j - i) + col])
                    continue
                a11, a12 = (lambda: prob(blk, 0, 2 * j)), (lambda: prob(blk, 0, 2 * j + 1))
                a21, a22 = (lambda: prob(blk, 1, 2 * j)), (lambda: prob(blk, 1, 2 * j + 1))
                lhs.append((
                    lambda: a11() + a22(), lambda: a21() + a22(), a11, a22,
                    lambda: a11() + a12(), lambda: a21() - a11(), lambda: a12() - a22())[t]())
                rhs.append(vt[j][t])
            x = nn(jnp.concatenate(lhs, axis=1).astype(BF16), bf([[r] for r in rhs]))
            blk.acc[t] = x if t not in blk.acc else x + blk.acc[t]
            rlog[-1] = x

        def lane_sums(i):
            out = []
            for half in range(2):
                tl = [p for (hf, _), p in blks[i].p.items() if hf == half]
                if i >= SUMPIN and INDEL:
                    tl[0] = jnp.where(never128, rlog[-INDEL - (INSTAG if half == 0 else 0)], tl[0])
                out.append(functools.reduce(jnp.add, tl))
            return out

        def normalise(i, lanes):
            m = blks[i].acc
            if i > 0:
                ctx = [[(m[0] + m[3]) + (m[6] - m[4]), (m[2] + m[4]) - m[7]],
                       [(m[1] + m[3]) - m[8], (m[0] + m[2]) + (m[5] - m[1])]]
            else:
                ctx = [[m[6], m[7]], [m[8], m[5]]]
            r = [_recip(jnp.sum(l, axis=1, keepdims=True)) for l in lanes]
            return _rhs_terms(ctx[0][0] * r[0], ctx[1][0] * r[1],
                              ctx[0][1] * r[0], ctx[1][1] * r[1])

        def sum_host(lanes, part, nparts):
            def host(lhs):
                n = 32 // nparts
                g0 = OS0 if part == 0 else 0
                slots = [(g, c) for g in range(g0, HM // 16) for c in range(len(lhs))]
                for k in range(n):
                    g, c = slots[len(slots) - 1 - ((n - 1 - k) * len(slots)) // n]
                    kk = part * n + k
                    l = lanes[kk // 16][8 * (kk % 16):8 * (kk % 16) + 8]
                    lhs[c][g] = jnp.where(never, pltpu.bitcast(l, U32), lhs[c][g])
            return host if lanes is not None else None

        rounds, events = _plan()
        ctx = None
        for r in range(max(events)):
            rlog.append(None)
            for u in (rounds[r] if r < len(rounds) else []):
                if u[0] == 'p':
                    pv_run(*u[1:])
                else:
                    s_run(r, *u)
            for kind, i in events.get(r + 1, []):
                if kind == 'm':
                    row_shift(i)
                    continue
                lanes = lane_sums(i)
                pins = lanes if i >= SUMPIN else None
                if i == NS - 1:
                    o = o_round_b(1 - slot, 0, ct0, singles[:1], sum_host(pins, 0, 1))
                    del singles[:1]
                elif i + 1 in SPLIT:
                    o = o_round_a(slot, i + 1, ctx, sum_host(pins, 0, 1))
                    singles += [(slot, i + 1, t, ctx[t]) for t in (5, 6, 0)]
                else:
                    o = o_round_a(slot, i + 1, ctx, sum_host(pins, 0, 2))
                    o_round_b(slot, i + 1, ctx, singles[:1], sum_host(pins, 1, 2))
                    del singles[:1]
                if pins is not None and XDEL:
                    lanes = [jnp.where(never128, o[c][:TQ], l) for c, l in enumerate(lanes)]
                ctx = normalise(i, lanes)
        assert [e[1:3] for e in singles] == CARRY
        for n, x in enumerate(ctx + [e[3] for e in singles]):
            ctxc_v[n] = x
        return 0

    with jax.named_scope('heads'):
        lax.fori_loop(0, H, head, 0)

    @jax.named_scope('epilogue')
    def _epilogue():
        for cp in w_copies(jnp.int32(H - 1), 0):
            cp.wait()
        ct0, singles = carried((H - 1) % 2)
        o_round_a((H - 1) % 2, 0, ct0)
        o_round_b((H - 1) % 2, 0, ct0, singles)

        def o_copy(c0, width):
            cols = pl.ds(c0, width)
            return pltpu.make_async_copy(acc_v.at[:, cols], out_hbm.at[:, cols], sem.at[0])

        def segment(s, c_cat, pieces):
            c0 = s * LSEG if isinstance(s, int) else pl.multiple_of(s * LSEG, LSEG)
            hs = jnp.concatenate(
                [h_v[kk, pl.ds(s, LSEG, stride=NSEG), :] for kk in range(7)],
                axis=1).astype(BF16)
            yt = lax.dot_general(c_cat, hs, NT, preferred_element_type=F32)
            w = LSEG // pieces
            for e in range(pieces):
                ce = c0 + e * w
                cols = pl.ds(ce, w)
                xf = xt_v[:, cols].astype(F32)
                dsk = jnp.concatenate([col_v[0]] * (w // 128), axis=1)
                gw = jnp.concatenate([col_v[1]] * (w // 128), axis=1)
                g = jax.nn.sigmoid(jnp.sum(xf * gw, axis=0, keepdims=True))
                y = yt[:, e * w:(e + 1) * w] + xf * dsk
                acc_v[:, cols] = g * acc_v[:, cols] + (1.0 - g) * y
                o_copy(ce, w).start()

        if EC == NSEG:
            c_cat = ccat_v[...]
            for s in range(NSEG - 1, -1, -1):
                segment(s, c_cat, 2 if s == 0 else 1)
        else:
            def out_step(it, _):
                c_cat = ccat_v[...]
                for e in range(EC):
                    segment(it * EC + e, c_cat, 1)
                return 0

            lax.fori_loop(0, NSEG // EC, out_step, 0)
        o_copy(0, S).wait()

    _epilogue()


@jax.jit
def pallas_gated_mix__compressed_kv_cla__ssm_conv_s5__prompt_kernel(
    A_x: jax.Array,
    A_c_kv: jax.Array,
    A_w_q: jax.Array,
    A_w_uk: jax.Array,
    A_w_uv: jax.Array,
    A_w_o: jax.Array,
    B_x: jax.Array,
    B_Lambda_re: jax.Array,
    B_Lambda_im: jax.Array,
    B_B_re: jax.Array,
    B_B_im: jax.Array,
    B_C_re: jax.Array,
    B_C_im: jax.Array,
    B_log_dt: jax.Array,
    B_Dskip: jax.Array,
    gate_w: jax.Array,
):
    del B_x
    hbm_spec = pl.BlockSpec(memory_space=pltpu.HBM)
    out_t = pl.pallas_call(
        _kernel,
        in_specs=[hbm_spec] * 15,
        out_specs=hbm_spec,
        out_shape=jax.ShapeDtypeStruct((M, S), F32),
        scratch_shapes=[
            pltpu.VMEM((M, S), BF16),
            pltpu.VMEM((7, 2, HS // 2, 128), U32),
            pltpu.VMEM((S, DC), BF16),
            pltpu.VMEM((7, 4, HS // 2, 128), U32),
            pltpu.VMEM((2, M // 2, D), U32),
            pltpu.VMEM((2, 7, M // 4, 128), U32),
            pltpu.VMEM((2, M, D), U32),
            pltpu.VMEM((2, DC, D), U32),
            pltpu.VMEM((2, DC, D), U32),
            pltpu.VMEM((4 * M, M), BF16),
            pltpu.VMEM((M, 2 * M), BF16),
            pltpu.VMEM((M,), BF16), pltpu.VMEM((M,), BF16), pltpu.VMEM((M,), BF16),
            pltpu.VMEM((M,), BF16), pltpu.VMEM((M,), BF16),
            pltpu.VMEM((2, M, 128), F32),
            pltpu.VMEM((2, 8, M), F32),
            pltpu.VMEM((8, NSEG * SEG_STRIDE, 128), F32),
            pltpu.VMEM((7, S, 128), F32),
            pltpu.VMEM((8, NSEG, 128), F32),
            pltpu.VMEM((8, NSEG, 128), F32),
            pltpu.VMEM((M, S), F32),
            pltpu.VMEM((7 + len(CARRY), TQ, 128), BF16),
            pltpu.VMEM((8, 128), jnp.int32),
            pltpu.SemaphoreType.DMA((SEM_X + NPRO,)),
        ],
        compiler_params=pltpu.CompilerParams(vmem_limit_bytes=110 * 1024 * 1024),
        name="gated_mix",
    )(
        A_x.reshape(S, M).T, A_c_kv.reshape(S, DC),
        A_w_q, A_w_uk, A_w_uv, jnp.swapaxes(A_w_o, 1, 2),
        B_Lambda_re, B_Lambda_im, B_B_re, B_B_im, B_C_re, B_C_im, B_log_dt,
        B_Dskip, gate_w,
    )
    return out_t.T.reshape(1, S, M)
```

```python
import functools
import math

import jax
import jax.numpy as jnp
from jax import lax
import jax.experimental.pallas as pl
import jax.experimental.pallas.tpu as pltpu

F32 = jnp.float32
BF16 = jnp.bfloat16
U32 = jnp.uint32

S = 2048
HS = S // 2
M = 448
HM = M // 2
DC = 1024
H = 16
D = 256
TQ = 128
NS = S // (2 * TQ)
NSEG = 8
LSEG = S // NSEG
SEG_STRIDE = LSEG + 8
STEPS = 2 * LSEG // H
MA = 384
MR = M - MA
NT = (((1,), (1,)), ((), ()))
NPRO = NSEG // 2
CW = 352
CSTEP = 336
CROWS = 32
SEM_W = 3
SEM_X = 5

XLO, XHI, CLO, CHI = 40, 420, 0, 420
QPIN, VPIN, VPIN2, SCAN_SPAN = 8, 12, 20, 3
PORDER = (2, 3, 0, 1, 5, 4, 6)
PGROUPS = [[(j, min(j + 4, i)) for j in range(0, i, 4)] for i in range(NS)]
PGROUPS[7] = [(0, 4), (4, 6), (6, 7)]
PGROUPS[3] = [(0, 2), (2, 3)]
LEAD0, LEAD, BAL, AGE, OS0 = 4, 5, 10, 3, 2
CAP, MCOST, OCOST, RATIO, PTAIL = 112, 32, 48, 0.85, 50
SPLIT = (7, 3)
CARRY = [(3, 0)]

_NEEDS = {0: ((0, 0), (1, 1)), 1: ((1, 0), (1, 1)), 2: ((0, 0),), 3: ((1, 1),),
          4: ((0, 0), (0, 1)), 5: ((1, 0), (0, 0)), 6: ((0, 1), (1, 1))}
_DIAG = {8: (1, 0), 5: (1, 1), 6: (0, 0), 7: (0, 1)}


def _plan():
    i = NS - 1
    sq = [(4, 'a', i, 0), (4, 'a', i, 1), (3, 'b', i, 0), (1, 's', i, (1, 5)),
          (4, 'a', i, 2), (3, 'b', i, 2), (1, 's', i, (1, 6)),
          (4, 'a', i, 3), (3, 'b', i, 3), (1, 's', i, (1, 0)),
          (4, 'a', i, 4), (4, 'a', i, 5), (3, 'b', i, 4), (1, 's', i, (5, 5)),
          (4, 'a', i, 6), (3, 'b', i, 6), (1, 's', i, (5, 6)),
          (2, 'd', i, (1, 0)), (2, 'd', i, (0, 0)),
          (4, 'a', i - 1, 0), (4, 'a', i - 1, 1),
          (1, 's', i, (5, 0)), (1, 's', i - 1, (1, 5)), (2, 'd', i, (1, 1)),
          (3, 'b', i - 1, 0), (1, 's', i - 1, (1, 6)),
          (4, 'a', i - 1, 2), (3, 'b', i - 1, 2), (1, 's', i - 1, (1, 0))]
    for i in range(NS - 2, -1, -1):
        for j in range(3 if i == NS - 2 else 0, i):
            sq += [(4, 'a', i, j), (3, 'b', i, j)]
        sq += [(2, 'd', i, hk) for hk in ((1, 0), (0, 0), (1, 1))]
    pq = {}
    for i in range(NS):
        pq[i] = [[j1 - j0, t, list(range(j0, j1))] for j0, j1 in PGROUPS[i] for t in PORDER]
        pq[i] += [[2, 8, [i, i + 1]], [2, 5, [i, i + 1]], [1, 6, [i]], [1, 7, [i]]]
    ready, rounds, events, seen = {}, [], {}, set()

    def needs(i, t, js):
        out = set()
        for j in js:
            out |= ({(i, _DIAG[t][0], i + j)} if j >= i else
                    {(i, hf, 2 * j + c) for hf, c in _NEEDS[t]})
        return out

    def p_fill(free, pi, first):
        left = {i: [list(u) for u in pq[i]] for i in (pi, pi - 1) if i >= 0}
        got, new = [], set()
        while free and pi in left and ready.get(pi, 1 << 30) <= len(rounds):
            us = left[pi]
            if first is not None:
                u, first = us[first], None
            else:
                size = min(free, max(v[0] for v in us))
                fit = [v for v in us if v[0] == size] or [
                    v for v in us if v[0] == min(w[0] for w in us if w[0] > size)]
                u = min(fit, key=lambda v: len(needs(pi, v[1], v[2][-size:]) - seen - new))
            size = min(free, u[0])
            got.append(('p', pi, u[1], u[2][-size:]))
            new |= needs(pi, u[1], u[2][-size:]) - seen
            u[2], u[0] = u[2][:len(u[2]) - size], u[0] - size
            if not u[0]:
                us.remove(u)
            free -= size
            if not us:
                pi -= 1
        return got, new, free, left, pi

    pi, prev = NS - 1, 0
    while sq or pi >= 0:
        cands = []
        if sq:
            n, free = 0, 4
            while n < len(sq) and sq[n][0] <= free and (
                    n == 0 or 's' in (sq[n][1], sq[n - 1][1])):
                free -= sq[n][0]
                n += 1
            cands.append((n,) + p_fill(free, pi, None))
            if free == 2 and n < len(sq) and sq[n][0] == 2:
                cands.append((n + 1,) + p_fill(0, pi, None))
        if pi >= 0:
            big = max(u[0] for u in pq[pi])
            grp = next(u[2] for u in pq[pi] if u[0] == big)
            cands += [(0,) + p_fill(4, pi, k) for k, u in enumerate(pq[pi]) if u[2] == grp]
        best = None
        for n, got, new, free, left, p2 in cands:
            s_left = sum(u[0] for u in sq[n:] if u[2] >= pi - 1)
            p_left = sum(u[0] for u in left.get(pi, []))
            s_all = sum(u[0] for u in sq[n:])
            p_all = sum(u[0] for i in range(pi + 1) for u in left.get(i, pq[i]))
            load = prev + 16 * len(new) + (MCOST if n and sq[0][1] == 'a' else 0)
            late = max(s_left + BAL - p_left, 0) if s_left else 0
            drift = abs(s_all - RATIO * max(p_all - PTAIL, 0))
            cost = 1000 * free + max(load - CAP, 0) + 2 * late + drift - len(new) + len(got)
            if best is None or cost < best[0]:
                best = (cost, n, got, new, left, p2)
        _, n, got, new, left, p2 = best
        cur = [u[1:] for u in sq[:n]] + got
        done = {u[2] for u in sq[:n]}
        del sq[:n]
        seen |= new
        pq.update(left)
        rounds.append(cur)
        for i in done:
            if all(v[2] != i for v in sq):
                events.setdefault(len(rounds), []).append(('m', i))
                ready[i] = len(rounds) + (LEAD0 if i == NS - 1 else LEAD)
        prev = sum({'a': 64, 'b': 32, 'd': 16, 's': 24, 'p': 16}[u[0]] for u in cur)
        for i in range(pi, p2, -1):
            events.setdefault(len(rounds), []).append(('o', i))
            prev = OCOST
        pi = p2
    return rounds, events


def _lhs_terms(a11, a12, a21, a22):
    return [t.astype(BF16) for t in
            (a11 + a22, a21 + a22, a11, a22, a11 + a12, a21 - a11, a12 - a22)]


def _rhs_terms(b11, b12, b21, b22):
    return [t.astype(BF16) for t in
            (b11 + b22, b11, b12 - b22, b21 - b11, b22, b11 + b12, b21 + b22)]


def _strassen(lhs, rhs, log):
    def mm(i):
        log.append(jnp.dot(lhs(i), rhs[i], preferred_element_type=F32))
        return log[-1]
    m1 = mm(0)
    m4 = mm(3)
    c11 = m1 + m4
    m2 = mm(1)
    c21 = m2 + m4
    c22 = m1 - m2
    m5 = mm(4)
    c11 = c11 - m5
    m3 = mm(2)
    c12 = m3 + m5
    c22 = c22 + m3
    c11 = c11 + mm(6)
    c22 = c22 + mm(5)
    return c11, c12, c21, c22


def _recip(l):
    r = pl.reciprocal(l, approx=True)
    return r * (2.0 - l * r)


def _cmul(pr, pi, hr, hi):
    return ([pr[t] * hr[t] - pi[t] * hi[t] for t in range(4)],
            [pr[t] * hi[t] + pi[t] * hr[t] for t in range(4)])


def _column(row):
    row = jnp.concatenate([row, jnp.zeros((1, 512 - M), F32)], axis=1)
    return jnp.broadcast_to(row, (128, 512)).T[:M]


def _kernel(xt_hbm, c_hbm, wq_hbm, wk_hbm, wv_hbm, wot_hbm,
            lre_hbm, lim_hbm, bre_hbm, bim_hbm, cre_hbm, cim_hbm, ldt_hbm,
            dsk_hbm, gw_hbm,
            out_hbm,
            xt_v, xs_v, c_v, cs_v, wot_v, wt_v, wq_b, wk_b, wv_b, bc_v, ccat_v,
            lre_v, lim_v, ldt_v, dsk_v, gw_v, col_v, coef_v,
            u_v, h_v, a_v, st_v, acc_v, ctxc_v, never_v, sem):
    wq32 = wq_hbm.bitcast(U32)
    wk32 = wk_hbm.bitcast(U32)
    wv32 = wv_hbm.bitcast(U32)
    wot32 = wot_hbm.bitcast(U32)

    def w_copies(h, sl):
        j = lax.shift_right_logical(h, 1)
        cps = [pltpu.make_async_copy(src.at[:, j, :], dst.at[sl], sem.at[SEM_W + sl])
               for src, dst in ((wq32, wq_b), (wk32, wk_b), (wv32, wv_b))]
        return cps + [pltpu.make_async_copy(wot32.at[h], wot_v.at[sl], sem.at[SEM_W + sl])]

    def x_copies(s):
        spans = [pl.ds(pl.multiple_of(s * LSEG + e * HS, LSEG), LSEG) for e in range(2)]
        return [pltpu.make_async_copy(xt_hbm.at[:, sp], xt_v.at[:, sp], sem.at[SEM_X + s])
                for sp in spans]

    def c_copies(start, rows, s):
        spans = [pl.ds(pl.multiple_of(start + e * HS, 16), rows) for e in range(2)]
        return [pltpu.make_async_copy(c_hbm.at[sp], c_v.at[sp], sem.at[SEM_X + s])
                for sp in spans]

    def stage_copies(s):
        return x_copies(s) + c_copies(CW - CSTEP + (s - 1) * CSTEP, CSTEP, s)

    first_cps = x_copies(0) + [
        pltpu.make_async_copy(bre_hbm.at[MA:M], bc_v.at[0:MR], sem.at[SEM_X]),
        pltpu.make_async_copy(bim_hbm.at[MA:M], bc_v.at[MR:2 * MR], sem.at[SEM_X]),
        pltpu.make_async_copy(bre_hbm.at[0:MA], bc_v.at[2 * MR:2 * MR + MA], sem.at[SEM_X]),
        pltpu.make_async_copy(bim_hbm.at[0:MA], bc_v.at[2 * MR + MA:2 * M], sem.at[SEM_X]),
    ] + c_copies(0, CW - CSTEP, 0)
    vec_cps = [pltpu.make_async_copy(src, dst, sem.at[1]) for src, dst in
               ((lre_hbm, lre_v), (lim_hbm, lim_v), (ldt_hbm, ldt_v), (dsk_hbm, dsk_v),
                (gw_hbm, gw_v))]
    late_cps = [pltpu.make_async_copy(cre_hbm, bc_v.at[2 * M:3 * M], sem.at[2]),
                pltpu.make_async_copy(cim_hbm, bc_v.at[3 * M:4 * M], sem.at[2])]

    def _prologue():
        zero = jnp.int32(0)
        first = vec_cps + first_cps
        for s in range(1, NPRO):
            first = first + stage_copies(s)
        for cp in first + w_copies(zero, 0) + late_cps:
            cp.start()
        acc_v[...] = jnp.zeros_like(acc_v)
        st_v[...] = jnp.zeros_like(st_v)
        ctxc_v[...] = jnp.zeros_like(ctxc_v)
        wt_v[1] = jnp.zeros(wt_v.shape[1:], U32)
        never_v[...] = jnp.zeros_like(never_v)

        for cp in vec_cps:
            cp.wait()
        lre = lre_v[...].astype(F32).reshape(1, M)
        lim = lim_v[...].astype(F32).reshape(1, M)
        dt = jnp.exp(ldt_v[...].astype(F32)).astype(BF16).astype(F32).reshape(1, M)
        er = jnp.exp(dt * lre)
        ar = er * jnp.cos(dt * lim)
        ai = er * jnp.sin(dt * lim)
        den = lre * lre + lim * lim
        coef_v[0] = jnp.broadcast_to(2.0 * ((ar - 1.0) * lre + ai * lim) / den, (8, M))
        coef_v[1] = jnp.broadcast_to(2.0 * (ai * lre - (ar - 1.0) * lim) / den, (8, M))

        def bc(v):
            return jnp.broadcast_to(v, (NSEG, 128))

        for t in range(3):
            a_v[t] = bc(ar[:, t * 128:(t + 1) * 128])
            a_v[4 + t] = bc(ai[:, t * 128:(t + 1) * 128])
        a_v[3] = bc(jnp.concatenate([ar[:, MA:], ar[:, MA:]], axis=1))
        a_v[7] = bc(jnp.concatenate([ai[:, MA:], -ai[:, MA:]], axis=1))
        col_v[0] = _column(dsk_v[...].astype(F32).reshape(1, M))
        col_v[1] = _column(gw_v[...].astype(F32).reshape(1, M))

        never = never_v[...] != 0

        def spread(us, rows, cols, lo, hi):
            out = []
            for c in range(cols):
                vr = []
                for g in range(rows):
                    n = lo + ((c * rows + g) * (hi - lo)) // (rows * cols)
                    e, t, rg = n // 224, (n % 224) // 32, n % 32
                    vr.append(us[e][8 * rg:8 * rg + 8, 128 * t:128 * t + 128])
                out.append(jnp.concatenate(vr, axis=0))
            mask = jnp.concatenate([jnp.concatenate([never] * rows, axis=0)] * cols, axis=1)
            return mask, jnp.concatenate(out, axis=1)

        def bu(s):
            b_cat = bc_v[0:2 * M, :]
            r = pl.ds(pl.multiple_of(s * (LSEG // 2), LSEG // 2), LSEG // 2)
            xs = []
            us = []
            for e in range(2):
                c0 = pl.multiple_of(s * LSEG + e * HS, LSEG)
                xe = xt_v[:, pl.ds(c0, LSEG)].T
                u = lax.dot_general(xe, b_cat, NT, preferred_element_type=F32)
                us.append(u)
                rows = pl.ds(pl.multiple_of((s + e * NPRO) * SEG_STRIDE, 8), LSEG)
                u_v[6, rows, :] = u[:, :128]
                u_v[7, rows, :] = pltpu.roll(u[:, :128], MR, 1)
                for t in range(6):
                    u_v[t, rows, :] = u[:, (t + 1) * 128:(t + 2) * 128]
                xe = xe.astype(F32)
                xs.append((xe[:, :D], jnp.concatenate(
                    [xe[:, D:], jnp.zeros((LSEG, 2 * D - M), F32)], axis=1)))
            mask, dep = spread(us, 32, 2, XLO, XHI)
            a11 = jnp.where(mask, dep, xs[0][0])
            a22 = jnp.where(mask, dep, xs[1][1])
            for i, t in enumerate(_lhs_terms(a11, xs[0][1], xs[1][0], a22)):
                t = pltpu.bitcast(t, U32)
                for kt in range(2):
                    xs_v[i, kt, r, :] = t[:, kt * 128:(kt + 1) * 128]
            return us

        def c_terms(s, us):
            hc = DC // 2
            r = pl.ds(pl.multiple_of(s * (CSTEP // 2), 8), CW // 2)
            rt = pl.ds(pl.multiple_of(s * CSTEP, 16), CW)
            rb = pl.ds(pl.multiple_of(s * CSTEP + HS, 16), CW)
            a11, a12, a21, a22 = c_v[rt, :hc], c_v[rt, hc:], c_v[rb, :hc], c_v[rb, hc:]
            mask, dep = spread(us, CW // 16, 4, CLO, CHI)
            dep = pltpu.bitcast(dep, U32)
            a11 = pltpu.bitcast(jnp.where(mask, dep, pltpu.bitcast(a11, U32)), BF16)
            a22 = pltpu.bitcast(jnp.where(mask, dep, pltpu.bitcast(a22, U32)), BF16)
            terms = _lhs_terms(*(a.astype(F32) for a in (a11, a12, a21, a22)))
            for i, t in enumerate(terms):
                t = pltpu.bitcast(t, U32)
                for kt in range(4):
                    cs_v[i, kt, r, :] = t[:, kt * 128:(kt + 1) * 128]

        for cp in first_cps:
            cp.wait()
        bu(0)

        def pro_step(s, _):
            for cp in stage_copies(s):
                cp.wait()
            c_terms(s - 1, bu(s))
            return 0

        lax.fori_loop(1, NPRO, pro_step, 0)

    _prologue()

    def o_tiles(jobs, host=None):
        lhs = [[wt_v[sl, t, 8 * g:8 * g + 8, :] for g in range(HM // 16)] for sl, t, _ in jobs]
        if host is not None:
            host(lhs)
        return [lax.dot_general(pltpu.bitcast(jnp.concatenate(l, axis=0), BF16),
                                c, NT, preferred_element_type=F32)
                for l, (_, _, c) in zip(lhs, jobs)]

    def o_add(i, quad, x):
        r0, c0 = (quad // 2) * HM, (2 * i + quad % 2) * TQ
        acc_v[r0:r0 + HM, c0:c0 + TQ] += x

    def o_finish_a(i, m2, m3, m4, m5):
        o_add(i, 0, m4 - m5)
        o_add(i, 1, m3 + m5)
        o_add(i, 2, m2 + m4)
        o_add(i, 3, m3 - m2)

    def o_round_a(sl, i, ct, host=None):
        o_finish_a(i, *o_tiles([(sl, t, ct[t]) for t in (1, 2, 3, 4)], host))

    def o_round_b(sl, i, ct, extra, host=None):
        ms = o_tiles([(sl, t, ct[t]) for t in (0, 5, 6)]
                     + [(e[0], e[2], e[3]) for e in extra], host)
        o_add(i, 0, ms[0] + ms[2])
        o_add(i, 3, ms[0] + ms[1])
        for (_, ie, t, _), m in zip(extra, ms[3:]):
            if t != 5:
                o_add(ie, 0, m)
            if t != 6:
                o_add(ie, 3, m)

    def carried(sl):
        ct = [ctxc_v[t] for t in range(7)]
        return ct, [(sl, i, t, ctxc_v[7 + n]) for n, (i, t) in enumerate(CARRY)]

    def head(h, _):
        slot = lax.bitwise_and(h, 1)

        @pl.when(h == H // 2)
        def _segment_carry():
            pr = [a_v[t] for t in range(4)]
            pi = [a_v[4 + t] for t in range(4)]
            for _ in range(int(math.log2(LSEG))):
                pr, pi = ([pr[t] * pr[t] - pi[t] * pi[t] for t in range(4)],
                          [2.0 * pr[t] * pi[t] for t in range(4)])
            row = lax.broadcasted_iota(jnp.int32, (NSEG, 128), 0)
            e_r = [st_v[t] for t in range(4)]
            e_i = [st_v[4 + t] for t in range(4)]
            ir = [jnp.zeros((NSEG, 128), F32)] * 4
            ii = ir
            for s in range(1, NSEG):
                mr, mi = _cmul(pr, pi, ir, ii)
                fr = [pltpu.roll(mr[k] + e_r[k], 1, 0) for k in range(4)]
                fi = [pltpu.roll(mi[k] + e_i[k], 1, 0) for k in range(4)]
                ir = [jnp.where(row == s, fr[k], ir[k]) for k in range(4)]
                ii = [jnp.where(row == s, fi[k], ii[k]) for k in range(4)]
            for t in range(4):
                st_v[t] = ir[t]
                st_v[4 + t] = ii[t]

        @pl.when(h == 1)
        def _():
            for cp in late_cps:
                cp.wait()

        for cp in w_copies(h, slot):
            cp.wait()

        o_prev = o_tiles([(1 - slot, t, ctxc_v[t]) for t in (1, 2, 3, 4)])
        for cp in w_copies(jnp.minimum(h + 1, H - 1), 1 - slot):
            cp.start()
        o_finish_a(0, *o_prev)
        ct0, singles = carried(1 - slot)

        up = ((1 - slot) * 16).astype(U32)
        never = never_v[...] != 0
        never64 = jnp.concatenate([never] * 8, axis=0)
        never128 = jnp.concatenate([never] * 16, axis=0)

        def weight(buf):
            return pltpu.bitcast((buf[slot] << up) & jnp.uint32(0xFFFF0000), F32)

        def quads(w, kh):
            return w[:kh, :128], w[:kh, 128:], w[kh:, :128], w[kh:, 128:]

        def bf(rows):
            return pltpu.bitcast(jnp.concatenate(
                [jnp.concatenate(r, axis=1) for r in rows], axis=0), BF16)

        def pk(x):
            return pltpu.bitcast(x.astype(BF16), U32)

        def nt(a, b):
            return lax.dot_general(a, b, NT, preferred_element_type=F32)

        def nn(a, b):
            return jnp.dot(a, b, preferred_element_type=F32)

        pin_list = []

        def lhs_term(ref, i, npin, order=range(8)):
            ncol = ref.shape[1]
            rows = [[ref[i, c, g * 64:(g + 1) * 64, :] for c in range(ncol)] for g in order]
            nr = len(rows) - 1
            npin = min(npin, len(pin_list), nr * ncol)
            for n in range(npin):
                g, c = 1 + (n * nr) // npin, n % ncol
                rows[g][c] = jnp.where(never64, pin_list.pop(0), rows[g][c])
            return bf(rows)

        def sup(cq, j):
            l, r = (cq[0], cq[1]) if j < NS // 2 else (cq[2], cq[3])
            r0 = (j % (NS // 2)) * 2 * TQ
            return l[r0:r0 + TQ], r[r0:r0 + TQ], l[r0 + TQ:r0 + 2 * TQ], r[r0 + TQ:r0 + 2 * TQ]

        def rhs_tiles(b11, b12, b21, b22, with_terms):
            plain = [pk(b11), pk(b12), pk(b21), pk(b22)]
            if not with_terms:
                return None, plain, plain
            extra = [pk(b11 + b22), pk(b12 - b22), pk(b21 - b11), pk(b11 + b12), pk(b21 + b22)]
            terms = [extra[0], plain[0], extra[1], extra[2], plain[3], extra[3], extra[4]]
            return terms, plain, plain + extra

        def lhs_tiles(a11, a12, a21, a22, with_terms):
            plain = [pk(a11), pk(a12), pk(a21), pk(a22)]
            if not with_terms:
                return None, plain, plain
            extra = [pk(a11 + a22), pk(a21 + a22), pk(a11 + a12), pk(a21 - a11), pk(a12 - a22)]
            terms = [extra[0], extra[1], plain[0], plain[3], extra[2], extra[3], extra[4]]
            return terms, plain, plain + extra

        klog = []
        kq = _strassen(lambda i: lhs_term(cs_v, i, 0),
                       _rhs_terms(*quads(weight(wk_b), DC // 2)), klog)
        kt, kp = [], []
        for j in range(NS):
            k11, k12, k21, k22 = sup(kq, j)
            t, p_, allt = rhs_tiles(k11, k21, k12, k22, j < NS - 1)
            kt.append(t)
            kp.append(p_)
            pin_list += allt

        r0 = pl.multiple_of(jnp.clip(h - 1, 0, M // CROWS - 1) * CROWS, CROWS)
        src = jnp.where(h == 0, 0, 2 * M) + r0
        cre = bc_v[pl.ds(pl.multiple_of(src, CROWS), CROWS), :].astype(F32)
        cim = bc_v[pl.ds(pl.multiple_of(src + M, CROWS), CROWS), :].astype(F32)
        cr = coef_v[0, 0:1, :]
        ci = coef_v[1, 0:1, :]
        c_r = cre * cr - cim * ci
        c_i = -(cre * ci + cim * cr)
        ccat_v[pl.ds(r0, CROWS), :] = jnp.concatenate(
            [c_r[:, :MA], c_i[:, :MA], c_r[:, MA:], c_i[:, MA:]], axis=1).astype(BF16)

        t0 = lax.bitwise_and(h, H // 2 - 1) * STEPS
        a_r = [a_v[t] for t in range(4)]
        a_i = [a_v[4 + t] for t in range(4)]
        hr = [st_v[t] for t in range(4)]
        hi = [st_v[4 + t] for t in range(4)]
        for j in range(STEPS):
            pos = (j * SCAN_SPAN * 128) // STEPS
            dep = klog[pos // 128][8 * (pos % 128):8 * (pos % 128) + 8]
            hr = [jnp.where(never, dep, x) for x in hr]
            us = [u_v[kk, pl.ds(t0 + j, NSEG, stride=SEG_STRIDE), :] for kk in range(8)]
            mr, mi = _cmul(a_r, a_i, hr, hi)
            hr = [mr[0] + us[0], mr[1] + us[1], mr[2] + us[2], mr[3] + us[6]]
            hi = [mi[0] + us[3], mi[1] + us[4], mi[2] + us[5], mi[3] + us[7]]
            r0 = pl.multiple_of((t0 + j) * NSEG, NSEG)
            for kk, val in enumerate(hr[:3] + hi[:3] + [hr[3]]):
                h_v[kk, pl.ds(r0, NSEG), :] = val
        for t in range(4):
            st_v[t] = hr[t]
            st_v[4 + t] = hi[t]

        wo = pltpu.bitcast(wot_v[slot], BF16).astype(F32)
        w11, w12, w21, w22 = quads(wo, HM)
        dep = jnp.concatenate([klog[5][32 * g:32 * g + 8] for g in range(HM // 8)], axis=0)
        nv = jnp.concatenate([never] * (HM // 8), axis=0)
        for t, val in enumerate(_lhs_terms(jnp.where(nv, dep, w11), w12, w21,
                                           jnp.where(nv, dep, w22))):
            wt_v[slot, t] = pltpu.bitcast(val, U32)

        qscale = (D ** -0.5) * math.log2(math.e)
        wq = jnp.concatenate([weight(wq_b), jnp.zeros((2 * D - M, D), F32)], axis=0)
        wqt = _rhs_terms(*quads(wq, D))
        m4, m1, m2, m3, m6, m5 = (nn(lhs_term(xs_v, i, QPIN), wqt[i]) for i in (3, 0, 1, 2, 5, 4))
        m7 = jnp.concatenate([nn(lhs_term(xs_v, 6, QPIN // 2, range(4)), wqt[6]),
                              nn(lhs_term(xs_v, 6, QPIN // 2, range(4, 8)), wqt[6])], axis=0)
        qq = [x * qscale for x in ((m1 + m4) + (m7 - m5), m3 + m5, m2 + m4, (m1 - m2) + (m3 + m6))]
        qt, qp = [None] * NS, [None] * NS
        for j in range(NS - 1, -1, -1):
            qt[j], qp[j], allt = lhs_tiles(*sup(qq, j), j > 0)
            pin_list += allt

        wvt = _rhs_terms(*quads(weight(wv_b), DC // 2))
        m1, m4, m2, m5, m3, m7 = (nn(lhs_term(cs_v, i, VPIN), wvt[i]) for i in (0, 3, 1, 4, 2, 6))
        vq = [(m1 + m4) + (m7 - m5), m3 + m5, m2 + m4, None]
        del pin_list[:]
        vt, vp = [None] * NS, [None] * NS
        for j in range(NS // 2):
            vt[j], vp[j], allt = rhs_tiles(*sup(vq, j), True)
            pin_list += allt
        vq[3] = ((m1 - m2) + m3) + nn(lhs_term(cs_v, 5, VPIN2), wvt[5])
        for j in range(NS // 2, NS):
            vt[j], vp[j], allt = rhs_tiles(*sup(vq, j), j < NS - 1)
            pin_list += allt

        vn = [[x ^ jnp.uint32(0x80008000) for x in t] for t in vp]
        causal = (lax.broadcasted_iota(jnp.int32, (TQ, TQ), 1)
                  <= lax.broadcasted_iota(jnp.int32, (TQ, TQ), 0))

        class Block:
            def __init__(self):
                self.tiles = [{}, {}]
                self.mx = [None, None]
                self.tmp, self.acc, self.p = {}, {}, {}

            def note(self, half, n, x):
                self.tiles[half][n] = x
                self.mx[half] = x if self.mx[half] is None else jnp.maximum(self.mx[half], x)

        blks = [Block() for _ in range(NS)]
        rlog = []
        snaps = []

        def host_tile(x):
            return jnp.where(never64, pin_list.pop(0), x) if pin_list else x

        def smm(i, j, t, lhs=None):
            lhs = host_tile(qt[i][t]) if lhs is None else lhs
            rlog[-1] = nt(bf([[lhs]]), bf([[host_tile(kt[j][t])]]))
            return rlog[-1]

        def host_max(r, lhs):
            old = [sn for sn in snaps if sn[0] <= r - AGE]
            if not old:
                return lhs
            pick = [sn for sn in old if sn[1] == old[0][1]][-1]
            snaps[:] = [sn for sn in snaps if sn[1] != pick[1] or sn[0] > pick[0]]
            t_, b_ = (pltpu.bitcast(x, U32) for x in pick[2])
            return [jnp.where(never64, x, y)
                    for x, y in zip((t_[:64], t_[64:], b_[:64], b_[64:]), lhs)]

        def s_run(r, kind, i, arg):
            blk = blks[i]
            if kind == 'a':
                lhs = host_max(r, [qt[i][t] for t in (1, 2, 3, 4)])
                m2, m3, m4, m5 = (smm(i, arg, t, x) for x, t in zip(lhs, (1, 2, 3, 4)))
                blk.tmp[arg] = [m4 - m5, m3 - m2, m3 + m5, m2 + m4]
                return
            if kind == 'd':
                half, kr = arg
                x = nt(bf([qp[i][2 * half:2 * half + 2]]), bf([[kp[i][kr], kp[i][2 + kr]]]))
                rlog[-1] = x
                blk.note(half, 2 * i + kr, jnp.where(causal, x, -1e9) if half == kr else x)
                if kr == 0:
                    return
            else:
                j = arg if kind == 'b' else arg[0]
                tmp = blk.tmp[j]
                if kind == 'b':
                    m1, m6, m7 = (smm(i, j, t) for t in (0, 5, 6))
                    c11, c22 = tmp[0] + (m1 + m7), tmp[1] + (m1 + m6)
                elif arg[1] == 0:
                    m1 = smm(i, j, 0)
                    c11, c22 = tmp[0] + m1, tmp[1] + m1
                else:
                    tmp[6 - arg[1]] = tmp[6 - arg[1]] + smm(i, j, arg[1])
                    return
                blk.note(0, 2 * j + 1, tmp[2])
                blk.note(1, 2 * j, tmp[3])
                blk.note(0, 2 * j, c11)
                blk.note(1, 2 * j + 1, c22)
            snaps.append((r, i, tuple(blk.mx)))

        def row_shift(i):
            blk = blks[i]
            blk.m = []
            for lane in blk.mx:
                m = jnp.max(lane, axis=1, keepdims=True)
                if i > 0:
                    m = m + jnp.log2(jnp.sum(jnp.exp2(lane - m), axis=1, keepdims=True))
                blk.m.append(m)

        def prob(blk, half, n):
            if (half, n) not in blk.p:
                blk.p[half, n] = jnp.exp2(blk.tiles[half][n] - blk.m[half])
            return blk.p[half, n]

        def pv_run(i, t, js):
            blk = blks[i]
            lhs, rhs = [], []
            for j in js:
                if j >= i:
                    half, col = _DIAG[t]
                    lhs.append(prob(blk, half, 2 * i + j - i))
                    rhs.append((vn if t > 6 and i > 0 else vp)[i][2 * (j - i) + col])
                    continue
                a11, a12 = (lambda: prob(blk, 0, 2 * j)), (lambda: prob(blk, 0, 2 * j + 1))
                a21, a22 = (lambda: prob(blk, 1, 2 * j)), (lambda: prob(blk, 1, 2 * j + 1))
                lhs.append((
                    lambda: a11() + a22(), lambda: a21() + a22(), a11, a22,
                    lambda: a11() + a12(), lambda: a21() - a11(), lambda: a12() - a22())[t]())
                rhs.append(vt[j][t])
            x = nn(jnp.concatenate(lhs, axis=1).astype(BF16), bf([[r] for r in rhs]))
            blk.acc[t] = x if t not in blk.acc else x + blk.acc[t]
            rlog[-1] = x

        def lane_sums(i):
            out = []
            for half in range(2):
                tl = [p for (hf, _), p in blks[i].p.items() if hf == half]
                if i > 0:
                    tl[0] = jnp.where(never128, rlog[half - 2], tl[0])
                out.append(functools.reduce(jnp.add, tl))
            return out

        def normalise(i, lanes):
            m = blks[i].acc
            if i > 0:
                ctx = [[(m[0] + m[3]) + (m[6] - m[4]), (m[2] + m[4]) - m[7]],
                       [(m[1] + m[3]) - m[8], (m[0] + m[2]) + (m[5] - m[1])]]
            else:
                ctx = [[m[6], m[7]], [m[8], m[5]]]
            r = [_recip(jnp.sum(l, axis=1, keepdims=True)) for l in lanes]
            return _rhs_terms(ctx[0][0] * r[0], ctx[1][0] * r[1],
                              ctx[0][1] * r[0], ctx[1][1] * r[1])

        def sum_host(lanes, part, nparts):
            def host(lhs):
                n = 32 // nparts
                g0 = OS0 if part == 0 else 0
                slots = [(g, c) for g in range(g0, HM // 16) for c in range(len(lhs))]
                for k in range(n):
                    g, c = slots[len(slots) - 1 - ((n - 1 - k) * len(slots)) // n]
                    kk = part * n + k
                    l = lanes[kk // 16][8 * (kk % 16):8 * (kk % 16) + 8]
                    lhs[c][g] = jnp.where(never, pltpu.bitcast(l, U32), lhs[c][g])
            return host if lanes is not None else None

        rounds, events = _plan()
        ctx = None
        for r, units in enumerate(rounds):
            rlog.append(None)
            for u in units:
                if u[0] == 'p':
                    pv_run(*u[1:])
                else:
                    s_run(r, *u)
            for kind, i in events.get(r + 1, []):
                if kind == 'm':
                    row_shift(i)
                    continue
                lanes = lane_sums(i)
                pins = lanes if i > 0 else None
                if i == NS - 1:
                    o_round_b(1 - slot, 0, ct0, singles[:1], sum_host(pins, 0, 1))
                    del singles[:1]
                elif i + 1 in SPLIT:
                    o_round_a(slot, i + 1, ctx, sum_host(pins, 0, 1))
                    singles += [(slot, i + 1, t, ctx[t]) for t in (5, 6, 0)]
                else:
                    o_round_a(slot, i + 1, ctx, sum_host(pins, 0, 2))
                    o_round_b(slot, i + 1, ctx, singles[:1], sum_host(pins, 1, 2))
                    del singles[:1]
                ctx = normalise(i, lanes)
        assert [e[1:3] for e in singles] == CARRY
        for n, x in enumerate(ctx + [e[3] for e in singles]):
            ctxc_v[n] = x
        return 0

    lax.fori_loop(0, H, head, 0)

    def _epilogue():
        for cp in w_copies(jnp.int32(H - 1), 0):
            cp.wait()
        ct0, singles = carried((H - 1) % 2)
        o_round_a((H - 1) % 2, 0, ct0)
        o_round_b((H - 1) % 2, 0, ct0, singles)

        def o_copy(c0, width):
            cols = pl.ds(c0, width)
            return pltpu.make_async_copy(acc_v.at[:, cols], out_hbm.at[:, cols], sem.at[0])

        c_cat = ccat_v[...]
        for s in range(NSEG - 1, -1, -1):
            hs = jnp.concatenate(
                [h_v[kk, pl.ds(s, LSEG, stride=NSEG), :] for kk in range(7)],
                axis=1).astype(BF16)
            yt = lax.dot_general(c_cat, hs, NT, preferred_element_type=F32)
            w = LSEG // 2 if s == 0 else LSEG
            for e in range(LSEG // w):
                cols = pl.ds(s * LSEG + e * w, w)
                xf = xt_v[:, cols].astype(F32)
                dsk = jnp.concatenate([col_v[0]] * (w // 128), axis=1)
                gw = jnp.concatenate([col_v[1]] * (w // 128), axis=1)
                g = jax.nn.sigmoid(jnp.sum(xf * gw, axis=0, keepdims=True))
                y = yt[:, e * w:(e + 1) * w] + xf * dsk
                acc_v[:, cols] = g * acc_v[:, cols] + (1.0 - g) * y
                o_copy(s * LSEG + e * w, w).start()
        o_copy(0, S).wait()

    _epilogue()


@jax.jit
def pallas_gated_mix__compressed_kv_cla__ssm_conv_s5__prompt_kernel(
    A_x: jax.Array,
    A_c_kv: jax.Array,
    A_w_q: jax.Array,
    A_w_uk: jax.Array,
    A_w_uv: jax.Array,
    A_w_o: jax.Array,
    B_x: jax.Array,
    B_Lambda_re: jax.Array,
    B_Lambda_im: jax.Array,
    B_B_re: jax.Array,
    B_B_im: jax.Array,
    B_C_re: jax.Array,
    B_C_im: jax.Array,
    B_log_dt: jax.Array,
    B_Dskip: jax.Array,
    gate_w: jax.Array,
):
    del B_x
    hbm_spec = pl.BlockSpec(memory_space=pltpu.HBM)
    out_t = pl.pallas_call(
        _kernel,
        in_specs=[hbm_spec] * 15,
        out_specs=hbm_spec,
        out_shape=jax.ShapeDtypeStruct((M, S), F32),
        scratch_shapes=[
            pltpu.VMEM((M, S), BF16),
            pltpu.VMEM((7, 2, HS // 2, 128), U32),
            pltpu.VMEM((S, DC), BF16),
            pltpu.VMEM((7, 4, HS // 2, 128), U32),
            pltpu.VMEM((2, M // 2, D), U32),
            pltpu.VMEM((2, 7, M // 4, 128), U32),
            pltpu.VMEM((2, M, D), U32),
            pltpu.VMEM((2, DC, D), U32),
            pltpu.VMEM((2, DC, D), U32),
            pltpu.VMEM((4 * M, M), BF16),
            pltpu.VMEM((M, 2 * M), BF16),
            pltpu.VMEM((M,), BF16), pltpu.VMEM((M,), BF16), pltpu.VMEM((M,), BF16),
            pltpu.VMEM((M,), BF16), pltpu.VMEM((M,), BF16),
            pltpu.VMEM((2, M, 128), F32),
            pltpu.VMEM((2, 8, M), F32),
            pltpu.VMEM((8, NSEG * SEG_STRIDE, 128), F32),
            pltpu.VMEM((7, S, 128), F32),
            pltpu.VMEM((8, NSEG, 128), F32),
            pltpu.VMEM((8, NSEG, 128), F32),
            pltpu.VMEM((M, S), F32),
            pltpu.VMEM((7 + len(CARRY), TQ, 128), BF16),
            pltpu.VMEM((8, 128), jnp.int32),
            pltpu.SemaphoreType.DMA((SEM_X + NPRO,)),
        ],
        compiler_params=pltpu.CompilerParams(vmem_limit_bytes=110 * 1024 * 1024),
        name="gated_mix",
    )(
        A_x.reshape(S, M).T, A_c_kv.reshape(S, DC),
        A_w_q, A_w_uk, A_w_uv, jnp.swapaxes(A_w_o, 1, 2),
        B_Lambda_re, B_Lambda_im, B_B_re, B_B_im, B_C_re, B_C_im, B_log_dt,
        B_Dskip, gate_w,
    )
    return out_t.T.reshape(1, S, M)
```

```python
import functools
import math

import jax
import jax.numpy as jnp
from jax import lax
import jax.experimental.pallas as pl
import jax.experimental.pallas.tpu as pltpu

F32 = jnp.float32
BF16 = jnp.bfloat16
U32 = jnp.uint32

S = 2048
HS = S // 2
QS = S // 4
M = 448
HM = M // 2
DC = 1024
H = 16
D = 256
TQ = 128
NS = S // (2 * TQ)
NSEG = 8
LSEG = S // NSEG
SEG_STRIDE = LSEG + 8
STEPS = 2 * LSEG // H
MA = 384
MR = M - MA
NT = (((1,), (1,)), ((), ()))
NPRO = NSEG // 2
CW = 192
CSTEP = 160
CROWS = 32
SEM_W = 3
SEM_X = 5

XLO, XHI, CLO, CHI = 230, 440, 0, 440
SCAN_SPAN, WODEP = 2, 1
OUTER = (4, 0, 3, 6, 1, 2, 5)
INNER = (3, 1, 4, 2, 0, 6, 5)
GPIN = (30, 20, 17, 0, 32, 32, 32)
WSH = (0, 0, 4, 8, 12, 16, 20, 24)
PORDER = (2, 3, 0, 1, 5, 4, 6)
PGROUPS = [[(j, min(j + 4, i)) for j in range(0, i, 4)] for i in range(NS)]
PGROUPS[7] = [(0, 4), (4, 6), (6, 7)]
PGROUPS[3] = [(0, 2), (2, 3)]
LEAD0, LEAD, BAL, AGE, OS0, INDEL, INSTAG = 4, 5, 10, 3, 2, 1, 1
CAP, MCOST, OCOST, RATIO, PTAIL, W_NEW, W_UNIT = 112, 32, 48, 0.85, 50, 1.0, 1.0
SPLIT = (7, 3)
CARRY = [(3, 0)]

_NEEDS = {0: ((0, 0), (1, 1)), 1: ((1, 0), (1, 1)), 2: ((0, 0),), 3: ((1, 1),),
          4: ((0, 0), (0, 1)), 5: ((1, 0), (0, 0)), 6: ((0, 1), (1, 1))}
_DIAG = {8: (1, 0), 5: (1, 1), 6: (0, 0), 7: (0, 1)}


def _plan():
    i = NS - 1
    sq = [(4, 'a', i, 0), (4, 'a', i, 1), (3, 'b', i, 0), (1, 's', i, (1, 5)),
          (4, 'a', i, 2), (3, 'b', i, 2), (1, 's', i, (1, 6)),
          (4, 'a', i, 3), (3, 'b', i, 3), (1, 's', i, (1, 0)),
          (4, 'a', i, 4), (4, 'a', i, 5), (3, 'b', i, 4), (1, 's', i, (5, 5)),
          (4, 'a', i, 6), (3, 'b', i, 6), (1, 's', i, (5, 6)),
          (2, 'd', i, (1, 0)), (2, 'd', i, (0, 0)),
          (4, 'a', i - 1, 0), (4, 'a', i - 1, 1),
          (1, 's', i, (5, 0)), (1, 's', i - 1, (1, 5)), (2, 'd', i, (1, 1)),
          (3, 'b', i - 1, 0), (1, 's', i - 1, (1, 6)),
          (4, 'a', i - 1, 2), (3, 'b', i - 1, 2), (1, 's', i - 1, (1, 0))]
    for i in range(NS - 2, -1, -1):
        for j in range(3 if i == NS - 2 else 0, i):
            sq += [(4, 'a', i, j), (3, 'b', i, j)]
        sq += [(2, 'd', i, hk) for hk in ((1, 0), (0, 0), (1, 1))]
    pq = {}
    for i in range(NS):
        pq[i] = [[j1 - j0, t, list(range(j0, j1))] for j0, j1 in PGROUPS[i] for t in PORDER]
        pq[i] += [[2, 8, [i, i + 1]], [2, 5, [i, i + 1]], [1, 6, [i]], [1, 7, [i]]]
    ready, rounds, events, seen = {}, [], {}, set()

    def needs(i, t, js):
        out = set()
        for j in js:
            out |= ({(i, _DIAG[t][0], i + j)} if j >= i else
                    {(i, hf, 2 * j + c) for hf, c in _NEEDS[t]})
        return out

    def p_fill(free, pi, first):
        left = {i: [list(u) for u in pq[i]] for i in (pi, pi - 1) if i >= 0}
        got, new = [], set()
        while free and pi in left and ready.get(pi, 1 << 30) <= len(rounds):
            us = left[pi]
            if first is not None:
                u, first = us[first], None
            else:
                size = min(free, max(v[0] for v in us))
                fit = [v for v in us if v[0] == size] or [
                    v for v in us if v[0] == min(w[0] for w in us if w[0] > size)]
                u = min(fit, key=lambda v: len(needs(pi, v[1], v[2][-size:]) - seen - new))
            size = min(free, u[0])
            got.append(('p', pi, u[1], u[2][-size:]))
            new |= needs(pi, u[1], u[2][-size:]) - seen
            u[2], u[0] = u[2][:len(u[2]) - size], u[0] - size
            if not u[0]:
                us.remove(u)
            free -= size
            if not us:
                pi -= 1
        return got, new, free, left, pi

    pi, prev = NS - 1, 0
    while sq or pi >= 0:
        cands = []
        if sq:
            n, free = 0, 4
            while n < len(sq) and sq[n][0] <= free and (
                    n == 0 or 's' in (sq[n][1], sq[n - 1][1])):
                free -= sq[n][0]
                n += 1
            cands.append((n,) + p_fill(free, pi, None))
            if free == 2 and n < len(sq) and sq[n][0] == 2:
                cands.append((n + 1,) + p_fill(0, pi, None))
        if pi >= 0:
            big = max(u[0] for u in pq[pi])
            grp = next(u[2] for u in pq[pi] if u[0] == big)
            cands += [(0,) + p_fill(4, pi, k) for k, u in enumerate(pq[pi]) if u[2] == grp]
        best = None
        for n, got, new, free, left, p2 in cands:
            s_left = sum(u[0] for u in sq[n:] if u[2] >= pi - 1)
            p_left = sum(u[0] for u in left.get(pi, []))
            s_all = sum(u[0] for u in sq[n:])
            p_all = sum(u[0] for i in range(pi + 1) for u in left.get(i, pq[i]))
            load = prev + 16 * len(new) + (MCOST if n and sq[0][1] == 'a' else 0)
            late = max(s_left + BAL - p_left, 0) if s_left else 0
            drift = abs(s_all - RATIO * max(p_all - PTAIL, 0))
            cost = (1000 * free + max(load - CAP, 0) + 2 * late + drift
                    - W_NEW * len(new) + W_UNIT * len(got))
            if best is None or cost < best[0]:
                best = (cost, n, got, new, left, p2)
        _, n, got, new, left, p2 = best
        cur = [u[1:] for u in sq[:n]] + got
        done = {u[2] for u in sq[:n]}
        del sq[:n]
        seen |= new
        pq.update(left)
        rounds.append(cur)
        for i in done:
            if all(v[2] != i for v in sq):
                events.setdefault(len(rounds), []).append(('m', i))
                ready[i] = len(rounds) + (LEAD0 if i == NS - 1 else LEAD)
        prev = sum({'a': 64, 'b': 32, 'd': 16, 's': 24, 'p': 16}[u[0]] for u in cur)
        for i in range(pi, p2, -1):
            events.setdefault(len(rounds), []).append(('o', i))
            prev = OCOST
        pi = p2
    return rounds, events


def _lhs_sums(a11, a12, a21, a22):
    return [a11 + a22, a21 + a22, a11, a22, a11 + a12, a21 - a11, a12 - a22]


def _rhs_sums(b11, b12, b21, b22):
    return [b11 + b22, b11, b12 - b22, b21 - b11, b22, b11 + b12, b21 + b22]


def _rhs_terms(*quad):
    return [t.astype(BF16) for t in _rhs_sums(*quad)]


def _unpack(w):
    return (pltpu.bitcast(w << jnp.uint32(16), F32),
            pltpu.bitcast(w & jnp.uint32(0xFFFF0000), F32))


def _pack(lo, hi):
    return pltpu.pack_elementwise([lo, hi], packed_dtype=BF16).astype(U32)


def _recip(l):
    r = pl.reciprocal(l, approx=True)
    return r * (2.0 - l * r)


def _cmul(pr, pi, hr, hi):
    return ([pr[t] * hr[t] - pi[t] * hi[t] for t in range(4)],
            [pr[t] * hi[t] + pi[t] * hr[t] for t in range(4)])


def _column(row):
    row = jnp.concatenate([row, jnp.zeros((1, 512 - M), F32)], axis=1)
    return jnp.broadcast_to(row, (128, 512)).T[:M]


def _kernel(xt_hbm, c_hbm, wq_hbm, wk_hbm, wv_hbm, wot_hbm,
            lre_hbm, lim_hbm, bre_hbm, bim_hbm, cre_hbm, cim_hbm, ldt_hbm,
            dsk_hbm, gw_hbm,
            out_hbm,
            xt_v, xs_v, c_v, cs_v, wot_v, wt_v, wq_b, wk_b, wv_b, bc_v, ccat_v,
            lre_v, lim_v, ldt_v, dsk_v, gw_v, col_v, coef_v,
            u_v, h_v, a_v, st_v, acc_v, ctxc_v, never_v, fac_v, sem):
    wq32 = wq_hbm.bitcast(U32)
    wk32 = wk_hbm.bitcast(U32)
    wv32 = wv_hbm.bitcast(U32)
    c32 = c_hbm.bitcast(U32)
    wot32 = wot_hbm.bitcast(U32)

    def w_copies(h, sl):
        j = lax.shift_right_logical(h, 1)
        cps = [pltpu.make_async_copy(src.at[:, j, :], dst.at[sl], sem.at[SEM_W + sl])
               for src, dst in ((wq32, wq_b), (wk32, wk_b), (wv32, wv_b))]
        return cps + [pltpu.make_async_copy(wot32.at[h], wot_v.at[sl], sem.at[SEM_W + sl])]

    def x_copies(s):
        spans = [pl.ds(pl.multiple_of(s * LSEG + e * HS, LSEG), LSEG) for e in range(2)]
        return [pltpu.make_async_copy(xt_hbm.at[:, sp], xt_v.at[:, sp], sem.at[SEM_X + s])
                for sp in spans]

    def c_copies(start, rows, s):
        spans = [pl.ds(pl.multiple_of(start + e * (QS // 2), 8), rows) for e in range(4)]
        return [pltpu.make_async_copy(c32.at[sp], c_v.at[sp], sem.at[SEM_X + s])
                for sp in spans]

    def stage_copies(s):
        return x_copies(s) + c_copies((CW - CSTEP) // 2 + (s - 1) * (CSTEP // 2), CSTEP // 2, s)

    first_cps = x_copies(0) + [
        pltpu.make_async_copy(bre_hbm.at[MA:M], bc_v.at[0:MR], sem.at[SEM_X]),
        pltpu.make_async_copy(bim_hbm.at[MA:M], bc_v.at[MR:2 * MR], sem.at[SEM_X]),
        pltpu.make_async_copy(bre_hbm.at[0:MA], bc_v.at[2 * MR:2 * MR + MA], sem.at[SEM_X]),
        pltpu.make_async_copy(bim_hbm.at[0:MA], bc_v.at[2 * MR + MA:2 * M], sem.at[SEM_X]),
    ] + c_copies(0, (CW - CSTEP) // 2, 0)
    vec_cps = [pltpu.make_async_copy(src, dst, sem.at[1]) for src, dst in
               ((lre_hbm, lre_v), (lim_hbm, lim_v), (ldt_hbm, ldt_v), (dsk_hbm, dsk_v),
                (gw_hbm, gw_v))]
    late_cps = [pltpu.make_async_copy(cre_hbm, bc_v.at[2 * M:3 * M], sem.at[2]),
                pltpu.make_async_copy(cim_hbm, bc_v.at[3 * M:4 * M], sem.at[2])]

    def _prologue():
        zero = jnp.int32(0)
        first = vec_cps + first_cps
        for s in range(1, NPRO):
            first = first + stage_copies(s)
        for cp in first + w_copies(zero, 0) + late_cps:
            cp.start()
        acc_v[...] = jnp.zeros_like(acc_v)
        st_v[...] = jnp.zeros_like(st_v)
        ctxc_v[...] = jnp.zeros_like(ctxc_v)
        wt_v[1] = jnp.zeros(wt_v.shape[1:], U32)
        never_v[...] = jnp.zeros_like(never_v)

        for cp in vec_cps:
            cp.wait()
        lre = lre_v[...].astype(F32).reshape(1, M)
        lim = lim_v[...].astype(F32).reshape(1, M)
        dt = jnp.exp(ldt_v[...].astype(F32)).astype(BF16).astype(F32).reshape(1, M)
        er = jnp.exp(dt * lre)
        ar = er * jnp.cos(dt * lim)
        ai = er * jnp.sin(dt * lim)
        den = lre * lre + lim * lim
        coef_v[0] = jnp.broadcast_to(2.0 * ((ar - 1.0) * lre + ai * lim) / den, (8, M))
        coef_v[1] = jnp.broadcast_to(2.0 * (ai * lre - (ar - 1.0) * lim) / den, (8, M))

        def bc(v):
            return jnp.broadcast_to(v, (NSEG, 128))

        for t in range(3):
            a_v[t] = bc(ar[:, t * 128:(t + 1) * 128])
            a_v[4 + t] = bc(ai[:, t * 128:(t + 1) * 128])
        a_v[3] = bc(jnp.concatenate([ar[:, MA:], ar[:, MA:]], axis=1))
        a_v[7] = bc(jnp.concatenate([ai[:, MA:], -ai[:, MA:]], axis=1))
        col_v[0] = _column(dsk_v[...].astype(F32).reshape(1, M))
        col_v[1] = _column(gw_v[...].astype(F32).reshape(1, M))

        never = never_v[...] != 0

        def spread(us, rows, cols, lo, hi, sub=0, nsub=1):
            out = []
            for c in range(cols):
                vr = []
                for g in range(rows):
                    n = lo + (((c * rows + g) * nsub + sub) * (hi - lo)) // (rows * cols * nsub)
                    e, t, rg = n // 224, (n % 224) // 32, n % 32
                    vr.append(us[e][8 * rg:8 * rg + 8, 128 * t:128 * t + 128])
                out.append(jnp.concatenate(vr, axis=0))
            mask = jnp.concatenate([jnp.concatenate([never] * rows, axis=0)] * cols, axis=1)
            return mask, jnp.concatenate(out, axis=1)

        def bu(s):
            b_cat = bc_v[0:2 * M, :]
            r = pl.ds(pl.multiple_of(s * (LSEG // 2), LSEG // 2), LSEG // 2)
            xs = []
            us = []
            for e in range(2):
                c0 = pl.multiple_of(s * LSEG + e * HS, LSEG)
                xe = xt_v[:, pl.ds(c0, LSEG)].T
                u = lax.dot_general(xe, b_cat, NT, preferred_element_type=F32)
                us.append(u)
                rows = pl.ds(pl.multiple_of((s + e * NPRO) * SEG_STRIDE, 8), LSEG)
                u_v[6, rows, :] = u[:, :128]
                u_v[7, rows, :] = pltpu.roll(u[:, :128], MR, 1)
                for t in range(6):
                    u_v[t, rows, :] = u[:, (t + 1) * 128:(t + 2) * 128]
                xw = pltpu.bitcast(xe, U32)
                xw = jnp.concatenate([xw, jnp.zeros((LSEG // 2, 2 * D - M), U32)], axis=1)
                xs.append((xw[:, :D], xw[:, D:]))
            mask, dep = spread(us, 16, 2, XLO, XHI)
            dep = pltpu.bitcast(dep, U32)
            quad = [_unpack(x) for x in (jnp.where(mask, dep, xs[0][0]), xs[0][1], xs[1][0],
                                         jnp.where(mask, dep, xs[1][1]))]
            par = [_lhs_sums(*(q[e] for q in quad)) for e in range(2)]
            for i, (lo, hi) in enumerate(zip(*par)):
                t = _pack(lo, hi)
                for kt in range(2):
                    xs_v[i, kt, r, :] = t[:, kt * 128:(kt + 1) * 128]
            return us

        def c_terms(s, us):
            nw = CW // 2
            r0 = s * (CSTEP // 2)
            blk = [[None] * 4 for _ in range(4)]
            for q in range(4):
                w = c_v[pl.ds(pl.multiple_of(r0 + q * (QS // 2), 8), nw), :]
                for k in range(4):
                    blk[q][k] = _unpack(w[:, k * D:(k + 1) * D])
            r = pl.ds(pl.multiple_of(r0, 8), nw)
            par = []
            for e in range(2):
                sub = [_lhs_sums(blk[a][c][e], blk[a][2 + c][e],
                                 blk[2 + a][c][e], blk[2 + a][2 + c][e])
                       for a in range(2) for c in range(2)]
                terms = []
                for i in range(7):
                    quad = [sub[n][i] for n in range(4)]
                    mask, dep = spread(us, nw // 8, 2, CLO, CHI, i, 7)
                    quad = [jnp.where(mask, dep, x) if n in (0, 3) else x
                            for n, x in enumerate(quad)]
                    terms += _lhs_sums(*quad)
                par.append(terms)
            for n, (lo, hi) in enumerate(zip(*par)):
                t = _pack(lo, hi)
                for kt in range(2):
                    cs_v[n, kt, r, :] = t[:, kt * 128:(kt + 1) * 128]

        for cp in first_cps:
            cp.wait()
        bu(0)

        def pro_step(s, _):
            for cp in stage_copies(s):
                cp.wait()
            c_terms(s - 1, bu(s))
            return 0

        lax.fori_loop(1, NPRO, pro_step, 0)

    _prologue()

    def o_tiles(jobs, host=None):
        lhs = [[wt_v[sl, t, 8 * g:8 * g + 8, :] for g in range(HM // 16)] for sl, t, _ in jobs]
        if host is not None:
            host(lhs)
        return [lax.dot_general(pltpu.bitcast(jnp.concatenate(l, axis=0), BF16),
                                c, NT, preferred_element_type=F32)
                for l, (_, _, c) in zip(lhs, jobs)]

    def o_add(i, quad, x):
        r0, c0 = (quad // 2) * HM, (2 * i + quad % 2) * TQ
        acc_v[r0:r0 + HM, c0:c0 + TQ] += x

    def o_finish_a(i, m2, m3, m4, m5):
        o_add(i, 0, m4 - m5)
        o_add(i, 1, m3 + m5)
        o_add(i, 2, m2 + m4)
        o_add(i, 3, m3 - m2)

    def o_round_a(sl, i, ct, host=None):
        o_finish_a(i, *o_tiles([(sl, t, ct[t]) for t in (1, 2, 3, 4)], host))

    def o_round_b(sl, i, ct, extra, host=None):
        ms = o_tiles([(sl, t, ct[t]) for t in (0, 5, 6)]
                     + [(e[0], e[2], e[3]) for e in extra], host)
        o_add(i, 0, ms[0] + ms[2])
        o_add(i, 3, ms[0] + ms[1])
        for (_, ie, t, _), m in zip(extra, ms[3:]):
            if t != 5:
                o_add(ie, 0, m)
            if t != 6:
                o_add(ie, 3, m)

    def carried(sl):
        ct = [ctxc_v[t] for t in range(7)]
        return ct, [(sl, i, t, ctxc_v[7 + n]) for n, (i, t) in enumerate(CARRY)]

    def kv_scale(sl, deps=None, never=None):
        ex = []
        for n, buf in enumerate((wk_b, wv_b)):
            acc = []
            for g in range(8):
                vs = [pltpu.bitcast(buf[sl, 128 * g + 32 * a:128 * g + 32 * a + 8,
                                        128 * c:128 * c + 128] & jnp.uint32(0x7FFF0000), F32)
                      for a in range(4) for c in range(2)]
                if deps is not None:
                    vs[0] = jnp.where(never, deps[n][128 * g:128 * g + 8], vs[0])
                acc.append(functools.reduce(jnp.add, vs))
            tot = jnp.sum(functools.reduce(jnp.add, acc), keepdims=True)
            ex.append(pltpu.bitcast(tot, jnp.int32) >> 23)
        de = jnp.broadcast_to(jnp.clip(ex[0] - ex[1], -60, 60), (8, 128))
        fac_v[0] = pltpu.bitcast((127 + de) << 23, F32)
        fac_v[1] = pltpu.bitcast((127 - de) << 23, F32)

    def head(h, _):
        slot = lax.bitwise_and(h, 1)

        @pl.when(h == H // 2)
        def _segment_carry():
            pr = [a_v[t] for t in range(4)]
            pi = [a_v[4 + t] for t in range(4)]
            for _ in range(int(math.log2(LSEG))):
                pr, pi = ([pr[t] * pr[t] - pi[t] * pi[t] for t in range(4)],
                          [2.0 * pr[t] * pi[t] for t in range(4)])
            row = lax.broadcasted_iota(jnp.int32, (NSEG, 128), 0)
            e_r = [st_v[t] for t in range(4)]
            e_i = [st_v[4 + t] for t in range(4)]
            ir = [jnp.zeros((NSEG, 128), F32)] * 4
            ii = ir
            for s in range(1, NSEG):
                mr, mi = _cmul(pr, pi, ir, ii)
                fr = [pltpu.roll(mr[k] + e_r[k], 1, 0) for k in range(4)]
                fi = [pltpu.roll(mi[k] + e_i[k], 1, 0) for k in range(4)]
                ir = [jnp.where(row == s, fr[k], ir[k]) for k in range(4)]
                ii = [jnp.where(row == s, fi[k], ii[k]) for k in range(4)]
            for t in range(4):
                st_v[t] = ir[t]
                st_v[4 + t] = ii[t]

        @pl.when(h == 1)
        def _():
            for cp in late_cps:
                cp.wait()

        for cp in w_copies(h, slot):
            cp.wait()

        @pl.when(h == 0)
        def _():
            kv_scale(0)

        o_prev = o_tiles([(1 - slot, t, ctxc_v[t]) for t in (1, 2, 3, 4)])
        for cp in w_copies(jnp.minimum(h + 1, H - 1), 1 - slot):
            cp.start()
        o_finish_a(0, *o_prev)
        ct0, singles = carried(1 - slot)
        v_up = jnp.concatenate([fac_v[0, 0:1, :]] * 2, axis=1)
        v_down = fac_v[1, 0:1, :]

        up = ((1 - slot) * 16).astype(U32)
        never = never_v[...] != 0
        never64 = jnp.concatenate([never] * 8, axis=0)
        never128 = jnp.concatenate([never] * 16, axis=0)

        def weight(buf):
            return pltpu.bitcast((buf[slot] << up) & jnp.uint32(0xFFFF0000), F32)

        def quads(w, kh):
            return w[:kh, :128], w[:kh, 128:], w[kh:, :128], w[kh:, 128:]

        def bf(rows):
            return pltpu.bitcast(jnp.concatenate(
                [jnp.concatenate(r, axis=1) for r in rows], axis=0), BF16)

        def pk(x):
            return pltpu.bitcast(x.astype(BF16), U32)

        def nt(a, b):
            return lax.dot_general(a, b, NT, preferred_element_type=F32)

        def nn(a, b):
            return jnp.dot(a, b, preferred_element_type=F32)

        pin_list = []

        def x_term(i, chunks=range(8)):
            return bf([[xs_v[i, c, g * 64:(g + 1) * 64, :] for c in range(2)] for g in chunks])

        def sup(cq, j):
            l, r = (cq[0], cq[1]) if j < NS // 2 else (cq[2], cq[3])
            r0 = (j % (NS // 2)) * 2 * TQ
            return l[r0:r0 + TQ], r[r0:r0 + TQ], l[r0 + TQ:r0 + 2 * TQ], r[r0 + TQ:r0 + 2 * TQ]

        def pki(x):
            return _pack(jnp.concatenate([x[16 * g:16 * g + 8] for g in range(8)], axis=0),
                         jnp.concatenate([x[16 * g + 8:16 * g + 16] for g in range(8)], axis=0))

        def rhs_tiles(b11, b12, b21, b22, with_terms):
            plain = [pki(b11), pki(b12), pki(b21), pki(b22)]
            if not with_terms:
                return None, plain, plain
            extra = [pki(x) for x in (b11 + b22, b12 - b22, b21 - b11, b11 + b12, b21 + b22)]
            terms = [extra[0], plain[0], extra[1], extra[2], plain[3], extra[3], extra[4]]
            return terms, plain, plain + extra

        def lhs_tiles(a11, a12, a21, a22, with_terms):
            plain = [pk(a11), pk(a12), pk(a21), pk(a22)]
            if not with_terms:
                return None, plain, plain
            extra = [pk(a11 + a22), pk(a21 + a22), pk(a11 + a12), pk(a21 - a11), pk(a12 - a22)]
            terms = [extra[0], extra[1], plain[0], plain[3], extra[2], extra[3], extra[4]]
            return terms, plain, plain + extra

        qscale = (D ** -0.5) * math.log2(math.e)
        wq = jnp.concatenate([weight(wq_b), jnp.zeros((2 * D - M, D), F32)], axis=0)
        wqt = _rhs_terms(*quads(wq, D))
        qlog = [nn(x_term(i), wqt[i]) for i in (3, 0, 1, 2, 5, 4)]
        m4, m1, m2, m3, m6, m5 = qlog
        m7 = jnp.concatenate([nn(x_term(6, o), wqt[6])
                              for o in (range(2), range(2, 4), range(4, 8))], axis=0)
        qq = [x * qscale for x in ((m1 + m4) + (m7 - m5), m3 + m5, m2 + m4, (m1 + m3) + (m6 - m2))]
        qt, qp = [None] * NS, [None] * NS
        for j in range(NS - 1, -1, -1):
            qt[j], qp[j], allt = lhs_tiles(*sup(qq, j), j > 0)
            pin_list += allt

        r0 = pl.multiple_of(jnp.clip(h - 1, 0, M // CROWS - 1) * CROWS, CROWS)
        src = jnp.where(h == 0, 0, 2 * M) + r0
        cre = bc_v[pl.ds(pl.multiple_of(src, CROWS), CROWS), :].astype(F32)
        cim = bc_v[pl.ds(pl.multiple_of(src + M, CROWS), CROWS), :].astype(F32)
        cr = coef_v[0, 0:1, :]
        ci = coef_v[1, 0:1, :]
        c_r = cre * cr - cim * ci
        c_i = -(cre * ci + cim * cr)
        ccat_v[pl.ds(r0, CROWS), :] = jnp.concatenate(
            [c_r[:, :MA], c_i[:, :MA], c_r[:, MA:], c_i[:, MA:]], axis=1).astype(BF16)

        t0 = lax.bitwise_and(h, H // 2 - 1) * STEPS
        a_r = [a_v[t] for t in range(4)]
        a_i = [a_v[4 + t] for t in range(4)]
        hr = [st_v[t] for t in range(4)]
        hi = [st_v[4 + t] for t in range(4)]
        for j in range(STEPS):
            pos = (j * SCAN_SPAN * 128) // STEPS
            dep = qlog[2 * (pos // 128)][8 * (pos % 128):8 * (pos % 128) + 8]
            hr = [jnp.where(never, dep, x) for x in hr]
            us = [u_v[kk, pl.ds(t0 + j, NSEG, stride=SEG_STRIDE), :] for kk in range(8)]
            mr, mi = _cmul(a_r, a_i, hr, hi)
            hr = [mr[0] + us[0], mr[1] + us[1], mr[2] + us[2], mr[3] + us[6]]
            hi = [mi[0] + us[3], mi[1] + us[4], mi[2] + us[5], mi[3] + us[7]]
            r0 = pl.multiple_of((t0 + j) * NSEG, NSEG)
            for kk, val in enumerate(hr[:3] + hi[:3] + [hr[3]]):
                h_v[kk, pl.ds(r0, NSEG), :] = val
        for t in range(4):
            st_v[t] = hr[t]
            st_v[4 + t] = hi[t]

        w11, w12, w21, w22 = quads(wot_v[slot], HM // 2)
        dep = pltpu.bitcast(jnp.concatenate(
            [qlog[WODEP][64 * g:64 * g + 8] for g in range(HM // 16)], axis=0), U32)
        nv = jnp.concatenate([never] * (HM // 16), axis=0)
        quad = [_unpack(x) for x in (jnp.where(nv, dep, w11), w12, w21, jnp.where(nv, dep, w22))]
        par = [_lhs_sums(*(q[e] * v_down for q in quad)) for e in range(2)]
        for t, (lo, hi) in enumerate(zip(*par)):
            wt_v[slot, t] = _pack(lo, hi)

        kv_scale(slot, [qlog[1], qlog[4]], never)
        wk, wv = weight(wk_b), weight(wv_b) * v_up
        hc = DC // 2
        outer = _rhs_sums(wk[:hc], wv[:hc], wk[hc:], wv[hc:])
        mo = {}
        mpins = []
        kt, kp, vt, vp = [None] * NS, [None] * NS, [None] * NS, [None] * NS

        def host_lhs(tiles, share, nt_):
            slots = [(g, c) for g in range(len(tiles)) for c in range(len(tiles[0]))]
            todo = [mpins.pop(0) for _ in range(min(share, len(mpins)))]
            todo += [pin_list.pop(0) for _ in range(min(nt_, len(pin_list), len(slots) - len(todo)))]
            for n, x in enumerate(todo):
                g, c = slots[len(slots) - 1 - ((len(todo) - 1 - n) * len(slots)) // len(todo)]
                tiles[g][c] = jnp.where(never64, x, tiles[g][c])
            return bf(tiles)

        def half_tiles(left, right, top, is_k):
            for jj in range(NS // 2):
                j = jj if top else NS // 2 + jj
                x11, x12, x21, x22 = sup((left, right, left, right), j)
                if is_k:
                    kt[j], kp[j], allt = rhs_tiles(x11, x21, x12, x22, j < NS - 1)
                else:
                    vt[j], vp[j], allt = rhs_tiles(x11, x12, x21, x22, j < NS - 1)
                pin_list.extend(allt)

        for n, i in enumerate(OUTER):
            rhs = _rhs_terms(*quads(outer[i], D))
            p = {}
            for e, t in enumerate(INNER):
                tiles = [[cs_v[7 * i + t, c, g * 64:(g + 1) * 64, :] for c in range(2)]
                         for g in range(4)]
                w0, w1 = WSH[e], WSH[e + 1]
                share = (32 * w1) // WSH[7] - (32 * w0) // WSH[7]
                extra = (GPIN[n] * w1) // WSH[7] - (GPIN[n] * w0) // WSH[7]
                p[t] = nn(host_lhs(tiles, share, extra), rhs[t])
            quad = [(p[0] + p[3]) + (p[6] - p[4]), p[2] + p[4],
                    p[1] + p[3], (p[0] + p[2]) + (p[5] - p[1])]
            mo[i] = [jnp.concatenate([quad[c], quad[2 + c]], axis=0) for c in range(2)]
            for x in (quad[2], quad[1], quad[0], quad[3]):
                x = pltpu.bitcast(x, U32)
                mpins += [x[g * 64:(g + 1) * 64] for g in range(8)]
            done = set(OUTER[:n + 1])
            for need, f, top, is_k in (
                    ({0, 3, 4, 6}, lambda c: (mo[0][c] + mo[3][c]) + (mo[6][c] - mo[4][c]), True, True),
                    ({1, 3}, lambda c: mo[1][c] + mo[3][c], False, True),
                    ({2, 4}, lambda c: mo[2][c] + mo[4][c], True, False),
                    ({0, 1, 2, 5}, lambda c: (mo[0][c] + mo[2][c]) + (mo[5][c] - mo[1][c]), False, False)):
                if i in need and need <= done:
                    del mpins[:]
                    half_tiles(f(0), f(1), top, is_k)

        vn = [[x ^ jnp.uint32(0x80008000) for x in t] for t in vp]
        col = lax.broadcasted_iota(jnp.int32, (TQ, TQ), 1)
        key = (col & ~15) | ((col & 1) << 3) | ((col & 15) >> 1)
        causal = key <= lax.broadcasted_iota(jnp.int32, (TQ, TQ), 0)

        class Block:
            def __init__(self):
                self.tiles = [{}, {}]
                self.mx = [None, None]
                self.tmp, self.acc, self.p = {}, {}, {}

            def note(self, half, n, x):
                self.tiles[half][n] = x
                self.mx[half] = x if self.mx[half] is None else jnp.maximum(self.mx[half], x)

        blks = [Block() for _ in range(NS)]
        rlog = []
        snaps = []

        def host_tile(x):
            return jnp.where(never64, pin_list.pop(0), x) if pin_list else x

        def smm(i, j, t, lhs=None):
            lhs = host_tile(qt[i][t]) if lhs is None else lhs
            rlog[-1] = nt(bf([[lhs]]), bf([[kt[j][t]]]))
            return rlog[-1]

        def host_max(r, lhs):
            old = [sn for sn in snaps if sn[0] <= r - AGE]
            if not old:
                return lhs
            pick = [sn for sn in old if sn[1] == old[0][1]][-1]
            snaps[:] = [sn for sn in snaps if sn[1] != pick[1] or sn[0] > pick[0]]
            t_, b_ = (pltpu.bitcast(x, U32) for x in pick[2])
            return [jnp.where(never64, x, y)
                    for x, y in zip((t_[:64], t_[64:], b_[:64], b_[64:]), lhs)]

        def s_run(r, kind, i, arg):
            blk = blks[i]
            if kind == 'a':
                lhs = host_max(r, [qt[i][t] for t in (1, 2, 3, 4)])
                m2, m3, m4, m5 = (smm(i, arg, t, x) for x, t in zip(lhs, (1, 2, 3, 4)))
                blk.tmp[arg] = [m4 - m5, m3 - m2, m3 + m5, m2 + m4]
                return
            if kind == 'd':
                half, kr = arg
                x = nt(bf([qp[i][2 * half:2 * half + 2]]), bf([[kp[i][kr], kp[i][2 + kr]]]))
                rlog[-1] = x
                blk.note(half, 2 * i + kr, jnp.where(causal, x, -1e9) if half == kr else x)
                if kr == 0:
                    return
            else:
                j = arg if kind == 'b' else arg[0]
                tmp = blk.tmp[j]
                if kind == 'b':
                    m1, m6, m7 = (smm(i, j, t) for t in (0, 5, 6))
                    c11, c22 = tmp[0] + (m1 + m7), tmp[1] + (m1 + m6)
                elif arg[1] == 0:
                    m1 = smm(i, j, 0)
                    c11, c22 = tmp[0] + m1, tmp[1] + m1
                else:
                    tmp[6 - arg[1]] = tmp[6 - arg[1]] + smm(i, j, arg[1])
                    return
                blk.note(0, 2 * j + 1, tmp[2])
                blk.note(1, 2 * j, tmp[3])
                blk.note(0, 2 * j, c11)
                blk.note(1, 2 * j + 1, c22)
            snaps.append((r, i, tuple(blk.mx)))

        def row_shift(i):
            blk = blks[i]
            blk.m = []
            for lane in blk.mx:
                m = jnp.max(lane, axis=1, keepdims=True)
                if i > 0:
                    m = m + jnp.log2(jnp.sum(jnp.exp2(lane - m), axis=1, keepdims=True))
                blk.m.append(m)

        def prob(blk, half, n):
            if (half, n) not in blk.p:
                blk.p[half, n] = jnp.exp2(blk.tiles[half][n] - blk.m[half])
            return blk.p[half, n]

        def pv_run(i, t, js):
            blk = blks[i]
            lhs, rhs = [], []
            for j in js:
                if j >= i:
                    half, col = _DIAG[t]
                    lhs.append(prob(blk, half, 2 * i + j - i))
                    rhs.append((vn if t > 6 and i > 0 else vp)[i][2 * (j - i) + col])
                    continue
                a11, a12 = (lambda: prob(blk, 0, 2 * j)), (lambda: prob(blk, 0, 2 * j + 1))
                a21, a22 = (lambda: prob(blk, 1, 2 * j)), (lambda: prob(blk, 1, 2 * j + 1))
                lhs.append((
                    lambda: a11() + a22(), lambda: a21() + a22(), a11, a22,
                    lambda: a11() + a12(), lambda: a21() - a11(), lambda: a12() - a22())[t]())
                rhs.append(vt[j][t])
            x = nn(jnp.concatenate(lhs, axis=1).astype(BF16), bf([[r] for r in rhs]))
            blk.acc[t] = x if t not in blk.acc else x + blk.acc[t]
            rlog[-1] = x

        def lane_sums(i):
            out = []
            for half in range(2):
                tl = [p for (hf, _), p in blks[i].p.items() if hf == half]
                if i > 0:
                    tl[0] = jnp.where(never128, rlog[-INDEL - (INSTAG if half == 0 else 0)], tl[0])
                out.append(functools.reduce(jnp.add, tl))
            return out

        def normalise(i, lanes):
            m = blks[i].acc
            if i > 0:
                ctx = [[(m[0] + m[3]) + (m[6] - m[4]), (m[2] + m[4]) - m[7]],
                       [(m[1] + m[3]) - m[8], (m[0] + m[2]) + (m[5] - m[1])]]
            else:
                ctx = [[m[6], m[7]], [m[8], m[5]]]
            r = [_recip(jnp.sum(l, axis=1, keepdims=True)) for l in lanes]
            return _rhs_terms(ctx[0][0] * r[0], ctx[1][0] * r[1],
                              ctx[0][1] * r[0], ctx[1][1] * r[1])

        def sum_host(lanes, part, nparts):
            def host(lhs):
                n = 32 // nparts
                g0 = OS0 if part == 0 else 0
                slots = [(g, c) for g in range(g0, HM // 16) for c in range(len(lhs))]
                for k in range(n):
                    g, c = slots[len(slots) - 1 - ((n - 1 - k) * len(slots)) // n]
                    kk = part * n + k
                    l = lanes[kk // 16][8 * (kk % 16):8 * (kk % 16) + 8]
                    lhs[c][g] = jnp.where(never, pltpu.bitcast(l, U32), lhs[c][g])
            return host if lanes is not None else None

        rounds, events = _plan()
        ctx = None
        for r, units in enumerate(rounds):
            rlog.append(None)
            for u in units:
                if u[0] == 'p':
                    pv_run(*u[1:])
                else:
                    s_run(r, *u)
            for kind, i in events.get(r + 1, []):
                if kind == 'm':
                    row_shift(i)
                    continue
                lanes = lane_sums(i)
                pins = lanes if i > 0 else None
                if i == NS - 1:
                    o_round_b(1 - slot, 0, ct0, singles[:1], sum_host(pins, 0, 1))
                    del singles[:1]
                elif i + 1 in SPLIT:
                    o_round_a(slot, i + 1, ctx, sum_host(pins, 0, 1))
                    singles += [(slot, i + 1, t, ctx[t]) for t in (5, 6, 0)]
                else:
                    o_round_a(slot, i + 1, ctx, sum_host(pins, 0, 2))
                    o_round_b(slot, i + 1, ctx, singles[:1], sum_host(pins, 1, 2))
                    del singles[:1]
                ctx = normalise(i, lanes)
        assert [e[1:3] for e in singles] == CARRY
        for n, x in enumerate(ctx + [e[3] for e in singles]):
            ctxc_v[n] = x
        return 0

    lax.fori_loop(0, H, head, 0)

    def _epilogue():
        for cp in w_copies(jnp.int32(H - 1), 0):
            cp.wait()
        ct0, singles = carried((H - 1) % 2)
        o_round_a((H - 1) % 2, 0, ct0)
        o_round_b((H - 1) % 2, 0, ct0, singles)

        def o_copy(c0, width):
            cols = pl.ds(c0, width)
            return pltpu.make_async_copy(acc_v.at[:, cols], out_hbm.at[:, cols], sem.at[0])

        c_cat = ccat_v[...]
        for s in range(NSEG - 1, -1, -1):
            hs = jnp.concatenate(
                [h_v[kk, pl.ds(s, LSEG, stride=NSEG), :] for kk in range(7)],
                axis=1).astype(BF16)
            yt = lax.dot_general(c_cat, hs, NT, preferred_element_type=F32)
            w = LSEG // 2 if s == 0 else LSEG
            for e in range(LSEG // w):
                cols = pl.ds(s * LSEG + e * w, w)
                xf = xt_v[:, cols].astype(F32)
                dsk = jnp.concatenate([col_v[0]] * (w // 128), axis=1)
                gw = jnp.concatenate([col_v[1]] * (w // 128), axis=1)
                g = jax.nn.sigmoid(jnp.sum(xf * gw, axis=0, keepdims=True))
                y = yt[:, e * w:(e + 1) * w] + xf * dsk
                acc_v[:, cols] = g * acc_v[:, cols] + (1.0 - g) * y
                o_copy(s * LSEG + e * w, w).start()
        o_copy(0, S).wait()

    _epilogue()


@jax.jit
def pallas_gated_mix__compressed_kv_cla__ssm_conv_s5__prompt_kernel(
    A_x: jax.Array,
    A_c_kv: jax.Array,
    A_w_q: jax.Array,
    A_w_uk: jax.Array,
    A_w_uv: jax.Array,
    A_w_o: jax.Array,
    B_x: jax.Array,
    B_Lambda_re: jax.Array,
    B_Lambda_im: jax.Array,
    B_B_re: jax.Array,
    B_B_im: jax.Array,
    B_C_re: jax.Array,
    B_C_im: jax.Array,
    B_log_dt: jax.Array,
    B_Dskip: jax.Array,
    gate_w: jax.Array,
):
    del B_x
    hbm_spec = pl.BlockSpec(memory_space=pltpu.HBM)
    out_t = pl.pallas_call(
        _kernel,
        in_specs=[hbm_spec] * 15,
        out_specs=hbm_spec,
        out_shape=jax.ShapeDtypeStruct((M, S), F32),
        scratch_shapes=[
            pltpu.VMEM((M, S), BF16),
            pltpu.VMEM((7, 2, HS // 2, 128), U32),
            pltpu.VMEM((HS, DC), U32),
            pltpu.VMEM((49, 2, QS // 2, 128), U32),
            pltpu.VMEM((2, M // 2, D), U32),
            pltpu.VMEM((2, 7, M // 4, 128), U32),
            pltpu.VMEM((2, M, D), U32),
            pltpu.VMEM((2, DC, D), U32),
            pltpu.VMEM((2, DC, D), U32),
            pltpu.VMEM((4 * M, M), BF16),
            pltpu.VMEM((M, 2 * M), BF16),
            pltpu.VMEM((M,), BF16), pltpu.VMEM((M,), BF16), pltpu.VMEM((M,), BF16),
            pltpu.VMEM((M,), BF16), pltpu.VMEM((M,), BF16),
            pltpu.VMEM((2, M, 128), F32),
            pltpu.VMEM((2, 8, M), F32),
            pltpu.VMEM((8, NSEG * SEG_STRIDE, 128), F32),
            pltpu.VMEM((7, S, 128), F32),
            pltpu.VMEM((8, NSEG, 128), F32),
            pltpu.VMEM((8, NSEG, 128), F32),
            pltpu.VMEM((M, S), F32),
            pltpu.VMEM((7 + len(CARRY), TQ, 128), BF16),
            pltpu.VMEM((8, 128), jnp.int32),
            pltpu.VMEM((2, 8, 128), F32),
            pltpu.SemaphoreType.DMA((SEM_X + NPRO,)),
        ],
        compiler_params=pltpu.CompilerParams(vmem_limit_bytes=110 * 1024 * 1024),
        name="gated_mix",
    )(
        A_x.reshape(S, M).T, A_c_kv.reshape(S, DC),
        A_w_q, A_w_uk, A_w_uv, jnp.swapaxes(A_w_o, 1, 2),
        B_Lambda_re, B_Lambda_im, B_B_re, B_B_im, B_C_re, B_C_im, B_log_dt,
        B_Dskip, gate_w,
    )
    return out_t.T.reshape(1, S, M)
```

```python
import functools
import math

import jax
import jax.numpy as jnp
from jax import lax
import jax.experimental.pallas as pl
import jax.experimental.pallas.tpu as pltpu

F32 = jnp.float32
BF16 = jnp.bfloat16
U32 = jnp.uint32

S = 2048
HS = S // 2
QS = S // 4
M = 448
HM = M // 2
DC = 1024
H = 16
D = 256
TQ = 128
NS = S // (2 * TQ)
NSEG = 8
LSEG = S // NSEG
SEG_STRIDE = LSEG + 8
STEPS = 2 * LSEG // H
MA = 384
MR = M - MA
NT = (((1,), (1,)), ((), ()))
NPRO = NSEG // 2
CW = 192
CSTEP = 160
CROWS = 32
SEM_W = 3
SEM_X = 5

XLO, XHI, CLO, CHI = 230, 440, 0, 440
SCAN_SPAN, WODEP = 2, 3
OUTER = (4, 0, 3, 6, 1, 2, 5)
INNER = (3, 1, 4, 2, 0, 6, 5)
GPIN = (24, 16, 14, 8, 32, 28, 32)
WSH = (0, 0, 4, 8, 12, 16, 20, 24)
PORDER = (2, 3, 0, 1, 5, 4, 6)
PGROUPS = [[(j, min(j + 4, i)) for j in range(0, i, 4)] for i in range(NS)]
PGROUPS[7] = [(0, 4), (4, 6), (6, 7)]
PGROUPS[3] = [(0, 2), (2, 3)]
LEAD, BAL, AGE, OS0 = 5, 16, 2, 2
CAP, ACOST, MCOST, OCOST, RATIO, PTAIL = 112, 48, 32, 48, 0.9, 26
SPLIT = (5, 1)
CARRY = [(1, 5), (1, 6), (1, 0)]

_NEEDS = {0: ((0, 0), (1, 1)), 1: ((1, 0), (1, 1)), 2: ((0, 0),), 3: ((1, 1),),
          4: ((0, 0), (0, 1)), 5: ((1, 0), (0, 0)), 6: ((0, 1), (1, 1))}


def _plan():
    def four(i, j):
        return [[('a', i, j)], [('a', i, j + 1)], [('b', i, j), ('s', i, (j + 1, 5))],
                [('a', i, j + 2)], [('b', i, j + 2), ('s', i, (j + 1, 6))],
                [('a', i, j + 3)], [('b', i, j + 3), ('s', i, (j + 1, 0))]]

    def weave(half, full):
        out = []
        for n, f in enumerate(full):
            out += half[2 * n:2 * n + 2] + [f]
        return out

    rounds = [[('d', 6, 0), ('d', 7, 0)]] + weave(four(7, 0) + four(7, 4), four(6, 0))
    events = {len(rounds) - 1: [('m', 7)]}
    rounds += [[('a', 6, 4)], [('a', 6, 5)], [('b', 6, 4), ('s', 6, (5, 5))]]
    rounds += weave([[('p', 7, t, list(range(j, j + 4)))] for j in (0, 4) for t in PORDER],
                    [[('a', 6, 6)], [('b', 6, 6), ('s', 6, (5, 6))], [('a', 5, 0)],
                     [('b', 5, 0), ('s', 6, (5, 0))], [('a', 5, 1)],
                     [('b', 5, 1), ('p', 7, 8, [8])], [('a', 5, 2)]])
    events[len(rounds) - 9] = [('m', 6)]
    rounds += [[('b', 5, 2), ('p', 7, 9, [8])]]
    events[len(rounds)] = [('o', 7)]
    sq = []
    for i in range(NS - 3, -1, -1):
        for j in range(3 if i == NS - 3 else 0, i + 1):
            sq += [(4, 'a', i, j), (3, 'b', i, j)]
        sq.append((2, 'd', i, 0))
    pq = {}
    for i in range(NS - 1):
        pq[i] = [[j1 - j0, t, list(range(j0, j1))] for j0, j1 in PGROUPS[i + 1] for t in PORDER]
        pq[i] += [[1, 8, [i + 1]], [1, 5, [i + 1]]]
    ready, seen = {NS - 2: 0}, set()

    def needs(i, t, js):
        out = set()
        for j in js:
            out |= {(i, 1, 2 * j)} if j > i else {(i, hf, 2 * j + c) for hf, c in _NEEDS[t]}
        return out

    def p_fill(free, pi, first):
        left = {i: [list(u) for u in pq[i]] for i in (pi, pi - 1) if i >= 0}
        got, new = [], set()
        while free and pi in left and ready.get(pi, 1 << 30) <= len(rounds):
            us = left[pi]
            if first is not None:
                u, first = us[first], None
            else:
                size = min(free, max(v[0] for v in us))
                fit = [v for v in us if v[0] == size] or [
                    v for v in us if v[0] == min(w[0] for w in us if w[0] > size)]
                u = min(fit, key=lambda v: len(needs(pi, v[1], v[2][-size:]) - seen - new))
            size = min(free, u[0])
            got.append(('p', pi, u[1], u[2][-size:]))
            new |= needs(pi, u[1], u[2][-size:]) - seen
            u[2], u[0] = u[2][:len(u[2]) - size], u[0] - size
            if not u[0]:
                us.remove(u)
            free -= size
            if not us:
                pi -= 1
        return got, new, free, left, pi

    pi, prev = NS - 2, OCOST
    while sq or pi >= 0:
        cands = []
        if sq:
            n, free = 0, 4
            while n < len(sq) and sq[n][0] <= free and (
                    n == 0 or 's' in (sq[n][1], sq[n - 1][1])):
                free -= sq[n][0]
                n += 1
            cands.append((n,) + p_fill(free, pi, None))
            if free == 2 and n < len(sq) and sq[n][0] == 2:
                cands.append((n + 1,) + p_fill(0, pi, None))
        if pi >= 0:
            big = max(u[0] for u in pq[pi])
            grp = next(u[2] for u in pq[pi] if u[0] == big)
            cands += [(0,) + p_fill(4, pi, k) for k, u in enumerate(pq[pi]) if u[2] == grp]
        best = None
        for n, got, new, free, left, p2 in cands:
            s_left = sum(u[0] for u in sq[n:] if u[2] >= pi - 1)
            p_left = sum(u[0] for u in left.get(pi, []))
            s_all = sum(u[0] for u in sq[n:])
            p_all = sum(u[0] for i in range(pi + 1) for u in left.get(i, pq[i]))
            load = prev + 16 * len(new) + (MCOST if n and sq[0][1] == 'a' else 0)
            late = max(s_left + BAL - p_left, 0) if s_left else 0
            drift = abs(s_all - RATIO * max(p_all - PTAIL, 0))
            cost = 1000 * free + max(load - CAP, 0) + 2 * late + drift - len(new) + len(got)
            if best is None or cost < best[0]:
                best = (cost, n, got, new, left, p2)
        _, n, got, new, left, p2 = best
        cur = [u[1:] for u in sq[:n]] + got
        done = {u[2] for u in sq[:n]}
        del sq[:n]
        seen |= new
        pq.update(left)
        rounds.append(cur)
        for i in done:
            if all(v[2] != i for v in sq):
                events.setdefault(len(rounds), []).append(('m', i))
                ready[i] = len(rounds) + LEAD
        prev = sum({'a': ACOST, 'b': 32, 'd': 16, 's': 24, 'p': 16}[u[0]] for u in cur)
        for i in range(pi, p2, -1):
            events.setdefault(len(rounds), []).append(('o', i))
            prev = OCOST
        pi = p2
    return rounds, events


def _lhs_sums(a11, a12, a21, a22):
    return [a11 + a22, a21 + a22, a11, a22, a11 + a12, a21 - a11, a12 - a22]


def _rhs_sums(b11, b12, b21, b22):
    return [b11 + b22, b11, b12 - b22, b21 - b11, b22, b11 + b12, b21 + b22]


def _rhs_terms(*quad):
    return [t.astype(BF16) for t in _rhs_sums(*quad)]


def _unpack(w):
    return (pltpu.bitcast(w << jnp.uint32(16), F32),
            pltpu.bitcast(w & jnp.uint32(0xFFFF0000), F32))


def _pack(lo, hi):
    return pltpu.pack_elementwise([lo, hi], packed_dtype=BF16).astype(U32)


def _recip(l):
    r = pl.reciprocal(l, approx=True)
    return r * (2.0 - l * r)


def _cmul(pr, pi, hr, hi):
    return ([pr[t] * hr[t] - pi[t] * hi[t] for t in range(4)],
            [pr[t] * hi[t] + pi[t] * hr[t] for t in range(4)])


def _column(row):
    row = jnp.concatenate([row, jnp.zeros((1, 512 - M), F32)], axis=1)
    return jnp.broadcast_to(row, (128, 512)).T[:M]


def _kernel(xt_hbm, c_hbm, wq_hbm, wk_hbm, wv_hbm, wot_hbm,
            lre_hbm, lim_hbm, bre_hbm, bim_hbm, cre_hbm, cim_hbm, ldt_hbm,
            dsk_hbm, gw_hbm,
            out_hbm,
            xt_v, xs_v, c_v, cs_v, wot_v, wt_v, wq_b, wk_b, wv_b, bc_v, ccat_v,
            lre_v, lim_v, ldt_v, dsk_v, gw_v, col_v, coef_v,
            u_v, h_v, a_v, st_v, acc_v, ctxc_v, never_v, fac_v, sem):
    wq32 = wq_hbm.bitcast(U32)
    wk32 = wk_hbm.bitcast(U32)
    wv32 = wv_hbm.bitcast(U32)
    c32 = c_hbm.bitcast(U32)
    wot32 = wot_hbm.bitcast(U32)

    def w_copies(h, sl):
        j = lax.shift_right_logical(h, 1)
        cps = [pltpu.make_async_copy(src.at[:, j, :], dst.at[sl], sem.at[SEM_W + sl])
               for src, dst in ((wq32, wq_b), (wk32, wk_b), (wv32, wv_b))]
        return cps + [pltpu.make_async_copy(wot32.at[h], wot_v.at[sl], sem.at[SEM_W + sl])]

    def x_copies(s):
        spans = [pl.ds(pl.multiple_of(s * LSEG + e * HS, LSEG), LSEG) for e in range(2)]
        return [pltpu.make_async_copy(xt_hbm.at[:, sp], xt_v.at[:, sp], sem.at[SEM_X + s])
                for sp in spans]

    def c_copies(start, rows, s):
        spans = [pl.ds(pl.multiple_of(start + e * (QS // 2), 8), rows) for e in range(4)]
        return [pltpu.make_async_copy(c32.at[sp], c_v.at[sp], sem.at[SEM_X + s])
                for sp in spans]

    def stage_copies(s):
        return x_copies(s) + c_copies((CW - CSTEP) // 2 + (s - 1) * (CSTEP // 2), CSTEP // 2, s)

    first_cps = x_copies(0) + [
        pltpu.make_async_copy(bre_hbm.at[MA:M], bc_v.at[0:MR], sem.at[SEM_X]),
        pltpu.make_async_copy(bim_hbm.at[MA:M], bc_v.at[MR:2 * MR], sem.at[SEM_X]),
        pltpu.make_async_copy(bre_hbm.at[0:MA], bc_v.at[2 * MR:2 * MR + MA], sem.at[SEM_X]),
        pltpu.make_async_copy(bim_hbm.at[0:MA], bc_v.at[2 * MR + MA:2 * M], sem.at[SEM_X]),
    ] + c_copies(0, (CW - CSTEP) // 2, 0)
    vec_cps = [pltpu.make_async_copy(src, dst, sem.at[1]) for src, dst in
               ((lre_hbm, lre_v), (lim_hbm, lim_v), (ldt_hbm, ldt_v), (dsk_hbm, dsk_v),
                (gw_hbm, gw_v))]
    late_cps = [pltpu.make_async_copy(cre_hbm, bc_v.at[2 * M:3 * M], sem.at[2]),
                pltpu.make_async_copy(cim_hbm, bc_v.at[3 * M:4 * M], sem.at[2])]

    def _prologue():
        zero = jnp.int32(0)
        first = vec_cps + first_cps
        for s in range(1, NPRO):
            first = first + stage_copies(s)
        for cp in first + w_copies(zero, 0) + late_cps:
            cp.start()
        acc_v[...] = jnp.zeros_like(acc_v)
        st_v[...] = jnp.zeros_like(st_v)
        ctxc_v[...] = jnp.zeros_like(ctxc_v)
        wt_v[1] = jnp.zeros(wt_v.shape[1:], U32)
        never_v[...] = jnp.zeros_like(never_v)

        for cp in vec_cps:
            cp.wait()
        lre = lre_v[...].astype(F32).reshape(1, M)
        lim = lim_v[...].astype(F32).reshape(1, M)
        dt = jnp.exp(ldt_v[...].astype(F32)).astype(BF16).astype(F32).reshape(1, M)
        er = jnp.exp(dt * lre)
        ar = er * jnp.cos(dt * lim)
        ai = er * jnp.sin(dt * lim)
        den = lre * lre + lim * lim
        coef_v[0] = jnp.broadcast_to(2.0 * ((ar - 1.0) * lre + ai * lim) / den, (8, M))
        coef_v[1] = jnp.broadcast_to(2.0 * (ai * lre - (ar - 1.0) * lim) / den, (8, M))

        def bc(v):
            return jnp.broadcast_to(v, (NSEG, 128))

        for t in range(3):
            a_v[t] = bc(ar[:, t * 128:(t + 1) * 128])
            a_v[4 + t] = bc(ai[:, t * 128:(t + 1) * 128])
        a_v[3] = bc(jnp.concatenate([ar[:, MA:], ar[:, MA:]], axis=1))
        a_v[7] = bc(jnp.concatenate([ai[:, MA:], -ai[:, MA:]], axis=1))
        col_v[0] = _column(dsk_v[...].astype(F32).reshape(1, M))
        col_v[1] = _column(gw_v[...].astype(F32).reshape(1, M))

        never = never_v[...] != 0

        def spread(us, rows, cols, lo, hi, sub=0, nsub=1):
            out = []
            for c in range(cols):
                vr = []
                for g in range(rows):
                    n = lo + (((c * rows + g) * nsub + sub) * (hi - lo)) // (rows * cols * nsub)
                    e, t, rg = n // 224, (n % 224) // 32, n % 32
                    vr.append(us[e][8 * rg:8 * rg + 8, 128 * t:128 * t + 128])
                out.append(jnp.concatenate(vr, axis=0))
            mask = jnp.concatenate([jnp.concatenate([never] * rows, axis=0)] * cols, axis=1)
            return mask, jnp.concatenate(out, axis=1)

        def bu(s):
            b_cat = bc_v[0:2 * M, :]
            r = pl.ds(pl.multiple_of(s * (LSEG // 2), LSEG // 2), LSEG // 2)
            xs = []
            us = []
            for e in range(2):
                c0 = pl.multiple_of(s * LSEG + e * HS, LSEG)
                xe = xt_v[:, pl.ds(c0, LSEG)].T
                u = lax.dot_general(xe, b_cat, NT, preferred_element_type=F32)
                us.append(u)
                rows = pl.ds(pl.multiple_of((s + e * NPRO) * SEG_STRIDE, 8), LSEG)
                u_v[6, rows, :] = u[:, :128]
                u_v[7, rows, :] = pltpu.roll(u[:, :128], MR, 1)
                for t in range(6):
                    u_v[t, rows, :] = u[:, (t + 1) * 128:(t + 2) * 128]
                xw = pltpu.bitcast(xe, U32)
                xw = jnp.concatenate([xw, jnp.zeros((LSEG // 2, 2 * D - M), U32)], axis=1)
                xs.append((xw[:, :D], xw[:, D:]))
            mask, dep = spread(us, 16, 2, XLO, XHI)
            dep = pltpu.bitcast(dep, U32)
            quad = [_unpack(x) for x in (jnp.where(mask, dep, xs[0][0]), xs[0][1], xs[1][0],
                                         jnp.where(mask, dep, xs[1][1]))]
            par = [_lhs_sums(*(q[e] for q in quad)) for e in range(2)]
            for i, (lo, hi) in enumerate(zip(*par)):
                t = _pack(lo, hi)
                for kt in range(2):
                    xs_v[i, kt, r, :] = t[:, kt * 128:(kt + 1) * 128]
            return us

        def c_terms(s, us):
            nw = CW // 2
            r0 = s * (CSTEP // 2)
            blk = [[None] * 4 for _ in range(4)]
            for q in range(4):
                w = c_v[pl.ds(pl.multiple_of(r0 + q * (QS // 2), 8), nw), :]
                for k in range(4):
                    blk[q][k] = _unpack(w[:, k * D:(k + 1) * D])
            r = pl.ds(pl.multiple_of(r0, 8), nw)
            par = []
            for e in range(2):
                sub = [_lhs_sums(blk[a][c][e], blk[a][2 + c][e],
                                 blk[2 + a][c][e], blk[2 + a][2 + c][e])
                       for a in range(2) for c in range(2)]
                terms = []
                for i in range(7):
                    quad = [sub[n][i] for n in range(4)]
                    mask, dep = spread(us, nw // 8, 2, CLO, CHI, i, 7)
                    quad = [jnp.where(mask, dep, x) if n in (0, 3) else x
                            for n, x in enumerate(quad)]
                    terms += _lhs_sums(*quad)
                par.append(terms)
            for n, (lo, hi) in enumerate(zip(*par)):
                t = _pack(lo, hi)
                for kt in range(2):
                    cs_v[n, kt, r, :] = t[:, kt * 128:(kt + 1) * 128]

        for cp in first_cps:
            cp.wait()
        bu(0)

        def pro_step(s, _):
            for cp in stage_copies(s):
                cp.wait()
            c_terms(s - 1, bu(s))
            return 0

        lax.fori_loop(1, NPRO, pro_step, 0)

    _prologue()

    def o_tiles(jobs, host=None):
        lhs = [[wt_v[sl, t, 8 * g:8 * g + 8, :] for g in range(HM // 16)] for sl, t, _ in jobs]
        if host is not None:
            host(lhs)
        return [lax.dot_general(pltpu.bitcast(jnp.concatenate(l, axis=0), BF16),
                                c, NT, preferred_element_type=F32)
                for l, (_, _, c) in zip(lhs, jobs)]

    def o_add(i, quad, x):
        r0, c0 = (quad // 2) * HM, ((2 * i + 1 + quad % 2) % (2 * NS)) * TQ
        acc_v[r0:r0 + HM, c0:c0 + TQ] += x

    def o_finish_a(i, m2, m3, m4, m5):
        o_add(i, 0, m4 - m5)
        o_add(i, 1, m3 + m5)
        o_add(i, 2, m2 + m4)
        o_add(i, 3, m3 - m2)

    def o_round_a(sl, i, ct, host=None):
        o_finish_a(i, *o_tiles([(sl, t, ct[t]) for t in (1, 2, 3, 4)], host))

    def o_round_b(sl, i, ct, extra, host=None):
        ms = o_tiles([(sl, t, ct[t]) for t in (0, 5, 6)]
                     + [(e[0], e[2], e[3]) for e in extra], host)
        o_add(i, 0, ms[0] + ms[2])
        o_add(i, 3, ms[0] + ms[1])
        for (_, ie, t, _), m in zip(extra, ms[3:]):
            if t != 5:
                o_add(ie, 0, m)
            if t != 6:
                o_add(ie, 3, m)

    def carried(sl):
        ct = [ctxc_v[t] for t in range(7)]
        return ct, [(sl, i, t, ctxc_v[7 + n]) for n, (i, t) in enumerate(CARRY)]

    def kv_scale(sl, deps=None, never=None):
        ex = []
        for n, buf in enumerate((wk_b, wv_b)):
            acc = []
            for g in range(8):
                vs = [pltpu.bitcast(buf[sl, 128 * g + 32 * a:128 * g + 32 * a + 8,
                                        128 * c:128 * c + 128] & jnp.uint32(0x7FFF0000), F32)
                      for a in range(4) for c in range(2)]
                if deps is not None:
                    vs[0] = jnp.where(never, deps[n][128 * g:128 * g + 8], vs[0])
                acc.append(functools.reduce(jnp.add, vs))
            tot = jnp.sum(functools.reduce(jnp.add, acc), keepdims=True)
            ex.append(pltpu.bitcast(tot, jnp.int32) >> 23)
        de = jnp.broadcast_to(jnp.clip(ex[0] - ex[1], -60, 60), (8, 128))
        fac_v[0] = pltpu.bitcast((127 + de) << 23, F32)
        fac_v[1] = pltpu.bitcast((127 - de) << 23, F32)

    def head(h, _):
        slot = lax.bitwise_and(h, 1)

        @pl.when(h == H // 2)
        def _segment_carry():
            pr = [a_v[t] for t in range(4)]
            pi = [a_v[4 + t] for t in range(4)]
            for _ in range(int(math.log2(LSEG))):
                pr, pi = ([pr[t] * pr[t] - pi[t] * pi[t] for t in range(4)],
                          [2.0 * pr[t] * pi[t] for t in range(4)])
            row = lax.broadcasted_iota(jnp.int32, (NSEG, 128), 0)
            e_r = [st_v[t] for t in range(4)]
            e_i = [st_v[4 + t] for t in range(4)]
            ir = [jnp.zeros((NSEG, 128), F32)] * 4
            ii = ir
            for s in range(1, NSEG):
                mr, mi = _cmul(pr, pi, ir, ii)
                fr = [pltpu.roll(mr[k] + e_r[k], 1, 0) for k in range(4)]
                fi = [pltpu.roll(mi[k] + e_i[k], 1, 0) for k in range(4)]
                ir = [jnp.where(row == s, fr[k], ir[k]) for k in range(4)]
                ii = [jnp.where(row == s, fi[k], ii[k]) for k in range(4)]
            for t in range(4):
                st_v[t] = ir[t]
                st_v[4 + t] = ii[t]

        @pl.when(h == 1)
        def _():
            for cp in late_cps:
                cp.wait()

        for cp in w_copies(h, slot):
            cp.wait()

        @pl.when(h == 0)
        def _():
            kv_scale(0)

        o_prev = o_tiles([(1 - slot, t, ctxc_v[t]) for t in (1, 2, 3, 4)])
        for cp in w_copies(jnp.minimum(h + 1, H - 1), 1 - slot):
            cp.start()
        o_finish_a(0, *o_prev)
        ct0, singles = carried(1 - slot)
        v_up = jnp.concatenate([fac_v[0, 0:1, :]] * 2, axis=1)
        v_down = fac_v[1, 0:1, :]

        up = ((1 - slot) * 16).astype(U32)
        never = never_v[...] != 0
        never64 = jnp.concatenate([never] * 8, axis=0)
        never128 = jnp.concatenate([never] * 16, axis=0)

        def weight(buf):
            return pltpu.bitcast((buf[slot] << up) & jnp.uint32(0xFFFF0000), F32)

        def quads(w, kh):
            return w[:kh, :128], w[:kh, 128:], w[kh:, :128], w[kh:, 128:]

        def bf(rows):
            return pltpu.bitcast(jnp.concatenate(
                [jnp.concatenate(r, axis=1) for r in rows], axis=0), BF16)

        def pk(x):
            return pltpu.bitcast(x.astype(BF16), U32)

        def nt(a, b):
            return lax.dot_general(a, b, NT, preferred_element_type=F32)

        def nn(a, b):
            return jnp.dot(a, b, preferred_element_type=F32)

        pin_list = []

        def x_term(i, chunks=range(8)):
            return bf([[xs_v[i, c, g * 64:(g + 1) * 64, :] for c in range(2)] for g in chunks])

        def sup(cq, j):
            l, r = (cq[0], cq[1]) if j < NS // 2 else (cq[2], cq[3])
            r0 = (j % (NS // 2)) * 2 * TQ
            return l[r0:r0 + TQ], r[r0:r0 + TQ], l[r0 + TQ:r0 + 2 * TQ], r[r0 + TQ:r0 + 2 * TQ]

        def pki(x):
            return _pack(jnp.concatenate([x[16 * g:16 * g + 8] for g in range(8)], axis=0),
                         jnp.concatenate([x[16 * g + 8:16 * g + 16] for g in range(8)], axis=0))

        qscale = (D ** -0.5) * math.log2(math.e)
        wq = jnp.concatenate([weight(wq_b), jnp.zeros((2 * D - M, D), F32)], axis=0)
        wqt = _rhs_terms(*quads(wq, D))
        qlog = [nn(x_term(i), wqt[i]) for i in (3, 0, 1, 2, 5, 4)]
        m4, m1, m2, m3, m6, m5 = qlog
        m7 = jnp.concatenate([nn(x_term(6, o), wqt[6])
                              for o in (range(2), range(2, 4), range(4, 8))], axis=0)
        qq = [x * qscale for x in ((m1 + m4) + (m7 - m5), m3 + m5, m2 + m4, (m1 + m3) + (m6 - m2))]
        ql, qr = (jnp.concatenate([qq[c], qq[2 + c]], axis=0) for c in range(2))
        qt, qp = [None] * NS, [None] * NS
        for j in range(NS - 1, -1, -1):
            r0, ht = (2 * j + 1) * TQ, (TQ if j < NS - 1 else TQ // 2)
            top, bot = slice(r0, r0 + ht), slice(r0 + ht, r0 + 2 * ht)
            qt[j] = [pk(x) for x in _lhs_sums(ql[top], qr[top], ql[bot], qr[bot])]
            if j < NS - 1:
                qp[j] = [pk(ql[bot]), qt[j][3]]
                pin_list += qt[j] + qp[j][:1]
            else:
                qp[j] = [pk(ql[:TQ]), pk(qr[:TQ])]
                pin_list += qp[j] + [jnp.concatenate([qt[j][t], qt[j][(t + 1) % 7]], axis=0)
                                     for t in (0, 2, 4, 6)]

        r0 = pl.multiple_of(jnp.clip(h - 1, 0, M // CROWS - 1) * CROWS, CROWS)
        src = jnp.where(h == 0, 0, 2 * M) + r0
        cre = bc_v[pl.ds(pl.multiple_of(src, CROWS), CROWS), :].astype(F32)
        cim = bc_v[pl.ds(pl.multiple_of(src + M, CROWS), CROWS), :].astype(F32)
        cr = coef_v[0, 0:1, :]
        ci = coef_v[1, 0:1, :]
        c_r = cre * cr - cim * ci
        c_i = -(cre * ci + cim * cr)
        ccat_v[pl.ds(r0, CROWS), :] = jnp.concatenate(
            [c_r[:, :MA], c_i[:, :MA], c_r[:, MA:], c_i[:, MA:]], axis=1).astype(BF16)

        t0 = lax.bitwise_and(h, H // 2 - 1) * STEPS
        a_r = [a_v[t] for t in range(4)]
        a_i = [a_v[4 + t] for t in range(4)]
        hr = [st_v[t] for t in range(4)]
        hi = [st_v[4 + t] for t in range(4)]
        for j in range(STEPS):
            pos = (j * SCAN_SPAN * 128) // STEPS
            dep = qlog[2 * (pos // 128)][8 * (pos % 128):8 * (pos % 128) + 8]
            hr = [jnp.where(never, dep, x) for x in hr]
            us = [u_v[kk, pl.ds(t0 + j, NSEG, stride=SEG_STRIDE), :] for kk in range(8)]
            mr, mi = _cmul(a_r, a_i, hr, hi)
            hr = [mr[0] + us[0], mr[1] + us[1], mr[2] + us[2], mr[3] + us[6]]
            hi = [mi[0] + us[3], mi[1] + us[4], mi[2] + us[5], mi[3] + us[7]]
            r0 = pl.multiple_of((t0 + j) * NSEG, NSEG)
            for kk, val in enumerate(hr[:3] + hi[:3] + [hr[3]]):
                h_v[kk, pl.ds(r0, NSEG), :] = val
        for t in range(4):
            st_v[t] = hr[t]
            st_v[4 + t] = hi[t]

        w11, w12, w21, w22 = quads(wot_v[slot], HM // 2)
        dep = pltpu.bitcast(jnp.concatenate(
            [qlog[WODEP][64 * g:64 * g + 8] for g in range(HM // 16)], axis=0), U32)
        nv = jnp.concatenate([never] * (HM // 16), axis=0)
        quad = [_unpack(x) for x in (jnp.where(nv, dep, w11), w12, w21, jnp.where(nv, dep, w22))]
        par = [_lhs_sums(*(q[e] * v_down for q in quad)) for e in range(2)]
        for t, (lo, hi) in enumerate(zip(*par)):
            wt_v[slot, t] = _pack(lo, hi)

        kv_scale(slot, [qlog[1], qlog[4]], never)
        wk, wv = weight(wk_b), weight(wv_b) * v_up
        hc = DC // 2
        outer = _rhs_sums(wk[:hc], wv[:hc], wk[hc:], wv[hc:])
        mo = {}
        mpins = []
        kt, kp, vt, vp = [None] * NS, [None] * NS, [None] * NS, [None] * NS

        def host_lhs(tiles, share, nt_):
            slots = [(g, c) for g in range(len(tiles)) for c in range(len(tiles[0]))]
            todo = [mpins.pop(0) for _ in range(min(share, len(mpins)))]
            todo += [pin_list.pop(0) for _ in range(min(nt_, len(pin_list), len(slots) - len(todo)))]
            for n, x in enumerate(todo):
                g, c = slots[len(slots) - 1 - ((len(todo) - 1 - n) * len(slots)) // len(todo)]
                tiles[g][c] = jnp.where(never64, x, tiles[g][c])
            return bf(tiles)

        def half_tiles(left, right, top, is_k):
            for jj in range(NS // 2):
                j = jj if top else NS // 2 + jj
                x11, x12, x21, x22 = sup((left, right, left, right), j)
                quad = (x11, x21, x12, x22) if is_k else (x11, x12, x21, x22)
                terms = [pki(x) for x in _rhs_sums(*quad)]
                plain = [terms[1], pki(x12)]
                (kt if is_k else vt)[j] = terms
                (kp if is_k else vp)[j] = plain
                pin_list.extend([terms[1], terms[4], plain[1]] + [terms[t] for t in (0, 2, 3, 5, 6)])

        for n, i in enumerate(OUTER):
            rhs = _rhs_terms(*quads(outer[i], D))
            p = {}
            nm = len(mpins)
            for e, t in enumerate(INNER):
                tiles = [[cs_v[7 * i + t, c, g * 64:(g + 1) * 64, :] for c in range(2)]
                         for g in range(4)]
                w0, w1 = WSH[e], WSH[e + 1]
                share = (nm * w1) // WSH[7] - (nm * w0) // WSH[7]
                extra = (GPIN[n] * w1) // WSH[7] - (GPIN[n] * w0) // WSH[7]
                p[t] = nn(host_lhs(tiles, share, extra), rhs[t])
            quad = [(p[0] + p[3]) + (p[6] - p[4]), p[2] + p[4],
                    p[1] + p[3], (p[0] + p[2]) + (p[5] - p[1])]
            mo[i] = [jnp.concatenate([quad[c], quad[2 + c]], axis=0) for c in range(2)]
            for x in (quad[2], quad[1], quad[0], quad[3]):
                x = pltpu.bitcast(x, U32)
                mpins += [x[g * 64:(g + 1) * 64] for g in range(8)]
            if n == 2:
                ktop = [(mo[0][c] + mo[3][c]) - mo[4][c] for c in range(2)]
                w = [pltpu.bitcast(x, U32) for x in ktop]
                mpins[:] = [x[g * 64:(g + 1) * 64] for g in range(16) for x in w]
            elif n == 3:
                w = pltpu.bitcast(outer[2], U32)
                mpins[:] = [w[g * 64:(g + 1) * 64, c * 128:(c + 1) * 128]
                            for g in range(8) for c in range(2)]
                half_tiles(*(ktop[c] + mo[6][c] for c in range(2)), True, True)
            elif n == 4:
                del mpins[:]
                vbot = [mo[0][c] - mo[1][c] for c in range(2)]
                half_tiles(*(mo[1][c] + mo[3][c] for c in range(2)), False, True)
            elif n == 5:
                del mpins[:]
                vbot = [vbot[c] + mo[2][c] for c in range(2)]
                half_tiles(*(mo[2][c] + mo[4][c] for c in range(2)), True, False)
            elif n == 6:
                half_tiles(*(vbot[c] + mo[5][c] for c in range(2)), False, False)

        col = lax.broadcasted_iota(jnp.int32, (TQ, TQ), 1)
        key = (col & ~15) | ((col & 1) << 3) | ((col & 15) >> 1)
        causal = key <= lax.broadcasted_iota(jnp.int32, (TQ, TQ), 0)

        class Block:
            def __init__(self):
                self.tiles = [{}, {}, {}]
                self.mx = [None, None, None]
                self.tmp, self.acc, self.p = {}, {}, {}

            def note(self, half, n, x):
                self.tiles[half][n] = x
                self.mx[half] = x if self.mx[half] is None else jnp.maximum(self.mx[half], x)

        blks = [Block() for _ in range(NS)]
        rlog = []
        snaps = []
        never32 = jnp.concatenate([never] * 4, axis=0)

        def host_tile(x):
            return jnp.where(never64, pin_list.pop(0), x) if pin_list else x

        def smm(i, j, t, lhs=None):
            rhs = kt[j][t]
            if lhs is None and i < NS - 1:
                lhs = host_tile(qt[i][t])
            elif lhs is None:
                lhs, rhs = qt[i][t], host_tile(rhs)
            rlog[-1] = nt(bf([[lhs]]), bf([[rhs]]))
            return rlog[-1]

        def host_max(r, i, lhs):
            old = [sn for sn in snaps if sn[0] <= r - AGE and (i < NS - 1 or sn[1] == i)]
            if not old:
                return lhs
            pick = [sn for sn in old if sn[1] == old[0][1]][-1]
            snaps[:] = [sn for sn in snaps if sn[1] != pick[1] or sn[0] > pick[0]]
            pn = pltpu.bitcast(jnp.concatenate(pick[2], axis=0), U32)
            k, n = pn.shape[0] // 4, lhs[0].shape[0]
            mask = never64 if k == 64 else never32
            out = []
            for e, y in enumerate(lhs):
                z = jnp.where(mask, pn[e * k:(e + 1) * k], y[n - k:])
                out.append(z if n == k else jnp.concatenate([y[:n - k], z], axis=0))
            return out

        def s_run(r, kind, i, arg):
            blk = blks[i]
            if kind == 'a':
                lhs = host_max(r, i, [qt[i][t] for t in (1, 2, 3, 4)])
                m2, m3, m4, m5 = (smm(i, arg, t, x) for x, t in zip(lhs, (1, 2, 3, 4)))
                c12, c21 = m3 + m5, m2 + m4
                blk.tmp[arg] = [c21, c12, c12, c21, m2 + m5]
                return
            if kind == 'd':
                x = nt(bf([qp[i]]), bf([kp[(i + 1) % NS]]))
                rlog[-1] = x
                blk.note(1 if i < NS - 1 else 2, 2 * i + 2, jnp.where(causal, x, -1e9))
                if blk.mx[0] is None:
                    return
            else:
                j = arg if kind == 'b' else arg[0]
                tmp = blk.tmp[j]
                if kind == 'b':
                    m1, m6, m7 = (smm(i, j, t) for t in (0, 5, 6))
                    z = m1 - tmp[4]
                    c11, c22 = tmp[0] + (z + m7), tmp[1] + (z + m6)
                elif arg[1] == 0:
                    z = smm(i, j, 0) - tmp[4]
                    c11, c22 = tmp[0] + z, tmp[1] + z
                else:
                    tmp[6 - arg[1]] = tmp[6 - arg[1]] + smm(i, j, arg[1])
                    return
                c12 = tmp[2]
                if j == i:
                    c12 = jnp.where(causal[:c12.shape[0]], c12, -1e9)
                    if i == NS - 1:
                        c22 = jnp.where(causal[TQ // 2:], c22, -1e9)
                blk.note(0, 2 * j + 1, c12)
                blk.note(1, 2 * j, tmp[3])
                blk.note(0, 2 * j, c11)
                blk.note(1, 2 * j + 1, c22)
            snaps.append((r, i, tuple(blk.mx[:2])))

        def row_shift(i):
            blk = blks[i]
            blk.m = []
            for half, lane in enumerate(blk.mx[:3 if i == NS - 1 else 2]):
                m = jnp.max(lane, axis=1, keepdims=True)
                if half < 2:
                    m = m + jnp.log2(jnp.sum(jnp.exp2(lane - m), axis=1, keepdims=True))
                blk.m.append(m)

        def prob(blk, half, n):
            if (half, n) not in blk.p:
                blk.p[half, n] = jnp.exp2(blk.tiles[half][n] - blk.m[half])
            return blk.p[half, n]

        def pv_run(i, t, js):
            blk = blks[i]
            lhs, rhs = [], []
            for j in js:
                if j > i:
                    lhs.append(prob(blk, 1 if i < NS - 1 else 2, 2 * j))
                    v = vp[j % NS][0 if t == 8 else 1]
                    rhs.append(v ^ jnp.uint32(0x80008000) if t == 8 and i < NS - 1 else v)
                    continue
                a11, a12 = (lambda: prob(blk, 0, 2 * j)), (lambda: prob(blk, 0, 2 * j + 1))
                a21, a22 = (lambda: prob(blk, 1, 2 * j)), (lambda: prob(blk, 1, 2 * j + 1))
                lhs.append((
                    lambda: a11() + a22(), lambda: a21() + a22(), a11, a22,
                    lambda: a11() + a12(), lambda: a21() - a11(), lambda: a12() - a22())[t]())
                rhs.append(vt[j][t])
            x = nn(jnp.concatenate(lhs, axis=1).astype(BF16), bf([[r] for r in rhs]))
            blk.acc[t] = x if t not in blk.acc else x + blk.acc[t]
            rlog[-1] = x

        def lane_sums(i):
            p = blks[i].p
            if i < NS - 1:
                rows = [[x for (hf, _), x in p.items() if hf == half] for half in range(2)]
            else:
                rows = [[jnp.concatenate([p[0, n], p[1, n]], axis=0) for n in range(2 * NS)],
                        [p[2, 2 * NS]]]
            out = []
            for half, tl in enumerate(rows):
                tl[0] = jnp.where(never128, rlog[half - 2], tl[0])
                out.append(functools.reduce(jnp.add, tl))
            return out

        def normalise(i, lanes):
            m = blks[i].acc
            ctx = [[(m[0] + m[3]) + (m[6] - m[4]), m[2] + m[4]],
                   [m[1] + m[3], (m[0] + m[2]) + (m[5] - m[1])]]
            if i < NS - 1:
                ctx[1][0] = ctx[1][0] - m[8]
            else:
                ctx = [[jnp.concatenate([ctx[0][c], ctx[1][c]], axis=0) for c in range(2)],
                       [m[8], m[9]]]
            r = [_recip(jnp.sum(l, axis=1, keepdims=True)) for l in lanes]
            return _rhs_terms(ctx[0][0] * r[0], ctx[1][0] * r[1],
                              ctx[0][1] * r[0], ctx[1][1] * r[1])

        def sum_host(lanes, part, nparts):
            def host(lhs):
                n = 32 // nparts
                g0 = OS0 if part == 0 else 0
                slots = [(g, c) for g in range(g0, HM // 16) for c in range(len(lhs))]
                for k in range(n):
                    g, c = slots[len(slots) - 1 - ((n - 1 - k) * len(slots)) // n]
                    kk = part * n + k
                    l = lanes[kk // 16][8 * (kk % 16):8 * (kk % 16) + 8]
                    lhs[c][g] = jnp.where(never, pltpu.bitcast(l, U32), lhs[c][g])
            return host

        rounds, events = _plan()
        ctx = None
        for r, units in enumerate(rounds):
            rlog.append(None)
            for u in units:
                if u[0] == 'p':
                    pv_run(*u[1:])
                else:
                    s_run(r, *u)
            for kind, i in events.get(r + 1, []):
                if kind == 'm':
                    row_shift(i)
                    continue
                lanes = lane_sums(i)
                if i == NS - 1:
                    o_round_b(1 - slot, 0, ct0, singles[:1], sum_host(lanes, 0, 1))
                    del singles[:1]
                elif i + 1 in SPLIT:
                    o_round_a(slot, i + 1, ctx, sum_host(lanes, 0, 1))
                    singles += [(slot, i + 1, t, ctx[t]) for t in (5, 6, 0)]
                else:
                    o_round_a(slot, i + 1, ctx, sum_host(lanes, 0, 2))
                    o_round_b(slot, i + 1, ctx, singles[:1], sum_host(lanes, 1, 2))
                    del singles[:1]
                ctx = normalise(i, lanes)
        assert [e[1:3] for e in singles] == CARRY
        for n, x in enumerate(ctx + [e[3] for e in singles]):
            ctxc_v[n] = x
        return 0

    lax.fori_loop(0, H, head, 0)

    def _epilogue():
        for cp in w_copies(jnp.int32(H - 1), 0):
            cp.wait()
        ct0, singles = carried((H - 1) % 2)
        o_round_a((H - 1) % 2, 0, ct0)
        o_round_b((H - 1) % 2, 0, ct0, singles)

        def o_copy(c0, width):
            cols = pl.ds(c0, width)
            return pltpu.make_async_copy(acc_v.at[:, cols], out_hbm.at[:, cols], sem.at[0])

        c_cat = ccat_v[...]
        for s in range(NSEG - 1, -1, -1):
            hs = jnp.concatenate(
                [h_v[kk, pl.ds(s, LSEG, stride=NSEG), :] for kk in range(7)],
                axis=1).astype(BF16)
            yt = lax.dot_general(c_cat, hs, NT, preferred_element_type=F32)
            w = LSEG // 2 if s == 0 else LSEG
            for e in range(LSEG // w):
                cols = pl.ds(s * LSEG + e * w, w)
                xf = xt_v[:, cols].astype(F32)
                dsk = jnp.concatenate([col_v[0]] * (w // 128), axis=1)
                gw = jnp.concatenate([col_v[1]] * (w // 128), axis=1)
                g = jax.nn.sigmoid(jnp.sum(xf * gw, axis=0, keepdims=True))
                y = yt[:, e * w:(e + 1) * w] + xf * dsk
                acc_v[:, cols] = g * acc_v[:, cols] + (1.0 - g) * y
                o_copy(s * LSEG + e * w, w).start()
        o_copy(0, S).wait()

    _epilogue()


@jax.jit
def pallas_gated_mix__compressed_kv_cla__ssm_conv_s5__prompt_kernel(
    A_x: jax.Array,
    A_c_kv: jax.Array,
    A_w_q: jax.Array,
    A_w_uk: jax.Array,
    A_w_uv: jax.Array,
    A_w_o: jax.Array,
    B_x: jax.Array,
    B_Lambda_re: jax.Array,
    B_Lambda_im: jax.Array,
    B_B_re: jax.Array,
    B_B_im: jax.Array,
    B_C_re: jax.Array,
    B_C_im: jax.Array,
    B_log_dt: jax.Array,
    B_Dskip: jax.Array,
    gate_w: jax.Array,
):
    del B_x
    hbm_spec = pl.BlockSpec(memory_space=pltpu.HBM)
    out_t = pl.pallas_call(
        _kernel,
        in_specs=[hbm_spec] * 15,
        out_specs=hbm_spec,
        out_shape=jax.ShapeDtypeStruct((M, S), F32),
        scratch_shapes=[
            pltpu.VMEM((M, S), BF16),
            pltpu.VMEM((7, 2, HS // 2, 128), U32),
            pltpu.VMEM((HS, DC), U32),
            pltpu.VMEM((49, 2, QS // 2, 128), U32),
            pltpu.VMEM((2, M // 2, D), U32),
            pltpu.VMEM((2, 7, M // 4, 128), U32),
            pltpu.VMEM((2, M, D), U32),
            pltpu.VMEM((2, DC, D), U32),
            pltpu.VMEM((2, DC, D), U32),
            pltpu.VMEM((4 * M, M), BF16),
            pltpu.VMEM((M, 2 * M), BF16),
            pltpu.VMEM((M,), BF16), pltpu.VMEM((M,), BF16), pltpu.VMEM((M,), BF16),
            pltpu.VMEM((M,), BF16), pltpu.VMEM((M,), BF16),
            pltpu.VMEM((2, M, 128), F32),
            pltpu.VMEM((2, 8, M), F32),
            pltpu.VMEM((8, NSEG * SEG_STRIDE, 128), F32),
            pltpu.VMEM((7, S, 128), F32),
            pltpu.VMEM((8, NSEG, 128), F32),
            pltpu.VMEM((8, NSEG, 128), F32),
            pltpu.VMEM((M, S), F32),
            pltpu.VMEM((7 + len(CARRY), TQ, 128), BF16),
            pltpu.VMEM((8, 128), jnp.int32),
            pltpu.VMEM((2, 8, 128), F32),
            pltpu.SemaphoreType.DMA((SEM_X + NPRO,)),
        ],
        compiler_params=pltpu.CompilerParams(vmem_limit_bytes=110 * 1024 * 1024),
        name="gated_mix",
    )(
        A_x.reshape(S, M).T, A_c_kv.reshape(S, DC),
        A_w_q, A_w_uk, A_w_uv, jnp.swapaxes(A_w_o, 1, 2),
        B_Lambda_re, B_Lambda_im, B_B_re, B_B_im, B_C_re, B_C_im, B_log_dt,
        B_Dskip, gate_w,
    )
    return out_t.T.reshape(1, S, M)
```

```python
import functools
import math

import jax
import jax.numpy as jnp
from jax import lax
import jax.experimental.pallas as pl
import jax.experimental.pallas.tpu as pltpu

F32 = jnp.float32
BF16 = jnp.bfloat16
U32 = jnp.uint32

S = 2048
HS = S // 2
QS = S // 4
M = 448
HM = M // 2
DC = 1024
H = 16
D = 256
TQ = 128
NS = S // (2 * TQ)
NSEG = 8
LSEG = S // NSEG
SEG_STRIDE = LSEG + 8
STEPS = 2 * LSEG // H
MA = 384
MR = M - MA
NT = (((1,), (1,)), ((), ()))
NPRO = NSEG // 2
C0, CSTEP = 16, 80
BSPLIT = 640
CROWS = 32
SEM_W = 3
SEM_X = 5

XLO, XHI, CLO, CHI = 230, 440, 10, 430
SCAN_SPAN, WODEP = 2, 3
OUTER = (4, 0, 3, 6, 1, 2, 5)
INNER = (3, 1, 4, 2, 0, 6, 5)
GPIN = (24, 16, 14, 8, 32, 28, 32)
WSH = (0, 0, 4, 8, 12, 16, 20, 24)
PORDER = (2, 3, 0, 1, 5, 4, 6)
PGROUPS = [[(j, min(j + 4, i)) for j in range(0, i, 4)] for i in range(NS)]
PGROUPS[7] = [(0, 4), (4, 6), (6, 7)]
PGROUPS[3] = [(0, 2), (2, 3)]
LEAD, BAL, AGE, OS0 = 5, 16, 2, 2
CAP, ACOST, MCOST, OCOST, RATIO, PTAIL = 112, 48, 32, 48, 0.9, 26
SPLIT = (5, 1)
CARRY = [(1, 5), (1, 6), (1, 0)]

_NEEDS = {0: ((0, 0), (1, 1)), 1: ((1, 0), (1, 1)), 2: ((0, 0),), 3: ((1, 1),),
          4: ((0, 0), (0, 1)), 5: ((1, 0), (0, 0)), 6: ((0, 1), (1, 1))}


def _plan():
    def four(i, j):
        return [[('a', i, j)], [('a', i, j + 1)], [('b', i, j), ('s', i, (j + 1, 5))],
                [('a', i, j + 2)], [('b', i, j + 2), ('s', i, (j + 1, 6))],
                [('a', i, j + 3)], [('b', i, j + 3), ('s', i, (j + 1, 0))]]

    def weave(half, full):
        out = []
        for n, f in enumerate(full):
            out += half[2 * n:2 * n + 2] + [f]
        return out

    rounds = [[('d', 6, 0), ('d', 7, 0)]] + weave(four(7, 0) + four(7, 4), four(6, 0))
    events = {len(rounds) - 1: [('m', 7)]}
    rounds += [[('a', 6, 4)], [('a', 6, 5)], [('b', 6, 4), ('s', 6, (5, 5))]]
    rounds += weave([[('p', 7, t, list(range(j, j + 4)))] for j in (0, 4) for t in PORDER],
                    [[('a', 6, 6)], [('b', 6, 6), ('s', 6, (5, 6))], [('a', 5, 0)],
                     [('b', 5, 0), ('s', 6, (5, 0))], [('a', 5, 1)],
                     [('b', 5, 1), ('p', 7, 8, [8])], [('a', 5, 2)]])
    events[len(rounds) - 9] = [('m', 6)]
    rounds += [[('b', 5, 2), ('p', 7, 9, [8])]]
    events[len(rounds)] = [('o', 7)]
    sq = []
    for i in range(NS - 3, -1, -1):
        for j in range(3 if i == NS - 3 else 0, i + 1):
            sq += [(4, 'a', i, j), (3, 'b', i, j)]
        sq.append((2, 'd', i, 0))
    pq = {}
    for i in range(NS - 1):
        pq[i] = [[j1 - j0, t, list(range(j0, j1))] for j0, j1 in PGROUPS[i + 1] for t in PORDER]
        pq[i] += [[1, 8, [i + 1]], [1, 5, [i + 1]]]
    ready, seen = {NS - 2: 0}, set()

    def needs(i, t, js):
        out = set()
        for j in js:
            out |= {(i, 1, 2 * j)} if j > i else {(i, hf, 2 * j + c) for hf, c in _NEEDS[t]}
        return out

    def p_fill(free, pi, first):
        left = {i: [list(u) for u in pq[i]] for i in (pi, pi - 1) if i >= 0}
        got, new = [], set()
        while free and pi in left and ready.get(pi, 1 << 30) <= len(rounds):
            us = left[pi]
            if first is not None:
                u, first = us[first], None
            else:
                size = min(free, max(v[0] for v in us))
                fit = [v for v in us if v[0] == size] or [
                    v for v in us if v[0] == min(w[0] for w in us if w[0] > size)]
                u = min(fit, key=lambda v: len(needs(pi, v[1], v[2][-size:]) - seen - new))
            size = min(free, u[0])
            got.append(('p', pi, u[1], u[2][-size:]))
            new |= needs(pi, u[1], u[2][-size:]) - seen
            u[2], u[0] = u[2][:len(u[2]) - size], u[0] - size
            if not u[0]:
                us.remove(u)
            free -= size
            if not us:
                pi -= 1
        return got, new, free, left, pi

    pi, prev = NS - 2, OCOST
    while sq or pi >= 0:
        cands = []
        if sq:
            n, free = 0, 4
            while n < len(sq) and sq[n][0] <= free and (
                    n == 0 or 's' in (sq[n][1], sq[n - 1][1])):
                free -= sq[n][0]
                n += 1
            cands.append((n,) + p_fill(free, pi, None))
            if free == 2 and n < len(sq) and sq[n][0] == 2:
                cands.append((n + 1,) + p_fill(0, pi, None))
        if pi >= 0:
            big = max(u[0] for u in pq[pi])
            grp = next(u[2] for u in pq[pi] if u[0] == big)
            cands += [(0,) + p_fill(4, pi, k) for k, u in enumerate(pq[pi]) if u[2] == grp]
        best = None
        for n, got, new, free, left, p2 in cands:
            s_left = sum(u[0] for u in sq[n:] if u[2] >= pi - 1)
            p_left = sum(u[0] for u in left.get(pi, []))
            s_all = sum(u[0] for u in sq[n:])
            p_all = sum(u[0] for i in range(pi + 1) for u in left.get(i, pq[i]))
            load = prev + 16 * len(new) + (MCOST if n and sq[0][1] == 'a' else 0)
            late = max(s_left + BAL - p_left, 0) if s_left else 0
            drift = abs(s_all - RATIO * max(p_all - PTAIL, 0))
            cost = 1000 * free + max(load - CAP, 0) + 2 * late + drift - len(new) + len(got)
            if best is None or cost < best[0]:
                best = (cost, n, got, new, left, p2)
        _, n, got, new, left, p2 = best
        cur = [u[1:] for u in sq[:n]] + got
        done = {u[2] for u in sq[:n]}
        del sq[:n]
        seen |= new
        pq.update(left)
        rounds.append(cur)
        for i in done:
            if all(v[2] != i for v in sq):
                events.setdefault(len(rounds), []).append(('m', i))
                ready[i] = len(rounds) + LEAD
        prev = sum({'a': ACOST, 'b': 32, 'd': 16, 's': 24, 'p': 16}[u[0]] for u in cur)
        for i in range(pi, p2, -1):
            events.setdefault(len(rounds), []).append(('o', i))
            prev = OCOST
        pi = p2
    return rounds, events


def _lhs_sums(a11, a12, a21, a22):
    return [a11 + a22, a21 + a22, a11, a22, a11 + a12, a21 - a11, a12 - a22]


def _rhs_sums(b11, b12, b21, b22):
    return [b11 + b22, b11, b12 - b22, b21 - b11, b22, b11 + b12, b21 + b22]


def _rhs_terms(*quad):
    return [t.astype(BF16) for t in _rhs_sums(*quad)]


def _unpack(w):
    return (pltpu.bitcast(w << jnp.uint32(16), F32),
            pltpu.bitcast(w & jnp.uint32(0xFFFF0000), F32))


def _pack(lo, hi):
    half = jnp.uint32(0x7FFF) + (lax.broadcasted_iota(U32, lo.shape, 1) & jnp.uint32(1))
    return (((pltpu.bitcast(lo, U32) + half) >> jnp.uint32(16))
            | ((pltpu.bitcast(hi, U32) + half) & jnp.uint32(0xFFFF0000)))


def _recip(l):
    r = pl.reciprocal(l, approx=True)
    return r * (2.0 - l * r)


def _cmul(pr, pi, hr, hi):
    return ([pr[t] * hr[t] - pi[t] * hi[t] for t in range(4)],
            [pr[t] * hi[t] + pi[t] * hr[t] for t in range(4)])


def _column(row):
    row = jnp.concatenate([row, jnp.zeros((1, 512 - M), F32)], axis=1)
    return jnp.broadcast_to(row, (128, 512)).T[:M]


def _kernel(xt_hbm, c_hbm, wq_hbm, wk_hbm, wv_hbm, wot_hbm,
            lre_hbm, lim_hbm, bre_hbm, bim_hbm, cre_hbm, cim_hbm, ldt_hbm,
            dsk_hbm, gw_hbm,
            out_hbm,
            xt_v, xs_v, c_v, cs_v, wot_v, wt_v, wq_b, wk_b, wv_b, bc_v, ccat_v,
            lre_v, lim_v, ldt_v, dsk_v, gw_v, col_v, coef_v,
            u_v, h_v, a_v, st_v, acc_v, ctxc_v, never_v, fac_v, sem):
    wq32 = wq_hbm.bitcast(U32)
    wk32 = wk_hbm.bitcast(U32)
    wv32 = wv_hbm.bitcast(U32)
    c32 = c_hbm.bitcast(U32)
    wot32 = wot_hbm.bitcast(U32)

    def w_copies(h, sl):
        j = lax.shift_right_logical(h, 1)
        cps = [pltpu.make_async_copy(src.at[:, j, :], dst.at[sl], sem.at[SEM_W + sl])
               for src, dst in ((wq32, wq_b), (wk32, wk_b), (wv32, wv_b))]
        return cps + [pltpu.make_async_copy(wot32.at[h], wot_v.at[sl], sem.at[SEM_W + sl])]

    def x_copies(s, halves=(0, 1)):
        spans = [pl.ds(pl.multiple_of(s * LSEG + e * HS, LSEG), LSEG) for e in halves]
        return [pltpu.make_async_copy(xt_hbm.at[:, sp], xt_v.at[:, sp], sem.at[SEM_X + s])
                for sp in spans]

    def c_copies(start, rows, s):
        spans = [pl.ds(pl.multiple_of(start + e * (QS // 2), 8), rows) for e in range(4)]
        return [pltpu.make_async_copy(c32.at[sp], c_v.at[sp], sem.at[SEM_X + s])
                for sp in spans]

    def stage_copies(s):
        return x_copies(s) + c_copies(C0 + (s - 1) * CSTEP, CSTEP, s)

    nb = BSPLIT - (2 * MR + MA)
    early_cps = [
        pltpu.make_async_copy(xt_hbm.at[:, 0:LSEG], xt_v.at[:, 0:LSEG], sem.at[0]),
        pltpu.make_async_copy(bre_hbm.at[MA:M], bc_v.at[0:MR], sem.at[0]),
        pltpu.make_async_copy(bim_hbm.at[MA:M], bc_v.at[MR:2 * MR], sem.at[0]),
        pltpu.make_async_copy(bre_hbm.at[0:MA], bc_v.at[2 * MR:2 * MR + MA], sem.at[0]),
        pltpu.make_async_copy(bim_hbm.at[0:nb], bc_v.at[2 * MR + MA:BSPLIT], sem.at[0]),
    ]
    first_cps = [
        pltpu.make_async_copy(bim_hbm.at[nb:MA], bc_v.at[BSPLIT:2 * M], sem.at[SEM_X]),
    ] + x_copies(0, (1,)) + c_copies(0, C0, 0)
    vec_cps = [pltpu.make_async_copy(src, dst, sem.at[1]) for src, dst in
               ((lre_hbm, lre_v), (lim_hbm, lim_v), (ldt_hbm, ldt_v), (dsk_hbm, dsk_v),
                (gw_hbm, gw_v))]
    late_cps = [pltpu.make_async_copy(cre_hbm, bc_v.at[2 * M:3 * M], sem.at[2]),
                pltpu.make_async_copy(cim_hbm, bc_v.at[3 * M:4 * M], sem.at[2])]

    def _prologue():
        zero = jnp.int32(0)
        first = vec_cps + early_cps + first_cps
        for s in range(1, NPRO):
            first = first + stage_copies(s)
        for cp in first + w_copies(zero, 0) + late_cps:
            cp.start()
        acc_v[...] = jnp.zeros_like(acc_v)
        st_v[...] = jnp.zeros_like(st_v)
        ctxc_v[...] = jnp.zeros_like(ctxc_v)
        wt_v[1] = jnp.zeros(wt_v.shape[1:], U32)
        never_v[...] = jnp.zeros_like(never_v)

        for cp in vec_cps:
            cp.wait()
        lre = lre_v[...].astype(F32).reshape(1, M)
        lim = lim_v[...].astype(F32).reshape(1, M)
        dt = jnp.exp(ldt_v[...].astype(F32)).astype(BF16).astype(F32).reshape(1, M)
        er = jnp.exp(dt * lre)
        ar = er * jnp.cos(dt * lim)
        ai = er * jnp.sin(dt * lim)
        den = lre * lre + lim * lim
        coef_v[0] = jnp.broadcast_to(2.0 * ((ar - 1.0) * lre + ai * lim) / den, (8, M))
        coef_v[1] = jnp.broadcast_to(2.0 * (ai * lre - (ar - 1.0) * lim) / den, (8, M))

        def bc(v):
            return jnp.broadcast_to(v, (NSEG, 128))

        for t in range(3):
            a_v[t] = bc(ar[:, t * 128:(t + 1) * 128])
            a_v[4 + t] = bc(ai[:, t * 128:(t + 1) * 128])
        a_v[3] = bc(jnp.concatenate([ar[:, MA:], ar[:, MA:]], axis=1))
        a_v[7] = bc(jnp.concatenate([ai[:, MA:], -ai[:, MA:]], axis=1))
        col_v[0] = _column(dsk_v[...].astype(F32).reshape(1, M))
        col_v[1] = _column(gw_v[...].astype(F32).reshape(1, M))

        never = never_v[...] != 0

        def spread(us, rows, cols, lo, hi, sub=0, nsub=1):
            out = []
            for c in range(cols):
                vr = []
                for g in range(rows):
                    n = lo + (((c * rows + g) * nsub + sub) * (hi - lo)) // (rows * cols * nsub)
                    n = (n * len(us)) // 14
                    vr.append(us[n // 32][8 * (n % 32):8 * (n % 32) + 8])
                out.append(jnp.concatenate(vr, axis=0))
            mask = jnp.concatenate([jnp.concatenate([never] * rows, axis=0)] * cols, axis=1)
            return mask, jnp.concatenate(out, axis=1)

        def store_u(seg, u, t0):
            rows = pl.ds(pl.multiple_of(seg * SEG_STRIDE, 8), LSEG)
            for t in range(t0, t0 + u.shape[1] // 128):
                ut = u[:, (t - t0) * 128:(t - t0 + 1) * 128]
                u_v[(t + 6) % 7, rows, :] = ut
                if t == 0:
                    u_v[7, rows, :] = pltpu.roll(ut, MR, 1)

        def bu(s, head_start=None):
            r = pl.ds(pl.multiple_of(s * (LSEG // 2), LSEG // 2), LSEG // 2)
            xs = []
            us = []
            for e in range(2):
                c0 = pl.multiple_of(s * LSEG + e * HS, LSEG)
                n0 = BSPLIT if head_start is not None and e == 0 else 0
                xe = head_start if n0 else xt_v[:, pl.ds(c0, LSEG)].T
                u = lax.dot_general(xe, bc_v[n0:2 * M, :], NT, preferred_element_type=F32)
                store_u(s + e * NPRO, u, n0 // 128)
                us += [u[:, t * 128:(t + 1) * 128] for t in range(u.shape[1] // 128)]
                xw = pltpu.bitcast(xe, U32)
                xw = jnp.concatenate([xw, jnp.zeros((LSEG // 2, 2 * D - M), U32)], axis=1)
                xs.append((xw[:, :D], xw[:, D:]))
            mask, dep = spread(us, 16, 2, XLO, XHI)
            dep = pltpu.bitcast(dep, U32)
            raw = {2: jnp.where(mask, dep, xs[0][0]), 3: jnp.where(mask, dep, xs[1][1])}
            quad = [_unpack(x) for x in (raw[2], xs[0][1], xs[1][0], raw[3])]
            par = [_lhs_sums(*(q[e] for q in quad)) for e in range(2)]
            for i, (lo, hi) in enumerate(zip(*par)):
                t = raw[i] if i in raw else _pack(lo, hi)
                for kt in range(2):
                    xs_v[i, kt, r, :] = t[:, kt * 128:(kt + 1) * 128]
            return us

        def c_terms(r0, nw, us):
            raw = {}
            blk = [[None] * 4 for _ in range(4)]
            for q in range(4):
                w = c_v[pl.ds(pl.multiple_of(r0 + q * (QS // 2), 8), nw), :]
                for k in range(4):
                    blk[q][k] = _unpack(w[:, k * D:(k + 1) * D])
                mask, dep = spread(us, nw // 8, 2, CLO, CHI, 2 + q // 2, 7)
                raw[7 * (2 + q // 2) + 2 + q % 2] = jnp.where(
                    mask, pltpu.bitcast(dep, U32), w[:, q * D:(q + 1) * D])
            r = pl.ds(pl.multiple_of(r0, 8), nw)
            par = []
            for e in range(2):
                sub = [_lhs_sums(blk[a][c][e], blk[a][2 + c][e],
                                 blk[2 + a][c][e], blk[2 + a][2 + c][e])
                       for a in range(2) for c in range(2)]
                terms = []
                for i in range(7):
                    quad = [sub[n][i] for n in range(4)]
                    mask, dep = spread(us, nw // 8, 2, CLO, CHI, i, 7)
                    quad = [jnp.where(mask, dep, x) if n in (0, 3) else x
                            for n, x in enumerate(quad)]
                    terms += _lhs_sums(*quad)
                par.append(terms)
            for n, (lo, hi) in enumerate(zip(*par)):
                t = raw[n] if n in raw else _pack(lo, hi)
                for kt in range(2):
                    cs_v[n, kt, r, :] = t[:, kt * 128:(kt + 1) * 128]

        for cp in early_cps:
            cp.wait()
        x0 = xt_v[:, 0:LSEG].T
        store_u(0, lax.dot_general(x0, bc_v[0:BSPLIT, :], NT, preferred_element_type=F32), 0)
        for cp in first_cps:
            cp.wait()
        c_terms(0, C0, bu(0, x0))

        def pro_step(s, _):
            for cp in stage_copies(s):
                cp.wait()
            c_terms(C0 + (s - 1) * CSTEP, CSTEP, bu(s))
            return 0

        lax.fori_loop(1, NPRO, pro_step, 0)

    _prologue()

    def o_tiles(jobs, host=None):
        lhs = [[wt_v[sl, t, 8 * g:8 * g + 8, :] for g in range(HM // 16)] for sl, t, _ in jobs]
        if host is not None:
            host(lhs)
        return [lax.dot_general(pltpu.bitcast(jnp.concatenate(l, axis=0), BF16),
                                c, NT, preferred_element_type=F32)
                for l, (_, _, c) in zip(lhs, jobs)]

    def o_add(i, quad, x):
        r0, c0 = (quad // 2) * HM, ((2 * i + 1 + quad % 2) % (2 * NS)) * TQ
        acc_v[r0:r0 + HM, c0:c0 + TQ] += x

    def o_finish_a(i, m2, m3, m4, m5):
        o_add(i, 0, m4 - m5)
        o_add(i, 1, m3 + m5)
        o_add(i, 2, m2 + m4)
        o_add(i, 3, m3 - m2)

    def o_round_a(sl, i, ct, host=None):
        o_finish_a(i, *o_tiles([(sl, t, ct[t]) for t in (1, 2, 3, 4)], host))

    def o_round_b(sl, i, ct, extra, host=None):
        ms = o_tiles([(sl, t, ct[t]) for t in (0, 5, 6)]
                     + [(e[0], e[2], e[3]) for e in extra], host)
        o_add(i, 0, ms[0] + ms[2])
        o_add(i, 3, ms[0] + ms[1])
        for (_, ie, t, _), m in zip(extra, ms[3:]):
            if t != 5:
                o_add(ie, 0, m)
            if t != 6:
                o_add(ie, 3, m)

    def carried(sl):
        ct = [ctxc_v[t] for t in range(7)]
        return ct, [(sl, i, t, ctxc_v[7 + n]) for n, (i, t) in enumerate(CARRY)]

    def kv_scale(sl, deps=None, never=None):
        ex = []
        for n, buf in enumerate((wk_b, wv_b)):
            acc = []
            for g in range(8):
                vs = [pltpu.bitcast(buf[sl, 128 * g + 32 * a:128 * g + 32 * a + 8,
                                        128 * c:128 * c + 128] & jnp.uint32(0x7FFF0000), F32)
                      for a in range(4) for c in range(2)]
                if deps is not None:
                    vs[0] = jnp.where(never, deps[n][128 * g:128 * g + 8], vs[0])
                acc.append(functools.reduce(jnp.add, vs))
            tot = jnp.sum(functools.reduce(jnp.add, acc), keepdims=True)
            ex.append(pltpu.bitcast(tot, jnp.int32) >> 23)
        de = jnp.broadcast_to(jnp.clip(ex[0] - ex[1], -60, 60), (8, 128))
        fac_v[0] = pltpu.bitcast((127 + de) << 23, F32)
        fac_v[1] = pltpu.bitcast((127 - de) << 23, F32)

    def head(h, _):
        slot = lax.bitwise_and(h, 1)

        @pl.when(h == H // 2)
        def _segment_carry():
            pr = [a_v[t] for t in range(4)]
            pi = [a_v[4 + t] for t in range(4)]
            for _ in range(int(math.log2(LSEG))):
                pr, pi = ([pr[t] * pr[t] - pi[t] * pi[t] for t in range(4)],
                          [2.0 * pr[t] * pi[t] for t in range(4)])
            row = lax.broadcasted_iota(jnp.int32, (NSEG, 128), 0)
            e_r = [st_v[t] for t in range(4)]
            e_i = [st_v[4 + t] for t in range(4)]
            ir = [jnp.zeros((NSEG, 128), F32)] * 4
            ii = ir
            for s in range(1, NSEG):
                mr, mi = _cmul(pr, pi, ir, ii)
                fr = [pltpu.roll(mr[k] + e_r[k], 1, 0) for k in range(4)]
                fi = [pltpu.roll(mi[k] + e_i[k], 1, 0) for k in range(4)]
                ir = [jnp.where(row == s, fr[k], ir[k]) for k in range(4)]
                ii = [jnp.where(row == s, fi[k], ii[k]) for k in range(4)]
            for t in range(4):
                st_v[t] = ir[t]
                st_v[4 + t] = ii[t]

        @pl.when(h == 1)
        def _():
            for cp in late_cps:
                cp.wait()

        for cp in w_copies(h, slot):
            cp.wait()

        @pl.when(h == 0)
        def _():
            kv_scale(0)

        o_prev = o_tiles([(1 - slot, t, ctxc_v[t]) for t in (1, 2, 3, 4)])
        for cp in w_copies(jnp.minimum(h + 1, H - 1), 1 - slot):
            cp.start()
        o_finish_a(0, *o_prev)
        ct0, singles = carried(1 - slot)
        v_up = jnp.concatenate([fac_v[0, 0:1, :]] * 2, axis=1)
        v_down = fac_v[1, 0:1, :]

        up = ((1 - slot) * 16).astype(U32)
        never = never_v[...] != 0
        never64 = jnp.concatenate([never] * 8, axis=0)
        never128 = jnp.concatenate([never] * 16, axis=0)

        def weight(buf):
            return pltpu.bitcast((buf[slot] << up) & jnp.uint32(0xFFFF0000), F32)

        def quads(w, kh):
            return w[:kh, :128], w[:kh, 128:], w[kh:, :128], w[kh:, 128:]

        def bf(rows):
            return pltpu.bitcast(jnp.concatenate(
                [jnp.concatenate(r, axis=1) for r in rows], axis=0), BF16)

        def pk(x):
            return pltpu.bitcast(x.astype(BF16), U32)

        def nt(a, b):
            return lax.dot_general(a, b, NT, preferred_element_type=F32)

        def nn(a, b):
            return jnp.dot(a, b, preferred_element_type=F32)

        pin_list = []

        def x_term(i, chunks=range(8)):
            return bf([[xs_v[i, c, g * 64:(g + 1) * 64, :] for c in range(2)] for g in chunks])

        def sup(cq, j):
            l, r = (cq[0], cq[1]) if j < NS // 2 else (cq[2], cq[3])
            r0 = (j % (NS // 2)) * 2 * TQ
            return l[r0:r0 + TQ], r[r0:r0 + TQ], l[r0 + TQ:r0 + 2 * TQ], r[r0 + TQ:r0 + 2 * TQ]

        qscale = (D ** -0.5) * math.log2(math.e)
        wq = jnp.concatenate([weight(wq_b), jnp.zeros((2 * D - M, D), F32)], axis=0)
        wqt = _rhs_terms(*quads(wq, D))
        qlog = [nn(x_term(i), wqt[i]) for i in (3, 0, 1, 2, 5, 4)]
        m4, m1, m2, m3, m6, m5 = qlog
        m7 = jnp.concatenate([nn(x_term(6, o), wqt[6])
                              for o in (range(2), range(2, 4), range(4, 8))], axis=0)
        qq = [x * qscale for x in ((m1 + m4) + (m7 - m5), m3 + m5, m2 + m4, (m1 + m3) + (m6 - m2))]
        ql, qr = (jnp.concatenate([qq[c], qq[2 + c]], axis=0) for c in range(2))
        qt, qp = [None] * NS, [None] * NS
        for j in range(NS - 1, -1, -1):
            r0, ht = (2 * j + 1) * TQ, (TQ if j < NS - 1 else TQ // 2)
            top, bot = slice(r0, r0 + ht), slice(r0 + ht, r0 + 2 * ht)
            qt[j] = [pk(x) for x in _lhs_sums(ql[top], qr[top], ql[bot], qr[bot])]
            if j < NS - 1:
                qp[j] = [pk(ql[bot]), qt[j][3]]
                pin_list += qt[j] + qp[j][:1]
            else:
                qp[j] = [pk(ql[:TQ]), pk(qr[:TQ])]
                pin_list += qp[j] + [jnp.concatenate([qt[j][t], qt[j][(t + 1) % 7]], axis=0)
                                     for t in (0, 2, 4, 6)]

        r0 = pl.multiple_of(jnp.clip(h - 1, 0, M // CROWS - 1) * CROWS, CROWS)
        src = jnp.where(h == 0, 0, 2 * M) + r0
        cre = bc_v[pl.ds(pl.multiple_of(src, CROWS), CROWS), :].astype(F32)
        cim = bc_v[pl.ds(pl.multiple_of(src + M, CROWS), CROWS), :].astype(F32)
        cr = coef_v[0, 0:1, :]
        ci = coef_v[1, 0:1, :]
        c_r = cre * cr - cim * ci
        c_i = -(cre * ci + cim * cr)
        ccat_v[pl.ds(r0, CROWS), :] = jnp.concatenate(
            [c_r[:, :MA], c_i[:, :MA], c_r[:, MA:], c_i[:, MA:]], axis=1).astype(BF16)

        t0 = lax.bitwise_and(h, H // 2 - 1) * STEPS
        a_r = [a_v[t] for t in range(4)]
        a_i = [a_v[4 + t] for t in range(4)]
        hr = [st_v[t] for t in range(4)]
        hi = [st_v[4 + t] for t in range(4)]
        for j in range(STEPS):
            pos = (j * SCAN_SPAN * 128) // STEPS
            dep = qlog[2 * (pos // 128)][8 * (pos % 128):8 * (pos % 128) + 8]
            hr = [jnp.where(never, dep, x) for x in hr]
            us = [u_v[kk, pl.ds(t0 + j, NSEG, stride=SEG_STRIDE), :] for kk in range(8)]
            mr, mi = _cmul(a_r, a_i, hr, hi)
            hr = [mr[0] + us[0], mr[1] + us[1], mr[2] + us[2], mr[3] + us[6]]
            hi = [mi[0] + us[3], mi[1] + us[4], mi[2] + us[5], mi[3] + us[7]]
            r0 = pl.multiple_of((t0 + j) * NSEG, NSEG)
            for kk, val in enumerate(hr[:3] + hi[:3] + [hr[3]]):
                h_v[kk, pl.ds(r0, NSEG), :] = val
        for t in range(4):
            st_v[t] = hr[t]
            st_v[4 + t] = hi[t]

        w11, w12, w21, w22 = quads(wot_v[slot], HM // 2)
        dep = pltpu.bitcast(jnp.concatenate(
            [qlog[WODEP][64 * g:64 * g + 8] for g in range(HM // 16)], axis=0), U32)
        nv = jnp.concatenate([never] * (HM // 16), axis=0)
        quad = [_unpack(x) for x in (jnp.where(nv, dep, w11), w12, w21, jnp.where(nv, dep, w22))]
        par = [_lhs_sums(*(q[e] * v_down for q in quad)) for e in range(2)]
        for t, (lo, hi) in enumerate(zip(*par)):
            wt_v[slot, t] = _pack(lo, hi)

        kv_scale(slot, [qlog[1], qlog[4]], never)
        wk, wv = weight(wk_b), weight(wv_b) * v_up
        hc = DC // 2
        outer = _rhs_sums(wk[:hc], wv[:hc], wk[hc:], wv[hc:])
        mo = {}
        mpins = []
        kt, kp, vt, vp = [None] * NS, [None] * NS, [None] * NS, [None] * NS

        def host_lhs(tiles, share, nt_):
            slots = [(g, c) for g in range(len(tiles)) for c in range(len(tiles[0]))]
            todo = [mpins.pop(0) for _ in range(min(share, len(mpins)))]
            todo += [pin_list.pop(0) for _ in range(min(nt_, len(pin_list), len(slots) - len(todo)))]
            for n, x in enumerate(todo):
                g, c = slots[len(slots) - 1 - ((len(todo) - 1 - n) * len(slots)) // len(todo)]
                tiles[g][c] = jnp.where(never64, x, tiles[g][c])
            return bf(tiles)

        def half_tiles(left, right, top, is_k):
            for jj in range(NS // 2):
                j = jj if top else NS // 2 + jj
                x11, x12, x21, x22 = sup((left, right, left, right), j)
                quad = (x11, x21, x12, x22) if is_k else (x11, x12, x21, x22)
                terms = [pk(x) for x in _rhs_sums(*quad)]
                plain = [terms[1], pk(x12)]
                (kt if is_k else vt)[j] = terms
                (kp if is_k else vp)[j] = plain
                pin_list.extend([terms[1], terms[4], plain[1]] + [terms[t] for t in (0, 2, 3, 5, 6)])

        for n, i in enumerate(OUTER):
            rhs = _rhs_terms(*quads(outer[i], D))
            p = {}
            nm = len(mpins)
            for e, t in enumerate(INNER):
                tiles = [[cs_v[7 * i + t, c, g * 64:(g + 1) * 64, :] for c in range(2)]
                         for g in range(4)]
                w0, w1 = WSH[e], WSH[e + 1]
                share = (nm * w1) // WSH[7] - (nm * w0) // WSH[7]
                extra = (GPIN[n] * w1) // WSH[7] - (GPIN[n] * w0) // WSH[7]
                p[t] = nn(host_lhs(tiles, share, extra), rhs[t])
            quad = [(p[0] + p[3]) + (p[6] - p[4]), p[2] + p[4],
                    p[1] + p[3], (p[0] + p[2]) + (p[5] - p[1])]
            mo[i] = [jnp.concatenate([quad[c], quad[2 + c]], axis=0) for c in range(2)]
            for x in (quad[2], quad[1], quad[0], quad[3]):
                x = pltpu.bitcast(x, U32)
                mpins += [x[g * 64:(g + 1) * 64] for g in range(8)]
            if n == 2:
                ktop = [(mo[0][c] + mo[3][c]) - mo[4][c] for c in range(2)]
                w = [pltpu.bitcast(x, U32) for x in ktop]
                mpins[:] = [x[g * 64:(g + 1) * 64] for g in range(16) for x in w]
            elif n == 3:
                w = pltpu.bitcast(outer[2], U32)
                mpins[:] = [w[g * 64:(g + 1) * 64, c * 128:(c + 1) * 128]
                            for g in range(8) for c in range(2)]
                half_tiles(*(ktop[c] + mo[6][c] for c in range(2)), True, True)
            elif n == 4:
                del mpins[:]
                vbot = [mo[0][c] - mo[1][c] for c in range(2)]
                half_tiles(*(mo[1][c] + mo[3][c] for c in range(2)), False, True)
            elif n == 5:
                del mpins[:]
                vbot = [vbot[c] + mo[2][c] for c in range(2)]
                half_tiles(*(mo[2][c] + mo[4][c] for c in range(2)), True, False)
            elif n == 6:
                half_tiles(*(vbot[c] + mo[5][c] for c in range(2)), False, False)

        col = lax.broadcasted_iota(jnp.int32, (TQ, TQ), 1)
        causal = col <= lax.broadcasted_iota(jnp.int32, (TQ, TQ), 0)

        class Block:
            def __init__(self):
                self.tiles = [{}, {}, {}]
                self.mx = [None, None, None]
                self.tmp, self.acc, self.p = {}, {}, {}

            def note(self, half, n, x):
                self.tiles[half][n] = x
                self.mx[half] = x if self.mx[half] is None else jnp.maximum(self.mx[half], x)

        blks = [Block() for _ in range(NS)]
        rlog = []
        snaps = []
        never32 = jnp.concatenate([never] * 4, axis=0)

        def host_tile(x):
            return jnp.where(never64, pin_list.pop(0), x) if pin_list else x

        def smm(i, j, t, lhs=None):
            rhs = kt[j][t]
            if lhs is None and i < NS - 1:
                lhs = host_tile(qt[i][t])
            elif lhs is None:
                lhs, rhs = qt[i][t], host_tile(rhs)
            rlog[-1] = nt(bf([[lhs]]), bf([[rhs]]))
            return rlog[-1]

        def host_max(r, i, lhs):
            old = [sn for sn in snaps if sn[0] <= r - AGE and (i < NS - 1 or sn[1] == i)]
            if not old:
                return lhs
            pick = [sn for sn in old if sn[1] == old[0][1]][-1]
            snaps[:] = [sn for sn in snaps if sn[1] != pick[1] or sn[0] > pick[0]]
            pn = pltpu.bitcast(jnp.concatenate(pick[2], axis=0), U32)
            k, n = pn.shape[0] // 4, lhs[0].shape[0]
            mask = never64 if k == 64 else never32
            out = []
            for e, y in enumerate(lhs):
                z = jnp.where(mask, pn[e * k:(e + 1) * k], y[n - k:])
                out.append(z if n == k else jnp.concatenate([y[:n - k], z], axis=0))
            return out

        def s_run(r, kind, i, arg):
            blk = blks[i]
            if kind == 'a':
                lhs = host_max(r, i, [qt[i][t] for t in (1, 2, 3, 4)])
                m2, m3, m4, m5 = (smm(i, arg, t, x) for x, t in zip(lhs, (1, 2, 3, 4)))
                c12, c21 = m3 + m5, m2 + m4
                blk.tmp[arg] = [c21, c12, c12, c21, m2 + m5]
                return
            if kind == 'd':
                x = nt(bf([qp[i]]), bf([kp[(i + 1) % NS]]))
                rlog[-1] = x
                blk.note(1 if i < NS - 1 else 2, 2 * i + 2, jnp.where(causal, x, -1e9))
                if blk.mx[0] is None:
                    return
            else:
                j = arg if kind == 'b' else arg[0]
                tmp = blk.tmp[j]
                if kind == 'b':
                    m1, m6, m7 = (smm(i, j, t) for t in (0, 5, 6))
                    z = m1 - tmp[4]
                    c11, c22 = tmp[0] + (z + m7), tmp[1] + (z + m6)
                elif arg[1] == 0:
                    z = smm(i, j, 0) - tmp[4]
                    c11, c22 = tmp[0] + z, tmp[1] + z
                else:
                    tmp[6 - arg[1]] = tmp[6 - arg[1]] + smm(i, j, arg[1])
                    return
                c12 = tmp[2]
                if j == i:
                    c12 = jnp.where(causal[:c12.shape[0]], c12, -1e9)
                    if i == NS - 1:
                        c22 = jnp.where(causal[TQ // 2:], c22, -1e9)
                blk.note(0, 2 * j + 1, c12)
                blk.note(1, 2 * j, tmp[3])
                blk.note(0, 2 * j, c11)
                blk.note(1, 2 * j + 1, c22)
            snaps.append((r, i, tuple(blk.mx[:2])))

        def row_shift(i):
            blk = blks[i]
            blk.m = []
            for half, lane in enumerate(blk.mx[:3 if i == NS - 1 else 2]):
                m = jnp.max(lane, axis=1, keepdims=True)
                if half < 2:
                    m = m + jnp.log2(jnp.sum(jnp.exp2(lane - m), axis=1, keepdims=True))
                blk.m.append(m)

        def prob(blk, half, n):
            if (half, n) not in blk.p:
                blk.p[half, n] = jnp.exp2(blk.tiles[half][n] - blk.m[half])
            return blk.p[half, n]

        def pv_run(i, t, js):
            blk = blks[i]
            lhs, rhs = [], []
            for j in js:
                if j > i:
                    lhs.append(prob(blk, 1 if i < NS - 1 else 2, 2 * j))
                    v = vp[j % NS][0 if t == 8 else 1]
                    rhs.append(v ^ jnp.uint32(0x80008000) if t == 8 and i < NS - 1 else v)
                    continue
                a11, a12 = (lambda: prob(blk, 0, 2 * j)), (lambda: prob(blk, 0, 2 * j + 1))
                a21, a22 = (lambda: prob(blk, 1, 2 * j)), (lambda: prob(blk, 1, 2 * j + 1))
                lhs.append((
                    lambda: a11() + a22(), lambda: a21() + a22(), a11, a22,
                    lambda: a11() + a12(), lambda: a21() - a11(), lambda: a12() - a22())[t]())
                rhs.append(vt[j][t])
            x = nn(jnp.concatenate(lhs, axis=1).astype(BF16), bf([[r] for r in rhs]))
            blk.acc[t] = x if t not in blk.acc else x + blk.acc[t]
            rlog[-1] = x

        def lane_sums(i):
            p = blks[i].p
            if i < NS - 1:
                rows = [[x for (hf, _), x in p.items() if hf == half] for half in range(2)]
            else:
                rows = [[jnp.concatenate([p[0, n], p[1, n]], axis=0) for n in range(2 * NS)],
                        [p[2, 2 * NS]]]
            out = []
            for half, tl in enumerate(rows):
                tl[0] = jnp.where(never128, rlog[half - 2], tl[0])
                out.append(functools.reduce(jnp.add, tl))
            return out

        def normalise(i, lanes):
            m = blks[i].acc
            ctx = [[(m[0] + m[3]) + (m[6] - m[4]), m[2] + m[4]],
                   [m[1] + m[3], (m[0] + m[2]) + (m[5] - m[1])]]
            if i < NS - 1:
                ctx[1][0] = ctx[1][0] - m[8]
            else:
                ctx = [[jnp.concatenate([ctx[0][c], ctx[1][c]], axis=0) for c in range(2)],
                       [m[8], m[9]]]
            r = [_recip(jnp.sum(l, axis=1, keepdims=True)) for l in lanes]
            return _rhs_terms(ctx[0][0] * r[0], ctx[1][0] * r[1],
                              ctx[0][1] * r[0], ctx[1][1] * r[1])

        def sum_host(lanes, part, nparts):
            def host(lhs):
                n = 32 // nparts
                g0 = OS0 if part == 0 else 0
                slots = [(g, c) for g in range(g0, HM // 16) for c in range(len(lhs))]
                for k in range(n):
                    g, c = slots[len(slots) - 1 - ((n - 1 - k) * len(slots)) // n]
                    kk = part * n + k
                    l = lanes[kk // 16][8 * (kk % 16):8 * (kk % 16) + 8]
                    lhs[c][g] = jnp.where(never, pltpu.bitcast(l, U32), lhs[c][g])
            return host

        rounds, events = _plan()
        ctx = None
        for r, units in enumerate(rounds):
            rlog.append(None)
            for u in units:
                if u[0] == 'p':
                    pv_run(*u[1:])
                else:
                    s_run(r, *u)
            for kind, i in events.get(r + 1, []):
                if kind == 'm':
                    row_shift(i)
                    continue
                lanes = lane_sums(i)
                if i == NS - 1:
                    o_round_b(1 - slot, 0, ct0, singles[:1], sum_host(lanes, 0, 1))
                    del singles[:1]
                elif i + 1 in SPLIT:
                    o_round_a(slot, i + 1, ctx, sum_host(lanes, 0, 1))
                    singles += [(slot, i + 1, t, ctx[t]) for t in (5, 6, 0)]
                else:
                    o_round_a(slot, i + 1, ctx, sum_host(lanes, 0, 2))
                    o_round_b(slot, i + 1, ctx, singles[:1], sum_host(lanes, 1, 2))
                    del singles[:1]
                ctx = normalise(i, lanes)
        assert [e[1:3] for e in singles] == CARRY
        for n, x in enumerate(ctx + [e[3] for e in singles]):
            ctxc_v[n] = x
        return 0

    lax.fori_loop(0, H, head, 0)

    def _epilogue():
        for cp in w_copies(jnp.int32(H - 1), 0):
            cp.wait()
        ct0, singles = carried((H - 1) % 2)
        o_round_a((H - 1) % 2, 0, ct0)
        o_round_b((H - 1) % 2, 0, ct0, singles)

        def o_copy(c0, width):
            cols = pl.ds(c0, width)
            return pltpu.make_async_copy(acc_v.at[:, cols], out_hbm.at[:, cols], sem.at[0])

        c_cat = ccat_v[...]
        for s in range(NSEG - 1, -1, -1):
            hs = jnp.concatenate(
                [h_v[kk, pl.ds(s, LSEG, stride=NSEG), :] for kk in range(7)],
                axis=1).astype(BF16)
            yt = lax.dot_general(c_cat, hs, NT, preferred_element_type=F32)
            w = LSEG // 2 if s == 0 else LSEG
            for e in range(LSEG // w):
                cols = pl.ds(s * LSEG + e * w, w)
                xf = xt_v[:, cols].astype(F32)
                dsk = jnp.concatenate([col_v[0]] * (w // 128), axis=1)
                gw = jnp.concatenate([col_v[1]] * (w // 128), axis=1)
                g = jax.nn.sigmoid(jnp.sum(xf * gw, axis=0, keepdims=True))
                y = yt[:, e * w:(e + 1) * w] + xf * dsk
                acc_v[:, cols] = g * acc_v[:, cols] + (1.0 - g) * y
                o_copy(s * LSEG + e * w, w).start()
        o_copy(0, S).wait()

    _epilogue()


@jax.jit
def pallas_gated_mix__compressed_kv_cla__ssm_conv_s5__prompt_kernel(
    A_x: jax.Array,
    A_c_kv: jax.Array,
    A_w_q: jax.Array,
    A_w_uk: jax.Array,
    A_w_uv: jax.Array,
    A_w_o: jax.Array,
    B_x: jax.Array,
    B_Lambda_re: jax.Array,
    B_Lambda_im: jax.Array,
    B_B_re: jax.Array,
    B_B_im: jax.Array,
    B_C_re: jax.Array,
    B_C_im: jax.Array,
    B_log_dt: jax.Array,
    B_Dskip: jax.Array,
    gate_w: jax.Array,
):
    del B_x
    hbm_spec = pl.BlockSpec(memory_space=pltpu.HBM)
    out_t = pl.pallas_call(
        _kernel,
        in_specs=[hbm_spec] * 15,
        out_specs=hbm_spec,
        out_shape=jax.ShapeDtypeStruct((M, S), F32),
        scratch_shapes=[
            pltpu.VMEM((M, S), BF16),
            pltpu.VMEM((7, 2, HS // 2, 128), U32),
            pltpu.VMEM((HS, DC), U32),
            pltpu.VMEM((49, 2, QS // 2, 128), U32),
            pltpu.VMEM((2, M // 2, D), U32),
            pltpu.VMEM((2, 7, M // 4, 128), U32),
            pltpu.VMEM((2, M, D), U32),
            pltpu.VMEM((2, DC, D), U32),
            pltpu.VMEM((2, DC, D), U32),
            pltpu.VMEM((4 * M, M), BF16),
            pltpu.VMEM((M, 2 * M), BF16),
            pltpu.VMEM((M,), BF16), pltpu.VMEM((M,), BF16), pltpu.VMEM((M,), BF16),
            pltpu.VMEM((M,), BF16), pltpu.VMEM((M,), BF16),
            pltpu.VMEM((2, M, 128), F32),
            pltpu.VMEM((2, 8, M), F32),
            pltpu.VMEM((8, NSEG * SEG_STRIDE, 128), F32),
            pltpu.VMEM((7, S, 128), F32),
            pltpu.VMEM((8, NSEG, 128), F32),
            pltpu.VMEM((8, NSEG, 128), F32),
            pltpu.VMEM((M, S), F32),
            pltpu.VMEM((7 + len(CARRY), TQ, 128), BF16),
            pltpu.VMEM((8, 128), jnp.int32),
            pltpu.VMEM((2, 8, 128), F32),
            pltpu.SemaphoreType.DMA((SEM_X + NPRO,)),
        ],
        compiler_params=pltpu.CompilerParams(vmem_limit_bytes=110 * 1024 * 1024),
        name="gated_mix",
    )(
        A_x.reshape(S, M).T, A_c_kv.reshape(S, DC),
        A_w_q, A_w_uk, A_w_uv, jnp.swapaxes(A_w_o, 1, 2),
        B_Lambda_re, B_Lambda_im, B_B_re, B_B_im, B_C_re, B_C_im, B_log_dt,
        B_Dskip, gate_w,
    )
    return out_t.T.reshape(1, S, M)
```

```python
import functools
import math

import jax
import jax.numpy as jnp
from jax import lax
import jax.experimental.pallas as pl
import jax.experimental.pallas.tpu as pltpu

F32 = jnp.float32
BF16 = jnp.bfloat16
U32 = jnp.uint32

S = 2048
HS = S // 2
QS = S // 4
M = 448
HM = M // 2
DC = 1024
H = 16
D = 256
TQ = 128
NS = S // (2 * TQ)
NSEG = 8
LSEG = S // NSEG
SEG_STRIDE = LSEG + 8
STEPS = 2 * LSEG // H
MA = 384
MR = M - MA
NT = (((1,), (1,)), ((), ()))
NPRO = NSEG // 2
C0, CSTEP = 16, 80
BSPLIT = 640
CROWS = 32
SEM_W = 3
SEM_X = 5

XLO, XHI, CLO, CHI = 230, 440, 10, 430
SCAN_SPAN, WODEP = 2, 3
OUTER = (4, 0, 3, 6, 1, 2, 5)
INNER = (3, 1, 4, 2, 0, 6, 5)
GPIN = (24, 16, 14, 8, 32, 28, 32)
WSH = (0, 0, 4, 8, 12, 16, 20, 24)
PORDER = (2, 3, 0, 1, 5, 4, 6)
PGROUPS = [[(j, min(j + 4, i)) for j in range(0, i, 4)] for i in range(NS)]
PGROUPS[7] = [(0, 4), (4, 6), (6, 7)]
PGROUPS[3] = [(0, 2), (2, 3)]
LEAD, BAL, AGE, OS0 = 5, 16, 2, 2
CAP, ACOST, MCOST, OCOST, RATIO, PTAIL = 112, 48, 32, 48, 0.9, 26
SPLIT = (5, 1)
CARRY = [(1, 5), (1, 6), (1, 0)]

_NEEDS = {0: ((0, 0), (1, 1)), 1: ((1, 0), (1, 1)), 2: ((0, 0),), 3: ((1, 1),),
          4: ((0, 0), (0, 1)), 5: ((1, 0), (0, 0)), 6: ((0, 1), (1, 1))}


def _plan():
    def four(i, j):
        return [[('a', i, j)], [('a', i, j + 1)], [('b', i, j), ('s', i, (j + 1, 5))],
                [('a', i, j + 2)], [('b', i, j + 2), ('s', i, (j + 1, 6))],
                [('a', i, j + 3)], [('b', i, j + 3), ('s', i, (j + 1, 0))]]

    def weave(half, full):
        out = []
        for n, f in enumerate(full):
            out += half[2 * n:2 * n + 2] + [f]
        return out

    rounds = [[('d', 6, 0), ('d', 7, 0)]] + weave(four(7, 0) + four(7, 4), four(6, 0))
    events = {len(rounds) - 1: [('m', 7)]}
    rounds += [[('a', 6, 4)], [('a', 6, 5)], [('b', 6, 4), ('s', 6, (5, 5))]]
    rounds += weave([[('p', 7, t, list(range(j, j + 4)))] for j in (0, 4) for t in PORDER],
                    [[('a', 6, 6)], [('b', 6, 6), ('s', 6, (5, 6))], [('a', 5, 0)],
                     [('b', 5, 0), ('s', 6, (5, 0))], [('a', 5, 1)],
                     [('b', 5, 1), ('p', 7, 8, [8])], [('a', 5, 2)]])
    events[len(rounds) - 9] = [('m', 6)]
    rounds += [[('b', 5, 2), ('p', 7, 9, [8])]]
    events[len(rounds)] = [('o', 7)]
    sq = []
    for i in range(NS - 3, -1, -1):
        for j in range(3 if i == NS - 3 else 0, i + 1):
            sq += [(4, 'a', i, j), (3, 'b', i, j)]
        sq.append((2, 'd', i, 0))
    pq = {}
    for i in range(NS - 1):
        pq[i] = [[j1 - j0, t, list(range(j0, j1))] for j0, j1 in PGROUPS[i + 1] for t in PORDER]
        pq[i] += [[1, 8, [i + 1]], [1, 5, [i + 1]]]
    ready, seen = {NS - 2: 0}, set()

    def needs(i, t, js):
        out = set()
        for j in js:
            out |= {(i, 1, 2 * j)} if j > i else {(i, hf, 2 * j + c) for hf, c in _NEEDS[t]}
        return out

    def p_fill(free, pi, first):
        left = {i: [list(u) for u in pq[i]] for i in (pi, pi - 1) if i >= 0}
        got, new = [], set()
        while free and pi in left and ready.get(pi, 1 << 30) <= len(rounds):
            us = left[pi]
            if first is not None:
                u, first = us[first], None
            else:
                size = min(free, max(v[0] for v in us))
                fit = [v for v in us if v[0] == size] or [
                    v for v in us if v[0] == min(w[0] for w in us if w[0] > size)]
                u = min(fit, key=lambda v: len(needs(pi, v[1], v[2][-size:]) - seen - new))
            size = min(free, u[0])
            got.append(('p', pi, u[1], u[2][-size:]))
            new |= needs(pi, u[1], u[2][-size:]) - seen
            u[2], u[0] = u[2][:len(u[2]) - size], u[0] - size
            if not u[0]:
                us.remove(u)
            free -= size
            if not us:
                pi -= 1
        return got, new, free, left, pi

    pi, prev = NS - 2, OCOST
    while sq or pi >= 0:
        cands = []
        if sq:
            n, free = 0, 4
            while n < len(sq) and sq[n][0] <= free and (
                    n == 0 or 's' in (sq[n][1], sq[n - 1][1])):
                free -= sq[n][0]
                n += 1
            cands.append((n,) + p_fill(free, pi, None))
            if free == 2 and n < len(sq) and sq[n][0] == 2:
                cands.append((n + 1,) + p_fill(0, pi, None))
        if pi >= 0:
            big = max(u[0] for u in pq[pi])
            grp = next(u[2] for u in pq[pi] if u[0] == big)
            cands += [(0,) + p_fill(4, pi, k) for k, u in enumerate(pq[pi]) if u[2] == grp]
        best = None
        for n, got, new, free, left, p2 in cands:
            s_left = sum(u[0] for u in sq[n:] if u[2] >= pi - 1)
            p_left = sum(u[0] for u in left.get(pi, []))
            s_all = sum(u[0] for u in sq[n:])
            p_all = sum(u[0] for i in range(pi + 1) for u in left.get(i, pq[i]))
            load = prev + 16 * len(new) + (MCOST if n and sq[0][1] == 'a' else 0)
            late = max(s_left + BAL - p_left, 0) if s_left else 0
            drift = abs(s_all - RATIO * max(p_all - PTAIL, 0))
            cost = 1000 * free + max(load - CAP, 0) + 2 * late + drift - len(new) + len(got)
            if best is None or cost < best[0]:
                best = (cost, n, got, new, left, p2)
        _, n, got, new, left, p2 = best
        cur = [u[1:] for u in sq[:n]] + got
        done = {u[2] for u in sq[:n]}
        del sq[:n]
        seen |= new
        pq.update(left)
        rounds.append(cur)
        for i in done:
            if all(v[2] != i for v in sq):
                events.setdefault(len(rounds), []).append(('m', i))
                ready[i] = len(rounds) + LEAD
        prev = sum({'a': ACOST, 'b': 32, 'd': 16, 's': 24, 'p': 16}[u[0]] for u in cur)
        for i in range(pi, p2, -1):
            events.setdefault(len(rounds), []).append(('o', i))
            prev = OCOST
        pi = p2
    return rounds, events


def _lhs_sums(a11, a12, a21, a22):
    return [a11 + a22, a21 + a22, a11, a22, a11 + a12, a21 - a11, a12 - a22]


def _rhs_sums(b11, b12, b21, b22):
    return [b11 + b22, b11, b12 - b22, b21 - b11, b22, b11 + b12, b21 + b22]


def _rhs_terms(*quad):
    return [t.astype(BF16) for t in _rhs_sums(*quad)]


def _unpack(w):
    return (pltpu.bitcast(w << jnp.uint32(16), F32),
            pltpu.bitcast(w & jnp.uint32(0xFFFF0000), F32))


def _pack(lo, hi):
    half = jnp.uint32(0x7FFF) + (lax.broadcasted_iota(U32, lo.shape, 1) & jnp.uint32(1))
    return (((pltpu.bitcast(lo, U32) + half) >> jnp.uint32(16))
            | ((pltpu.bitcast(hi, U32) + half) & jnp.uint32(0xFFFF0000)))


def _recip(l):
    r = pl.reciprocal(l, approx=True)
    return r * (2.0 - l * r)


def _cmul(pr, pi, hr, hi):
    return ([pr[t] * hr[t] - pi[t] * hi[t] for t in range(4)],
            [pr[t] * hi[t] + pi[t] * hr[t] for t in range(4)])


def _column(row):
    row = jnp.concatenate([row, jnp.zeros((1, 512 - M), F32)], axis=1)
    return jnp.broadcast_to(row, (128, 512)).T[:M]


def _kernel(xt_hbm, c_hbm, wq_hbm, wk_hbm, wv_hbm, wot_hbm,
            lre_hbm, lim_hbm, bre_hbm, bim_hbm, cre_hbm, cim_hbm, ldt_hbm,
            dsk_hbm, gw_hbm,
            out_hbm,
            xt_v, xs_v, c_v, cs_v, wot_v, wt_v, wq_b, wk_b, wv_b, bc_v, ccat_v,
            lre_v, lim_v, ldt_v, dsk_v, gw_v, col_v, coef_v,
            u_v, h_v, a_v, st_v, acc_v, ctxc_v, never_v, fac_v, sem):
    wq32 = wq_hbm.bitcast(U32)
    wk32 = wk_hbm.bitcast(U32)
    wv32 = wv_hbm.bitcast(U32)
    c32 = c_hbm.bitcast(U32)
    wot32 = wot_hbm.bitcast(U32)

    def w_copies(h, sl):
        j = lax.shift_right_logical(h, 1)
        cps = [pltpu.make_async_copy(src.at[:, j, :], dst.at[sl], sem.at[SEM_W + sl])
               for src, dst in ((wq32, wq_b), (wk32, wk_b), (wv32, wv_b))]
        return cps + [pltpu.make_async_copy(wot32.at[h], wot_v.at[sl], sem.at[SEM_W + sl])]

    def x_copies(s, halves=(0, 1)):
        spans = [pl.ds(pl.multiple_of(s * LSEG + e * HS, LSEG), LSEG) for e in halves]
        return [pltpu.make_async_copy(xt_hbm.at[:, sp], xt_v.at[:, sp], sem.at[SEM_X + s])
                for sp in spans]

    def c_copies(start, rows, s):
        spans = [pl.ds(pl.multiple_of(start + e * (QS // 2), 8), rows) for e in range(4)]
        return [pltpu.make_async_copy(c32.at[sp], c_v.at[sp], sem.at[SEM_X + s])
                for sp in spans]

    def stage_copies(s):
        return x_copies(s) + c_copies(C0 + (s - 1) * CSTEP, CSTEP, s)

    nb = BSPLIT - (2 * MR + MA)
    early_cps = [
        pltpu.make_async_copy(xt_hbm.at[:, 0:LSEG], xt_v.at[:, 0:LSEG], sem.at[0]),
        pltpu.make_async_copy(bre_hbm.at[MA:M], bc_v.at[0:MR], sem.at[0]),
        pltpu.make_async_copy(bim_hbm.at[MA:M], bc_v.at[MR:2 * MR], sem.at[0]),
        pltpu.make_async_copy(bre_hbm.at[0:MA], bc_v.at[2 * MR:2 * MR + MA], sem.at[0]),
        pltpu.make_async_copy(bim_hbm.at[0:nb], bc_v.at[2 * MR + MA:BSPLIT], sem.at[0]),
    ]
    first_cps = [
        pltpu.make_async_copy(bim_hbm.at[nb:MA], bc_v.at[BSPLIT:2 * M], sem.at[SEM_X]),
    ] + x_copies(0, (1,)) + c_copies(0, C0, 0)
    vec_cps = [pltpu.make_async_copy(src, dst, sem.at[1]) for src, dst in
               ((lre_hbm, lre_v), (lim_hbm, lim_v), (ldt_hbm, ldt_v), (dsk_hbm, dsk_v),
                (gw_hbm, gw_v))]
    late_cps = [pltpu.make_async_copy(cre_hbm, bc_v.at[2 * M:3 * M], sem.at[2]),
                pltpu.make_async_copy(cim_hbm, bc_v.at[3 * M:4 * M], sem.at[2])]

    def _prologue():
        zero = jnp.int32(0)
        first = vec_cps + early_cps + first_cps
        for s in range(1, NPRO):
            first = first + stage_copies(s)
        for cp in first + w_copies(zero, 0) + late_cps:
            cp.start()
        acc_v[...] = jnp.zeros_like(acc_v)
        st_v[...] = jnp.zeros_like(st_v)
        ctxc_v[...] = jnp.zeros_like(ctxc_v)
        wt_v[1] = jnp.zeros(wt_v.shape[1:], U32)
        never_v[...] = jnp.zeros_like(never_v)

        for cp in vec_cps:
            cp.wait()
        lre = lre_v[...].astype(F32).reshape(1, M)
        lim = lim_v[...].astype(F32).reshape(1, M)
        dt = jnp.exp(ldt_v[...].astype(F32)).astype(BF16).astype(F32).reshape(1, M)
        er = jnp.exp(dt * lre)
        ar = er * jnp.cos(dt * lim)
        ai = er * jnp.sin(dt * lim)
        den = lre * lre + lim * lim
        coef_v[0] = jnp.broadcast_to(2.0 * ((ar - 1.0) * lre + ai * lim) / den, (8, M))
        coef_v[1] = jnp.broadcast_to(2.0 * (ai * lre - (ar - 1.0) * lim) / den, (8, M))

        def bc(v):
            return jnp.broadcast_to(v, (NSEG, 128))

        for t in range(3):
            a_v[t] = bc(ar[:, t * 128:(t + 1) * 128])
            a_v[4 + t] = bc(ai[:, t * 128:(t + 1) * 128])
        a_v[3] = bc(jnp.concatenate([ar[:, MA:], ar[:, MA:]], axis=1))
        a_v[7] = bc(jnp.concatenate([ai[:, MA:], -ai[:, MA:]], axis=1))
        col_v[0] = _column(dsk_v[...].astype(F32).reshape(1, M))
        col_v[1] = _column(gw_v[...].astype(F32).reshape(1, M))

        never = never_v[...] != 0

        def spread(us, rows, cols, lo, hi, sub=0, nsub=1):
            out = []
            for c in range(cols):
                vr = []
                for g in range(rows):
                    n = lo + (((c * rows + g) * nsub + sub) * (hi - lo)) // (rows * cols * nsub)
                    n = (n * len(us)) // 14
                    vr.append(us[n // 32][8 * (n % 32):8 * (n % 32) + 8])
                out.append(jnp.concatenate(vr, axis=0))
            mask = jnp.concatenate([jnp.concatenate([never] * rows, axis=0)] * cols, axis=1)
            return mask, jnp.concatenate(out, axis=1)

        def store_u(seg, u, t0):
            rows = pl.ds(pl.multiple_of(seg * SEG_STRIDE, 8), LSEG)
            for t in range(t0, t0 + u.shape[1] // 128):
                ut = u[:, (t - t0) * 128:(t - t0 + 1) * 128]
                u_v[(t + 6) % 7, rows, :] = ut
                if t == 0:
                    u_v[7, rows, :] = pltpu.roll(ut, MR, 1)

        def bu(s, head_start=None):
            r = pl.ds(pl.multiple_of(s * (LSEG // 2), LSEG // 2), LSEG // 2)
            xs = []
            us = []
            for e in range(2):
                c0 = pl.multiple_of(s * LSEG + e * HS, LSEG)
                n0 = BSPLIT if head_start is not None and e == 0 else 0
                xe = head_start if n0 else xt_v[:, pl.ds(c0, LSEG)].T
                u = lax.dot_general(xe, bc_v[n0:2 * M, :], NT, preferred_element_type=F32)
                store_u(s + e * NPRO, u, n0 // 128)
                us += [u[:, t * 128:(t + 1) * 128] for t in range(u.shape[1] // 128)]
                xw = pltpu.bitcast(xe, U32)
                xw = jnp.concatenate([xw, jnp.zeros((LSEG // 2, 2 * D - M), U32)], axis=1)
                xs.append((xw[:, :D], xw[:, D:]))
            mask, dep = spread(us, 16, 2, XLO, XHI)
            dep = pltpu.bitcast(dep, U32)
            raw = {2: jnp.where(mask, dep, xs[0][0]), 3: jnp.where(mask, dep, xs[1][1])}
            quad = [_unpack(x) for x in (raw[2], xs[0][1], xs[1][0], raw[3])]
            par = [_lhs_sums(*(q[e] for q in quad)) for e in range(2)]
            for i, (lo, hi) in enumerate(zip(*par)):
                t = raw[i] if i in raw else _pack(lo, hi)
                for kt in range(2):
                    xs_v[i, kt, r, :] = t[:, kt * 128:(kt + 1) * 128]
            return us

        def c_terms(r0, nw, us):
            raw = {}
            blk = [[None] * 4 for _ in range(4)]
            for q in range(4):
                w = c_v[pl.ds(pl.multiple_of(r0 + q * (QS // 2), 8), nw), :]
                for k in range(4):
                    blk[q][k] = _unpack(w[:, k * D:(k + 1) * D])
                mask, dep = spread(us, nw // 8, 2, CLO, CHI, 2 + q // 2, 7)
                raw[7 * (2 + q // 2) + 2 + q % 2] = jnp.where(
                    mask, pltpu.bitcast(dep, U32), w[:, q * D:(q + 1) * D])
            r = pl.ds(pl.multiple_of(r0, 8), nw)
            par = []
            for e in range(2):
                sub = [_lhs_sums(blk[a][c][e], blk[a][2 + c][e],
                                 blk[2 + a][c][e], blk[2 + a][2 + c][e])
                       for a in range(2) for c in range(2)]
                terms = []
                for i in range(7):
                    quad = [sub[n][i] for n in range(4)]
                    mask, dep = spread(us, nw // 8, 2, CLO, CHI, i, 7)
                    quad = [jnp.where(mask, dep, x) if n in (0, 3) else x
                            for n, x in enumerate(quad)]
                    terms += _lhs_sums(*quad)
                par.append(terms)
            for n, (lo, hi) in enumerate(zip(*par)):
                t = raw[n] if n in raw else _pack(lo, hi)
                for kt in range(2):
                    cs_v[n, kt, r, :] = t[:, kt * 128:(kt + 1) * 128]

        for cp in early_cps:
            cp.wait()
        x0 = xt_v[:, 0:LSEG].T
        store_u(0, lax.dot_general(x0, bc_v[0:BSPLIT, :], NT, preferred_element_type=F32), 0)
        for cp in first_cps:
            cp.wait()
        c_terms(0, C0, bu(0, x0))

        def pro_step(s, _):
            for cp in stage_copies(s):
                cp.wait()
            c_terms(C0 + (s - 1) * CSTEP, CSTEP, bu(s))
            return 0

        lax.fori_loop(1, NPRO, pro_step, 0)

    _prologue()

    def o_tiles(jobs, host=None):
        lhs = [[wt_v[sl, t, 8 * g:8 * g + 8, :] for g in range(HM // 16)] for sl, t, _ in jobs]
        if host is not None:
            host(lhs)
        return [lax.dot_general(pltpu.bitcast(jnp.concatenate(l, axis=0), BF16),
                                c, NT, preferred_element_type=F32)
                for l, (_, _, c) in zip(lhs, jobs)]

    def o_add(i, quad, x):
        r0, c0 = (quad // 2) * HM, ((2 * i + 1 + quad % 2) % (2 * NS)) * TQ
        acc_v[r0:r0 + HM, c0:c0 + TQ] += x

    def o_finish_a(i, m2, m3, m4, m5):
        o_add(i, 0, m4 - m5)
        o_add(i, 1, m3 + m5)
        o_add(i, 2, m2 + m4)
        o_add(i, 3, m3 - m2)

    def o_round_a(sl, i, ct, host=None):
        o_finish_a(i, *o_tiles([(sl, t, ct[t]) for t in (1, 2, 3, 4)], host))

    def o_round_b(sl, i, ct, extra, host=None):
        ms = o_tiles([(sl, t, ct[t]) for t in (0, 5, 6)]
                     + [(e[0], e[2], e[3]) for e in extra], host)
        o_add(i, 0, ms[0] + ms[2])
        o_add(i, 3, ms[0] + ms[1])
        for (_, ie, t, _), m in zip(extra, ms[3:]):
            if t != 5:
                o_add(ie, 0, m)
            if t != 6:
                o_add(ie, 3, m)

    def carried(sl):
        ct = [ctxc_v[t] for t in range(7)]
        return ct, [(sl, i, t, ctxc_v[7 + n]) for n, (i, t) in enumerate(CARRY)]

    def kv_scale(sl, deps=None, never=None):
        ex = []
        for n, buf in enumerate((wk_b, wv_b)):
            acc = []
            for g in range(8):
                vs = [pltpu.bitcast(buf[sl, 128 * g + 32 * a:128 * g + 32 * a + 8,
                                        128 * c:128 * c + 128] & jnp.uint32(0x7FFF0000), F32)
                      for a in range(4) for c in range(2)]
                if deps is not None:
                    vs[0] = jnp.where(never, deps[n][128 * g:128 * g + 8], vs[0])
                acc.append(functools.reduce(jnp.add, vs))
            tot = jnp.sum(functools.reduce(jnp.add, acc), keepdims=True)
            ex.append(pltpu.bitcast(tot, jnp.int32) >> 23)
        de = jnp.broadcast_to(jnp.clip(ex[0] - ex[1], -60, 60), (8, 128))
        fac_v[0] = pltpu.bitcast((127 + de) << 23, F32)
        fac_v[1] = pltpu.bitcast((127 - de) << 23, F32)

    def head(h, _):
        slot = lax.bitwise_and(h, 1)

        @pl.when(h == H // 2)
        def _segment_carry():
            pr = [a_v[t] for t in range(4)]
            pi = [a_v[4 + t] for t in range(4)]
            for _ in range(int(math.log2(LSEG))):
                pr, pi = ([pr[t] * pr[t] - pi[t] * pi[t] for t in range(4)],
                          [2.0 * pr[t] * pi[t] for t in range(4)])
            row = lax.broadcasted_iota(jnp.int32, (NSEG, 128), 0)
            e_r = [st_v[t] for t in range(4)]
            e_i = [st_v[4 + t] for t in range(4)]
            ir = [jnp.zeros((NSEG, 128), F32)] * 4
            ii = ir
            for s in range(1, NSEG):
                mr, mi = _cmul(pr, pi, ir, ii)
                fr = [pltpu.roll(mr[k] + e_r[k], 1, 0) for k in range(4)]
                fi = [pltpu.roll(mi[k] + e_i[k], 1, 0) for k in range(4)]
                ir = [jnp.where(row == s, fr[k], ir[k]) for k in range(4)]
                ii = [jnp.where(row == s, fi[k], ii[k]) for k in range(4)]
            for t in range(4):
                st_v[t] = ir[t]
                st_v[4 + t] = ii[t]

        @pl.when(h == 1)
        def _():
            for cp in late_cps:
                cp.wait()

        for cp in w_copies(h, slot):
            cp.wait()

        @pl.when(h == 0)
        def _():
            kv_scale(0)

        o_prev = o_tiles([(1 - slot, t, ctxc_v[t]) for t in (1, 2, 3, 4)])
        for cp in w_copies(jnp.minimum(h + 1, H - 1), 1 - slot):
            cp.start()
        o_finish_a(0, *o_prev)
        ct0, singles = carried(1 - slot)
        v_up = jnp.concatenate([fac_v[0, 0:1, :]] * 2, axis=1)
        v_down = fac_v[1, 0:1, :]

        up = ((1 - slot) * 16).astype(U32)
        never = never_v[...] != 0
        never64 = jnp.concatenate([never] * 8, axis=0)
        never128 = jnp.concatenate([never] * 16, axis=0)

        def weight(buf):
            return pltpu.bitcast((buf[slot] << up) & jnp.uint32(0xFFFF0000), F32)

        def quads(w, kh):
            return w[:kh, :128], w[:kh, 128:], w[kh:, :128], w[kh:, 128:]

        def bf(rows):
            return pltpu.bitcast(jnp.concatenate(
                [jnp.concatenate(r, axis=1) for r in rows], axis=0), BF16)

        def pk(x):
            return pltpu.bitcast(x.astype(BF16), U32)

        def nt(a, b):
            return lax.dot_general(a, b, NT, preferred_element_type=F32)

        def nn(a, b):
            return jnp.dot(a, b, preferred_element_type=F32)

        pin_list = []

        def x_term(i, chunks=range(8)):
            return bf([[xs_v[i, c, g * 64:(g + 1) * 64, :] for c in range(2)] for g in chunks])

        def sup(cq, j):
            l, r = (cq[0], cq[1]) if j < NS // 2 else (cq[2], cq[3])
            r0 = (j % (NS // 2)) * 2 * TQ
            return l[r0:r0 + TQ], r[r0:r0 + TQ], l[r0 + TQ:r0 + 2 * TQ], r[r0 + TQ:r0 + 2 * TQ]

        qscale = (D ** -0.5) * math.log2(math.e)
        wq = jnp.concatenate([weight(wq_b), jnp.zeros((2 * D - M, D), F32)], axis=0)
        wqt = _rhs_terms(*quads(wq, D))
        qlog = [nn(x_term(i), wqt[i]) for i in (3, 0, 1, 2, 5, 4)]
        m4, m1, m2, m3, m6, m5 = qlog
        m7 = jnp.concatenate([nn(x_term(6, o), wqt[6])
                              for o in (range(2), range(2, 4), range(4, 8))], axis=0)
        qq = [x * qscale for x in ((m1 + m4) + (m7 - m5), m3 + m5, m2 + m4, (m1 + m3) + (m6 - m2))]
        ql, qr = (jnp.concatenate([qq[c], qq[2 + c]], axis=0) for c in range(2))
        qt, qp = [None] * NS, [None] * NS
        for j in range(NS - 1, -1, -1):
            r0, ht = (2 * j + 1) * TQ, (TQ if j < NS - 1 else TQ // 2)
            top, bot = slice(r0, r0 + ht), slice(r0 + ht, r0 + 2 * ht)
            qt[j] = [pk(x) for x in _lhs_sums(ql[top], qr[top], ql[bot], qr[bot])]
            if j < NS - 1:
                qp[j] = [pk(ql[bot]), qt[j][3]]
                pin_list += qt[j] + qp[j][:1]
            else:
                qp[j] = [pk(ql[:TQ]), pk(qr[:TQ])]
                pin_list += qp[j] + [jnp.concatenate([qt[j][t], qt[j][(t + 1) % 7]], axis=0)
                                     for t in (0, 2, 4, 6)]

        r0 = pl.multiple_of(jnp.clip(h - 1, 0, M // CROWS - 1) * CROWS, CROWS)
        src = jnp.where(h == 0, 0, 2 * M) + r0
        cre = bc_v[pl.ds(pl.multiple_of(src, CROWS), CROWS), :].astype(F32)
        cim = bc_v[pl.ds(pl.multiple_of(src + M, CROWS), CROWS), :].astype(F32)
        cr = coef_v[0, 0:1, :]
        ci = coef_v[1, 0:1, :]
        c_r = cre * cr - cim * ci
        c_i = -(cre * ci + cim * cr)
        ccat_v[pl.ds(r0, CROWS), :] = jnp.concatenate(
            [c_r[:, :MA], c_i[:, :MA], c_r[:, MA:], c_i[:, MA:]], axis=1).astype(BF16)

        t0 = lax.bitwise_and(h, H // 2 - 1) * STEPS
        a_r = [a_v[t] for t in range(4)]
        a_i = [a_v[4 + t] for t in range(4)]
        hr = [st_v[t] for t in range(4)]
        hi = [st_v[4 + t] for t in range(4)]
        for j in range(STEPS):
            pos = (j * SCAN_SPAN * 128) // STEPS
            dep = qlog[2 * (pos // 128)][8 * (pos % 128):8 * (pos % 128) + 8]
            hr = [jnp.where(never, dep, x) for x in hr]
            us = [u_v[kk, pl.ds(t0 + j, NSEG, stride=SEG_STRIDE), :] for kk in range(8)]
            mr, mi = _cmul(a_r, a_i, hr, hi)
            hr = [mr[0] + us[0], mr[1] + us[1], mr[2] + us[2], mr[3] + us[6]]
            hi = [mi[0] + us[3], mi[1] + us[4], mi[2] + us[5], mi[3] + us[7]]
            r0 = pl.multiple_of((t0 + j) * NSEG, NSEG)
            for kk, val in enumerate(hr[:3] + hi[:3] + [hr[3]]):
                h_v[kk, pl.ds(r0, NSEG), :] = val
        for t in range(4):
            st_v[t] = hr[t]
            st_v[4 + t] = hi[t]

        w11, w12, w21, w22 = quads(wot_v[slot], HM // 2)
        dep = pltpu.bitcast(jnp.concatenate(
            [qlog[WODEP][64 * g:64 * g + 8] for g in range(HM // 16)], axis=0), U32)
        nv = jnp.concatenate([never] * (HM // 16), axis=0)
        quad = [_unpack(x) for x in (jnp.where(nv, dep, w11), w12, w21, jnp.where(nv, dep, w22))]
        par = [_lhs_sums(*(q[e] * v_down for q in quad)) for e in range(2)]
        for t, (lo, hi) in enumerate(zip(*par)):
            wt_v[slot, t] = _pack(lo, hi)

        kv_scale(slot, [qlog[1], qlog[4]], never)
        wk, wv = weight(wk_b), weight(wv_b) * v_up
        hc = DC // 2
        outer = _rhs_sums(wk[:hc], wv[:hc], wk[hc:], wv[hc:])
        mo = {}
        mpins = []
        kt, kp, vt, vp = [None] * NS, [None] * NS, [None] * NS, [None] * NS

        def host_lhs(tiles, share, nt_):
            slots = [(g, c) for g in range(len(tiles)) for c in range(len(tiles[0]))]
            todo = [mpins.pop(0) for _ in range(min(share, len(mpins)))]
            todo += [pin_list.pop(0) for _ in range(min(nt_, len(pin_list), len(slots) - len(todo)))]
            for n, x in enumerate(todo):
                g, c = slots[len(slots) - 1 - ((len(todo) - 1 - n) * len(slots)) // len(todo)]
                tiles[g][c] = jnp.where(never64, x, tiles[g][c])
            return bf(tiles)

        def half_tiles(left, right, top, is_k):
            for jj in range(NS // 2):
                j = jj if top else NS // 2 + jj
                x11, x12, x21, x22 = sup((left, right, left, right), j)
                quad = (x11, x21, x12, x22) if is_k else (x11, x12, x21, x22)
                terms = [pk(x) for x in _rhs_sums(*quad)]
                plain = [terms[1], pk(x12)]
                (kt if is_k else vt)[j] = terms
                (kp if is_k else vp)[j] = plain
                pin_list.extend([terms[1], terms[4], plain[1]] + [terms[t] for t in (0, 2, 3, 5, 6)])

        for n, i in enumerate(OUTER):
            rhs = _rhs_terms(*quads(outer[i], D))
            p = {}
            nm = len(mpins)
            for e, t in enumerate(INNER):
                tiles = [[cs_v[7 * i + t, c, g * 64:(g + 1) * 64, :] for c in range(2)]
                         for g in range(4)]
                w0, w1 = WSH[e], WSH[e + 1]
                share = (nm * w1) // WSH[7] - (nm * w0) // WSH[7]
                extra = (GPIN[n] * w1) // WSH[7] - (GPIN[n] * w0) // WSH[7]
                p[t] = nn(host_lhs(tiles, share, extra), rhs[t])
            quad = [(p[0] + p[3]) + (p[6] - p[4]), p[2] + p[4],
                    p[1] + p[3], (p[0] + p[2]) + (p[5] - p[1])]
            mo[i] = [jnp.concatenate([quad[c], quad[2 + c]], axis=0) for c in range(2)]
            for x in (quad[2], quad[1], quad[0], quad[3]):
                x = pltpu.bitcast(x, U32)
                mpins += [x[g * 64:(g + 1) * 64] for g in range(8)]
            if n == 2:
                ktop = [(mo[0][c] + mo[3][c]) - mo[4][c] for c in range(2)]
                w = [pltpu.bitcast(x, U32) for x in ktop]
                mpins[:] = [x[g * 64:(g + 1) * 64] for g in range(16) for x in w]
            elif n == 3:
                w = pltpu.bitcast(outer[2], U32)
                mpins[:] = [w[g * 64:(g + 1) * 64, c * 128:(c + 1) * 128]
                            for g in range(8) for c in range(2)]
                half_tiles(*(ktop[c] + mo[6][c] for c in range(2)), True, True)
            elif n == 4:
                del mpins[:]
                vbot = [mo[0][c] - mo[1][c] for c in range(2)]
                half_tiles(*(mo[1][c] + mo[3][c] for c in range(2)), False, True)
            elif n == 5:
                del mpins[:]
                vbot = [vbot[c] + mo[2][c] for c in range(2)]
                half_tiles(*(mo[2][c] + mo[4][c] for c in range(2)), True, False)
            elif n == 6:
                half_tiles(*(vbot[c] + mo[5][c] for c in range(2)), False, False)

        col = lax.broadcasted_iota(jnp.int32, (TQ, TQ), 1)
        causal = col <= lax.broadcasted_iota(jnp.int32, (TQ, TQ), 0)

        class Block:
            def __init__(self):
                self.tiles = [{}, {}, {}]
                self.mx = [None, None, None]
                self.tmp, self.acc, self.p = {}, {}, {}

            def note(self, half, n, x):
                self.tiles[half][n] = x
                self.mx[half] = x if self.mx[half] is None else jnp.maximum(self.mx[half], x)

        blks = [Block() for _ in range(NS)]
        rlog = []
        snaps = []
        never32 = jnp.concatenate([never] * 4, axis=0)

        def host_tile(x):
            return jnp.where(never64, pin_list.pop(0), x) if pin_list else x

        def smm(i, j, t, lhs=None):
            rhs = kt[j][t]
            if lhs is None and i < NS - 1:
                lhs = host_tile(qt[i][t])
            elif lhs is None:
                lhs, rhs = qt[i][t], host_tile(rhs)
            rlog[-1] = nt(bf([[lhs]]), bf([[rhs]]))
            return rlog[-1]

        def host_max(r, i, lhs):
            old = [sn for sn in snaps if sn[0] <= r - AGE and (i < NS - 1 or sn[1] == i)]
            if not old:
                return lhs
            pick = [sn for sn in old if sn[1] == old[0][1]][-1]
            snaps[:] = [sn for sn in snaps if sn[1] != pick[1] or sn[0] > pick[0]]
            pn = pltpu.bitcast(jnp.concatenate(pick[2], axis=0), U32)
            k, n = pn.shape[0] // 4, lhs[0].shape[0]
            mask = never64 if k == 64 else never32
            out = []
            for e, y in enumerate(lhs):
                z = jnp.where(mask, pn[e * k:(e + 1) * k], y[n - k:])
                out.append(z if n == k else jnp.concatenate([y[:n - k], z], axis=0))
            return out

        def s_run(r, kind, i, arg):
            blk = blks[i]
            if kind == 'a':
                lhs = host_max(r, i, [qt[i][t] for t in (1, 2, 3, 4)])
                m2, m3, m4, m5 = (smm(i, arg, t, x) for x, t in zip(lhs, (1, 2, 3, 4)))
                c12, c21 = m3 + m5, m2 + m4
                blk.tmp[arg] = [c21, c12, c12, c21, m2 + m5]
                return
            if kind == 'd':
                x = nt(bf([qp[i]]), bf([kp[(i + 1) % NS]]))
                rlog[-1] = x
                blk.note(1 if i < NS - 1 else 2, 2 * i + 2, jnp.where(causal, x, -1e9))
                if blk.mx[0] is None:
                    return
            else:
                j = arg if kind == 'b' else arg[0]
                tmp = blk.tmp[j]
                if kind == 'b':
                    m1, m6, m7 = (smm(i, j, t) for t in (0, 5, 6))
                    z = m1 - tmp[4]
                    c11, c22 = tmp[0] + (z + m7), tmp[1] + (z + m6)
                elif arg[1] == 0:
                    z = smm(i, j, 0) - tmp[4]
                    c11, c22 = tmp[0] + z, tmp[1] + z
                else:
                    tmp[6 - arg[1]] = tmp[6 - arg[1]] + smm(i, j, arg[1])
                    return
                c12 = tmp[2]
                if j == i:
                    c12 = jnp.where(causal[:c12.shape[0]], c12, -1e9)
                    if i == NS - 1:
                        c22 = jnp.where(causal[TQ // 2:], c22, -1e9)
                blk.note(0, 2 * j + 1, c12)
                blk.note(1, 2 * j, tmp[3])
                blk.note(0, 2 * j, c11)
                blk.note(1, 2 * j + 1, c22)
            snaps.append((r, i, tuple(blk.mx[:2])))

        def row_shift(i):
            blk = blks[i]
            blk.m = []
            for half, lane in enumerate(blk.mx[:3 if i == NS - 1 else 2]):
                m = jnp.max(lane, axis=1, keepdims=True)
                if half < 2:
                    est = jnp.sum(jnp.exp2(lane - m), axis=1, keepdims=True)
                    m = m + ((pltpu.bitcast(est, jnp.int32) >> 23) - 127).astype(F32)
                blk.m.append(m)

        def prob(blk, half, n):
            if (half, n) not in blk.p:
                blk.p[half, n] = jnp.exp2(blk.tiles[half][n] - blk.m[half])
            return blk.p[half, n]

        def pv_run(i, t, js):
            blk = blks[i]
            lhs, rhs = [], []
            for j in js:
                if j > i:
                    lhs.append(prob(blk, 1 if i < NS - 1 else 2, 2 * j))
                    v = vp[j % NS][0 if t == 8 else 1]
                    rhs.append(v ^ jnp.uint32(0x80008000) if t == 8 and i < NS - 1 else v)
                    continue
                a11, a12 = (lambda: prob(blk, 0, 2 * j)), (lambda: prob(blk, 0, 2 * j + 1))
                a21, a22 = (lambda: prob(blk, 1, 2 * j)), (lambda: prob(blk, 1, 2 * j + 1))
                lhs.append((
                    lambda: a11() + a22(), lambda: a21() + a22(), a11, a22,
                    lambda: a11() + a12(), lambda: a21() - a11(), lambda: a12() - a22())[t]())
                rhs.append(vt[j][t])
            x = nn(jnp.concatenate(lhs, axis=1).astype(BF16), bf([[r] for r in rhs]))
            blk.acc[t] = x if t not in blk.acc else x + blk.acc[t]
            rlog[-1] = x

        def lane_sums(i):
            p = blks[i].p
            if i < NS - 1:
                rows = [[x for (hf, _), x in p.items() if hf == half] for half in range(2)]
            else:
                rows = [[jnp.concatenate([p[0, n], p[1, n]], axis=0) for n in range(2 * NS)],
                        [p[2, 2 * NS]]]
            out = []
            for half, tl in enumerate(rows):
                tl[0] = jnp.where(never128, rlog[half - 2], tl[0])
                out.append(functools.reduce(jnp.add, tl))
            return out

        def normalise(i, lanes):
            m = blks[i].acc
            ctx = [[(m[0] + m[3]) + (m[6] - m[4]), m[2] + m[4]],
                   [m[1] + m[3], (m[0] + m[2]) + (m[5] - m[1])]]
            if i < NS - 1:
                ctx[1][0] = ctx[1][0] - m[8]
            else:
                ctx = [[jnp.concatenate([ctx[0][c], ctx[1][c]], axis=0) for c in range(2)],
                       [m[8], m[9]]]
            r = [_recip(jnp.sum(l, axis=1, keepdims=True)) for l in lanes]
            return _rhs_terms(ctx[0][0] * r[0], ctx[1][0] * r[1],
                              ctx[0][1] * r[0], ctx[1][1] * r[1])

        def sum_host(lanes, part, nparts):
            def host(lhs):
                n = 32 // nparts
                g0 = OS0 if part == 0 else 0
                slots = [(g, c) for g in range(g0, HM // 16) for c in range(len(lhs))]
                for k in range(n):
                    g, c = slots[len(slots) - 1 - ((n - 1 - k) * len(slots)) // n]
                    kk = part * n + k
                    l = lanes[kk // 16][8 * (kk % 16):8 * (kk % 16) + 8]
                    lhs[c][g] = jnp.where(never, pltpu.bitcast(l, U32), lhs[c][g])
            return host

        rounds, events = _plan()
        ctx = None
        for r, units in enumerate(rounds):
            rlog.append(None)
            for u in units:
                if u[0] == 'p':
                    pv_run(*u[1:])
                else:
                    s_run(r, *u)
            for kind, i in events.get(r + 1, []):
                if kind == 'm':
                    row_shift(i)
                    continue
                lanes = lane_sums(i)
                if i == NS - 1:
                    o_round_b(1 - slot, 0, ct0, singles[:1], sum_host(lanes, 0, 1))
                    del singles[:1]
                elif i + 1 in SPLIT:
                    o_round_a(slot, i + 1, ctx, sum_host(lanes, 0, 1))
                    singles += [(slot, i + 1, t, ctx[t]) for t in (5, 6, 0)]
                else:
                    o_round_a(slot, i + 1, ctx, sum_host(lanes, 0, 2))
                    o_round_b(slot, i + 1, ctx, singles[:1], sum_host(lanes, 1, 2))
                    del singles[:1]
                ctx = normalise(i, lanes)
        assert [e[1:3] for e in singles] == CARRY
        for n, x in enumerate(ctx + [e[3] for e in singles]):
            ctxc_v[n] = x
        return 0

    lax.fori_loop(0, H, head, 0)

    def _epilogue():
        for cp in w_copies(jnp.int32(H - 1), 0):
            cp.wait()
        ct0, singles = carried((H - 1) % 2)
        o_round_a((H - 1) % 2, 0, ct0)
        o_round_b((H - 1) % 2, 0, ct0, singles)

        def o_copy(rows, cols):
            return pltpu.make_async_copy(acc_v.at[rows, cols], out_hbm.at[rows, cols], sem.at[0])

        c_cat = ccat_v[...]
        for s in range(NSEG - 1, -1, -1):
            hs = jnp.concatenate(
                [h_v[kk, pl.ds(s, LSEG, stride=NSEG), :] for kk in range(7)],
                axis=1).astype(BF16)
            yt = lax.dot_general(c_cat, hs, NT, preferred_element_type=F32)
            w = LSEG // 2 if s == 0 else LSEG
            for e in range(LSEG // w):
                cols = pl.ds(s * LSEG + e * w, w)
                xf = xt_v[:, cols].astype(F32)
                dsk = jnp.concatenate([col_v[0]] * (w // 128), axis=1)
                gw = jnp.concatenate([col_v[1]] * (w // 128), axis=1)
                g = jax.nn.sigmoid(jnp.sum(xf * gw, axis=0, keepdims=True))
                y = yt[:, e * w:(e + 1) * w] + xf * dsk
                nr = M // 4 if (s, e) == (0, 1) else M
                for r in range(0, M, nr):
                    rows = slice(r, r + nr)
                    acc_v[rows, cols] = g * acc_v[rows, cols] + (1.0 - g) * y[rows]
                    o_copy(rows, cols).start()
        pltpu.make_async_copy(acc_v, out_hbm, sem.at[0]).wait()

    _epilogue()


@jax.jit
def pallas_gated_mix__compressed_kv_cla__ssm_conv_s5__prompt_kernel(
    A_x: jax.Array,
    A_c_kv: jax.Array,
    A_w_q: jax.Array,
    A_w_uk: jax.Array,
    A_w_uv: jax.Array,
    A_w_o: jax.Array,
    B_x: jax.Array,
    B_Lambda_re: jax.Array,
    B_Lambda_im: jax.Array,
    B_B_re: jax.Array,
    B_B_im: jax.Array,
    B_C_re: jax.Array,
    B_C_im: jax.Array,
    B_log_dt: jax.Array,
    B_Dskip: jax.Array,
    gate_w: jax.Array,
):
    del B_x
    hbm_spec = pl.BlockSpec(memory_space=pltpu.HBM)
    out_t = pl.pallas_call(
        _kernel,
        in_specs=[hbm_spec] * 15,
        out_specs=hbm_spec,
        out_shape=jax.ShapeDtypeStruct((M, S), F32),
        scratch_shapes=[
            pltpu.VMEM((M, S), BF16),
            pltpu.VMEM((7, 2, HS // 2, 128), U32),
            pltpu.VMEM((HS, DC), U32),
            pltpu.VMEM((49, 2, QS // 2, 128), U32),
            pltpu.VMEM((2, M // 2, D), U32),
            pltpu.VMEM((2, 7, M // 4, 128), U32),
            pltpu.VMEM((2, M, D), U32),
            pltpu.VMEM((2, DC, D), U32),
            pltpu.VMEM((2, DC, D), U32),
            pltpu.VMEM((4 * M, M), BF16),
            pltpu.VMEM((M, 2 * M), BF16),
            pltpu.VMEM((M,), BF16), pltpu.VMEM((M,), BF16), pltpu.VMEM((M,), BF16),
            pltpu.VMEM((M,), BF16), pltpu.VMEM((M,), BF16),
            pltpu.VMEM((2, M, 128), F32),
            pltpu.VMEM((2, 8, M), F32),
            pltpu.VMEM((8, NSEG * SEG_STRIDE, 128), F32),
            pltpu.VMEM((7, S, 128), F32),
            pltpu.VMEM((8, NSEG, 128), F32),
            pltpu.VMEM((8, NSEG, 128), F32),
            pltpu.VMEM((M, S), F32),
            pltpu.VMEM((7 + len(CARRY), TQ, 128), BF16),
            pltpu.VMEM((8, 128), jnp.int32),
            pltpu.VMEM((2, 8, 128), F32),
            pltpu.SemaphoreType.DMA((SEM_X + NPRO,)),
        ],
        compiler_params=pltpu.CompilerParams(vmem_limit_bytes=110 * 1024 * 1024),
        name="gated_mix",
    )(
        A_x.reshape(S, M).T, A_c_kv.reshape(S, DC),
        A_w_q, A_w_uk, A_w_uv, jnp.swapaxes(A_w_o, 1, 2),
        B_Lambda_re, B_Lambda_im, B_B_re, B_B_im, B_C_re, B_C_im, B_log_dt,
        B_Dskip, gate_w,
    )
    return out_t.T.reshape(1, S, M)
```

```python
import functools
import math

import jax
import jax.numpy as jnp
from jax import lax
import jax.experimental.pallas as pl
import jax.experimental.pallas.tpu as pltpu

F32 = jnp.float32
BF16 = jnp.bfloat16
U32 = jnp.uint32

S = 2048
HS = S // 2
QS = S // 4
M = 448
HM = M // 2
DC = 1024
H = 16
D = 256
TQ = 128
NS = S // (2 * TQ)
NSEG = 8
LSEG = S // NSEG
SEG_STRIDE = LSEG + 8
STEPS = 2 * LSEG // H
MA = 384
MR = M - MA
NT = (((1,), (1,)), ((), ()))
NPRO = NSEG // 2
C0, CSTEP = 16, 80
BSPLIT = 640
CROWS = 32
SEM_W = 3
SEM_X = 4

XLO, XHI, CLO, CHI = 230, 440, 10, 430
SCAN_SPAN, WODEP = 2, 3
OUTER = (4, 0, 3, 6, 1, 2, 5)
INNER = (3, 1, 4, 2, 0, 6, 5)
GPIN = (24, 16, 14, 8, 32, 28, 32)
WSH = (0, 0, 4, 8, 12, 16, 20, 24)
PORDER = (2, 3, 0, 1, 5, 4, 6)
PGROUPS = [[(j, min(j + 4, i)) for j in range(0, i, 4)] for i in range(NS)]
PGROUPS[7] = [(0, 4), (4, 6), (6, 7)]
PGROUPS[3] = [(0, 2), (2, 3)]
LEAD, BAL, AGE, OS0 = 5, 16, 2, 2
CAP, ACOST, MCOST, OCOST, RATIO, PTAIL = 112, 48, 32, 48, 0.9, 26
SPLIT = (5, 1)
CARRY = [(1, 5), (1, 6), (1, 0)]

_NEEDS = {0: ((0, 0), (1, 1)), 1: ((1, 0), (1, 1)), 2: ((0, 0),), 3: ((1, 1),),
          4: ((0, 0), (0, 1)), 5: ((1, 0), (0, 0)), 6: ((0, 1), (1, 1))}


def _plan():
    def four(i, j):
        return [[('a', i, j)], [('a', i, j + 1)], [('b', i, j), ('s', i, (j + 1, 5))],
                [('a', i, j + 2)], [('b', i, j + 2), ('s', i, (j + 1, 6))],
                [('a', i, j + 3)], [('b', i, j + 3), ('s', i, (j + 1, 0))]]

    def weave(half, full):
        out = []
        for n, f in enumerate(full):
            out += half[2 * n:2 * n + 2] + [f]
        return out

    rounds = [[('d', 6, 0), ('d', 7, 0)]] + weave(four(7, 0) + four(7, 4), four(6, 0))
    events = {len(rounds) - 1: [('m', 7)]}
    rounds += [[('a', 6, 4)], [('a', 6, 5)], [('b', 6, 4), ('s', 6, (5, 5))]]
    rounds += weave([[('p', 7, t, list(range(j, j + 4)))] for j in (0, 4) for t in PORDER],
                    [[('a', 6, 6)], [('b', 6, 6), ('s', 6, (5, 6))], [('a', 5, 0)],
                     [('b', 5, 0), ('s', 6, (5, 0))], [('a', 5, 1)],
                     [('b', 5, 1), ('p', 7, 8, [8])], [('a', 5, 2)]])
    events[len(rounds) - 9] = [('m', 6)]
    rounds += [[('b', 5, 2), ('p', 7, 9, [8])]]
    events[len(rounds)] = [('o', 7)]
    sq = []
    for i in range(NS - 3, -1, -1):
        for j in range(3 if i == NS - 3 else 0, i + 1):
            sq += [(4, 'a', i, j), (3, 'b', i, j)]
        sq.append((2, 'd', i, 0))
    pq = {}
    for i in range(NS - 1):
        pq[i] = [[j1 - j0, t, list(range(j0, j1))] for j0, j1 in PGROUPS[i + 1] for t in PORDER]
        pq[i] += [[1, 8, [i + 1]], [1, 5, [i + 1]]]
    ready, seen = {NS - 2: 0}, set()

    def needs(i, t, js):
        out = set()
        for j in js:
            out |= {(i, 1, 2 * j)} if j > i else {(i, hf, 2 * j + c) for hf, c in _NEEDS[t]}
        return out

    def p_fill(free, pi, first):
        left = {i: [list(u) for u in pq[i]] for i in (pi, pi - 1) if i >= 0}
        got, new = [], set()
        while free and pi in left and ready.get(pi, 1 << 30) <= len(rounds):
            us = left[pi]
            if first is not None:
                u, first = us[first], None
            else:
                size = min(free, max(v[0] for v in us))
                fit = [v for v in us if v[0] == size] or [
                    v for v in us if v[0] == min(w[0] for w in us if w[0] > size)]
                u = min(fit, key=lambda v: len(needs(pi, v[1], v[2][-size:]) - seen - new))
            size = min(free, u[0])
            got.append(('p', pi, u[1], u[2][-size:]))
            new |= needs(pi, u[1], u[2][-size:]) - seen
            u[2], u[0] = u[2][:len(u[2]) - size], u[0] - size
            if not u[0]:
                us.remove(u)
            free -= size
            if not us:
                pi -= 1
        return got, new, free, left, pi

    pi, prev = NS - 2, OCOST
    while sq or pi >= 0:
        cands = []
        if sq:
            n, free = 0, 4
            while n < len(sq) and sq[n][0] <= free and (
                    n == 0 or 's' in (sq[n][1], sq[n - 1][1])):
                free -= sq[n][0]
                n += 1
            cands.append((n,) + p_fill(free, pi, None))
            if free == 2 and n < len(sq) and sq[n][0] == 2:
                cands.append((n + 1,) + p_fill(0, pi, None))
        if pi >= 0:
            big = max(u[0] for u in pq[pi])
            grp = next(u[2] for u in pq[pi] if u[0] == big)
            cands += [(0,) + p_fill(4, pi, k) for k, u in enumerate(pq[pi]) if u[2] == grp]
        best = None
        for n, got, new, free, left, p2 in cands:
            s_left = sum(u[0] for u in sq[n:] if u[2] >= pi - 1)
            p_left = sum(u[0] for u in left.get(pi, []))
            s_all = sum(u[0] for u in sq[n:])
            p_all = sum(u[0] for i in range(pi + 1) for u in left.get(i, pq[i]))
            load = prev + 16 * len(new) + (MCOST if n and sq[0][1] == 'a' else 0)
            late = max(s_left + BAL - p_left, 0) if s_left else 0
            drift = abs(s_all - RATIO * max(p_all - PTAIL, 0))
            cost = 1000 * free + max(load - CAP, 0) + 2 * late + drift - len(new) + len(got)
            if best is None or cost < best[0]:
                best = (cost, n, got, new, left, p2)
        _, n, got, new, left, p2 = best
        cur = [u[1:] for u in sq[:n]] + got
        done = {u[2] for u in sq[:n]}
        del sq[:n]
        seen |= new
        pq.update(left)
        rounds.append(cur)
        for i in done:
            if all(v[2] != i for v in sq):
                events.setdefault(len(rounds), []).append(('m', i))
                ready[i] = len(rounds) + LEAD
        prev = sum({'a': ACOST, 'b': 32, 'd': 16, 's': 24, 'p': 16}[u[0]] for u in cur)
        for i in range(pi, p2, -1):
            events.setdefault(len(rounds), []).append(('o', i))
            prev = OCOST
        pi = p2
    return rounds, events


def _lhs_sums(a11, a12, a21, a22):
    return [a11 + a22, a21 + a22, a11, a22, a11 + a12, a21 - a11, a12 - a22]


def _rhs_sums(b11, b12, b21, b22):
    return [b11 + b22, b11, b12 - b22, b21 - b11, b22, b11 + b12, b21 + b22]


def _rhs_terms(*quad):
    return [t.astype(BF16) for t in _rhs_sums(*quad)]


def _unpack(w):
    return (pltpu.bitcast(w << jnp.uint32(16), F32),
            pltpu.bitcast(w & jnp.uint32(0xFFFF0000), F32))


def _pack(lo, hi):
    half = jnp.uint32(0x7FFF) + (lax.broadcasted_iota(U32, lo.shape, 1) & jnp.uint32(1))
    return (((pltpu.bitcast(lo, U32) + half) >> jnp.uint32(16))
            | ((pltpu.bitcast(hi, U32) + half) & jnp.uint32(0xFFFF0000)))


def _recip(l):
    r = pl.reciprocal(l, approx=True)
    return r * (2.0 - l * r)


def _cmul(pr, pi, hr, hi):
    return ([pr[t] * hr[t] - pi[t] * hi[t] for t in range(4)],
            [pr[t] * hi[t] + pi[t] * hr[t] for t in range(4)])


def _column(row):
    row = jnp.concatenate([row, jnp.zeros((1, 512 - M), F32)], axis=1)
    return jnp.broadcast_to(row, (128, 512)).T[:M]


def _kernel(xt_hbm, c_hbm, wq_hbm, wk_hbm, wv_hbm, wot_hbm,
            lre_hbm, lim_hbm, bre_hbm, bim_hbm, cre_hbm, cim_hbm, ldt_hbm,
            dsk_hbm, gw_hbm,
            out_hbm,
            xt_v, xs_v, c_v, cs_v, wot_v, wt_v, wq_b, wk_b, wv_b, bc_v, ccat_v,
            lre_v, lim_v, ldt_v, dsk_v, gw_v, col_v, coef_v,
            u_v, h_v, a_v, st_v, acc_v, ctxc_v, never_v, fac_v, sem):
    wq32 = wq_hbm.bitcast(U32)
    wk32 = wk_hbm.bitcast(U32)
    wv32 = wv_hbm.bitcast(U32)
    c32 = c_hbm.bitcast(U32)
    wot32 = wot_hbm.bitcast(U32)

    def w_copies(h, buf, sm=SEM_W):
        j = lax.shift_right_logical(h, 1)
        cps = [pltpu.make_async_copy(src.at[:, j, :], dst.at[buf], sem.at[sm])
               for src, dst in ((wq32, wq_b), (wk32, wk_b), (wv32, wv_b))]
        return cps + [pltpu.make_async_copy(wot32.at[h], wot_v.at[buf], sem.at[sm])]

    def x_copies(s, halves=(0, 1)):
        spans = [pl.ds(pl.multiple_of(s * LSEG + e * HS, LSEG), LSEG) for e in halves]
        return [pltpu.make_async_copy(xt_hbm.at[:, sp], xt_v.at[:, sp], sem.at[SEM_X + s])
                for sp in spans]

    def c_copies(start, rows, s):
        spans = [pl.ds(pl.multiple_of(start + e * (QS // 2), 8), rows) for e in range(4)]
        return [pltpu.make_async_copy(c32.at[sp], c_v.at[sp], sem.at[SEM_X + s])
                for sp in spans]

    def stage_copies(s):
        return x_copies(s) + c_copies(C0 + (s - 1) * CSTEP, CSTEP, s)

    nb = BSPLIT - (2 * MR + MA)
    early_cps = [
        pltpu.make_async_copy(xt_hbm.at[:, 0:LSEG], xt_v.at[:, 0:LSEG], sem.at[0]),
        pltpu.make_async_copy(bre_hbm.at[MA:M], bc_v.at[0:MR], sem.at[0]),
        pltpu.make_async_copy(bim_hbm.at[MA:M], bc_v.at[MR:2 * MR], sem.at[0]),
        pltpu.make_async_copy(bre_hbm.at[0:MA], bc_v.at[2 * MR:2 * MR + MA], sem.at[0]),
        pltpu.make_async_copy(bim_hbm.at[0:nb], bc_v.at[2 * MR + MA:BSPLIT], sem.at[0]),
    ]
    first_cps = [
        pltpu.make_async_copy(bim_hbm.at[nb:MA], bc_v.at[BSPLIT:2 * M], sem.at[SEM_X]),
    ] + x_copies(0, (1,)) + c_copies(0, C0, 0)
    vec_cps = [pltpu.make_async_copy(src, dst, sem.at[1]) for src, dst in
               ((lre_hbm, lre_v), (lim_hbm, lim_v), (ldt_hbm, ldt_v), (dsk_hbm, dsk_v),
                (gw_hbm, gw_v))]
    late_cps = [pltpu.make_async_copy(cre_hbm, bc_v.at[2 * M:3 * M], sem.at[2]),
                pltpu.make_async_copy(cim_hbm, bc_v.at[3 * M:4 * M], sem.at[2])]
    late_cps += w_copies(jnp.int32(1), 1, 2)

    def _prologue():
        zero = jnp.int32(0)
        first = vec_cps + early_cps + first_cps
        for s in range(1, NPRO):
            first = first + stage_copies(s)
        for cp in first + w_copies(zero, 0) + late_cps:
            cp.start()
        acc_v[...] = jnp.zeros_like(acc_v)
        st_v[...] = jnp.zeros_like(st_v)
        ctxc_v[...] = jnp.zeros_like(ctxc_v)
        wt_v[1] = jnp.zeros(wt_v.shape[1:], U32)
        never_v[...] = jnp.zeros_like(never_v)

        for cp in vec_cps:
            cp.wait()
        lre = lre_v[...].astype(F32).reshape(1, M)
        lim = lim_v[...].astype(F32).reshape(1, M)
        dt = jnp.exp(ldt_v[...].astype(F32)).astype(BF16).astype(F32).reshape(1, M)
        er = jnp.exp(dt * lre)
        ar = er * jnp.cos(dt * lim)
        ai = er * jnp.sin(dt * lim)
        den = lre * lre + lim * lim
        coef_v[0] = jnp.broadcast_to(2.0 * ((ar - 1.0) * lre + ai * lim) / den, (8, M))
        coef_v[1] = jnp.broadcast_to(2.0 * (ai * lre - (ar - 1.0) * lim) / den, (8, M))

        def bc(v):
            return jnp.broadcast_to(v, (NSEG, 128))

        for t in range(3):
            a_v[t] = bc(ar[:, t * 128:(t + 1) * 128])
            a_v[4 + t] = bc(ai[:, t * 128:(t + 1) * 128])
        a_v[3] = bc(jnp.concatenate([ar[:, MA:], ar[:, MA:]], axis=1))
        a_v[7] = bc(jnp.concatenate([ai[:, MA:], -ai[:, MA:]], axis=1))
        col_v[0] = _column(dsk_v[...].astype(F32).reshape(1, M))
        col_v[1] = _column(gw_v[...].astype(F32).reshape(1, M))

        never = never_v[...] != 0

        def spread(us, rows, cols, lo, hi, sub=0, nsub=1):
            out = []
            for c in range(cols):
                vr = []
                for g in range(rows):
                    n = lo + (((c * rows + g) * nsub + sub) * (hi - lo)) // (rows * cols * nsub)
                    n = (n * len(us)) // 14
                    vr.append(us[n // 32][8 * (n % 32):8 * (n % 32) + 8])
                out.append(jnp.concatenate(vr, axis=0))
            mask = jnp.concatenate([jnp.concatenate([never] * rows, axis=0)] * cols, axis=1)
            return mask, jnp.concatenate(out, axis=1)

        def store_u(seg, u, t0):
            rows = pl.ds(pl.multiple_of(seg * SEG_STRIDE, 8), LSEG)
            for t in range(t0, t0 + u.shape[1] // 128):
                ut = u[:, (t - t0) * 128:(t - t0 + 1) * 128]
                u_v[(t + 6) % 7, rows, :] = ut
                if t == 0:
                    u_v[7, rows, :] = pltpu.roll(ut, MR, 1)

        def bu(s, head_start=None):
            r = pl.ds(pl.multiple_of(s * (LSEG // 2), LSEG // 2), LSEG // 2)
            xs = []
            us = []
            for e in range(2):
                c0 = pl.multiple_of(s * LSEG + e * HS, LSEG)
                n0 = BSPLIT if head_start is not None and e == 0 else 0
                xe = head_start if n0 else xt_v[:, pl.ds(c0, LSEG)].T
                u = lax.dot_general(xe, bc_v[n0:2 * M, :], NT, preferred_element_type=F32)
                store_u(s + e * NPRO, u, n0 // 128)
                us += [u[:, t * 128:(t + 1) * 128] for t in range(u.shape[1] // 128)]
                xw = pltpu.bitcast(xe, U32)
                xw = jnp.concatenate([xw, jnp.zeros((LSEG // 2, 2 * D - M), U32)], axis=1)
                xs.append((xw[:, :D], xw[:, D:]))
            mask, dep = spread(us, 16, 2, XLO, XHI)
            dep = pltpu.bitcast(dep, U32)
            raw = {2: jnp.where(mask, dep, xs[0][0]), 3: jnp.where(mask, dep, xs[1][1])}
            quad = [_unpack(x) for x in (raw[2], xs[0][1], xs[1][0], raw[3])]
            par = [_lhs_sums(*(q[e] for q in quad)) for e in range(2)]
            for i, (lo, hi) in enumerate(zip(*par)):
                t = raw[i] if i in raw else _pack(lo, hi)
                for kt in range(2):
                    xs_v[i, kt, r, :] = t[:, kt * 128:(kt + 1) * 128]
            return us

        def c_terms(r0, nw, us):
            raw = {}
            blk = [[None] * 4 for _ in range(4)]
            for q in range(4):
                w = c_v[pl.ds(pl.multiple_of(r0 + q * (QS // 2), 8), nw), :]
                for k in range(4):
                    blk[q][k] = _unpack(w[:, k * D:(k + 1) * D])
                mask, dep = spread(us, nw // 8, 2, CLO, CHI, 2 + q // 2, 7)
                raw[7 * (2 + q // 2) + 2 + q % 2] = jnp.where(
                    mask, pltpu.bitcast(dep, U32), w[:, q * D:(q + 1) * D])
            r = pl.ds(pl.multiple_of(r0, 8), nw)
            par = []
            for e in range(2):
                sub = [_lhs_sums(blk[a][c][e], blk[a][2 + c][e],
                                 blk[2 + a][c][e], blk[2 + a][2 + c][e])
                       for a in range(2) for c in range(2)]
                terms = []
                for i in range(7):
                    quad = [sub[n][i] for n in range(4)]
                    mask, dep = spread(us, nw // 8, 2, CLO, CHI, i, 7)
                    quad = [jnp.where(mask, dep, x) if n in (0, 3) else x
                            for n, x in enumerate(quad)]
                    terms += _lhs_sums(*quad)
                par.append(terms)
            for n, (lo, hi) in enumerate(zip(*par)):
                t = raw[n] if n in raw else _pack(lo, hi)
                for kt in range(2):
                    cs_v[n, kt, r, :] = t[:, kt * 128:(kt + 1) * 128]

        for cp in early_cps:
            cp.wait()
        x0 = xt_v[:, 0:LSEG].T
        store_u(0, lax.dot_general(x0, bc_v[0:BSPLIT, :], NT, preferred_element_type=F32), 0)
        for cp in first_cps:
            cp.wait()
        c_terms(0, C0, bu(0, x0))

        def pro_step(s, _):
            for cp in stage_copies(s):
                cp.wait()
            c_terms(C0 + (s - 1) * CSTEP, CSTEP, bu(s))
            return 0

        lax.fori_loop(1, NPRO, pro_step, 0)

    _prologue()

    def o_tiles(jobs, host=None):
        lhs = [[wt_v[sl, t, 8 * g:8 * g + 8, :] for g in range(HM // 16)] for sl, t, _ in jobs]
        if host is not None:
            host(lhs)
        return [lax.dot_general(pltpu.bitcast(jnp.concatenate(l, axis=0), BF16),
                                c, NT, preferred_element_type=F32)
                for l, (_, _, c) in zip(lhs, jobs)]

    def o_add(i, quad, x):
        r0, c0 = (quad // 2) * HM, ((2 * i + 1 + quad % 2) % (2 * NS)) * TQ
        acc_v[r0:r0 + HM, c0:c0 + TQ] += x

    def o_finish_a(i, m2, m3, m4, m5):
        o_add(i, 0, m4 - m5)
        o_add(i, 1, m3 + m5)
        o_add(i, 2, m2 + m4)
        o_add(i, 3, m3 - m2)

    def o_round_a(sl, i, ct, host=None):
        o_finish_a(i, *o_tiles([(sl, t, ct[t]) for t in (1, 2, 3, 4)], host))

    def o_round_b(sl, i, ct, extra, host=None):
        ms = o_tiles([(sl, t, ct[t]) for t in (0, 5, 6)]
                     + [(e[0], e[2], e[3]) for e in extra], host)
        o_add(i, 0, ms[0] + ms[2])
        o_add(i, 3, ms[0] + ms[1])
        for (_, ie, t, _), m in zip(extra, ms[3:]):
            if t != 5:
                o_add(ie, 0, m)
            if t != 6:
                o_add(ie, 3, m)

    def carried(sl):
        ct = [ctxc_v[t] for t in range(7)]
        return ct, [(sl, i, t, ctxc_v[7 + n]) for n, (i, t) in enumerate(CARRY)]

    def kv_scale(buf, up, deps=None, never=None):
        ex = []
        for n, ref in enumerate((wk_b, wv_b)):
            acc = []
            for g in range(16):
                r0 = g * (DC // 16)
                vs = [ref[buf, r0 + 8 * a:r0 + 8 * a + 8, 128 * (a % 2):128 * (a % 2) + 128]
                      for a in range(DC // 16 // 8)]
                vs = [pltpu.bitcast((w << up) & jnp.uint32(0x7FFF0000), F32) for w in vs]
                if deps is not None:
                    vs[0] = jnp.where(never, deps[n][r0:r0 + 8], vs[0])
                acc.append(functools.reduce(jnp.add, vs))
            tot = jnp.sum(functools.reduce(jnp.add, acc), keepdims=True)
            ex.append(pltpu.bitcast(tot, jnp.int32) >> 23)
        de = jnp.broadcast_to(jnp.clip(ex[0] - ex[1], -60, 60), (8, 128))
        fac_v[0] = pltpu.bitcast((127 + de) << 23, F32)
        fac_v[1] = pltpu.bitcast((127 - de) << 23, F32)

    def head(h, cur):
        slot = lax.bitwise_and(h, 1)

        @pl.when(h == H // 2)
        def _segment_carry():
            pr = [a_v[t] for t in range(4)]
            pi = [a_v[4 + t] for t in range(4)]
            for _ in range(int(math.log2(LSEG))):
                pr, pi = ([pr[t] * pr[t] - pi[t] * pi[t] for t in range(4)],
                          [2.0 * pr[t] * pi[t] for t in range(4)])
            row = lax.broadcasted_iota(jnp.int32, (NSEG, 128), 0)
            e_r = [st_v[t] for t in range(4)]
            e_i = [st_v[4 + t] for t in range(4)]
            ir = [jnp.zeros((NSEG, 128), F32)] * 4
            ii = ir
            for s in range(1, NSEG):
                mr, mi = _cmul(pr, pi, ir, ii)
                fr = [pltpu.roll(mr[k] + e_r[k], 1, 0) for k in range(4)]
                fi = [pltpu.roll(mi[k] + e_i[k], 1, 0) for k in range(4)]
                ir = [jnp.where(row == s, fr[k], ir[k]) for k in range(4)]
                ii = [jnp.where(row == s, fi[k], ii[k]) for k in range(4)]
            for t in range(4):
                st_v[t] = ir[t]
                st_v[4 + t] = ii[t]

        @pl.when(h == 1)
        def _():
            for cp in late_cps:
                cp.wait()

        inc = jnp.where(cur == 2, 0, cur + 1)
        nxt = jnp.where(h == 0, 0, inc)
        for cp in w_copies(jnp.where(h == 0, 0, jnp.minimum(h + 1, H - 1)), nxt):
            cp.wait()

        @pl.when(h == 0)
        def _():
            kv_scale(0, jnp.uint32(16))

        o_prev = o_tiles([(1 - slot, t, ctxc_v[t]) for t in (1, 2, 3, 4)])
        for cp in w_copies(jnp.minimum(h + 2, H - 1), 3 - cur - inc):
            cp.start()
        o_finish_a(0, *o_prev)
        ct0, singles = carried(1 - slot)
        v_up = jnp.concatenate([fac_v[0, 0:1, :]] * 2, axis=1)
        v_down = fac_v[1, 0:1, :]

        up = ((1 - slot) * 16).astype(U32)
        never = never_v[...] != 0
        never64 = jnp.concatenate([never] * 8, axis=0)
        never128 = jnp.concatenate([never] * 16, axis=0)

        def weight(buf):
            return pltpu.bitcast((buf[cur] << up) & jnp.uint32(0xFFFF0000), F32)

        def quads(w, kh):
            return w[:kh, :128], w[:kh, 128:], w[kh:, :128], w[kh:, 128:]

        def bf(rows):
            return pltpu.bitcast(jnp.concatenate(
                [jnp.concatenate(r, axis=1) for r in rows], axis=0), BF16)

        def pk(x):
            return pltpu.bitcast(x.astype(BF16), U32)

        def nt(a, b):
            return lax.dot_general(a, b, NT, preferred_element_type=F32)

        def nn(a, b):
            return jnp.dot(a, b, preferred_element_type=F32)

        pin_list = []

        def x_term(i, chunks=range(8)):
            return bf([[xs_v[i, c, g * 64:(g + 1) * 64, :] for c in range(2)] for g in chunks])

        def sup(cq, j):
            l, r = (cq[0], cq[1]) if j < NS // 2 else (cq[2], cq[3])
            r0 = (j % (NS // 2)) * 2 * TQ
            return l[r0:r0 + TQ], r[r0:r0 + TQ], l[r0 + TQ:r0 + 2 * TQ], r[r0 + TQ:r0 + 2 * TQ]

        qscale = (D ** -0.5) * math.log2(math.e)
        wq = jnp.concatenate([weight(wq_b), jnp.zeros((2 * D - M, D), F32)], axis=0)
        wqt = _rhs_terms(*quads(wq, D))
        qlog = [nn(x_term(i), wqt[i]) for i in (3, 0, 1, 2, 5, 4)]
        m4, m1, m2, m3, m6, m5 = qlog
        m7 = jnp.concatenate([nn(x_term(6, o), wqt[6])
                              for o in (range(2), range(2, 4), range(4, 8))], axis=0)
        qq = [x * qscale for x in ((m1 + m4) + (m7 - m5), m3 + m5, m2 + m4, (m1 + m3) + (m6 - m2))]
        ql, qr = (jnp.concatenate([qq[c], qq[2 + c]], axis=0) for c in range(2))
        qt, qp = [None] * NS, [None] * NS
        for j in range(NS - 1, -1, -1):
            r0, ht = (2 * j + 1) * TQ, (TQ if j < NS - 1 else TQ // 2)
            top, bot = slice(r0, r0 + ht), slice(r0 + ht, r0 + 2 * ht)
            qt[j] = [pk(x) for x in _lhs_sums(ql[top], qr[top], ql[bot], qr[bot])]
            if j < NS - 1:
                qp[j] = [pk(ql[bot]), qt[j][3]]
                pin_list += qt[j] + qp[j][:1]
            else:
                qp[j] = [pk(ql[:TQ]), pk(qr[:TQ])]
                pin_list += qp[j] + [jnp.concatenate([qt[j][t], qt[j][(t + 1) % 7]], axis=0)
                                     for t in (0, 2, 4, 6)]

        r0 = pl.multiple_of(jnp.clip(h - 1, 0, M // CROWS - 1) * CROWS, CROWS)
        src = jnp.where(h == 0, 0, 2 * M) + r0
        cre = bc_v[pl.ds(pl.multiple_of(src, CROWS), CROWS), :].astype(F32)
        cim = bc_v[pl.ds(pl.multiple_of(src + M, CROWS), CROWS), :].astype(F32)
        cr = coef_v[0, 0:1, :]
        ci = coef_v[1, 0:1, :]
        c_r = cre * cr - cim * ci
        c_i = -(cre * ci + cim * cr)
        ccat_v[pl.ds(r0, CROWS), :] = jnp.concatenate(
            [c_r[:, :MA], c_i[:, :MA], c_r[:, MA:], c_i[:, MA:]], axis=1).astype(BF16)

        t0 = lax.bitwise_and(h, H // 2 - 1) * STEPS
        a_r = [a_v[t] for t in range(4)]
        a_i = [a_v[4 + t] for t in range(4)]
        hr = [st_v[t] for t in range(4)]
        hi = [st_v[4 + t] for t in range(4)]
        for j in range(STEPS):
            pos = (j * SCAN_SPAN * 128) // STEPS
            dep = qlog[2 * (pos // 128)][8 * (pos % 128):8 * (pos % 128) + 8]
            hr = [jnp.where(never, dep, x) for x in hr]
            us = [u_v[kk, pl.ds(t0 + j, NSEG, stride=SEG_STRIDE), :] for kk in range(8)]
            mr, mi = _cmul(a_r, a_i, hr, hi)
            hr = [mr[0] + us[0], mr[1] + us[1], mr[2] + us[2], mr[3] + us[6]]
            hi = [mi[0] + us[3], mi[1] + us[4], mi[2] + us[5], mi[3] + us[7]]
            r0 = pl.multiple_of((t0 + j) * NSEG, NSEG)
            for kk, val in enumerate(hr[:3] + hi[:3] + [hr[3]]):
                h_v[kk, pl.ds(r0, NSEG), :] = val
        for t in range(4):
            st_v[t] = hr[t]
            st_v[4 + t] = hi[t]

        w11, w12, w21, w22 = quads(wot_v[cur], HM // 2)
        dep = pltpu.bitcast(jnp.concatenate(
            [qlog[WODEP][64 * g:64 * g + 8] for g in range(HM // 16)], axis=0), U32)
        nv = jnp.concatenate([never] * (HM // 16), axis=0)
        quad = [_unpack(x) for x in (jnp.where(nv, dep, w11), w12, w21, jnp.where(nv, dep, w22))]
        par = [_lhs_sums(*(q[e] * v_down for q in quad)) for e in range(2)]
        for t, (lo, hi) in enumerate(zip(*par)):
            wt_v[slot, t] = _pack(lo, hi)

        kv_scale(nxt, (slot * 16).astype(U32), [qlog[1], qlog[4]], never)
        wk, wv = weight(wk_b), weight(wv_b) * v_up
        hc = DC // 2
        outer = _rhs_sums(wk[:hc], wv[:hc], wk[hc:], wv[hc:])
        mo = {}
        mpins = []
        kt, kp, vt, vp = [None] * NS, [None] * NS, [None] * NS, [None] * NS

        def host_lhs(tiles, share, nt_):
            slots = [(g, c) for g in range(len(tiles)) for c in range(len(tiles[0]))]
            todo = [mpins.pop(0) for _ in range(min(share, len(mpins)))]
            todo += [pin_list.pop(0) for _ in range(min(nt_, len(pin_list), len(slots) - len(todo)))]
            for n, x in enumerate(todo):
                g, c = slots[len(slots) - 1 - ((len(todo) - 1 - n) * len(slots)) // len(todo)]
                tiles[g][c] = jnp.where(never64, x, tiles[g][c])
            return bf(tiles)

        def half_tiles(left, right, top, is_k):
            for jj in range(NS // 2):
                j = jj if top else NS // 2 + jj
                x11, x12, x21, x22 = sup((left, right, left, right), j)
                quad = (x11, x21, x12, x22) if is_k else (x11, x12, x21, x22)
                terms = [pk(x) for x in _rhs_sums(*quad)]
                plain = [terms[1], pk(x12)]
                (kt if is_k else vt)[j] = terms
                (kp if is_k else vp)[j] = plain
                pin_list.extend([terms[1], terms[4], plain[1]] + [terms[t] for t in (0, 2, 3, 5, 6)])

        for n, i in enumerate(OUTER):
            rhs = _rhs_terms(*quads(outer[i], D))
            p = {}
            nm = len(mpins)
            for e, t in enumerate(INNER):
                tiles = [[cs_v[7 * i + t, c, g * 64:(g + 1) * 64, :] for c in range(2)]
                         for g in range(4)]
                w0, w1 = WSH[e], WSH[e + 1]
                share = (nm * w1) // WSH[7] - (nm * w0) // WSH[7]
                extra = (GPIN[n] * w1) // WSH[7] - (GPIN[n] * w0) // WSH[7]
                p[t] = nn(host_lhs(tiles, share, extra), rhs[t])
            quad = [(p[0] + p[3]) + (p[6] - p[4]), p[2] + p[4],
                    p[1] + p[3], (p[0] + p[2]) + (p[5] - p[1])]
            mo[i] = [jnp.concatenate([quad[c], quad[2 + c]], axis=0) for c in range(2)]
            for x in (quad[2], quad[1], quad[0], quad[3]):
                x = pltpu.bitcast(x, U32)
                mpins += [x[g * 64:(g + 1) * 64] for g in range(8)]
            if n == 2:
                ktop = [(mo[0][c] + mo[3][c]) - mo[4][c] for c in range(2)]
                w = [pltpu.bitcast(x, U32) for x in ktop]
                mpins[:] = [x[g * 64:(g + 1) * 64] for g in range(16) for x in w]
            elif n == 3:
                w = pltpu.bitcast(outer[2], U32)
                mpins[:] = [w[g * 64:(g + 1) * 64, c * 128:(c + 1) * 128]
                            for g in range(8) for c in range(2)]
                half_tiles(*(ktop[c] + mo[6][c] for c in range(2)), True, True)
            elif n == 4:
                del mpins[:]
                vbot = [mo[0][c] - mo[1][c] for c in range(2)]
                half_tiles(*(mo[1][c] + mo[3][c] for c in range(2)), False, True)
            elif n == 5:
                del mpins[:]
                vbot = [vbot[c] + mo[2][c] for c in range(2)]
                half_tiles(*(mo[2][c] + mo[4][c] for c in range(2)), True, False)
            elif n == 6:
                half_tiles(*(vbot[c] + mo[5][c] for c in range(2)), False, False)

        col = lax.broadcasted_iota(jnp.int32, (TQ, TQ), 1)
        causal = col <= lax.broadcasted_iota(jnp.int32, (TQ, TQ), 0)

        class Block:
            def __init__(self):
                self.tiles = [{}, {}, {}]
                self.mx = [None, None, None]
                self.tmp, self.acc, self.p = {}, {}, {}

            def note(self, half, n, x):
                self.tiles[half][n] = x
                self.mx[half] = x if self.mx[half] is None else jnp.maximum(self.mx[half], x)

        blks = [Block() for _ in range(NS)]
        rlog = []
        snaps = []
        never32 = jnp.concatenate([never] * 4, axis=0)

        def host_tile(x):
            return jnp.where(never64, pin_list.pop(0), x) if pin_list else x

        def smm(i, j, t, lhs=None):
            rhs = kt[j][t]
            if lhs is None and i < NS - 1:
                lhs = host_tile(qt[i][t])
            elif lhs is None:
                lhs, rhs = qt[i][t], host_tile(rhs)
            rlog[-1] = nt(bf([[lhs]]), bf([[rhs]]))
            return rlog[-1]

        def host_max(r, i, lhs):
            old = [sn for sn in snaps if sn[0] <= r - AGE and (i < NS - 1 or sn[1] == i)]
            if not old:
                return lhs
            pick = [sn for sn in old if sn[1] == old[0][1]][-1]
            snaps[:] = [sn for sn in snaps if sn[1] != pick[1] or sn[0] > pick[0]]
            pn = pltpu.bitcast(jnp.concatenate(pick[2], axis=0), U32)
            k, n = pn.shape[0] // 4, lhs[0].shape[0]
            mask = never64 if k == 64 else never32
            out = []
            for e, y in enumerate(lhs):
                z = jnp.where(mask, pn[e * k:(e + 1) * k], y[n - k:])
                out.append(z if n == k else jnp.concatenate([y[:n - k], z], axis=0))
            return out

        def s_run(r, kind, i, arg):
            blk = blks[i]
            if kind == 'a':
                lhs = host_max(r, i, [qt[i][t] for t in (1, 2, 3, 4)])
                m2, m3, m4, m5 = (smm(i, arg, t, x) for x, t in zip(lhs, (1, 2, 3, 4)))
                c12, c21 = m3 + m5, m2 + m4
                blk.tmp[arg] = [c21, c12, c12, c21, m2 + m5]
                return
            if kind == 'd':
                x = nt(bf([qp[i]]), bf([kp[(i + 1) % NS]]))
                rlog[-1] = x
                blk.note(1 if i < NS - 1 else 2, 2 * i + 2, jnp.where(causal, x, -1e9))
                if blk.mx[0] is None:
                    return
            else:
                j = arg if kind == 'b' else arg[0]
                tmp = blk.tmp[j]
                if kind == 'b':
                    m1, m6, m7 = (smm(i, j, t) for t in (0, 5, 6))
                    z = m1 - tmp[4]
                    c11, c22 = tmp[0] + (z + m7), tmp[1] + (z + m6)
                elif arg[1] == 0:
                    z = smm(i, j, 0) - tmp[4]
                    c11, c22 = tmp[0] + z, tmp[1] + z
                else:
                    tmp[6 - arg[1]] = tmp[6 - arg[1]] + smm(i, j, arg[1])
                    return
                c12 = tmp[2]
                if j == i:
                    c12 = jnp.where(causal[:c12.shape[0]], c12, -1e9)
                    if i == NS - 1:
                        c22 = jnp.where(causal[TQ // 2:], c22, -1e9)
                blk.note(0, 2 * j + 1, c12)
                blk.note(1, 2 * j, tmp[3])
                blk.note(0, 2 * j, c11)
                blk.note(1, 2 * j + 1, c22)
            snaps.append((r, i, tuple(blk.mx[:2])))

        def row_shift(i):
            blk = blks[i]
            blk.m = []
            for half, lane in enumerate(blk.mx[:3 if i == NS - 1 else 2]):
                m = jnp.max(lane, axis=1, keepdims=True)
                if half < 2:
                    est = jnp.sum(jnp.exp2(lane - m), axis=1, keepdims=True)
                    m = m + ((pltpu.bitcast(est, jnp.int32) >> 23) - 127).astype(F32)
                blk.m.append(m)

        def prob(blk, half, n):
            if (half, n) not in blk.p:
                blk.p[half, n] = jnp.exp2(blk.tiles[half][n] - blk.m[half])
            return blk.p[half, n]

        def pv_run(i, t, js):
            blk = blks[i]
            lhs, rhs = [], []
            for j in js:
                if j > i:
                    lhs.append(prob(blk, 1 if i < NS - 1 else 2, 2 * j))
                    v = vp[j % NS][0 if t == 8 else 1]
                    rhs.append(v ^ jnp.uint32(0x80008000) if t == 8 and i < NS - 1 else v)
                    continue
                a11, a12 = (lambda: prob(blk, 0, 2 * j)), (lambda: prob(blk, 0, 2 * j + 1))
                a21, a22 = (lambda: prob(blk, 1, 2 * j)), (lambda: prob(blk, 1, 2 * j + 1))
                lhs.append((
                    lambda: a11() + a22(), lambda: a21() + a22(), a11, a22,
                    lambda: a11() + a12(), lambda: a21() - a11(), lambda: a12() - a22())[t]())
                rhs.append(vt[j][t])
            x = nn(jnp.concatenate(lhs, axis=1).astype(BF16), bf([[r] for r in rhs]))
            blk.acc[t] = x if t not in blk.acc else x + blk.acc[t]
            rlog[-1] = x

        def lane_sums(i):
            p = blks[i].p
            if i < NS - 1:
                rows = [[x for (hf, _), x in p.items() if hf == half] for half in range(2)]
            else:
                rows = [[jnp.concatenate([p[0, n], p[1, n]], axis=0) for n in range(2 * NS)],
                        [p[2, 2 * NS]]]
            out = []
            for half, tl in enumerate(rows):
                tl[0] = jnp.where(never128, rlog[half - 2], tl[0])
                out.append(functools.reduce(jnp.add, tl))
            return out

        def normalise(i, lanes):
            m = blks[i].acc
            ctx = [[(m[0] + m[3]) + (m[6] - m[4]), m[2] + m[4]],
                   [m[1] + m[3], (m[0] + m[2]) + (m[5] - m[1])]]
            if i < NS - 1:
                ctx[1][0] = ctx[1][0] - m[8]
            else:
                ctx = [[jnp.concatenate([ctx[0][c], ctx[1][c]], axis=0) for c in range(2)],
                       [m[8], m[9]]]
            r = [_recip(jnp.sum(l, axis=1, keepdims=True)) for l in lanes]
            return _rhs_terms(ctx[0][0] * r[0], ctx[1][0] * r[1],
                              ctx[0][1] * r[0], ctx[1][1] * r[1])

        def sum_host(lanes, part, nparts):
            def host(lhs):
                n = 32 // nparts
                g0 = OS0 if part == 0 else 0
                slots = [(g, c) for g in range(g0, HM // 16) for c in range(len(lhs))]
                for k in range(n):
                    g, c = slots[len(slots) - 1 - ((n - 1 - k) * len(slots)) // n]
                    kk = part * n + k
                    l = lanes[kk // 16][8 * (kk % 16):8 * (kk % 16) + 8]
                    lhs[c][g] = jnp.where(never, pltpu.bitcast(l, U32), lhs[c][g])
            return host

        rounds, events = _plan()
        ctx = None
        for r, units in enumerate(rounds):
            rlog.append(None)
            for u in units:
                if u[0] == 'p':
                    pv_run(*u[1:])
                else:
                    s_run(r, *u)
            for kind, i in events.get(r + 1, []):
                if kind == 'm':
                    row_shift(i)
                    continue
                lanes = lane_sums(i)
                if i == NS - 1:
                    o_round_b(1 - slot, 0, ct0, singles[:1], sum_host(lanes, 0, 1))
                    del singles[:1]
                elif i + 1 in SPLIT:
                    o_round_a(slot, i + 1, ctx, sum_host(lanes, 0, 1))
                    singles += [(slot, i + 1, t, ctx[t]) for t in (5, 6, 0)]
                else:
                    o_round_a(slot, i + 1, ctx, sum_host(lanes, 0, 2))
                    o_round_b(slot, i + 1, ctx, singles[:1], sum_host(lanes, 1, 2))
                    del singles[:1]
                ctx = normalise(i, lanes)
        assert [e[1:3] for e in singles] == CARRY
        for n, x in enumerate(ctx + [e[3] for e in singles]):
            ctxc_v[n] = x
        return inc

    lax.fori_loop(0, H, head, jnp.int32(0))

    def _epilogue():
        for cp in w_copies(jnp.int32(H - 1), (H + 1) % 3):
            cp.wait()
        ct0, singles = carried((H - 1) % 2)
        o_round_a((H - 1) % 2, 0, ct0)
        o_round_b((H - 1) % 2, 0, ct0, singles)

        def o_copy(rows, cols):
            return pltpu.make_async_copy(acc_v.at[rows, cols], out_hbm.at[rows, cols], sem.at[0])

        c_cat = ccat_v[...]
        for s in range(NSEG - 1, -1, -1):
            hs = jnp.concatenate(
                [h_v[kk, pl.ds(s, LSEG, stride=NSEG), :] for kk in range(7)],
                axis=1).astype(BF16)
            yt = lax.dot_general(c_cat, hs, NT, preferred_element_type=F32)
            w = LSEG // 2 if s == 0 else LSEG
            for e in range(LSEG // w):
                cols = pl.ds(s * LSEG + e * w, w)
                xf = xt_v[:, cols].astype(F32)
                dsk = jnp.concatenate([col_v[0]] * (w // 128), axis=1)
                gw = jnp.concatenate([col_v[1]] * (w // 128), axis=1)
                g = jax.nn.sigmoid(jnp.sum(xf * gw, axis=0, keepdims=True))
                y = yt[:, e * w:(e + 1) * w] + xf * dsk
                nr = M // 4 if (s, e) == (0, 1) else M
                for r in range(0, M, nr):
                    rows = slice(r, r + nr)
                    acc_v[rows, cols] = g * acc_v[rows, cols] + (1.0 - g) * y[rows]
                    o_copy(rows, cols).start()
        pltpu.make_async_copy(acc_v, out_hbm, sem.at[0]).wait()

    _epilogue()


@jax.jit
def pallas_gated_mix__compressed_kv_cla__ssm_conv_s5__prompt_kernel(
    A_x: jax.Array,
    A_c_kv: jax.Array,
    A_w_q: jax.Array,
    A_w_uk: jax.Array,
    A_w_uv: jax.Array,
    A_w_o: jax.Array,
    B_x: jax.Array,
    B_Lambda_re: jax.Array,
    B_Lambda_im: jax.Array,
    B_B_re: jax.Array,
    B_B_im: jax.Array,
    B_C_re: jax.Array,
    B_C_im: jax.Array,
    B_log_dt: jax.Array,
    B_Dskip: jax.Array,
    gate_w: jax.Array,
):
    del B_x
    hbm_spec = pl.BlockSpec(memory_space=pltpu.HBM)
    out_t = pl.pallas_call(
        _kernel,
        in_specs=[hbm_spec] * 15,
        out_specs=hbm_spec,
        out_shape=jax.ShapeDtypeStruct((M, S), F32),
        scratch_shapes=[
            pltpu.VMEM((M, S), BF16),
            pltpu.VMEM((7, 2, HS // 2, 128), U32),
            pltpu.VMEM((HS, DC), U32),
            pltpu.VMEM((49, 2, QS // 2, 128), U32),
            pltpu.VMEM((3, M // 2, D), U32),
            pltpu.VMEM((2, 7, M // 4, 128), U32),
            pltpu.VMEM((3, M, D), U32),
            pltpu.VMEM((3, DC, D), U32),
            pltpu.VMEM((3, DC, D), U32),
            pltpu.VMEM((4 * M, M), BF16),
            pltpu.VMEM((M, 2 * M), BF16),
            pltpu.VMEM((M,), BF16), pltpu.VMEM((M,), BF16), pltpu.VMEM((M,), BF16),
            pltpu.VMEM((M,), BF16), pltpu.VMEM((M,), BF16),
            pltpu.VMEM((2, M, 128), F32),
            pltpu.VMEM((2, 8, M), F32),
            pltpu.VMEM((8, (NSEG + 1) * SEG_STRIDE, 128), F32),
            pltpu.VMEM((7, S + NSEG, 128), F32),
            pltpu.VMEM((8, NSEG, 128), F32),
            pltpu.VMEM((8, NSEG, 128), F32),
            pltpu.VMEM((M, S), F32),
            pltpu.VMEM((7 + len(CARRY), TQ, 128), BF16),
            pltpu.VMEM((8, 128), jnp.int32),
            pltpu.VMEM((2, 8, 128), F32),
            pltpu.SemaphoreType.DMA((SEM_X + NPRO,)),
        ],
        compiler_params=pltpu.CompilerParams(vmem_limit_bytes=110 * 1024 * 1024),
        name="gated_mix",
    )(
        A_x.reshape(S, M).T, A_c_kv.reshape(S, DC),
        A_w_q, A_w_uk, A_w_uv, jnp.swapaxes(A_w_o, 1, 2),
        B_Lambda_re, B_Lambda_im, B_B_re, B_B_im, B_C_re, B_C_im, B_log_dt,
        B_Dskip, gate_w,
    )
    return out_t.T.reshape(1, S, M)
```
